```python
import jax
import jax.numpy as jnp

def _softmax(x, axis=-1):
    return jax.nn.softmax(x, axis=axis)

def _gelu(x):
    return jax.nn.gelu(x, approximate=True)

def _silu(x):
    return jax.nn.silu(x)

def _sigmoid(x):
    return jax.nn.sigmoid(x)

def _layernorm(x, axis=-1, eps=1e-05):
    m = jnp.mean(x, axis=axis, keepdims=True)
    v = jnp.var(x, axis=axis, keepdims=True)
    return (x - m) / jnp.sqrt(v + eps)

def _scatter_add(tgt, idx, src, axis=0):
    return tgt.at[idx].add(src)

def _segment_sum(src, seg, n):
    return jax.ops.segment_sum(src, seg, n)

class _Rng:

    def __init__(self, key):
        self._k = key

    def _next(self):
        self._k, sub = jax.random.split(self._k)
        return sub

    def normal(self, shape):
        return jax.random.normal(self._next(), shape, dtype=jnp.bfloat16)

    def randint(self, lo, hi, shape):
        return jax.random.randint(self._next(), shape, lo, hi, dtype=jnp.int32)

    def uniform(self, shape, lo=0.0, hi=1.0):
        return jax.random.uniform(self._next(), shape, jnp.bfloat16, lo, hi)

    def permutation(self, n):
        return jax.random.permutation(self._next(), n)
kernel_name = 'adaLN_cond__compressed_kv_cla__mixer_s_mlp__prompt'

def setup_inputs():
    _rng = _Rng(jax.random.key(int.from_bytes(__import__("os").urandom(4), "little")))
    _w = lambda a: (lambda t: t.astype(jnp.bfloat16) if jnp.issubdtype(t.dtype, jnp.floating) else t)(jnp.asarray(a))

    def _A_setup():
        B, H, Sq, Sk, D, M = (1, 32, 2048, 2048, 128, 640)
        Dc = 4 * D
        return {'x': _w((lambda *s: _rng.normal(s) * 0.05)(B, Sq, M)), 'c_kv': _w((lambda *s: _rng.normal(s) * 0.05)(B, Sk, Dc)), 'w_q': _w((lambda *s: _rng.normal(s) * 0.05)(M, H, D) * M ** (-0.5)), 'w_uk': _w((lambda *s: _rng.normal(s) * 0.05)(Dc, H, D) * Dc ** (-0.5)), 'w_uv': _w((lambda *s: _rng.normal(s) * 0.05)(Dc, H, D) * Dc ** (-0.5)), 'w_o': _w((lambda *s: _rng.normal(s) * 0.05)(H, D, M) * (H * D) ** (-0.5))}
    _A_in = _A_setup()

    def _B_setup():
        B, S, D, F = (1, 2048, 640, 1728)
        return {'x': _w((lambda *s: _rng.normal(s) * 0.05)(B, S, D)), 'w1': _w((lambda *s: _rng.normal(s) * 0.05)(D, D) * D ** (-0.5)), 'w2': _w((lambda *s: _rng.normal(s) * 0.05)(D, D) * D ** (-0.5)), 'w3': _w((lambda *s: _rng.normal(s) * 0.05)(D, F) * D ** (-0.5)), 'w4': _w((lambda *s: _rng.normal(s) * 0.05)(F, D) * F ** (-0.5))}
    _B_in = _B_setup()
    return {'A_x': _A_in['x'], 'A_c_kv': _A_in['c_kv'], 'A_w_q': _A_in['w_q'], 'A_w_uk': _A_in['w_uk'], 'A_w_uv': _A_in['w_uv'], 'A_w_o': _A_in['w_o'], 'B_x': _B_in['x'], 'B_w1': _B_in['w1'], 'B_w2': _B_in['w2'], 'B_w3': _B_in['w3'], 'B_w4': _B_in['w4'], 'c': _w((lambda *s: _rng.normal(s) * 0.05)(1, 640)), 'w_mod': _w((lambda *s: _rng.normal(s) * 0.05)(640, 6 * 640) * 640 ** (-0.5))}

def reference(A_x, A_c_kv, A_w_q, A_w_uk, A_w_uv, A_w_o, B_x, B_w1, B_w2, B_w3, B_w4, c, w_mod):

    def _A_ref(x, c_kv, w_q, w_uk, w_uv, w_o):
        B, Sq, M = (x.shape[0], x.shape[1], x.shape[2])
        Sk = c_kv.shape[1]
        H, D = (w_q.shape[1], w_q.shape[2])
        q = jnp.einsum('bqm,mhd->bhqd', x, w_q)
        k = jnp.einsum('bkc,chd->bhkd', c_kv, w_uk)
        v = jnp.einsum('bkc,chd->bhkd', c_kv, w_uv)
        scores = jnp.einsum('bhqd,bhkd->bhqk', q, k) * D ** (-0.5)
        off = Sk - Sq
        qi = jnp.arange(Sq)[:, None]
        kj = jnp.arange(Sk)[None, :]
        cmask = kj <= qi + off
        scores = jnp.where(cmask[None, None], scores, -1000000000.0)
        p = _softmax(scores, axis=-1)
        ctx = jnp.einsum('bhqk,bhkd->bhqd', p, v)
        return jnp.einsum('bhqd,hdm->bqm', ctx, w_o)

    def _B_ref(x, w1, w2, w3, w4):
        B, S, D = x.shape
        h = _gelu(_layernorm(x, axis=-1) @ w1)
        c = D // 4
        g0 = jnp.pad(h[:, :, 0 * c:1 * c], ((0, 0), (1, 0), (0, 0)))[:, :S, :]
        g1 = jnp.pad(h[:, :, 1 * c:2 * c], ((0, 0), (0, 1), (0, 0)))[:, 1:, :]
        g2 = jnp.pad(h[:, :, 2 * c:3 * c], ((0, 0), (2, 0), (0, 0)))[:, :S, :]
        g3 = jnp.pad(h[:, :, 3 * c:], ((0, 0), (0, 2), (0, 0)))[:, 2:, :]
        hs = jnp.concatenate([g0, g1, g2, g3], axis=-1) @ w2
        x1 = x + hs
        h2 = _gelu(_layernorm(x1, axis=-1) @ w3) @ w4
        return x1 + h2
    x = A_x
    mod = (_silu(c) @ w_mod).reshape(c.shape[0], 6, 1, -1)
    sa, ca, ga, sb, cb, gb = (mod[:, 0].copy(), mod[:, 1].copy(), mod[:, 2].copy(), mod[:, 3].copy(), mod[:, 4].copy(), mod[:, 5].copy())
    h = _layernorm(x, axis=-1) * (1 + ca) + sa
    x = x + ga * _A_ref(h, A_c_kv, A_w_q, A_w_uk, A_w_uv, A_w_o)
    h = _layernorm(x, axis=-1) * (1 + cb) + sb
    x = x + gb * _B_ref(h, B_w1, B_w2, B_w3, B_w4)
    return x
```

```python
import functools
import math

import jax
import jax.numpy as jnp
from jax import lax
import jax.experimental.pallas as pl
import jax.experimental.pallas.tpu as pltpu

F32 = jnp.float32
BF16 = jnp.bfloat16
NT = (((1,), (1,)), ((), ()))
NEG = -1000000000.0
EPS = 1e-05
TQ = 128
TR = 256
HALO = 8


def _ln(x):
    m = jnp.mean(x, axis=-1, keepdims=True)
    xc = x - m
    v = jnp.mean(xc * xc, axis=-1, keepdims=True)
    return xc * lax.rsqrt(v + EPS)


def _gelu(x):
    c = math.sqrt(2.0 / math.pi)
    return 0.5 * x * (1.0 + jnp.tanh(c * (x + 0.044715 * (x * x * x))))


def _split_pair(w):
    m, _, d = w.shape
    u = pltpu.bitcast(w.reshape(2 * m, d), jnp.uint32)
    lo = pltpu.bitcast(u << 16, F32).astype(BF16)
    hi = pltpu.bitcast(u & jnp.uint32(0xFFFF0000), F32).astype(BF16)
    return lo, hi


def _kernel(x_ref, ckv_ref, wq_ref, wk_ref, wv_ref, wo_ref,
            w1_ref, w2_ref, w3_ref, w4_ref, c_ref, wmod_ref,
            o_ref,
            mod_ref, h_ref, wqp_ref, wkvp_ref, kv_ref, acc_ref, t_ref, x1_ref, hb_ref,
            *, S, M, D, NP):
    j = pl.program_id(0)
    nq = S // TQ
    qscale = (D ** -0.5) * math.log2(math.e)

    @pl.when(j == 0)
    def _prologue():
        c = c_ref[...].astype(F32)
        sc = c * jax.nn.sigmoid(c)
        sc8 = jnp.broadcast_to(sc, (8, M)).astype(BF16)
        mod_ref[...] = jnp.dot(sc8, wmod_ref[...], preferred_element_type=F32)

        def body(t, carry):
            r = pl.multiple_of(t * TR, TR)
            x = x_ref[pl.ds(r, TR), :].astype(F32)
            sa = mod_ref[0:1, 0:M]
            ca = mod_ref[0:1, M:2 * M]
            h_ref[pl.ds(r, TR), :] = (_ln(x) * (1.0 + ca) + sa).astype(BF16)
            acc_ref[pl.ds(r, TR), :] = jnp.zeros((TR, M), F32)
            return carry
        lax.fori_loop(0, S // TR, body, 0)

    qa, qb = _split_pair(wq_ref[...])
    wqp_ref[:, 0:D] = qa
    wqp_ref[:, D:2 * D] = qb
    ka, kb = _split_pair(wk_ref[...])
    wkvp_ref[:, 0:D] = ka
    wkvp_ref[:, D:2 * D] = kb
    va, vb = _split_pair(wv_ref[...])
    wkvp_ref[:, 2 * D:3 * D] = va
    wkvp_ref[:, 3 * D:4 * D] = vb

    row = lax.broadcasted_iota(jnp.int32, (TQ, TQ), 0)
    col = lax.broadcasted_iota(jnp.int32, (TQ, TQ), 1)
    tri = col <= row

    def proj(i):
        rows = slice(i * TQ, (i + 1) * TQ)
        kv = jnp.dot(ckv_ref[rows, :], wkvp_ref[...], preferred_element_type=F32)
        kv_ref[rows, :] = kv.astype(BF16)
        q = jnp.dot(h_ref[rows, :], wqp_ref[...], preferred_element_type=F32)
        return (q * qscale).astype(BF16)

    def scores(q, hh, i):
        k = kv_ref[0:(i + 1) * TQ, hh * D:(hh + 1) * D]
        s = lax.dot_general(q[:, hh * D:(hh + 1) * D], k, NT, preferred_element_type=F32)
        sd = jnp.where(tri, s[:, i * TQ:], NEG)
        if i > 0:
            return jnp.concatenate([s[:, :i * TQ], sd], axis=1)
        return sd

    def softmax_pv(s, hh, i):
        m = jnp.max(s, axis=1, keepdims=True)
        p = jnp.exp2(s - m)
        l = jnp.sum(p, axis=1, keepdims=True)
        v = kv_ref[0:(i + 1) * TQ, (2 + hh) * D:(3 + hh) * D]
        o = jnp.dot(p.astype(BF16), v, preferred_element_type=F32)
        return (o * pl.reciprocal(l, approx=False)).astype(BF16)

    def oproj(ctx, i):
        rows = slice(i * TQ, (i + 1) * TQ)
        acc_ref[rows, :] += jnp.dot(ctx, wo_ref[...], preferred_element_type=F32)

    q = {0: proj(0)}
    s = {}
    ctx = {}
    for i in range(nq + 2):
        if i + 1 < nq:
            q[i + 1] = proj(i + 1)
        if i < nq:
            s[(i, 0)] = scores(q[i], 0, i)
        if 0 <= i - 1 < nq:
            ctx[(i - 1, 0)] = softmax_pv(s.pop((i - 1, 0)), 0, i - 1)
        if i < nq:
            s[(i, 1)] = scores(q.pop(i), 1, i)
        if 0 <= i - 1 < nq:
            ctx[(i - 1, 1)] = softmax_pv(s.pop((i - 1, 1)), 1, i - 1)
        if 0 <= i - 2 < nq:
            oproj(jnp.concatenate([ctx.pop((i - 2, 0)), ctx.pop((i - 2, 1))], axis=1), i - 2)

    @pl.when(j == NP - 1)
    def _epilogue():
        ga = mod_ref[0:1, 2 * M:3 * M]
        sb = mod_ref[0:1, 3 * M:4 * M]
        cb = mod_ref[0:1, 4 * M:5 * M]
        gb = mod_ref[0:1, 5 * M:6 * M]
        t_ref[0:HALO, :] = jnp.zeros((HALO, M), F32)
        t_ref[S + HALO:S + 2 * HALO, :] = jnp.zeros((HALO, M), F32)

        def stage_a(t, carry):
            r = pl.multiple_of(t * TR, TR)
            x1 = x_ref[pl.ds(r, TR), :].astype(F32) + ga * acc_ref[pl.ds(r, TR), :]
            x1_ref[pl.ds(r, TR), :] = x1
            h = _ln(x1) * (1.0 + cb) + sb
            hb_ref[pl.ds(r, TR), :] = h
            u = _ln(h).astype(BF16)
            t_ref[pl.ds(HALO + r, TR), :] = _gelu(jnp.dot(u, w1_ref[...], preferred_element_type=F32))
            return carry
        lax.fori_loop(0, S // TR, stage_a, 0)

        G = M // 4
        lane = lax.broadcasted_iota(jnp.int32, (TR, M), 1)

        def stage_b(t, carry):
            r = pl.multiple_of(t * TR, TR)
            win = t_ref[pl.ds(r, TR + 2 * HALO), :]
            g0 = win[HALO - 1:HALO - 1 + TR]
            g1 = win[HALO + 1:HALO + 1 + TR]
            g2 = win[HALO - 2:HALO - 2 + TR]
            g3 = win[HALO + 2:HALO + 2 + TR]
            sh = jnp.where(lane < 2 * G, jnp.where(lane < G, g0, g1),
                           jnp.where(lane < 3 * G, g2, g3)).astype(BF16)
            y = hb_ref[pl.ds(r, TR), :] + jnp.dot(sh, w2_ref[...], preferred_element_type=F32)
            u = _ln(y).astype(BF16)
            f = _gelu(jnp.dot(u, w3_ref[...], preferred_element_type=F32)).astype(BF16)
            h2 = jnp.dot(f, w4_ref[...], preferred_element_type=F32)
            o_ref[pl.ds(r, TR), :] = (x1_ref[pl.ds(r, TR), :] + gb * (y + h2)).astype(o_ref.dtype)
            return carry
        lax.fori_loop(0, S // TR, stage_b, 0)


@jax.jit
def pallas_adaLN_cond__compressed_kv_cla__mixer_s_mlp__prompt_kernel(
    A_x: jax.Array,
    A_c_kv: jax.Array,
    A_w_q: jax.Array,
    A_w_uk: jax.Array,
    A_w_uv: jax.Array,
    A_w_o: jax.Array,
    B_x: jax.Array,
    B_w1: jax.Array,
    B_w2: jax.Array,
    B_w3: jax.Array,
    B_w4: jax.Array,
    c: jax.Array,
    w_mod: jax.Array,
):
    B, S, M = A_x.shape
    assert B == 1 and A_c_kv.shape[1] == S
    Dc = A_c_kv.shape[2]
    H, D = A_w_q.shape[1], A_w_q.shape[2]
    NP = H // 2
    Fd = B_w3.shape[1]

    def whole(shape):
        return pl.BlockSpec(shape, lambda j: (0,) * len(shape), pipeline_mode=pl.Buffered(1))

    def pair(rows):
        return pl.BlockSpec((rows, None, 2, D), lambda j: (0, j, 0, 0))

    out = pl.pallas_call(
        functools.partial(_kernel, S=S, M=M, D=D, NP=NP),
        grid=(NP,),
        in_specs=[
            whole((S, M)), whole((S, Dc)),
            pair(M), pair(Dc), pair(Dc),
            pl.BlockSpec((2 * D, M), lambda j: (j, 0)),
            whole((M, M)), whole((M, M)), whole((M, Fd)), whole((Fd, M)),
            whole((1, M)), whole((M, 6 * M)),
        ],
        out_specs=pl.BlockSpec((S, M), lambda j: (0, 0)),
        out_shape=jax.ShapeDtypeStruct((S, M), A_x.dtype),
        scratch_shapes=[
            pltpu.VMEM((8, 6 * M), F32),
            pltpu.VMEM((S, M), BF16),
            pltpu.VMEM((M, 2 * D), BF16),
            pltpu.VMEM((Dc, 4 * D), BF16),
            pltpu.VMEM((S, 4 * D), BF16),
            pltpu.VMEM((S, M), F32),
            pltpu.VMEM((S + 2 * HALO, M), F32),
            pltpu.VMEM((S, M), F32),
            pltpu.VMEM((S, M), F32),
        ],
        compiler_params=pltpu.CompilerParams(
            dimension_semantics=("arbitrary",),
            vmem_limit_bytes=100 * 1024 * 1024,
        ),
    )(
        A_x.reshape(S, M), A_c_kv.reshape(S, Dc),
        A_w_q.reshape(M, NP, 2, D), A_w_uk.reshape(Dc, NP, 2, D), A_w_uv.reshape(Dc, NP, 2, D),
        A_w_o.reshape(H * D, M),
        B_w1, B_w2, B_w3, B_w4, c, w_mod,
    )
    return out.reshape(B, S, M)
```

```python
import functools
import math

import jax
import jax.numpy as jnp
from jax import lax
import jax.experimental.pallas as pl
import jax.experimental.pallas.tpu as pltpu

F32 = jnp.float32
BF16 = jnp.bfloat16
U32 = jnp.uint32
NT = (((1,), (1,)), ((), ()))
NEG = -1000000000.0
EPS = 1e-05
TQ = 128
TA = 256
TB = 256
XC = 4
HALO = 8
ORDER = list(range(2, 16)) + [1, 0]


def _ln(x):
    m = jnp.mean(x, axis=-1, keepdims=True)
    xc = x - m
    v = jnp.mean(xc * xc, axis=-1, keepdims=True)
    return xc * lax.rsqrt(v + EPS)


def _gelu(x):
    c = math.sqrt(2.0 / math.pi)
    return 0.5 * x * (1.0 + jnp.tanh(c * (x + 0.044715 * (x * x * x))))


def _as_bf16(u):
    return pltpu.bitcast(u, BF16)


def _as_u32(b):
    return pltpu.bitcast(b, U32)


def _split_pair(u):
    lo = pltpu.bitcast(u << 16, F32).astype(BF16)
    hi = pltpu.bitcast(u & jnp.uint32(0xFFFF0000), F32).astype(BF16)
    return _as_u32(lo), _as_u32(hi)


def _kernel(x_hbm, ckv_hbm, wq_hbm, wk_hbm, wv_hbm, wo_hbm,
            w1_hbm, w2_hbm, w3t_hbm, w4_hbm, c_hbm, wmod_hbm,
            o_hbm,
            x_ref, ckv_ref, wqr_ref, wkr_ref, wvr_ref, wo_ref,
            w1_ref, w2_ref, w3t_ref, w4_ref, c_ref, wmoda_ref, wmodb_ref,
            mod_ref, h_ref, wqp_ref, wkvp_ref, kv_ref, acc_ref,
            t_ref, hb_ref, y_ref, u3_ref, ob_ref,
            xsem, ssem, psem, osem,
            *, S, M, D, NP):
    j = pl.program_id(0)
    slot = j % 2
    nq = S // TQ
    HQ = TQ // 2
    qscale = (D ** -0.5) * math.log2(math.e)
    XR = S // XC

    def x_copy(i):
        return pltpu.make_async_copy(x_hbm.at[pl.ds(i * XR, XR), :],
                                     x_ref.at[pl.ds(i * XR, XR), :], xsem.at[i])

    wmod_u = wmod_hbm.bitcast(U32)
    c_copy = pltpu.make_async_copy(c_hbm, c_ref, ssem.at[0])
    wmoda_copy = pltpu.make_async_copy(wmod_u.at[:, pl.ds(0, 2 * M)], wmoda_ref, ssem.at[1])
    ckv_copy = pltpu.make_async_copy(ckv_hbm.bitcast(U32), ckv_ref, ssem.at[2])
    wmodb_copy = pltpu.make_async_copy(wmod_u.at[:, pl.ds(2 * M, 4 * M)], wmodb_ref, ssem.at[3])
    late_copies = [
        pltpu.make_async_copy(w1_hbm.bitcast(U32), w1_ref, ssem.at[4]),
        pltpu.make_async_copy(w2_hbm.bitcast(U32), w2_ref, ssem.at[5]),
        pltpu.make_async_copy(w3t_hbm.bitcast(U32), w3t_ref, ssem.at[6]),
        pltpu.make_async_copy(w4_hbm.bitcast(U32), w4_ref, ssem.at[7]),
    ]

    def pair_copies(p, sl):
        return [
            pltpu.make_async_copy(wk_hbm.bitcast(U32).at[:, p, :], wkr_ref.at[sl], psem.at[sl, 0]),
            pltpu.make_async_copy(wv_hbm.bitcast(U32).at[:, p, :], wvr_ref.at[sl], psem.at[sl, 1]),
            pltpu.make_async_copy(wq_hbm.bitcast(U32).at[:, p, :], wqr_ref.at[sl], psem.at[sl, 2]),
            pltpu.make_async_copy(wo_hbm.bitcast(U32).at[pl.ds(pl.multiple_of(p * D, D), D), :],
                                  wo_ref.at[sl], psem.at[sl, 3]),
        ]

    def silu_c():
        c = c_ref[...].astype(F32)
        return jnp.broadcast_to(c * jax.nn.sigmoid(c), (16, M)).astype(BF16)

    @pl.when(j == 0)
    def _prologue():
        c_copy.start()
        wmoda_copy.start()
        for i in range(XC):
            x_copy(i).start()
        for cp in pair_copies(0, 0):
            cp.start()
        ckv_copy.start()
        acc_ref[...] = jnp.zeros(acc_ref.shape, F32)
        c_copy.wait()
        wmoda_copy.wait()
        mod_ref[:, 0:2 * M] = jnp.dot(silu_c(), _as_bf16(wmoda_ref[...]),
                                      preferred_element_type=F32)[0:8]
        sa = mod_ref[0:1, 0:M]
        ca1 = 1.0 + mod_ref[0:1, M:2 * M]
        for i in range(XC):
            x_copy(i).wait()

            def body(t, carry):
                r = pl.multiple_of(i * XR + t * TQ, TQ)
                rh = pl.multiple_of(i * (XR // 2) + t * HQ, HQ)
                x = x_ref[pl.ds(r, TQ), :].astype(F32)
                h_ref[pl.ds(rh, HQ), :] = _as_u32((_ln(x) * ca1 + sa).astype(BF16))
                return carry
            lax.fori_loop(0, XR // TQ, body, 0)
        ckv_copy.wait()

    @pl.when(j == 1)
    def _late_start():
        wmodb_copy.start()
        for cp in late_copies:
            cp.start()

    for cp in pair_copies(j, slot):
        cp.wait()

    @pl.when(j + 1 < NP)
    def _prefetch():
        for cp in pair_copies(j + 1, 1 - slot):
            cp.start()

    ka, kb = _split_pair(wkr_ref[slot])
    wkvp_ref[:, 0:D] = ka
    wkvp_ref[:, D:2 * D] = kb
    va, vb = _split_pair(wvr_ref[slot])
    wkvp_ref[:, 2 * D:3 * D] = va
    wkvp_ref[:, 3 * D:4 * D] = vb
    qa, qb = _split_pair(wqr_ref[slot])
    wqp_ref[:, 0:D] = qa
    wqp_ref[:, D:2 * D] = qb

    row = lax.broadcasted_iota(jnp.int32, (TQ, TQ), 0)
    col = lax.broadcasted_iota(jnp.int32, (TQ, TQ), 1)
    tri = col <= row

    def proj_kv(i):
        rows = slice(i * HQ, (i + 1) * HQ)
        kv = jnp.dot(_as_bf16(ckv_ref[rows, :]), _as_bf16(wkvp_ref[...]), preferred_element_type=F32)
        kv_ref[rows, :] = _as_u32(kv.astype(BF16))

    def proj_q(i):
        rows = slice(i * HQ, (i + 1) * HQ)
        q = jnp.dot(_as_bf16(h_ref[rows, :]), _as_bf16(wqp_ref[...]), preferred_element_type=F32)
        return (q * qscale).astype(BF16)

    def scores(q, hh, i):
        k = _as_bf16(kv_ref[0:(i + 1) * HQ, hh * D:(hh + 1) * D])
        s = lax.dot_general(q[:, hh * D:(hh + 1) * D], k, NT, preferred_element_type=F32)
        sd = jnp.where(tri, s[:, i * TQ:], NEG)
        if i > 0:
            return jnp.concatenate([s[:, :i * TQ], sd], axis=1)
        return sd

    def softmax_pv(s, hh, i):
        m = jnp.max(s, axis=1, keepdims=True)
        p = jnp.exp2(s - m)
        l = jnp.sum(p, axis=1, keepdims=True)
        v = _as_bf16(kv_ref[0:(i + 1) * HQ, (2 + hh) * D:(3 + hh) * D])
        o = jnp.dot(p.astype(BF16), v, preferred_element_type=F32)
        return (o * pl.reciprocal(l, approx=False, full_range=False)).astype(BF16)

    def oproj(ctx, i):
        rows = slice(i * TQ, (i + 1) * TQ)
        acc_ref[rows, :] += jnp.dot(ctx, _as_bf16(wo_ref[slot]), preferred_element_type=F32)

    kv_done = 0

    def need_kv(i):
        nonlocal kv_done
        while kv_done <= i:
            proj_kv(kv_done)
            kv_done += 1

    order = ORDER
    q, s, ctx = {}, {}, {}
    need_kv(order[0])
    q[0] = proj_q(order[0])
    for n in range(nq + 2):
        if n + 1 < nq:
            need_kv(order[n + 1])
            q[n + 1] = proj_q(order[n + 1])
        if n < nq:
            s[(n, 0)] = scores(q[n], 0, order[n])
        if 0 <= n - 1 < nq:
            ctx[(n - 1, 0)] = softmax_pv(s.pop((n - 1, 0)), 0, order[n - 1])
        if n < nq:
            s[(n, 1)] = scores(q.pop(n), 1, order[n])
        if 0 <= n - 1 < nq:
            ctx[(n - 1, 1)] = softmax_pv(s.pop((n - 1, 1)), 1, order[n - 1])
        if 0 <= n - 2 < nq:
            oproj(jnp.concatenate([ctx.pop((n - 2, 0)), ctx.pop((n - 2, 1))], axis=1), order[n - 2])

    @pl.when(j == NP - 1)
    def _epilogue():
        wmodb_copy.wait()
        for cp in late_copies:
            cp.wait()
        mod_ref[:, 2 * M:6 * M] = jnp.dot(silu_c(), _as_bf16(wmodb_ref[...]),
                                          preferred_element_type=F32)[0:8]
        ga = mod_ref[0:1, 2 * M:3 * M]
        sb = mod_ref[0:1, 3 * M:4 * M]
        cb1 = 1.0 + mod_ref[0:1, 4 * M:5 * M]
        t_ref[0:HALO, :] = jnp.zeros((HALO, M), F32)
        t_ref[S + HALO:S + 2 * HALO, :] = jnp.zeros((HALO, M), F32)

        def pre(t):
            rows = slice(t * TA, (t + 1) * TA)
            x1 = x_ref[rows, :].astype(F32) + ga * acc_ref[rows, :]
            acc_ref[rows, :] = x1
            h = _ln(x1) * cb1 + sb
            hb_ref[rows, :] = h
            return _ln(h).astype(BF16)

        for t in range(S // TA):
            u = pre(t)
            t_ref[HALO + t * TA:HALO + (t + 1) * TA, :] = _gelu(
                jnp.dot(u, _as_bf16(w1_ref[...]), preferred_element_type=F32))

        G = M // 4
        HB = TB // 2
        lane = lax.broadcasted_iota(jnp.int32, (TB, M), 1)

        def mm2(t, sl):
            r = t * TB if isinstance(t, int) else pl.multiple_of(t * TB, TB)
            win = t_ref[pl.ds(r, TB + 2 * HALO), :]
            g0 = win[HALO - 1:HALO - 1 + TB]
            g1 = win[HALO + 1:HALO + 1 + TB]
            g2 = win[HALO - 2:HALO - 2 + TB]
            g3 = win[HALO + 2:HALO + 2 + TB]
            sh = jnp.where(lane < 2 * G, jnp.where(lane < G, g0, g1),
                           jnp.where(lane < 3 * G, g2, g3)).astype(BF16)
            y = hb_ref[pl.ds(r, TB), :] + jnp.dot(sh, _as_bf16(w2_ref[...]), preferred_element_type=F32)
            y_ref[sl] = y
            u3_ref[sl] = _as_u32(_ln(y).astype(BF16))

        def out_copy(t, sl):
            r = t * TB if isinstance(t, int) else pl.multiple_of(t * TB, TB)
            return pltpu.make_async_copy(ob_ref.at[sl], o_hbm.at[pl.ds(r, TB), :], osem.at[sl])

        def stage_b(t, sl, nxt):
            r = t * TB if isinstance(t, int) else pl.multiple_of(t * TB, TB)
            gb = mod_ref[0:1, 5 * M:6 * M]
            f = _gelu(lax.dot_general(_as_bf16(u3_ref[sl]), _as_bf16(w3t_ref[...]), NT,
                                      preferred_element_type=F32)).astype(BF16)
            y = y_ref[sl]
            if nxt:
                mm2(t + 1, 1 - sl)
            h2 = jnp.dot(f, _as_bf16(w4_ref[...]), preferred_element_type=F32)
            ob_ref[sl] = (acc_ref[pl.ds(r, TB), :] + gb * (y + h2)).astype(ob_ref.dtype)
            out_copy(t, sl).start()

        nb = S // TB
        mm2(0, 0)

        def loop_b(t, carry):
            sl = t % 2

            @pl.when(t >= 2)
            def _():
                out_copy(t - 2, sl).wait()
            stage_b(t, sl, True)
            return carry
        lax.fori_loop(0, nb - 1, loop_b, 0)
        out_copy(nb - 3, (nb - 1) % 2).wait()
        stage_b(nb - 1, (nb - 1) % 2, False)
        out_copy(nb - 2, (nb - 2) % 2).wait()
        out_copy(nb - 1, (nb - 1) % 2).wait()


@jax.jit
def pallas_adaLN_cond__compressed_kv_cla__mixer_s_mlp__prompt_kernel(
    A_x: jax.Array,
    A_c_kv: jax.Array,
    A_w_q: jax.Array,
    A_w_uk: jax.Array,
    A_w_uv: jax.Array,
    A_w_o: jax.Array,
    B_x: jax.Array,
    B_w1: jax.Array,
    B_w2: jax.Array,
    B_w3: jax.Array,
    B_w4: jax.Array,
    c: jax.Array,
    w_mod: jax.Array,
):
    B, S, M = A_x.shape
    assert B == 1 and A_c_kv.shape[1] == S
    Dc = A_c_kv.shape[2]
    H, D = A_w_q.shape[1], A_w_q.shape[2]
    NP = H // 2
    Fd = B_w3.shape[1]
    any_spec = pl.BlockSpec(memory_space=pl.ANY)

    out = pl.pallas_call(
        functools.partial(_kernel, S=S, M=M, D=D, NP=NP),
        grid=(NP,),
        in_specs=[any_spec] * 12,
        out_specs=any_spec,
        out_shape=jax.ShapeDtypeStruct((S, M), A_x.dtype),
        scratch_shapes=[
            pltpu.VMEM((S, M), BF16),
            pltpu.VMEM((S // 2, Dc), U32),
            pltpu.VMEM((2, M, D), U32),
            pltpu.VMEM((2, Dc, D), U32),
            pltpu.VMEM((2, Dc, D), U32),
            pltpu.VMEM((2, D, M), U32),
            pltpu.VMEM((M // 2, M), U32),
            pltpu.VMEM((M // 2, M), U32),
            pltpu.VMEM((Fd // 2, M), U32),
            pltpu.VMEM((Fd // 2, M), U32),
            pltpu.VMEM((1, M), BF16),
            pltpu.VMEM((M // 2, 2 * M), U32),
            pltpu.VMEM((M // 2, 4 * M), U32),
            pltpu.VMEM((8, 6 * M), F32),
            pltpu.VMEM((S // 2, M), U32),
            pltpu.VMEM((M // 2, 2 * D), U32),
            pltpu.VMEM((Dc // 2, 4 * D), U32),
            pltpu.VMEM((S // 2, 4 * D), U32),
            pltpu.VMEM((S, M), F32),
            pltpu.VMEM((S + 2 * HALO, M), F32),
            pltpu.VMEM((S, M), F32),
            pltpu.VMEM((2, TB, M), F32),
            pltpu.VMEM((2, TB // 2, M), U32),
            pltpu.VMEM((2, TB, M), BF16),
            pltpu.SemaphoreType.DMA((XC,)),
            pltpu.SemaphoreType.DMA((8,)),
            pltpu.SemaphoreType.DMA((2, 4)),
            pltpu.SemaphoreType.DMA((2,)),
        ],
        compiler_params=pltpu.CompilerParams(
            dimension_semantics=("arbitrary",),
            vmem_limit_bytes=100 * 1024 * 1024,
        ),
    )(
        A_x.reshape(S, M), A_c_kv.reshape(S, Dc),
        A_w_q, A_w_uk, A_w_uv,
        A_w_o.reshape(H * D, M),
        B_w1, B_w2, B_w3.T, B_w4, c, w_mod,
    )
    return out.reshape(B, S, M)
```

```python
import functools
import math

import jax
import jax.numpy as jnp
from jax import lax
import jax.experimental.pallas as pl
import jax.experimental.pallas.tpu as pltpu

F32 = jnp.float32
BF16 = jnp.bfloat16
U32 = jnp.uint32
NT = (((1,), (1,)), ((), ()))
NEG = -1000000000.0
EPS = 1e-05
TQ = 128
TB = 256
XC = 4
HALO = 8
ORDER = list(range(2, 16)) + [1, 0]


def _ln(x):
    m = jnp.mean(x, axis=-1, keepdims=True)
    xc = x - m
    v = jnp.mean(xc * xc, axis=-1, keepdims=True)
    return xc * lax.rsqrt(v + EPS)


def _gelu(x):
    c = math.sqrt(2.0 / math.pi)
    return 0.5 * x * (1.0 + jnp.tanh(c * (x + 0.044715 * (x * x * x))))


def _as_bf16(u):
    return pltpu.bitcast(u, BF16)


def _as_u32(b):
    return pltpu.bitcast(b, U32)


def _split_pair(u):
    lo = pltpu.bitcast(u << 16, F32).astype(BF16)
    hi = pltpu.bitcast(u & jnp.uint32(0xFFFF0000), F32).astype(BF16)
    return _as_u32(lo), _as_u32(hi)


def _kernel(x_hbm, ckv_hbm, wq_hbm, wk_hbm, wv_hbm, wo_hbm,
            w1_hbm, w2_hbm, w3t_hbm, w4_hbm, c_hbm, wmod_hbm,
            o_hbm,
            x_ref, ckv_ref, wqr_ref, wkr_ref, wvr_ref, wo_ref,
            w1_ref, w2_ref, w3t_ref, w4_ref, c_ref, wmoda_ref, wmodb_ref,
            mod_ref, h_ref, wqp_ref, wkvp_ref, kv_ref, acc_ref,
            x1_ref, y_ref, u3_ref, ob_ref,
            xsem, ssem, psem, osem,
            *, S, M, D, NP, Fd):
    j = pl.program_id(0)
    slot = j % 2
    nq = S // TQ
    HQ = TQ // 2
    qscale = (D ** -0.5) * math.log2(math.e)
    XR = S // XC

    def x_copy(i):
        return pltpu.make_async_copy(x_hbm.at[pl.ds(i * XR, XR), :],
                                     x_ref.at[pl.ds(HALO + i * XR, XR), :], xsem.at[i])

    wmod_u = wmod_hbm.bitcast(U32)
    c_copy = pltpu.make_async_copy(c_hbm, c_ref, ssem.at[0])
    wmoda_copy = pltpu.make_async_copy(wmod_u.at[:, pl.ds(0, 2 * M)], wmoda_ref, ssem.at[1])
    ckv_copy = pltpu.make_async_copy(ckv_hbm.bitcast(U32), ckv_ref, ssem.at[2])
    wmodb_copy = pltpu.make_async_copy(wmod_u.at[:, pl.ds(2 * M, 4 * M)], wmodb_ref, ssem.at[3])
    late_copies = [
        pltpu.make_async_copy(w1_hbm.bitcast(U32), w1_ref, ssem.at[4]),
        pltpu.make_async_copy(w2_hbm.bitcast(U32), w2_ref, ssem.at[5]),
        pltpu.make_async_copy(w3t_hbm.bitcast(U32), w3t_ref, ssem.at[6]),
        pltpu.make_async_copy(w4_hbm.bitcast(U32), w4_ref, ssem.at[7]),
    ]

    def pair_copies(p, sl):
        return [
            pltpu.make_async_copy(wk_hbm.bitcast(U32).at[:, p, :], wkr_ref.at[sl], psem.at[sl, 0]),
            pltpu.make_async_copy(wv_hbm.bitcast(U32).at[:, p, :], wvr_ref.at[sl], psem.at[sl, 1]),
            pltpu.make_async_copy(wq_hbm.bitcast(U32).at[:, p, :], wqr_ref.at[sl], psem.at[sl, 2]),
            pltpu.make_async_copy(wo_hbm.bitcast(U32).at[pl.ds(pl.multiple_of(p * D, D), D), :],
                                  wo_ref.at[sl], psem.at[sl, 3]),
        ]

    def silu_c():
        c = c_ref[...].astype(F32)
        return jnp.broadcast_to(c * jax.nn.sigmoid(c), (16, M)).astype(BF16)

    @pl.when(j == 0)
    def _prologue():
        c_copy.start()
        wmoda_copy.start()
        for i in range(XC):
            x_copy(i).start()
        for cp in pair_copies(0, 0):
            cp.start()
        ckv_copy.start()
        acc_ref[...] = jnp.zeros(acc_ref.shape, F32)
        x_ref[0:HALO, :] = jnp.zeros((HALO, M), BF16)
        x_ref[S + HALO:S + 2 * HALO, :] = jnp.zeros((HALO, M), BF16)
        c_copy.wait()
        wmoda_copy.wait()
        mod_ref[:, 0:2 * M] = jnp.dot(silu_c(), _as_bf16(wmoda_ref[...]),
                                      preferred_element_type=F32)[0:8]
        sa = mod_ref[0:1, 0:M]
        ca1 = 1.0 + mod_ref[0:1, M:2 * M]
        for i in range(XC):
            x_copy(i).wait()

            def body(t, carry):
                r = pl.multiple_of(i * XR + t * TQ, TQ)
                rh = pl.multiple_of(i * (XR // 2) + t * HQ, HQ)
                x = x_ref[pl.ds(HALO + r, TQ), :].astype(F32)
                h_ref[pl.ds(rh, HQ), :] = _as_u32((_ln(x) * ca1 + sa).astype(BF16))
                return carry
            lax.fori_loop(0, XR // TQ, body, 0)
        ckv_copy.wait()

    @pl.when(j == 1)
    def _late_start():
        wmodb_copy.start()
        for cp in late_copies:
            cp.start()

    for cp in pair_copies(j, slot):
        cp.wait()

    @pl.when(j + 1 < NP)
    def _prefetch():
        for cp in pair_copies(j + 1, 1 - slot):
            cp.start()

    ka, kb = _split_pair(wkr_ref[slot])
    wkvp_ref[:, 0:D] = ka
    wkvp_ref[:, D:2 * D] = kb
    va, vb = _split_pair(wvr_ref[slot])
    wkvp_ref[:, 2 * D:3 * D] = va
    wkvp_ref[:, 3 * D:4 * D] = vb
    qa, qb = _split_pair(wqr_ref[slot])
    wqp_ref[:, 0:D] = qa
    wqp_ref[:, D:2 * D] = qb

    row = lax.broadcasted_iota(jnp.int32, (TQ, TQ), 0)
    col = lax.broadcasted_iota(jnp.int32, (TQ, TQ), 1)
    tri = col <= row

    def proj_kv(i):
        rows = slice(i * HQ, (i + 1) * HQ)
        kv = jnp.dot(_as_bf16(ckv_ref[rows, :]), _as_bf16(wkvp_ref[...]), preferred_element_type=F32)
        kv_ref[rows, :] = _as_u32(kv.astype(BF16))

    def proj_q(i):
        rows = slice(i * HQ, (i + 1) * HQ)
        q = jnp.dot(_as_bf16(h_ref[rows, :]), _as_bf16(wqp_ref[...]), preferred_element_type=F32)
        return (q * qscale).astype(BF16)

    def scores(q, hh, i):
        k = _as_bf16(kv_ref[0:(i + 1) * HQ, hh * D:(hh + 1) * D])
        s = lax.dot_general(q[:, hh * D:(hh + 1) * D], k, NT, preferred_element_type=F32)
        sd = jnp.where(tri, s[:, i * TQ:], NEG)
        if i > 0:
            return jnp.concatenate([s[:, :i * TQ], sd], axis=1)
        return sd

    def softmax_pv(s, hh, i):
        m = jnp.max(s, axis=1, keepdims=True)
        p = jnp.exp2(s - m)
        l = jnp.sum(p, axis=1, keepdims=True)
        v = _as_bf16(kv_ref[0:(i + 1) * HQ, (2 + hh) * D:(3 + hh) * D])
        o = jnp.dot(p.astype(BF16), v, preferred_element_type=F32)
        return (o * pl.reciprocal(l, approx=False, full_range=False)).astype(BF16)

    def oproj(ctx, i):
        rows = slice(HALO + i * TQ, HALO + (i + 1) * TQ)
        acc_ref[rows, :] += jnp.dot(ctx, _as_bf16(wo_ref[slot]), preferred_element_type=F32)

    kv_done = 0

    def need_kv(i):
        nonlocal kv_done
        while kv_done <= i:
            proj_kv(kv_done)
            kv_done += 1

    order = ORDER
    q, s, ctx = {}, {}, {}
    need_kv(order[0])
    q[0] = proj_q(order[0])
    for n in range(nq + 2):
        if n + 1 < nq:
            need_kv(order[n + 1])
            q[n + 1] = proj_q(order[n + 1])
        if n < nq:
            s[(n, 0)] = scores(q[n], 0, order[n])
        if 0 <= n - 1 < nq:
            ctx[(n - 1, 0)] = softmax_pv(s.pop((n - 1, 0)), 0, order[n - 1])
        if n < nq:
            s[(n, 1)] = scores(q.pop(n), 1, order[n])
        if 0 <= n - 1 < nq:
            ctx[(n - 1, 1)] = softmax_pv(s.pop((n - 1, 1)), 1, order[n - 1])
        if 0 <= n - 2 < nq:
            oproj(jnp.concatenate([ctx.pop((n - 2, 0)), ctx.pop((n - 2, 1))], axis=1), order[n - 2])

    @pl.when(j == NP - 1)
    def _epilogue():
        wmodb_copy.wait()
        for cp in late_copies:
            cp.wait()
        sc = silu_c()
        for g in range(4):
            mod_ref[:, (2 + g) * M:(3 + g) * M] = jnp.dot(
                sc, _as_bf16(wmodb_ref[:, g * M:(g + 1) * M]), preferred_element_type=F32)[0:8]

        G = M // 4
        TH = TB + 2 * HALO
        FH = (Fd // 2 + 127) // 128 * 128
        lane = lax.broadcasted_iota(jnp.int32, (TB, M), 1)
        hrow = lax.broadcasted_iota(jnp.int32, (TH, M), 0)

        def start_row(t):
            return t * TB if isinstance(t, int) else pl.multiple_of(t * TB, TB)

        def front_a(t, sl):
            r = start_row(t)
            ga = mod_ref[0:1, 2 * M:3 * M]
            sb = mod_ref[0:1, 3 * M:4 * M]
            cb1 = 1.0 + mod_ref[0:1, 4 * M:5 * M]
            x1 = x_ref[pl.ds(r, TH), :].astype(F32) + ga * acc_ref[pl.ds(r, TH), :]
            x1_ref[sl] = x1[HALO:HALO + TB]
            h = _ln(x1) * cb1 + sb
            tt = _gelu(jnp.dot(_ln(h).astype(BF16), _as_bf16(w1_ref[...]),
                               preferred_element_type=F32))
            grow = hrow + (r - HALO)
            tt = jnp.where(jnp.logical_and(grow >= 0, grow < S), tt, 0.0)
            return h[HALO:HALO + TB], tt

        def front_b(h, tt, sl):
            g0 = tt[HALO - 1:HALO - 1 + TB]
            g1 = tt[HALO + 1:HALO + 1 + TB]
            g2 = tt[HALO - 2:HALO - 2 + TB]
            g3 = tt[HALO + 2:HALO + 2 + TB]
            sh = jnp.where(lane < 2 * G, jnp.where(lane < G, g0, g1),
                           jnp.where(lane < 3 * G, g2, g3)).astype(BF16)
            y = h + jnp.dot(sh, _as_bf16(w2_ref[...]), preferred_element_type=F32)
            y_ref[sl] = y
            u3_ref[sl] = _as_u32(_ln(y).astype(BF16))

        def out_copy(t, sl):
            return pltpu.make_async_copy(ob_ref.at[sl], o_hbm.at[pl.ds(start_row(t), TB), :],
                                         osem.at[sl])

        def mm3(sl, lo, hi):
            return _gelu(lax.dot_general(_as_bf16(u3_ref[sl]), _as_bf16(w3t_ref[lo // 2:hi // 2, :]),
                                         NT, preferred_element_type=F32)).astype(BF16)

        def stage(t, sl, nxt):
            gb = mod_ref[0:1, 5 * M:6 * M]
            f0 = mm3(sl, 0, FH)
            if nxt:
                h, tt = front_a(t + 1, 1 - sl)
            f1 = mm3(sl, FH, Fd)
            if nxt:
                front_b(h, tt, 1 - sl)
            h2 = jnp.dot(jnp.concatenate([f0, f1], axis=1), _as_bf16(w4_ref[...]),
                         preferred_element_type=F32)
            ob_ref[sl] = (x1_ref[sl] + gb * (y_ref[sl] + h2)).astype(ob_ref.dtype)
            out_copy(t, sl).start()

        nb = S // TB
        front_b(*front_a(0, 0), 0)

        def loop_b(t, carry):
            sl = t % 2

            @pl.when(t >= 2)
            def _():
                out_copy(t - 2, sl).wait()
            stage(t, sl, True)
            return carry
        lax.fori_loop(0, nb - 1, loop_b, 0)
        out_copy(nb - 3, (nb - 1) % 2).wait()
        stage(nb - 1, (nb - 1) % 2, False)
        out_copy(nb - 2, (nb - 2) % 2).wait()
        out_copy(nb - 1, (nb - 1) % 2).wait()


@jax.jit
def pallas_adaLN_cond__compressed_kv_cla__mixer_s_mlp__prompt_kernel(
    A_x: jax.Array,
    A_c_kv: jax.Array,
    A_w_q: jax.Array,
    A_w_uk: jax.Array,
    A_w_uv: jax.Array,
    A_w_o: jax.Array,
    B_x: jax.Array,
    B_w1: jax.Array,
    B_w2: jax.Array,
    B_w3: jax.Array,
    B_w4: jax.Array,
    c: jax.Array,
    w_mod: jax.Array,
):
    B, S, M = A_x.shape
    assert B == 1 and A_c_kv.shape[1] == S
    Dc = A_c_kv.shape[2]
    H, D = A_w_q.shape[1], A_w_q.shape[2]
    NP = H // 2
    Fd = B_w3.shape[1]
    any_spec = pl.BlockSpec(memory_space=pl.ANY)

    out = pl.pallas_call(
        functools.partial(_kernel, S=S, M=M, D=D, NP=NP, Fd=Fd),
        grid=(NP,),
        in_specs=[any_spec] * 12,
        out_specs=any_spec,
        out_shape=jax.ShapeDtypeStruct((S, M), A_x.dtype),
        scratch_shapes=[
            pltpu.VMEM((S + 2 * HALO, M), BF16),
            pltpu.VMEM((S // 2, Dc), U32),
            pltpu.VMEM((2, M, D), U32),
            pltpu.VMEM((2, Dc, D), U32),
            pltpu.VMEM((2, Dc, D), U32),
            pltpu.VMEM((2, D, M), U32),
            pltpu.VMEM((M // 2, M), U32),
            pltpu.VMEM((M // 2, M), U32),
            pltpu.VMEM((Fd // 2, M), U32),
            pltpu.VMEM((Fd // 2, M), U32),
            pltpu.VMEM((1, M), BF16),
            pltpu.VMEM((M // 2, 2 * M), U32),
            pltpu.VMEM((M // 2, 4 * M), U32),
            pltpu.VMEM((8, 6 * M), F32),
            pltpu.VMEM((S // 2, M), U32),
            pltpu.VMEM((M // 2, 2 * D), U32),
            pltpu.VMEM((Dc // 2, 4 * D), U32),
            pltpu.VMEM((S // 2, 4 * D), U32),
            pltpu.VMEM((S + 2 * HALO, M), F32),
            pltpu.VMEM((2, TB, M), F32),
            pltpu.VMEM((2, TB, M), F32),
            pltpu.VMEM((2, TB // 2, M), U32),
            pltpu.VMEM((2, TB, M), BF16),
            pltpu.SemaphoreType.DMA((XC,)),
            pltpu.SemaphoreType.DMA((8,)),
            pltpu.SemaphoreType.DMA((2, 4)),
            pltpu.SemaphoreType.DMA((2,)),
        ],
        compiler_params=pltpu.CompilerParams(
            dimension_semantics=("arbitrary",),
            vmem_limit_bytes=100 * 1024 * 1024,
        ),
    )(
        A_x.reshape(S, M), A_c_kv.reshape(S, Dc),
        A_w_q, A_w_uk, A_w_uv,
        A_w_o.reshape(H * D, M),
        B_w1, B_w2, B_w3.T, B_w4, c, w_mod,
    )
    return out.reshape(B, S, M)
```

```python
import functools
import math

import jax
import jax.numpy as jnp
from jax import lax
import jax.experimental.pallas as pl
import jax.experimental.pallas.tpu as pltpu

F32 = jnp.float32
BF16 = jnp.bfloat16
U32 = jnp.uint32
NT = (((1,), (1,)), ((), ()))
NEG = -1000000000.0
EPS = 1e-05
TQ = 128
TB = 256
TC = 64
XC = 4
HALO = 8
ORDER = list(range(2, 16)) + [1, 0]


def _ln(x):
    m = jnp.mean(x, axis=-1, keepdims=True)
    xc = x - m
    v = jnp.mean(xc * xc, axis=-1, keepdims=True)
    return xc * lax.rsqrt(v + EPS)


def _gelu(x):
    c = math.sqrt(2.0 / math.pi)
    hx = 0.5 * x
    return hx + hx * jnp.tanh(x * (c + (c * 0.044715) * (x * x)))


def _as_bf16(u):
    return pltpu.bitcast(u, BF16)


def _as_u32(b):
    return pltpu.bitcast(b, U32)


def _split_pair(u):
    lo = pltpu.bitcast(u << 16, F32).astype(BF16)
    hi = pltpu.bitcast(u & jnp.uint32(0xFFFF0000), F32).astype(BF16)
    return _as_u32(lo), _as_u32(hi)


def _kernel(x_hbm, ckv_hbm, wq_hbm, wk_hbm, wv_hbm, wo_hbm,
            w1_hbm, w2_hbm, w3t_hbm, w4_hbm, c_hbm, wmod_hbm,
            o_hbm,
            x_ref, ckv_ref, wqr_ref, wkr_ref, wvr_ref, wo_ref,
            w1_ref, w2_ref, w3t_ref, w4_ref, c_ref, wmoda_ref, wmodb_ref,
            mod_ref, h_ref, wqp_ref, wkvp_ref, kv_ref, acc_ref,
            z_ref, u3_ref, ob_ref,
            xsem, ssem, psem, osem,
            *, S, M, D, NP, Fd):
    j = pl.program_id(0)
    slot = j % 2
    nq = S // TQ
    HQ = TQ // 2
    qscale = (D ** -0.5) * math.log2(math.e)
    XR = S // XC

    def x_copy(i):
        return pltpu.make_async_copy(x_hbm.at[pl.ds(i * XR, XR), :],
                                     x_ref.at[pl.ds(HALO + i * XR, XR), :], xsem.at[i])

    wmod_u = wmod_hbm.bitcast(U32)
    c_copy = pltpu.make_async_copy(c_hbm, c_ref, ssem.at[0])
    wmoda_copy = pltpu.make_async_copy(wmod_u.at[:, pl.ds(0, 2 * M)], wmoda_ref, ssem.at[1])
    ckv_copy = pltpu.make_async_copy(ckv_hbm.bitcast(U32), ckv_ref, ssem.at[2])
    wmodb_copy = pltpu.make_async_copy(wmod_u.at[:, pl.ds(2 * M, 4 * M)], wmodb_ref, ssem.at[3])
    late_copies = [
        pltpu.make_async_copy(w1_hbm.bitcast(U32), w1_ref, ssem.at[4]),
        pltpu.make_async_copy(w2_hbm.bitcast(U32), w2_ref, ssem.at[5]),
        pltpu.make_async_copy(w3t_hbm.bitcast(U32), w3t_ref, ssem.at[6]),
        pltpu.make_async_copy(w4_hbm.bitcast(U32), w4_ref, ssem.at[7]),
    ]

    def pair_copies(p, sl):
        return [
            pltpu.make_async_copy(wk_hbm.bitcast(U32).at[:, p, :], wkr_ref.at[sl], psem.at[sl, 0]),
            pltpu.make_async_copy(wv_hbm.bitcast(U32).at[:, p, :], wvr_ref.at[sl], psem.at[sl, 1]),
            pltpu.make_async_copy(wq_hbm.bitcast(U32).at[:, p, :], wqr_ref.at[sl], psem.at[sl, 2]),
            pltpu.make_async_copy(wo_hbm.bitcast(U32).at[pl.ds(pl.multiple_of(p * D, D), D), :],
                                  wo_ref.at[sl], psem.at[sl, 3]),
        ]

    def silu_c():
        c = c_ref[...].astype(F32)
        return jnp.broadcast_to(c * jax.nn.sigmoid(c), (16, M)).astype(BF16)

    @pl.when(j == 0)
    def _prologue():
        c_copy.start()
        wmoda_copy.start()
        for i in range(XC):
            x_copy(i).start()
        for cp in pair_copies(0, 0):
            cp.start()
        ckv_copy.start()
        acc_ref[...] = jnp.zeros(acc_ref.shape, F32)
        x_ref[0:HALO, :] = jnp.zeros((HALO, M), BF16)
        x_ref[S + HALO:S + 2 * HALO, :] = jnp.zeros((HALO, M), BF16)
        c_copy.wait()
        wmoda_copy.wait()
        mod_ref[:, 0:2 * M] = jnp.dot(silu_c(), _as_bf16(wmoda_ref[...]),
                                      preferred_element_type=F32)[0:8]
        sa = mod_ref[0:1, 0:M]
        ca1 = 1.0 + mod_ref[0:1, M:2 * M]
        for i in range(XC):
            x_copy(i).wait()

            def body(t, carry):
                r = pl.multiple_of(i * XR + t * TQ, TQ)
                rh = pl.multiple_of(i * (XR // 2) + t * HQ, HQ)
                x = x_ref[pl.ds(HALO + r, TQ), :].astype(F32)
                h_ref[pl.ds(rh, HQ), :] = _as_u32((_ln(x) * ca1 + sa).astype(BF16))
                return carry
            lax.fori_loop(0, XR // TQ, body, 0)
        ckv_copy.wait()
        wmodb_copy.start()
        for cp in late_copies:
            cp.start()

    @pl.when(j + 1 < NP)
    def _prefetch():
        for cp in pair_copies(j + 1, 1 - slot):
            cp.start()

    for cp in pair_copies(j, slot):
        cp.wait()

    ka, kb = _split_pair(wkr_ref[slot])
    wkvp_ref[:, 0:D] = ka
    wkvp_ref[:, D:2 * D] = kb
    va, vb = _split_pair(wvr_ref[slot])
    wkvp_ref[:, 2 * D:3 * D] = va
    wkvp_ref[:, 3 * D:4 * D] = vb
    qa, qb = _split_pair(wqr_ref[slot])
    wqp_ref[:, 0:D] = qa
    wqp_ref[:, D:2 * D] = qb

    row = lax.broadcasted_iota(jnp.int32, (TQ, TQ), 0)
    col = lax.broadcasted_iota(jnp.int32, (TQ, TQ), 1)
    tri = col <= row

    def proj_kv(i):
        rows = slice(i * HQ, (i + 1) * HQ)
        kv = jnp.dot(_as_bf16(ckv_ref[rows, :]), _as_bf16(wkvp_ref[...]), preferred_element_type=F32)
        kv_ref[rows, :] = _as_u32(kv.astype(BF16))

    def proj_q(i):
        rows = slice(i * HQ, (i + 1) * HQ)
        q = jnp.dot(_as_bf16(h_ref[rows, :]), _as_bf16(wqp_ref[...]), preferred_element_type=F32)
        return (q * qscale).astype(BF16)

    def scores(q, hh, i):
        k = _as_bf16(kv_ref[0:(i + 1) * HQ, hh * D:(hh + 1) * D])
        s = lax.dot_general(q[:, hh * D:(hh + 1) * D], k, NT, preferred_element_type=F32)
        sd = jnp.where(tri, s[:, i * TQ:], NEG)
        if i > 0:
            return jnp.concatenate([s[:, :i * TQ], sd], axis=1)
        return sd

    def softmax_pv(s, hh, i):
        m = jnp.max(s, axis=1, keepdims=True)
        p = jnp.exp2(s - m)
        l = jnp.sum(p, axis=1, keepdims=True)
        v = _as_bf16(kv_ref[0:(i + 1) * HQ, (2 + hh) * D:(3 + hh) * D])
        o = jnp.dot(p.astype(BF16), v, preferred_element_type=F32)
        return (o * pl.reciprocal(l, approx=False, full_range=False)).astype(BF16)

    def oproj(ctx, i):
        rows = slice(HALO + i * TQ, HALO + (i + 1) * TQ)
        acc_ref[rows, :] += jnp.dot(ctx, _as_bf16(wo_ref[slot]), preferred_element_type=F32)

    kv_done = 0

    def need_kv(i):
        nonlocal kv_done
        while kv_done <= i:
            proj_kv(kv_done)
            kv_done += 1

    order = ORDER
    q, s, ctx = {}, {}, {}
    need_kv(order[0])
    q[0] = proj_q(order[0])
    for n in range(nq + 2):
        if n + 1 < nq:
            need_kv(order[n + 1])
            q[n + 1] = proj_q(order[n + 1])
        if n < nq:
            s[(n, 0)] = scores(q[n], 0, order[n])
        if 0 <= n - 1 < nq:
            ctx[(n - 1, 0)] = softmax_pv(s.pop((n - 1, 0)), 0, order[n - 1])
        if n < nq:
            s[(n, 1)] = scores(q.pop(n), 1, order[n])
        if 0 <= n - 1 < nq:
            ctx[(n - 1, 1)] = softmax_pv(s.pop((n - 1, 1)), 1, order[n - 1])
        if 0 <= n - 2 < nq:
            oproj(jnp.concatenate([ctx.pop((n - 2, 0)), ctx.pop((n - 2, 1))], axis=1), order[n - 2])

    @pl.when(j == NP - 1)
    def _epilogue():
        wmodb_copy.wait()
        for cp in late_copies:
            cp.wait()
        sc = silu_c()
        for g in range(4):
            mod_ref[:, (2 + g) * M:(3 + g) * M] = jnp.dot(
                sc, _as_bf16(wmodb_ref[:, g * M:(g + 1) * M]), preferred_element_type=F32)[0:8]

        G = M // 4
        NC = TB // TC
        TH = TB + 2 * HALO
        hsplit = [0] + [2 * HALO + (k + 1) * TC for k in range(NC)]
        ntile = (Fd + 127) // 128
        fsplit = [min(Fd, ((k * ntile + NC - 1) // NC) * 128) for k in range(NC + 1)]

        def start_row(t):
            return t * TB if isinstance(t, int) else pl.multiple_of(t * TB, TB)

        def front_a(t, k):
            lo, hi = hsplit[k], hsplit[k + 1]
            r = start_row(t)
            ga = mod_ref[0:1, 2 * M:3 * M]
            sb = mod_ref[0:1, 3 * M:4 * M]
            cb1 = 1.0 + mod_ref[0:1, 4 * M:5 * M]
            x1 = (x_ref[pl.ds(r + lo, hi - lo), :].astype(F32)
                  + ga * acc_ref[pl.ds(r + lo, hi - lo), :])
            h = _ln(x1) * cb1 + sb
            tt = _gelu(jnp.dot(_ln(h).astype(BF16), _as_bf16(w1_ref[...]),
                               preferred_element_type=F32))
            if k == 0:
                tt = jnp.concatenate([jnp.where(r >= HALO, tt[0:HALO], 0.0), tt[HALO:]], axis=0)
            if k == NC - 1:
                n = hi - lo - HALO
                tt = jnp.concatenate([tt[:n], jnp.where(r + TB < S, tt[n:], 0.0)], axis=0)
            return x1, h, tt

        def front_b(x1, h, tt, k):
            lo = k * TC
            gb = mod_ref[0:1, 5 * M:6 * M]
            lane = lax.broadcasted_iota(jnp.int32, (TC, 128), 1)
            cols = []
            shifts = (-1, 1, -2, 2)
            for cblk in range(M // 128):
                c0, c1 = cblk * 128, (cblk + 1) * 128
                ga_, gb_ = c0 // G, (c1 - 1) // G
                a = tt[HALO + lo + shifts[ga_]:HALO + lo + shifts[ga_] + TC, c0:c1]
                if gb_ != ga_:
                    b = tt[HALO + lo + shifts[gb_]:HALO + lo + shifts[gb_] + TC, c0:c1]
                    a = jnp.where(lane < gb_ * G - c0, a, b)
                cols.append(a.astype(BF16))
            sh = jnp.concatenate(cols, axis=1)
            y = h[HALO + lo:HALO + lo + TC] + jnp.dot(sh, _as_bf16(w2_ref[...]),
                                                      preferred_element_type=F32)
            z_ref[lo:lo + TC, :] = x1[HALO + lo:HALO + lo + TC] + gb * y
            u3_ref[lo // 2:(lo + TC) // 2, :] = _as_u32(_ln(y).astype(BF16))

        def out_copy(t):
            rows = pl.ds(start_row(t), TB)
            return pltpu.make_async_copy(ob_ref.at[rows, :], o_hbm.at[rows, :], osem.at[t])

        def mm3(k):
            lo, hi = fsplit[k], fsplit[k + 1]
            return _gelu(lax.dot_general(_as_bf16(u3_ref[...]), _as_bf16(w3t_ref[lo // 2:hi // 2, :]),
                                         NT, preferred_element_type=F32)).astype(BF16)

        def mm4(t, f, z, k):
            lo = k * TC
            gb = mod_ref[0:1, 5 * M:6 * M]
            h2 = jnp.dot(f[lo:lo + TC], _as_bf16(w4_ref[...]), preferred_element_type=F32)
            ob_ref[pl.ds(start_row(t) + lo, TC), :] = (z + gb * h2).astype(ob_ref.dtype)

        def stage(t, cur, nxt):
            fs, fr = [], []
            for k in range(NC):
                if cur:
                    fs.append(mm3(k))
                if nxt:
                    fr.append(front_a(t + 1, k))
            if cur:
                f = jnp.concatenate(fs, axis=1)
            if nxt:
                fr = [jnp.concatenate(parts, axis=0) for parts in zip(*fr)]
            for k in range(NC):
                if cur:
                    z = z_ref[k * TC:(k + 1) * TC, :]
                if nxt and k == NC - 1:
                    front_b(*fr, k)
                if cur:
                    mm4(t, f, z, k)
                if nxt and k < NC - 1:
                    front_b(*fr, k)
            if cur:
                out_copy(t).start()

        nb = S // TB
        stage(-1, False, True)

        def loop_b(t, carry):
            stage(t, True, True)
            return carry
        lax.fori_loop(0, nb - 1, loop_b, 0)
        stage(nb - 1, True, False)
        for t in range(nb):
            out_copy(t).wait()


@jax.jit
def pallas_adaLN_cond__compressed_kv_cla__mixer_s_mlp__prompt_kernel(
    A_x: jax.Array,
    A_c_kv: jax.Array,
    A_w_q: jax.Array,
    A_w_uk: jax.Array,
    A_w_uv: jax.Array,
    A_w_o: jax.Array,
    B_x: jax.Array,
    B_w1: jax.Array,
    B_w2: jax.Array,
    B_w3: jax.Array,
    B_w4: jax.Array,
    c: jax.Array,
    w_mod: jax.Array,
):
    B, S, M = A_x.shape
    assert B == 1 and A_c_kv.shape[1] == S
    Dc = A_c_kv.shape[2]
    H, D = A_w_q.shape[1], A_w_q.shape[2]
    NP = H // 2
    Fd = B_w3.shape[1]
    any_spec = pl.BlockSpec(memory_space=pl.ANY)

    out = pl.pallas_call(
        functools.partial(_kernel, S=S, M=M, D=D, NP=NP, Fd=Fd),
        grid=(NP,),
        in_specs=[any_spec] * 12,
        out_specs=any_spec,
        out_shape=jax.ShapeDtypeStruct((S, M), A_x.dtype),
        scratch_shapes=[
            pltpu.VMEM((S + 2 * HALO, M), BF16),
            pltpu.VMEM((S // 2, Dc), U32),
            pltpu.VMEM((2, M, D), U32),
            pltpu.VMEM((2, Dc, D), U32),
            pltpu.VMEM((2, Dc, D), U32),
            pltpu.VMEM((2, D, M), U32),
            pltpu.VMEM((M // 2, M), U32),
            pltpu.VMEM((M // 2, M), U32),
            pltpu.VMEM((Fd // 2, M), U32),
            pltpu.VMEM((Fd // 2, M), U32),
            pltpu.VMEM((1, M), BF16),
            pltpu.VMEM((M // 2, 2 * M), U32),
            pltpu.VMEM((M // 2, 4 * M), U32),
            pltpu.VMEM((8, 6 * M), F32),
            pltpu.VMEM((S // 2, M), U32),
            pltpu.VMEM((M // 2, 2 * D), U32),
            pltpu.VMEM((Dc // 2, 4 * D), U32),
            pltpu.VMEM((S // 2, 4 * D), U32),
            pltpu.VMEM((S + 2 * HALO, M), F32),
            pltpu.VMEM((TB, M), F32),
            pltpu.VMEM((TB // 2, M), U32),
            pltpu.VMEM((S, M), BF16),
            pltpu.SemaphoreType.DMA((XC,)),
            pltpu.SemaphoreType.DMA((8,)),
            pltpu.SemaphoreType.DMA((2, 4)),
            pltpu.SemaphoreType.DMA((S // TB,)),
        ],
        compiler_params=pltpu.CompilerParams(
            dimension_semantics=("arbitrary",),
            vmem_limit_bytes=100 * 1024 * 1024,
            disable_bounds_checks=True,
        ),
    )(
        A_x.reshape(S, M), A_c_kv.reshape(S, Dc),
        A_w_q, A_w_uk, A_w_uv,
        A_w_o.reshape(H * D, M),
        B_w1, B_w2, B_w3.T, B_w4, c, w_mod,
    )
    return out.reshape(B, S, M)
```

```python
import functools
import math

import jax
import jax.numpy as jnp
from jax import lax
import jax.experimental.pallas as pl
import jax.experimental.pallas.tpu as pltpu

F32 = jnp.float32
BF16 = jnp.bfloat16
U32 = jnp.uint32
NT = (((1,), (1,)), ((), ()))
NEG = -1000000000.0
EPS = 1e-05
TQ = 128
TB = 256
TC = 64
KP = 2
TK = 256
NL = 4
HALO = 8
ORDER = list(range(2, 16)) + [1, 0]


def _ln(x):
    m = jnp.mean(x, axis=-1, keepdims=True)
    xc = x - m
    v = jnp.mean(xc * xc, axis=-1, keepdims=True)
    return xc * lax.rsqrt(v + EPS)


def _gelu(x):
    c = math.sqrt(2.0 / math.pi)
    hx = 0.5 * x
    return hx + hx * jnp.tanh(x * (c + (c * 0.044715) * (x * x)))


def _as_bf16(u):
    return pltpu.bitcast(u, BF16)


def _as_u32(b):
    return pltpu.bitcast(b, U32)


def _split_pair(u):
    lo = pltpu.bitcast(u << 16, F32).astype(BF16)
    hi = pltpu.bitcast(u & jnp.uint32(0xFFFF0000), F32).astype(BF16)
    return _as_u32(lo), _as_u32(hi)


def _after(lhs, dep, zero):
    t = None
    for r in range(0, dep.shape[0], 8):
        for c in range(0, dep.shape[1], 128):
            tile = dep[r:r + 8, c:c + 128]
            t = tile if t is None else t | tile
    head = jnp.concatenate([lhs[0:8, 0:128] | (t & zero), lhs[0:8, 128:]], axis=1)
    return jnp.concatenate([head, lhs[8:]], axis=0)


def _kernel(x_hbm, ckv_hbm, wq_hbm, wk_hbm, wv_hbm, wo_hbm,
            w1_hbm, w2_hbm, w3t_hbm, w4_hbm, c_hbm, wmod_hbm,
            o_hbm,
            x_ref, ckv_ref, wqr_ref, wkr_ref, wvr_ref, wo_ref,
            w1_ref, w2_ref, w3t_ref, w4_ref, c_ref, wmod_ref,
            mod_ref, h_ref, wqp_ref, wkp_ref, wvp_ref, k_ref, v_ref, acc_ref,
            z_ref, u3_ref, ob_ref,
            ssem, ksem, psem, osem,
            *, S, M, D, NP, Fd):
    step = pl.program_id(0)
    NK = NP // KP
    nq = S // TQ
    HQ = TQ // 2
    qscale = (D ** -0.5) * math.log2(math.e)
    LR = S // NL

    ckv_copy = pltpu.make_async_copy(ckv_hbm.bitcast(U32), ckv_ref, ssem.at[0])
    mid_copies = [
        pltpu.make_async_copy(c_hbm, c_ref, ssem.at[1]),
        pltpu.make_async_copy(wmod_hbm.bitcast(U32), wmod_ref, ssem.at[2]),
        pltpu.make_async_copy(x_hbm, x_ref.at[pl.ds(HALO, S), :], ssem.at[3]),
    ]
    late_copies = [
        pltpu.make_async_copy(w1_hbm.bitcast(U32), w1_ref, ssem.at[4]),
        pltpu.make_async_copy(w2_hbm.bitcast(U32), w2_ref, ssem.at[5]),
        pltpu.make_async_copy(w3t_hbm.bitcast(U32), w3t_ref, ssem.at[6]),
        pltpu.make_async_copy(w4_hbm.bitcast(U32), w4_ref, ssem.at[7]),
    ]

    def wk_copy(p):
        return pltpu.make_async_copy(wk_hbm.bitcast(U32).at[:, p, :], wkr_ref.at[p], ksem.at[p])

    def pair_copies(p, sl):
        return [
            pltpu.make_async_copy(wv_hbm.bitcast(U32).at[:, p, :], wvr_ref.at[sl], psem.at[sl, 0]),
            pltpu.make_async_copy(wq_hbm.bitcast(U32).at[:, p, :], wqr_ref.at[sl], psem.at[sl, 1]),
            pltpu.make_async_copy(wo_hbm.bitcast(U32).at[pl.ds(pl.multiple_of(p * D, D), D), :],
                                  wo_ref.at[sl], psem.at[sl, 2]),
        ]

    @pl.when(step == 0)
    def _prologue():
        for p in range(KP):
            wk_copy(p).start()
        ckv_copy.start()
        for p in range(KP, NP):
            wk_copy(p).start()
        for cp in mid_copies:
            cp.start()
        x_ref[0:HALO, :] = jnp.zeros((HALO, M), BF16)
        x_ref[S + HALO:, :] = jnp.zeros((HALO + LR, M), BF16)
        mod_ref[...] = jnp.zeros(mod_ref.shape, F32)

        def zero_acc(t, carry):
            acc_ref[pl.ds(pl.multiple_of(t * 16, 16), 16), :] = jnp.zeros((16, M), F32)
            return carry
        lax.fori_loop(0, (S + 2 * HALO) // 16, zero_acc, 0)
        ckv_copy.wait()

    @pl.when(step == NK - NL)
    def _modulation():
        for cp in mid_copies:
            cp.wait()
        for cp in pair_copies(0, 0):
            cp.start()
        for cp in late_copies:
            cp.start()
        c = c_ref[...].astype(F32)
        sc = jnp.broadcast_to(c * jax.nn.sigmoid(c), (16, M)).astype(BF16)
        mod_ref[...] = jnp.dot(sc, _as_bf16(wmod_ref[...]), preferred_element_type=F32)[0:8]

    @pl.when(step < NK)
    def _keys():
        for u in range(KP):
            wk_copy(step * KP + u).wait()
        for u in range(KP):
            ka, kb = _split_pair(wkr_ref[step * KP + u])
            wkp_ref[:, 2 * u * D:(2 * u + 1) * D] = ka
            wkp_ref[:, (2 * u + 1) * D:(2 * u + 2) * D] = kb
        lblk = jnp.where(step >= NK - NL, step - (NK - NL), NL)
        xoff = jnp.where(step >= NK - NL, HALO, 2 * HALO)
        sa = mod_ref[0:1, 0:M]
        ca1 = 1.0 + mod_ref[0:1, M:2 * M]
        zero = pltpu.bitcast(acc_ref[0:8, 0:128], U32)
        nk = S // TK
        lc = LR // nk
        hu = None
        for i in range(nk):
            rows = slice(i * TK // 2, (i + 1) * TK // 2)
            lhs = ckv_ref[rows, :]
            if hu is not None:
                lhs = _after(lhs, hu, zero)
            k = jnp.dot(_as_bf16(lhs), _as_bf16(wkp_ref[...]), preferred_element_type=F32)
            ku = _as_u32(k.astype(BF16))
            for u in range(KP):
                k_ref[step * KP + u, rows, :] = ku[:, 2 * u * D:(2 * u + 2) * D]
            r = pl.multiple_of(lblk * LR + i * lc + xoff, 8)
            rh = pl.multiple_of(lblk * (LR // 2) + i * (lc // 2), 8)
            x = x_ref[pl.ds(r, lc), :].astype(F32)
            hu = _as_u32((_ln(x) * ca1 + sa).astype(BF16))
            h_ref[pl.ds(rh, lc // 2), :] = hu

    @pl.when(step >= NK)
    def _attention():
        j = step - NK
        slot = j % 2

        @pl.when(j + 1 < NP)
        def _prefetch():
            for cp in pair_copies(j + 1, 1 - slot):
                cp.start()

        for cp in pair_copies(j, slot):
            cp.wait()

        qa, qb = _split_pair(wqr_ref[slot])
        wqp_ref[:, 0:D] = qa
        wqp_ref[:, D:2 * D] = qb
        va, vb = _split_pair(wvr_ref[slot])
        wvp_ref[:, 0:D] = va
        wvp_ref[:, D:2 * D] = vb

        row = lax.broadcasted_iota(jnp.int32, (TQ, TQ), 0)
        col = lax.broadcasted_iota(jnp.int32, (TQ, TQ), 1)
        tri = col <= row

        def proj_v(i):
            rows = slice(i * HQ, (i + 1) * HQ)
            v = jnp.dot(_as_bf16(ckv_ref[rows, :]), _as_bf16(wvp_ref[...]), preferred_element_type=F32)
            v_ref[rows, :] = _as_u32(v.astype(BF16))

        def proj_q(i):
            rows = slice(i * HQ, (i + 1) * HQ)
            q = jnp.dot(_as_bf16(h_ref[rows, :]), _as_bf16(wqp_ref[...]), preferred_element_type=F32)
            return (q * qscale).astype(BF16)

        def scores(q, hh, i):
            k = _as_bf16(k_ref[j, 0:(i + 1) * HQ, hh * D:(hh + 1) * D])
            s = lax.dot_general(q[:, hh * D:(hh + 1) * D], k, NT, preferred_element_type=F32)
            sd = jnp.where(tri, s[:, i * TQ:], NEG)
            if i > 0:
                return jnp.concatenate([s[:, :i * TQ], sd], axis=1)
            return sd

        def softmax_pv(s, hh, i):
            m = jnp.max(s, axis=1, keepdims=True)
            p = jnp.exp2(s - m)
            l = jnp.sum(p, axis=1, keepdims=True)
            v = _as_bf16(v_ref[0:(i + 1) * HQ, hh * D:(hh + 1) * D])
            o = jnp.dot(p.astype(BF16), v, preferred_element_type=F32)
            return (o * pl.reciprocal(l, approx=False, full_range=False)).astype(BF16)

        def oproj(ctx, i):
            rows = slice(HALO + i * TQ, HALO + (i + 1) * TQ)
            acc_ref[rows, :] += jnp.dot(ctx, _as_bf16(wo_ref[slot]), preferred_element_type=F32)

        v_done = 0

        def need_v(i):
            nonlocal v_done
            while v_done <= i:
                proj_v(v_done)
                v_done += 1

        order = ORDER
        q, s, ctx = {}, {}, {}
        q[0] = proj_q(order[0])
        for n in range(nq + 2):
            if n + 1 < nq:
                q[n + 1] = proj_q(order[n + 1])
            if n < nq:
                need_v(order[n])
                s[(n, 0)] = scores(q[n], 0, order[n])
            if 0 <= n - 1 < nq:
                ctx[(n - 1, 0)] = softmax_pv(s.pop((n - 1, 0)), 0, order[n - 1])
            if n < nq:
                s[(n, 1)] = scores(q.pop(n), 1, order[n])
            if 0 <= n - 1 < nq:
                ctx[(n - 1, 1)] = softmax_pv(s.pop((n - 1, 1)), 1, order[n - 1])
            if 0 <= n - 2 < nq:
                oproj(jnp.concatenate([ctx.pop((n - 2, 0)), ctx.pop((n - 2, 1))], axis=1),
                      order[n - 2])

    @pl.when(step == NK + NP - 1)
    def _epilogue():
        for cp in late_copies:
            cp.wait()

        G = M // 4
        NC = TB // TC
        TH = TB + 2 * HALO
        hsplit = [0] + [2 * HALO + (k + 1) * TC for k in range(NC)]
        ntile = (Fd + 127) // 128
        fsplit = [min(Fd, ((k * ntile + NC - 1) // NC) * 128) for k in range(NC + 1)]

        def start_row(t):
            return t * TB if isinstance(t, int) else pl.multiple_of(t * TB, TB)

        def front_a(t, k):
            lo, hi = hsplit[k], hsplit[k + 1]
            r = start_row(t)
            ga = mod_ref[0:1, 2 * M:3 * M]
            sb = mod_ref[0:1, 3 * M:4 * M]
            cb1 = 1.0 + mod_ref[0:1, 4 * M:5 * M]
            x1 = (x_ref[pl.ds(r + lo, hi - lo), :].astype(F32)
                  + ga * acc_ref[pl.ds(r + lo, hi - lo), :])
            h = _ln(x1) * cb1 + sb
            tt = _gelu(jnp.dot(_ln(h).astype(BF16), _as_bf16(w1_ref[...]),
                               preferred_element_type=F32))
            if k == 0:
                tt = jnp.concatenate([jnp.where(r >= HALO, tt[0:HALO], 0.0), tt[HALO:]], axis=0)
            if k == NC - 1:
                n = hi - lo - HALO
                tt = jnp.concatenate([tt[:n], jnp.where(r + TB < S, tt[n:], 0.0)], axis=0)
            return x1, h, tt

        def front_b(x1, h, tt, k):
            lo = k * TC
            gb = mod_ref[0:1, 5 * M:6 * M]
            lane = lax.broadcasted_iota(jnp.int32, (TC, 128), 1)
            cols = []
            shifts = (-1, 1, -2, 2)
            for cblk in range(M // 128):
                c0, c1 = cblk * 128, (cblk + 1) * 128
                ga_, gb_ = c0 // G, (c1 - 1) // G
                a = tt[HALO + lo + shifts[ga_]:HALO + lo + shifts[ga_] + TC, c0:c1]
                if gb_ != ga_:
                    b = tt[HALO + lo + shifts[gb_]:HALO + lo + shifts[gb_] + TC, c0:c1]
                    a = jnp.where(lane < gb_ * G - c0, a, b)
                cols.append(a.astype(BF16))
            sh = jnp.concatenate(cols, axis=1)
            y = h[HALO + lo:HALO + lo + TC] + jnp.dot(sh, _as_bf16(w2_ref[...]),
                                                      preferred_element_type=F32)
            z_ref[lo:lo + TC, :] = x1[HALO + lo:HALO + lo + TC] + gb * y
            u3_ref[lo // 2:(lo + TC) // 2, :] = _as_u32(_ln(y).astype(BF16))

        def out_copy(t):
            rows = pl.ds(start_row(t), TB)
            return pltpu.make_async_copy(ob_ref.at[rows, :], o_hbm.at[rows, :], osem.at[t])

        def mm3(k):
            lo, hi = fsplit[k], fsplit[k + 1]
            return _gelu(lax.dot_general(_as_bf16(u3_ref[...]), _as_bf16(w3t_ref[lo // 2:hi // 2, :]),
                                         NT, preferred_element_type=F32)).astype(BF16)

        def mm4(t, f, z, k):
            lo = k * TC
            gb = mod_ref[0:1, 5 * M:6 * M]
            h2 = jnp.dot(f[lo:lo + TC], _as_bf16(w4_ref[...]), preferred_element_type=F32)
            ob_ref[pl.ds(start_row(t) + lo, TC), :] = (z + gb * h2).astype(ob_ref.dtype)

        def stage(t, cur, nxt):
            fs, fr = [], []
            for k in range(NC):
                if cur:
                    fs.append(mm3(k))
                if nxt:
                    fr.append(front_a(t + 1, k))
            if cur:
                f = jnp.concatenate(fs, axis=1)
            if nxt:
                fr = [jnp.concatenate(parts, axis=0) for parts in zip(*fr)]
            for k in range(NC):
                if cur:
                    z = z_ref[k * TC:(k + 1) * TC, :]
                if nxt and k == NC - 1:
                    front_b(*fr, k)
                if cur:
                    mm4(t, f, z, k)
                if nxt and k < NC - 1:
                    front_b(*fr, k)
            if cur:
                out_copy(t).start()

        nb = S // TB
        stage(-1, False, True)

        def loop_b(t, carry):
            stage(t, True, True)
            return carry
        lax.fori_loop(0, nb - 1, loop_b, 0)
        stage(nb - 1, True, False)
        for t in range(nb):
            out_copy(t).wait()


@jax.jit
def pallas_adaLN_cond__compressed_kv_cla__mixer_s_mlp__prompt_kernel(
    A_x: jax.Array,
    A_c_kv: jax.Array,
    A_w_q: jax.Array,
    A_w_uk: jax.Array,
    A_w_uv: jax.Array,
    A_w_o: jax.Array,
    B_x: jax.Array,
    B_w1: jax.Array,
    B_w2: jax.Array,
    B_w3: jax.Array,
    B_w4: jax.Array,
    c: jax.Array,
    w_mod: jax.Array,
):
    B, S, M = A_x.shape
    assert B == 1 and A_c_kv.shape[1] == S
    Dc = A_c_kv.shape[2]
    H, D = A_w_q.shape[1], A_w_q.shape[2]
    NP = H // 2
    Fd = B_w3.shape[1]
    any_spec = pl.BlockSpec(memory_space=pl.ANY)

    out = pl.pallas_call(
        functools.partial(_kernel, S=S, M=M, D=D, NP=NP, Fd=Fd),
        grid=(NP // KP + NP,),
        in_specs=[any_spec] * 12,
        out_specs=any_spec,
        out_shape=jax.ShapeDtypeStruct((S, M), A_x.dtype),
        scratch_shapes=[
            pltpu.VMEM((S + 2 * HALO + S // NL, M), BF16),
            pltpu.VMEM((S // 2, Dc), U32),
            pltpu.VMEM((2, M, D), U32),
            pltpu.VMEM((NP, Dc, D), U32),
            pltpu.VMEM((2, Dc, D), U32),
            pltpu.VMEM((2, D, M), U32),
            pltpu.VMEM((M // 2, M), U32),
            pltpu.VMEM((M // 2, M), U32),
            pltpu.VMEM((Fd // 2, M), U32),
            pltpu.VMEM((Fd // 2, M), U32),
            pltpu.VMEM((1, M), BF16),
            pltpu.VMEM((M // 2, 6 * M), U32),
            pltpu.VMEM((8, 6 * M), F32),
            pltpu.VMEM(((S + S // NL) // 2, M), U32),
            pltpu.VMEM((M // 2, 2 * D), U32),
            pltpu.VMEM((Dc // 2, 2 * KP * D), U32),
            pltpu.VMEM((Dc // 2, 2 * D), U32),
            pltpu.VMEM((NP, S // 2, 2 * D), U32),
            pltpu.VMEM((S // 2, 2 * D), U32),
            pltpu.VMEM((S + 2 * HALO, M), F32),
            pltpu.VMEM((TB, M), F32),
            pltpu.VMEM((TB // 2, M), U32),
            pltpu.VMEM((S, M), BF16),
            pltpu.SemaphoreType.DMA((8,)),
            pltpu.SemaphoreType.DMA((NP,)),
            pltpu.SemaphoreType.DMA((2, 3)),
            pltpu.SemaphoreType.DMA((S // TB,)),
        ],
        compiler_params=pltpu.CompilerParams(
            dimension_semantics=("arbitrary",),
            vmem_limit_bytes=100 * 1024 * 1024,
            disable_bounds_checks=True,
        ),
    )(
        A_x.reshape(S, M), A_c_kv.reshape(S, Dc),
        A_w_q, A_w_uk, A_w_uv,
        A_w_o.reshape(H * D, M),
        B_w1, B_w2, B_w3.T, B_w4, c, w_mod,
    )
    return out.reshape(B, S, M)
```

```python
import functools
import math

import jax
import jax.numpy as jnp
from jax import lax
import jax.experimental.pallas as pl
import jax.experimental.pallas.tpu as pltpu

F32 = jnp.float32
BF16 = jnp.bfloat16
U32 = jnp.uint32
NT = (((1,), (1,)), ((), ()))
NEG = -1000000000.0
EPS = 1e-05
TQ = 128
TB = 256
TC = 64
KP = 2
TK = 256
NL = 4
HALO = 8


def _ln(x):
    m = jnp.mean(x, axis=-1, keepdims=True)
    xc = x - m
    v = jnp.mean(xc * xc, axis=-1, keepdims=True)
    return xc * lax.rsqrt(v + EPS)


def _gelu(x):
    c = math.sqrt(2.0 / math.pi)
    hx = 0.5 * x
    return hx + hx * jnp.tanh(x * (c + (c * 0.044715) * (x * x)))


def _as_bf16(u):
    return pltpu.bitcast(u, BF16)


def _as_u32(b):
    return pltpu.bitcast(b, U32)


def _split_pair(u):
    lo = pltpu.bitcast(u << 16, F32).astype(BF16)
    hi = pltpu.bitcast(u & jnp.uint32(0xFFFF0000), F32).astype(BF16)
    return _as_u32(lo), _as_u32(hi)


def _attention_schedule(nq):
    order = list(range(nq - 1, -1, -1))
    ops = [("q", order[0])]
    for n in range(nq + 2):
        if n < nq:
            ops.append(("s", order[n], 0))
        if 0 <= n - 1 < nq:
            ops.append(("pv", order[n - 1], 0))
        if n + 1 < nq:
            ops.append(("q", order[n + 1]))
        if n == 0:
            ops.extend(("v", i) for i in range(nq))
        if n < nq:
            ops.append(("s", order[n], 1))
        if 0 <= n - 1 < nq:
            ops.append(("pv", order[n - 1], 1))
        if 0 <= n - 2 < nq:
            ops.append(("o", order[n - 2]))
    return ops


def _after(lhs, dep, zero):
    t = None
    for r in range(0, dep.shape[0], 8):
        for c in range(0, dep.shape[1], 128):
            tile = dep[r:r + 8, c:c + 128]
            t = tile if t is None else t | tile
    head = lhs[0:8, 0:128] | (t & zero)
    if lhs.shape[1] > 128:
        head = jnp.concatenate([head, lhs[0:8, 128:]], axis=1)
    return jnp.concatenate([head, lhs[8:]], axis=0)


def _kernel(x_hbm, ckv_hbm, wq_hbm, wk_hbm, wv_hbm, wo_hbm,
            w1_hbm, w2_hbm, w3t_hbm, w4_hbm, c_hbm, wmod_hbm,
            o_hbm,
            x_ref, ckv_ref, wqr_ref, wkr_ref, wvr_ref, wo_ref,
            w1_ref, w2_ref, w3t_ref, w4_ref, c_ref, wmod_ref,
            mod_ref, h_ref, wqp_ref, wkp_ref, wvp_ref, k_ref, v_ref, acc_ref,
            z_ref, u3_ref, ob_ref,
            ssem, ksem, psem, osem,
            *, S, M, D, NP, Fd):
    step = pl.program_id(0)
    NK = NP // KP
    nq = S // TQ
    HQ = TQ // 2
    qscale = (D ** -0.5) * math.log2(math.e)
    LR = S // NL

    ckv_copy = pltpu.make_async_copy(ckv_hbm.bitcast(U32), ckv_ref, ssem.at[0])
    mid_copies = [
        pltpu.make_async_copy(c_hbm, c_ref, ssem.at[1]),
        pltpu.make_async_copy(wmod_hbm.bitcast(U32), wmod_ref, ssem.at[2]),
        pltpu.make_async_copy(x_hbm, x_ref.at[pl.ds(HALO, S), :], ssem.at[3]),
    ]
    late_copies = [
        pltpu.make_async_copy(w1_hbm.bitcast(U32), w1_ref, ssem.at[4]),
        pltpu.make_async_copy(w2_hbm.bitcast(U32), w2_ref, ssem.at[5]),
        pltpu.make_async_copy(w3t_hbm.bitcast(U32), w3t_ref, ssem.at[6]),
        pltpu.make_async_copy(w4_hbm.bitcast(U32), w4_ref, ssem.at[7]),
    ]

    def wk_copy(p):
        return pltpu.make_async_copy(wk_hbm.bitcast(U32).at[:, p, :], wkr_ref.at[p], ksem.at[p])

    def pair_copies(p, sl):
        return [
            pltpu.make_async_copy(wv_hbm.bitcast(U32).at[:, p, :], wvr_ref.at[sl], psem.at[sl, 0]),
            pltpu.make_async_copy(wq_hbm.bitcast(U32).at[:, p, :], wqr_ref.at[sl], psem.at[sl, 1]),
            pltpu.make_async_copy(wo_hbm.bitcast(U32).at[pl.ds(pl.multiple_of(p * D, D), D), :],
                                  wo_ref.at[sl], psem.at[sl, 2]),
        ]

    @pl.when(step == 0)
    def _prologue():
        for p in range(KP):
            wk_copy(p).start()
        ckv_copy.start()
        for p in range(KP, NP):
            wk_copy(p).start()
        for cp in mid_copies:
            cp.start()
        x_ref[0:HALO, :] = jnp.zeros((HALO, M), BF16)
        x_ref[S + HALO:, :] = jnp.zeros((HALO + LR, M), BF16)
        mod_ref[...] = jnp.zeros(mod_ref.shape, F32)

        def zero_acc(t, carry):
            acc_ref[pl.ds(pl.multiple_of(t * 16, 16), 16), :] = jnp.zeros((16, M), F32)
            return carry
        lax.fori_loop(0, (S + 2 * HALO) // 16, zero_acc, 0)
        ckv_copy.wait()

    @pl.when(step == NK - NL)
    def _modulation():
        for cp in mid_copies:
            cp.wait()
        for cp in pair_copies(0, 0):
            cp.start()
        for cp in late_copies:
            cp.start()
        c = c_ref[...].astype(F32)
        sc = jnp.broadcast_to(c * jax.nn.sigmoid(c), (16, M)).astype(BF16)
        mod_ref[...] = jnp.dot(sc, _as_bf16(wmod_ref[...]), preferred_element_type=F32)[0:8]

    @pl.when(step < NK)
    def _keys():
        for u in range(KP):
            wk_copy(step * KP + u).wait()
        for u in range(KP):
            ka, kb = _split_pair(wkr_ref[step * KP + u])
            wkp_ref[:, 2 * u * D:(2 * u + 1) * D] = ka
            wkp_ref[:, (2 * u + 1) * D:(2 * u + 2) * D] = kb
        lblk = jnp.where(step >= NK - NL, step - (NK - NL), NL)
        xoff = jnp.where(step >= NK - NL, HALO, 2 * HALO)
        sa = mod_ref[0:1, 0:M]
        ca1 = 1.0 + mod_ref[0:1, M:2 * M]
        zero = pltpu.bitcast(acc_ref[0:8, 0:128], U32)
        nk = S // TK
        lc = LR // nk
        hu = None
        for i in range(nk):
            rows = slice(i * TK // 2, (i + 1) * TK // 2)
            lhs = ckv_ref[rows, :]
            if hu is not None:
                lhs = _after(lhs, hu, zero)
            k = jnp.dot(_as_bf16(lhs), _as_bf16(wkp_ref[...]), preferred_element_type=F32)
            ku = _as_u32(k.astype(BF16))
            for u in range(KP):
                k_ref[step * KP + u, rows, :] = ku[:, 2 * u * D:(2 * u + 2) * D]
            r = pl.multiple_of(lblk * LR + i * lc + xoff, 8)
            rh = pl.multiple_of(lblk * (LR // 2) + i * (lc // 2), 8)
            x = x_ref[pl.ds(r, lc), :].astype(F32)
            hu = _as_u32((_ln(x) * ca1 + sa).astype(BF16))
            h_ref[pl.ds(rh, lc // 2), :] = hu

    @pl.when(step >= NK)
    def _attention():
        j = step - NK
        slot = j % 2

        @pl.when(j + 1 < NP)
        def _prefetch():
            for cp in pair_copies(j + 1, 1 - slot):
                cp.start()

        for cp in pair_copies(j, slot):
            cp.wait()

        qa, qb = _split_pair(wqr_ref[slot])
        wqp_ref[:, 0:D] = qa
        wqp_ref[:, D:2 * D] = qb
        va, vb = _split_pair(wvr_ref[slot])
        wvp_ref[:, 0:D] = va
        wvp_ref[:, D:2 * D] = vb

        row = lax.broadcasted_iota(jnp.int32, (TQ, TQ), 0)
        col = lax.broadcasted_iota(jnp.int32, (TQ, TQ), 1)
        tri = col <= row

        def proj_v(i):
            rows = slice(i * HQ, (i + 1) * HQ)
            v = jnp.dot(_as_bf16(ckv_ref[rows, :]), _as_bf16(wvp_ref[...]), preferred_element_type=F32)
            v_ref[rows, :] = _as_u32(v.astype(BF16))

        def proj_q(i):
            rows = slice(i * HQ, (i + 1) * HQ)
            q = jnp.dot(_as_bf16(h_ref[rows, :]), _as_bf16(wqp_ref[...]), preferred_element_type=F32)
            q = q * qscale
            return [q[:, 0:D].astype(BF16), q[:, D:2 * D].astype(BF16)]

        def scores(q, hh, i):
            k = _as_bf16(k_ref[j, 0:(i + 1) * HQ, hh * D:(hh + 1) * D])
            s = lax.dot_general(q[hh], k, NT, preferred_element_type=F32)
            sd = jnp.where(tri, s[:, i * TQ:], NEG)
            if i > 0:
                return jnp.concatenate([s[:, :i * TQ], sd], axis=1)
            return sd

        def softmax_pv(s, hh, i):
            m = jnp.max(s, axis=1, keepdims=True)
            p = jnp.exp2(s - m).astype(BF16)
            l = jnp.sum(p.astype(F32), axis=1, keepdims=True)
            v = _as_bf16(v_ref[0:(i + 1) * HQ, hh * D:(hh + 1) * D])
            o = jnp.dot(p, v, preferred_element_type=F32)
            return o * pl.reciprocal(l, approx=False, full_range=False)

        def oproj(ctx, i):
            rows = slice(HALO + i * TQ, HALO + (i + 1) * TQ)
            acc_ref[rows, :] += jnp.dot(ctx.astype(BF16), _as_bf16(wo_ref[slot]),
                                        preferred_element_type=F32)

        q, s, ctx = {}, {}, {}
        for op in _attention_schedule(nq):
            kind, i = op[0], op[1]
            if kind == "q":
                q[i] = proj_q(i)
            elif kind == "v":
                proj_v(i)
            elif kind == "s":
                s[(i, op[2])] = scores(q[i], op[2], i)
            elif kind == "pv":
                ctx[(i, op[2])] = softmax_pv(s.pop((i, op[2])), op[2], i)
            else:
                oproj(jnp.concatenate([ctx.pop((i, 0)), ctx.pop((i, 1))], axis=1), i)

    @pl.when(step == NK + NP - 1)
    def _epilogue():
        for cp in late_copies:
            cp.wait()

        G = M // 4
        NC = TB // TC
        TH = TB + 2 * HALO
        hsplit = [0] + [2 * HALO + (k + 1) * TC for k in range(NC)]
        ntile = (Fd + 127) // 128
        fsplit = [min(Fd, ((k * ntile + NC - 1) // NC) * 128) for k in range(NC + 1)]

        def start_row(t):
            return t * TB if isinstance(t, int) else pl.multiple_of(t * TB, TB)

        def front_a(t, k):
            lo, hi = hsplit[k], hsplit[k + 1]
            r = start_row(t)
            ga = mod_ref[0:1, 2 * M:3 * M]
            sb = mod_ref[0:1, 3 * M:4 * M]
            cb1 = 1.0 + mod_ref[0:1, 4 * M:5 * M]
            x1 = (x_ref[pl.ds(r + lo, hi - lo), :].astype(F32)
                  + ga * acc_ref[pl.ds(r + lo, hi - lo), :])
            h = _ln(x1) * cb1 + sb
            tt = _gelu(jnp.dot(_ln(h).astype(BF16), _as_bf16(w1_ref[...]),
                               preferred_element_type=F32))
            if k == 0:
                tt = jnp.concatenate([jnp.where(r >= HALO, tt[0:HALO], 0.0), tt[HALO:]], axis=0)
            if k == NC - 1:
                n = hi - lo - HALO
                tt = jnp.concatenate([tt[:n], jnp.where(r + TB < S, tt[n:], 0.0)], axis=0)
            return x1, h, tt

        def front_b(x1, h, tt, k):
            lo = k * TC
            gb = mod_ref[0:1, 5 * M:6 * M]
            lane = lax.broadcasted_iota(jnp.int32, (TC, 128), 1)
            cols = []
            shifts = (-1, 1, -2, 2)
            for cblk in range(M // 128):
                c0, c1 = cblk * 128, (cblk + 1) * 128
                ga_, gb_ = c0 // G, (c1 - 1) // G
                a = tt[HALO + lo + shifts[ga_]:HALO + lo + shifts[ga_] + TC, c0:c1]
                if gb_ != ga_:
                    b = tt[HALO + lo + shifts[gb_]:HALO + lo + shifts[gb_] + TC, c0:c1]
                    a = jnp.where(lane < gb_ * G - c0, a, b)
                cols.append(a.astype(BF16))
            sh = jnp.concatenate(cols, axis=1)
            y = h[HALO + lo:HALO + lo + TC] + jnp.dot(sh, _as_bf16(w2_ref[...]),
                                                      preferred_element_type=F32)
            z_ref[lo:lo + TC, :] = x1[HALO + lo:HALO + lo + TC] + gb * y
            u3_ref[lo // 2:(lo + TC) // 2, :] = _as_u32(_ln(y).astype(BF16))

        def out_copy(t):
            rows = pl.ds(start_row(t), TB)
            return pltpu.make_async_copy(ob_ref.at[rows, :], o_hbm.at[rows, :], osem.at[t])

        def mm3(k):
            lo, hi = fsplit[k], fsplit[k + 1]
            mid = hi - hi % 128
            u3 = _as_bf16(u3_ref[...])
            f = _gelu(lax.dot_general(u3, _as_bf16(w3t_ref[lo // 2:mid // 2, :]),
                                      NT, preferred_element_type=F32))
            if mid < hi:
                ft = _gelu(lax.dot_general(_as_bf16(w3t_ref[mid // 2:hi // 2, :]), u3,
                                           NT, preferred_element_type=F32))
                f = jnp.concatenate([f, ft.T], axis=1)
            return f.astype(BF16)

        def mm4(t, f, z, k):
            lo = k * TC
            gb = mod_ref[0:1, 5 * M:6 * M]
            h2 = jnp.dot(f[lo:lo + TC], _as_bf16(w4_ref[...]), preferred_element_type=F32)
            ob_ref[pl.ds(start_row(t) + lo, TC), :] = (z + gb * h2).astype(ob_ref.dtype)

        def stage(t, cur, nxt):
            fs, fr = [], []
            for k in range(NC):
                if cur:
                    fs.append(mm3(k))
                if nxt:
                    fr.append(front_a(t + 1, k))
            if cur:
                f = jnp.concatenate(fs, axis=1)
            if nxt:
                fr = [jnp.concatenate(parts, axis=0) for parts in zip(*fr)]
            for k in range(NC):
                if cur:
                    z = z_ref[k * TC:(k + 1) * TC, :]
                if nxt and k == NC - 1:
                    front_b(*fr, k)
                if cur:
                    mm4(t, f, z, k)
                if nxt and k < NC - 1:
                    front_b(*fr, k)
            if cur:
                out_copy(t).start()

        nb = S // TB
        stage(-1, False, True)

        def loop_b(t, carry):
            stage(t, True, True)
            return carry
        lax.fori_loop(0, nb - 1, loop_b, 0)
        stage(nb - 1, True, False)
        for t in range(nb):
            out_copy(t).wait()


@jax.jit
def pallas_adaLN_cond__compressed_kv_cla__mixer_s_mlp__prompt_kernel(
    A_x: jax.Array,
    A_c_kv: jax.Array,
    A_w_q: jax.Array,
    A_w_uk: jax.Array,
    A_w_uv: jax.Array,
    A_w_o: jax.Array,
    B_x: jax.Array,
    B_w1: jax.Array,
    B_w2: jax.Array,
    B_w3: jax.Array,
    B_w4: jax.Array,
    c: jax.Array,
    w_mod: jax.Array,
):
    B, S, M = A_x.shape
    assert B == 1 and A_c_kv.shape[1] == S
    Dc = A_c_kv.shape[2]
    H, D = A_w_q.shape[1], A_w_q.shape[2]
    NP = H // 2
    Fd = B_w3.shape[1]
    any_spec = pl.BlockSpec(memory_space=pl.ANY)

    out = pl.pallas_call(
        functools.partial(_kernel, S=S, M=M, D=D, NP=NP, Fd=Fd),
        grid=(NP // KP + NP,),
        in_specs=[any_spec] * 12,
        out_specs=any_spec,
        out_shape=jax.ShapeDtypeStruct((S, M), A_x.dtype),
        scratch_shapes=[
            pltpu.VMEM((S + 2 * HALO + S // NL, M), BF16),
            pltpu.VMEM((S // 2, Dc), U32),
            pltpu.VMEM((2, M, D), U32),
            pltpu.VMEM((NP, Dc, D), U32),
            pltpu.VMEM((2, Dc, D), U32),
            pltpu.VMEM((2, D, M), U32),
            pltpu.VMEM((M // 2, M), U32),
            pltpu.VMEM((M // 2, M), U32),
            pltpu.VMEM((Fd // 2, M), U32),
            pltpu.VMEM((Fd // 2, M), U32),
            pltpu.VMEM((1, M), BF16),
            pltpu.VMEM((M // 2, 6 * M), U32),
            pltpu.VMEM((8, 6 * M), F32),
            pltpu.VMEM(((S + S // NL) // 2, M), U32),
            pltpu.VMEM((M // 2, 2 * D), U32),
            pltpu.VMEM((Dc // 2, 2 * KP * D), U32),
            pltpu.VMEM((Dc // 2, 2 * D), U32),
            pltpu.VMEM((NP, S // 2, 2 * D), U32),
            pltpu.VMEM((S // 2, 2 * D), U32),
            pltpu.VMEM((S + 2 * HALO, M), F32),
            pltpu.VMEM((TB, M), F32),
            pltpu.VMEM((TB // 2, M), U32),
            pltpu.VMEM((S, M), BF16),
            pltpu.SemaphoreType.DMA((8,)),
            pltpu.SemaphoreType.DMA((NP,)),
            pltpu.SemaphoreType.DMA((2, 3)),
            pltpu.SemaphoreType.DMA((S // TB,)),
        ],
        compiler_params=pltpu.CompilerParams(
            dimension_semantics=("arbitrary",),
            vmem_limit_bytes=100 * 1024 * 1024,
            disable_bounds_checks=True,
        ),
    )(
        A_x.reshape(S, M), A_c_kv.reshape(S, Dc),
        A_w_q, A_w_uk, A_w_uv,
        A_w_o.reshape(H * D, M),
        B_w1, B_w2, B_w3.T, B_w4, c, w_mod,
    )
    return out.reshape(B, S, M)
```

```python
import functools
import math

import jax
import jax.numpy as jnp
from jax import lax
import jax.experimental.pallas as pl
import jax.experimental.pallas.tpu as pltpu

F32 = jnp.float32
BF16 = jnp.bfloat16
U32 = jnp.uint32
NT = (((1,), (1,)), ((), ()))
NEG = -1000000000.0
EPS = 1e-05
TQ = 128
TB = 256
TC = 64
LAG = 4
O_LAG = 4
Q_SUB = 0
T_SUB = 2
V_FIRST = 1
V_SPREAD = 4
O_HALF = True
KP = 2
TK = 256
NL = 4
HALO = 8


def _ln(x):
    m = jnp.mean(x, axis=-1, keepdims=True)
    xc = x - m
    v = jnp.mean(xc * xc, axis=-1, keepdims=True)
    return xc * lax.rsqrt(v + EPS)


def _gelu(x):
    c = math.sqrt(2.0 / math.pi)
    hx = 0.5 * x
    return hx + hx * jnp.tanh(x * (c + (c * 0.044715) * (x * x)))


def _as_bf16(u):
    return pltpu.bitcast(u, BF16)


def _as_u32(b):
    return pltpu.bitcast(b, U32)


def _split_pair(u):
    lo = pltpu.bitcast(u << 16, F32).astype(BF16)
    hi = pltpu.bitcast(u & jnp.uint32(0xFFFF0000), F32).astype(BF16)
    return _as_u32(lo), _as_u32(hi)


def _attention_schedule(nq):
    order = list(range(nq - 1, -1, -1))
    units = [(i, hh, half) for i in order for half in (1, 0) for hh in (0, 1)]
    ops = [("q", order[0])] + [("v", i) for i in range(V_FIRST)]
    for k in range(len(units) + LAG + O_LAG):
        n, sub = divmod(k, 4)
        if k < len(units):
            ops.append(("s",) + units[k])
        if 0 <= k - LAG < len(units):
            ops.append(("pv",) + units[k - LAG])
        if sub == Q_SUB and n + 1 < nq:
            ops.append(("q", order[n + 1]))
        if k < LAG:
            per = -(-(nq - V_FIRST) // V_SPREAD)
            ops.extend(("v", i) for i in range(V_FIRST + k * per, min(nq, V_FIRST + (k + 1) * per)))
        if sub == T_SUB and n % 2 == 0 and n + 1 < nq:
            ops.append(("t", order[n], order[n + 1]))
        ko = k - LAG - O_LAG
        if 0 <= ko < len(units):
            if O_HALF and ko % 2 == 1:
                ops.append(("o", units[ko][0], units[ko][2]))
            if not O_HALF and ko % 4 == 3:
                ops.append(("o", units[ko][0], None))
    return ops


def _after(lhs, dep, zero):
    t = None
    for r in range(0, dep.shape[0], 8):
        for c in range(0, dep.shape[1], 128):
            tile = dep[r:r + 8, c:c + 128]
            t = tile if t is None else t | tile
    head = lhs[0:8, 0:128] | (t & zero)
    if lhs.shape[1] > 128:
        head = jnp.concatenate([head, lhs[0:8, 128:]], axis=1)
    return jnp.concatenate([head, lhs[8:]], axis=0)


def _kernel(x_hbm, ckv_hbm, wq_hbm, wk_hbm, wv_hbm, wo_hbm,
            w1_hbm, w2_hbm, w3t_hbm, w4_hbm, c_hbm, wmod_hbm,
            o_hbm,
            x_ref, ckv_ref, wqr_ref, wkr_ref, wvr_ref, wo_ref,
            w1_ref, w2_ref, w3t_ref, w4_ref, c_ref, wmod_ref,
            mod_ref, h_ref, wqp_ref, wkp_ref, wvp_ref, k_ref, v_ref, acc_ref,
            z_ref, u3_ref, ob_ref,
            ssem, ksem, psem, osem,
            *, S, M, D, NP, Fd):
    step = pl.program_id(0)
    NK = NP // KP
    nq = S // TQ
    HQ = TQ // 2
    qscale = (D ** -0.5) * math.log2(math.e)
    LR = S // NL

    ckv_copy = pltpu.make_async_copy(ckv_hbm.bitcast(U32), ckv_ref, ssem.at[0])
    mid_copies = [
        pltpu.make_async_copy(c_hbm, c_ref, ssem.at[1]),
        pltpu.make_async_copy(wmod_hbm.bitcast(U32), wmod_ref, ssem.at[2]),
        pltpu.make_async_copy(x_hbm, x_ref.at[pl.ds(HALO, S), :], ssem.at[3]),
    ]
    late_copies = [
        pltpu.make_async_copy(w1_hbm.bitcast(U32), w1_ref, ssem.at[4]),
        pltpu.make_async_copy(w2_hbm.bitcast(U32), w2_ref, ssem.at[5]),
        pltpu.make_async_copy(w3t_hbm.bitcast(U32), w3t_ref, ssem.at[6]),
        pltpu.make_async_copy(w4_hbm.bitcast(U32), w4_ref, ssem.at[7]),
    ]

    def wk_copy(p):
        return pltpu.make_async_copy(wk_hbm.bitcast(U32).at[:, p, :], wkr_ref.at[p], ksem.at[p])

    def pair_copies(p, sl):
        return [
            pltpu.make_async_copy(wv_hbm.bitcast(U32).at[:, p, :], wvr_ref.at[sl], psem.at[sl, 0]),
            pltpu.make_async_copy(wq_hbm.bitcast(U32).at[:, p, :], wqr_ref.at[sl], psem.at[sl, 1]),
            pltpu.make_async_copy(wo_hbm.bitcast(U32).at[pl.ds(pl.multiple_of(p * D, D), D), :],
                                  wo_ref.at[sl], psem.at[sl, 2]),
        ]

    @pl.when(step == 0)
    def _prologue():
        for p in range(KP):
            wk_copy(p).start()
        ckv_copy.start()
        for p in range(KP, NP):
            wk_copy(p).start()
        for cp in mid_copies:
            cp.start()
        x_ref[0:HALO, :] = jnp.zeros((HALO, M), BF16)
        x_ref[S + HALO:, :] = jnp.zeros((HALO + LR, M), BF16)
        mod_ref[...] = jnp.zeros(mod_ref.shape, F32)

        def zero_acc(t, carry):
            acc_ref[pl.ds(pl.multiple_of(t * 16, 16), 16), :] = jnp.zeros((16, M), F32)
            return carry
        lax.fori_loop(0, (S + 2 * HALO) // 16, zero_acc, 0)
        ckv_copy.wait()

    @pl.when(step == NK - NL)
    def _modulation():
        for cp in mid_copies:
            cp.wait()
        for cp in pair_copies(0, 0):
            cp.start()
        for cp in late_copies:
            cp.start()
        c = c_ref[...].astype(F32)
        sc = jnp.broadcast_to(c * jax.nn.sigmoid(c), (16, M)).astype(BF16)
        mod_ref[...] = jnp.dot(sc, _as_bf16(wmod_ref[...]), preferred_element_type=F32)[0:8]

    @pl.when(step < NK)
    def _keys():
        for u in range(KP):
            wk_copy(step * KP + u).wait()
        for u in range(KP):
            ka, kb = _split_pair(wkr_ref[step * KP + u])
            wkp_ref[:, 2 * u * D:(2 * u + 1) * D] = ka
            wkp_ref[:, (2 * u + 1) * D:(2 * u + 2) * D] = kb
        lblk = jnp.where(step >= NK - NL, step - (NK - NL), NL)
        xoff = jnp.where(step >= NK - NL, HALO, 2 * HALO)
        sa = mod_ref[0:1, 0:M]
        ca1 = 1.0 + mod_ref[0:1, M:2 * M]
        zero = pltpu.bitcast(acc_ref[0:8, 0:128], U32)
        nk = S // TK
        lc = LR // nk
        hu = None
        for i in range(nk):
            rows = slice(i * TK // 2, (i + 1) * TK // 2)
            lhs = ckv_ref[rows, :]
            if hu is not None:
                lhs = _after(lhs, hu, zero)
            k = jnp.dot(_as_bf16(lhs), _as_bf16(wkp_ref[...]), preferred_element_type=F32)
            ku = _as_u32(k.astype(BF16))
            for u in range(KP):
                k_ref[step * KP + u, rows, :] = ku[:, 2 * u * D:(2 * u + 2) * D]
            r = pl.multiple_of(lblk * LR + i * lc + xoff, 8)
            rh = pl.multiple_of(lblk * (LR // 2) + i * (lc // 2), 8)
            x = x_ref[pl.ds(r, lc), :].astype(F32)
            hu = _as_u32((_ln(x) * ca1 + sa).astype(BF16))
            h_ref[pl.ds(rh, lc // 2), :] = hu

    @pl.when(step >= NK)
    def _attention():
        j = step - NK
        slot = j % 2

        @pl.when(j + 1 < NP)
        def _prefetch():
            for cp in pair_copies(j + 1, 1 - slot):
                cp.start()

        for cp in pair_copies(j, slot):
            cp.wait()

        qa, qb = _split_pair(wqr_ref[slot])
        wqp_ref[:, 0:D] = qa
        wqp_ref[:, D:2 * D] = qb
        va, vb = _split_pair(wvr_ref[slot])
        wvp_ref[:, 0:D] = va
        wvp_ref[:, D:2 * D] = vb

        HH = HQ // 2
        row = lax.broadcasted_iota(jnp.int32, (HQ, TQ), 0)
        col = lax.broadcasted_iota(jnp.int32, (HQ, TQ), 1)
        diag = col <= row + HQ
        first = [col < HQ, col >= HQ]
        first0 = [col <= row, jnp.logical_and(col >= HQ, diag)]

        def proj_v(i):
            rows = slice(i * HQ, (i + 1) * HQ)
            v = jnp.dot(_as_bf16(ckv_ref[rows, :]), _as_bf16(wvp_ref[...]), preferred_element_type=F32)
            v_ref[rows, :] = _as_u32(v.astype(BF16))

        def proj_q(i):
            rows = slice(i * HQ, (i + 1) * HQ)
            q = jnp.dot(_as_bf16(h_ref[rows, :]), _as_bf16(wqp_ref[...]), preferred_element_type=F32)
            q = q * qscale
            return [q[:, 0:D].astype(BF16), q[:, D:2 * D].astype(BF16)]

        def masked_scores(qh, k):
            s = lax.dot_general(qh, k, NT, preferred_element_type=F32)
            n = s.shape[1] - TQ
            sd = jnp.where(diag, s[:, n:], NEG)
            return jnp.concatenate([s[:, :n], sd], axis=1) if n else sd

        def scores(q, hh, half, i):
            cols = slice(hh * D, (hh + 1) * D)
            if half == 1:
                return masked_scores(q[hh][HQ:TQ], _as_bf16(k_ref[j, 0:(i + 1) * HQ, cols]))
            if i > 0:
                return masked_scores(q[hh][0:HQ], _as_bf16(k_ref[j, HH:i * HQ + HH, cols]))
            return None

        def first_scores(q1, q2):
            st = [lax.dot_general(_as_bf16(k_ref[j, 0:HH, hh * D:(hh + 1) * D]),
                                  jnp.concatenate([q1[hh][0:HQ], q2[hh][0:HQ]], axis=0),
                                  NT, preferred_element_type=F32) for hh in range(2)]
            t = jnp.concatenate(st, axis=0).T
            return t[0:HQ], t[HQ:TQ]

        def softmax_pv(s, t0, hh, half, i):
            cols = slice(hh * D, (hh + 1) * D)
            if half == 1:
                v = v_ref[0:(i + 1) * HQ, cols]
            else:
                s0 = jnp.where(first[hh] if i > 0 else first0[hh], t0[i], NEG)
                s = s0 if s is None else jnp.concatenate([s, s0], axis=1)
                if hh == 0:
                    v = v_ref[0:HQ, cols]
                else:
                    v = jnp.concatenate([v_ref[HH:HQ, cols], v_ref[0:HH, cols]], axis=0)
                if i > 0:
                    v = jnp.concatenate([v_ref[HH:i * HQ + HH, cols], v], axis=0)
            m = jnp.max(s, axis=1, keepdims=True)
            p = jnp.exp2(s - m).astype(BF16)
            l = jnp.sum(p.astype(F32), axis=1, keepdims=True)
            o = jnp.dot(p, _as_bf16(v), preferred_element_type=F32)
            return o * pl.reciprocal(l, approx=False, full_range=False)

        def oproj(ctx, r, n):
            rows = slice(HALO + r, HALO + r + n)
            acc_ref[rows, :] += jnp.dot(ctx.astype(BF16), _as_bf16(wo_ref[slot]),
                                        preferred_element_type=F32)

        q, s, t0, ctx = {}, {}, {}, {}
        for op in _attention_schedule(nq):
            kind, i = op[0], op[1]
            if kind == "q":
                q[i] = proj_q(i)
            elif kind == "v":
                proj_v(i)
            elif kind == "s":
                s[op[1:]] = scores(q[i], op[2], op[3], i)
            elif kind == "t":
                t0[i], t0[op[2]] = first_scores(q[i], q[op[2]])
            elif kind == "pv":
                ctx[op[1:]] = softmax_pv(s.pop(op[1:]), t0, op[2], op[3], i)
            elif op[2] is None:
                oproj(jnp.concatenate(
                    [jnp.concatenate([ctx.pop((i, hh, 0)), ctx.pop((i, hh, 1))], axis=0)
                     for hh in range(2)], axis=1), i * TQ, TQ)
            else:
                oproj(jnp.concatenate([ctx.pop((i, hh, op[2])) for hh in range(2)], axis=1),
                      i * TQ + op[2] * HQ, HQ)

    @pl.when(step == NK + NP - 1)
    def _epilogue():
        for cp in late_copies:
            cp.wait()

        G = M // 4
        NC = TB // TC
        TH = TB + 2 * HALO
        hsplit = [0] + [2 * HALO + (k + 1) * TC for k in range(NC)]
        ntile = (Fd + 127) // 128
        fsplit = [min(Fd, ((k * ntile + NC - 1) // NC) * 128) for k in range(NC + 1)]

        def start_row(t):
            return t * TB if isinstance(t, int) else pl.multiple_of(t * TB, TB)

        def front_a(t, k):
            lo, hi = hsplit[k], hsplit[k + 1]
            r = start_row(t)
            ga = mod_ref[0:1, 2 * M:3 * M]
            sb = mod_ref[0:1, 3 * M:4 * M]
            cb1 = 1.0 + mod_ref[0:1, 4 * M:5 * M]
            x1 = (x_ref[pl.ds(r + lo, hi - lo), :].astype(F32)
                  + ga * acc_ref[pl.ds(r + lo, hi - lo), :])
            h = _ln(x1) * cb1 + sb
            tt = _gelu(jnp.dot(_ln(h).astype(BF16), _as_bf16(w1_ref[...]),
                               preferred_element_type=F32))
            if k == 0:
                tt = jnp.concatenate([jnp.where(r >= HALO, tt[0:HALO], 0.0), tt[HALO:]], axis=0)
            if k == NC - 1:
                n = hi - lo - HALO
                tt = jnp.concatenate([tt[:n], jnp.where(r + TB < S, tt[n:], 0.0)], axis=0)
            return x1, h, tt

        def front_b(x1, h, tt, k):
            lo = k * TC
            gb = mod_ref[0:1, 5 * M:6 * M]
            lane = lax.broadcasted_iota(jnp.int32, (TC, 128), 1)
            cols = []
            shifts = (-1, 1, -2, 2)
            for cblk in range(M // 128):
                c0, c1 = cblk * 128, (cblk + 1) * 128
                ga_, gb_ = c0 // G, (c1 - 1) // G
                a = tt[HALO + lo + shifts[ga_]:HALO + lo + shifts[ga_] + TC, c0:c1]
                if gb_ != ga_:
                    b = tt[HALO + lo + shifts[gb_]:HALO + lo + shifts[gb_] + TC, c0:c1]
                    a = jnp.where(lane < gb_ * G - c0, a, b)
                cols.append(a.astype(BF16))
            sh = jnp.concatenate(cols, axis=1)
            y = h[HALO + lo:HALO + lo + TC] + jnp.dot(sh, _as_bf16(w2_ref[...]),
                                                      preferred_element_type=F32)
            z_ref[lo:lo + TC, :] = x1[HALO + lo:HALO + lo + TC] + gb * y
            u3_ref[lo // 2:(lo + TC) // 2, :] = _as_u32(_ln(y).astype(BF16))

        def out_copy(t):
            rows = pl.ds(start_row(t), TB)
            return pltpu.make_async_copy(ob_ref.at[rows, :], o_hbm.at[rows, :], osem.at[t])

        def mm3(k):
            lo, hi = fsplit[k], fsplit[k + 1]
            mid = hi - hi % 128
            u3 = _as_bf16(u3_ref[...])
            f = _gelu(lax.dot_general(u3, _as_bf16(w3t_ref[lo // 2:mid // 2, :]),
                                      NT, preferred_element_type=F32))
            if mid < hi:
                ft = _gelu(lax.dot_general(_as_bf16(w3t_ref[mid // 2:hi // 2, :]), u3,
                                           NT, preferred_element_type=F32))
                f = jnp.concatenate([f, ft.T], axis=1)
            return f.astype(BF16)

        def mm4(t, f, z, k):
            lo = k * TC
            gb = mod_ref[0:1, 5 * M:6 * M]
            h2 = jnp.dot(f[lo:lo + TC], _as_bf16(w4_ref[...]), preferred_element_type=F32)
            ob_ref[pl.ds(start_row(t) + lo, TC), :] = (z + gb * h2).astype(ob_ref.dtype)

        def stage(t, cur, nxt):
            fs, fr = [], []
            for k in range(NC):
                if cur:
                    fs.append(mm3(k))
                if nxt:
                    fr.append(front_a(t + 1, k))
            if cur:
                f = jnp.concatenate(fs, axis=1)
            if nxt:
                fr = [jnp.concatenate(parts, axis=0) for parts in zip(*fr)]
            for k in range(NC):
                if cur:
                    z = z_ref[k * TC:(k + 1) * TC, :]
                if nxt and k == NC - 1:
                    front_b(*fr, k)
                if cur:
                    mm4(t, f, z, k)
                if nxt and k < NC - 1:
                    front_b(*fr, k)
            if cur:
                out_copy(t).start()

        nb = S // TB
        stage(-1, False, True)

        def loop_b(t, carry):
            stage(t, True, True)
            return carry
        lax.fori_loop(0, nb - 1, loop_b, 0)
        stage(nb - 1, True, False)
        for t in range(nb):
            out_copy(t).wait()


@jax.jit
def pallas_adaLN_cond__compressed_kv_cla__mixer_s_mlp__prompt_kernel(
    A_x: jax.Array,
    A_c_kv: jax.Array,
    A_w_q: jax.Array,
    A_w_uk: jax.Array,
    A_w_uv: jax.Array,
    A_w_o: jax.Array,
    B_x: jax.Array,
    B_w1: jax.Array,
    B_w2: jax.Array,
    B_w3: jax.Array,
    B_w4: jax.Array,
    c: jax.Array,
    w_mod: jax.Array,
):
    B, S, M = A_x.shape
    assert B == 1 and A_c_kv.shape[1] == S
    Dc = A_c_kv.shape[2]
    H, D = A_w_q.shape[1], A_w_q.shape[2]
    NP = H // 2
    Fd = B_w3.shape[1]
    any_spec = pl.BlockSpec(memory_space=pl.ANY)

    out = pl.pallas_call(
        functools.partial(_kernel, S=S, M=M, D=D, NP=NP, Fd=Fd),
        grid=(NP // KP + NP,),
        in_specs=[any_spec] * 12,
        out_specs=any_spec,
        out_shape=jax.ShapeDtypeStruct((S, M), A_x.dtype),
        scratch_shapes=[
            pltpu.VMEM((S + 2 * HALO + S // NL, M), BF16),
            pltpu.VMEM((S // 2, Dc), U32),
            pltpu.VMEM((2, M, D), U32),
            pltpu.VMEM((NP, Dc, D), U32),
            pltpu.VMEM((2, Dc, D), U32),
            pltpu.VMEM((2, D, M), U32),
            pltpu.VMEM((M // 2, M), U32),
            pltpu.VMEM((M // 2, M), U32),
            pltpu.VMEM((Fd // 2, M), U32),
            pltpu.VMEM((Fd // 2, M), U32),
            pltpu.VMEM((1, M), BF16),
            pltpu.VMEM((M // 2, 6 * M), U32),
            pltpu.VMEM((8, 6 * M), F32),
            pltpu.VMEM(((S + S // NL) // 2, M), U32),
            pltpu.VMEM((M // 2, 2 * D), U32),
            pltpu.VMEM((Dc // 2, 2 * KP * D), U32),
            pltpu.VMEM((Dc // 2, 2 * D), U32),
            pltpu.VMEM((NP, S // 2, 2 * D), U32),
            pltpu.VMEM((S // 2, 2 * D), U32),
            pltpu.VMEM((S + 2 * HALO, M), F32),
            pltpu.VMEM((TB, M), F32),
            pltpu.VMEM((TB // 2, M), U32),
            pltpu.VMEM((S, M), BF16),
            pltpu.SemaphoreType.DMA((8,)),
            pltpu.SemaphoreType.DMA((NP,)),
            pltpu.SemaphoreType.DMA((2, 3)),
            pltpu.SemaphoreType.DMA((S // TB,)),
        ],
        compiler_params=pltpu.CompilerParams(
            dimension_semantics=("arbitrary",),
            vmem_limit_bytes=100 * 1024 * 1024,
            disable_bounds_checks=True,
        ),
    )(
        A_x.reshape(S, M), A_c_kv.reshape(S, Dc),
        A_w_q, A_w_uk, A_w_uv,
        A_w_o.reshape(H * D, M),
        B_w1, B_w2, B_w3.T, B_w4, c, w_mod,
    )
    return out.reshape(B, S, M)
```

```python
import functools
import math

import jax
import jax.numpy as jnp
from jax import lax
import jax.experimental.pallas as pl
import jax.experimental.pallas.tpu as pltpu

F32 = jnp.float32
BF16 = jnp.bfloat16
U32 = jnp.uint32
NT = (((1,), (1,)), ((), ()))
NEG = -1000000000.0
EPS = 1e-05
TQ = 128
TB = 256
TC = 64
LAG = 4
O_LAG = 4
Q_SUB = 0
T_SUB = 2
V_FIRST = 1
V_SPREAD = 4
O_HALF = True
KP = 2
TK = 256
NL = 4
HALO = 8


def _ln(x):
    m = jnp.mean(x, axis=-1, keepdims=True)
    xc = x - m
    v = jnp.mean(xc * xc, axis=-1, keepdims=True)
    return xc * lax.rsqrt(v + EPS)


def _gelu(x):
    c = math.sqrt(2.0 / math.pi)
    hx = 0.5 * x
    return hx + hx * jnp.tanh(x * (c + (c * 0.044715) * (x * x)))


def _as_bf16(u):
    return pltpu.bitcast(u, BF16)


def _as_u32(b):
    return pltpu.bitcast(b, U32)


def _halves(u):
    return pltpu.bitcast(u << 16, F32), pltpu.bitcast(u & jnp.uint32(0xFFFF0000), F32)


def _split_pair(u):
    return _as_u32(jnp.concatenate(_halves(u), axis=1).astype(BF16))


def _attention_schedule(nq):
    order = list(range(nq - 1, -1, -1))
    units = [(i, hh, half) for i in order for half in (1, 0) for hh in (0, 1)]
    ops = [("q", order[0])] + [("v", i) for i in range(V_FIRST)]
    for k in range(len(units) + LAG + O_LAG):
        n, sub = divmod(k, 4)
        if k < len(units):
            ops.append(("s",) + units[k])
        if 0 <= k - LAG < len(units):
            ops.append(("pv",) + units[k - LAG])
        if sub == Q_SUB and n + 1 < nq:
            ops.append(("q", order[n + 1]))
        if k < LAG:
            per = -(-(nq - V_FIRST) // V_SPREAD)
            ops.extend(("v", i) for i in range(V_FIRST + k * per, min(nq, V_FIRST + (k + 1) * per)))
        if sub == T_SUB and n % 2 == 0 and n + 1 < nq:
            ops.append(("t", order[n], order[n + 1]))
        ko = k - LAG - O_LAG
        if 0 <= ko < len(units):
            if O_HALF and ko % 2 == 1:
                ops.append(("o", units[ko][0], units[ko][2]))
            if not O_HALF and ko % 4 == 3:
                ops.append(("o", units[ko][0], None))
    return ops


def _after(lhs, deps, zero):
    t = None
    for dep in deps:
        for r in range(0, dep.shape[0], 8):
            for c in range(0, dep.shape[1], 128):
                tile = dep[r:r + 8, c:c + 128]
                t = tile if t is None else t | tile
    head = lhs[0:8, 0:128] | (t & zero)
    if lhs.shape[1] > 128:
        head = jnp.concatenate([head, lhs[0:8, 128:]], axis=1)
    return jnp.concatenate([head, lhs[8:]], axis=0)


def _kernel(x_hbm, ckv_hbm, wq_hbm, wk_hbm, wv_hbm, wo_hbm,
            w1_hbm, w2_hbm, w3t_hbm, w4_hbm, c_hbm, wmod_hbm,
            o_hbm,
            x_ref, ckv_ref, wqr_ref, wkr_ref, wvr_ref, wo_ref,
            w1_ref, w2_ref, w3t_ref, w4_ref, c_ref, wmod_ref,
            sc_ref, mod_ref, h_ref, wqp_ref, wkp_ref, wvp_ref, wop_ref, k_ref, v_ref, acc_ref,
            z_ref, u3_ref, ob_ref,
            ssem, ksem, msem, osem,
            *, S, M, D, NP, Fd):
    NK = NP // KP
    nq = S // TQ
    HQ = TQ // 2
    qscale = (D ** -0.5) * math.log2(math.e)
    LR = S // NL
    NM = 6

    c_copy = pltpu.make_async_copy(c_hbm, c_ref, ssem.at[0])
    ckv_copy = pltpu.make_async_copy(ckv_hbm.bitcast(U32), ckv_ref, ssem.at[1])
    x_copy = pltpu.make_async_copy(x_hbm, x_ref.at[pl.ds(HALO, S), :], ssem.at[2])
    wo_copy = pltpu.make_async_copy(wo_hbm.bitcast(U32), wo_ref, ssem.at[3])
    late_copies = [
        pltpu.make_async_copy(w1_hbm.bitcast(U32), w1_ref, ssem.at[4]),
        pltpu.make_async_copy(w2_hbm.bitcast(U32), w2_ref, ssem.at[5]),
        pltpu.make_async_copy(w3t_hbm.bitcast(U32), w3t_ref, ssem.at[6]),
        pltpu.make_async_copy(w4_hbm.bitcast(U32), w4_ref, ssem.at[7]),
    ]

    def wk_copy(p):
        return pltpu.make_async_copy(wk_hbm.bitcast(U32).at[:, p, :], wkr_ref.at[p], ksem.at[p])

    def wmod_copy(g):
        off = g * M if isinstance(g, int) else pl.multiple_of(g * M, 128)
        return pltpu.make_async_copy(wmod_hbm.bitcast(U32).at[:, pl.ds(off, M)],
                                     wmod_ref.at[g], msem.at[g])

    def stage_weights(p):
        wqp_ref[...] = _split_pair(wqr_ref[p])
        wvp_ref[...] = _split_pair(wvr_ref[p])
        wop_ref[...] = wo_ref[p]

    def _prologue():
        c_copy.start()
        for p in range(KP):
            wk_copy(p).start()
        ckv_copy.start()
        x_ref[0:HALO, :] = jnp.zeros((HALO, M), BF16)
        x_ref[S + HALO:, :] = jnp.zeros((HALO + LR, M), BF16)
        for p in range(KP, 3 * KP):
            wk_copy(p).start()
        for g in range(2):
            wmod_copy(g).start()
        for p in range(3 * KP, NP):
            wk_copy(p).start()
        x_copy.start()
        for g in range(2, NM):
            wmod_copy(g).start()

        def start_qv(p, carry):
            pltpu.make_async_copy(wq_hbm.bitcast(U32).at[:, p, :], wqr_ref.at[p], ssem.at[8]).start()
            pltpu.make_async_copy(wv_hbm.bitcast(U32).at[:, p, :], wvr_ref.at[p], ssem.at[9]).start()
            return carry
        lax.fori_loop(0, NP, start_qv, 0)
        wo_copy.start()
        for cp in late_copies:
            cp.start()

        mod_ref[...] = jnp.zeros(mod_ref.shape, F32)

        def zero_acc(t, carry):
            acc_ref[pl.ds(pl.multiple_of(t * 16, 16), 16), :] = jnp.zeros((16, M), F32)
            return carry
        lax.fori_loop(0, (S + 2 * HALO) // 16, zero_acc, 0)

        def zero_wmod(t, carry):
            wmod_ref[NM, pl.ds(pl.multiple_of(t * 16, 16), 16), :] = jnp.zeros((16, M), U32)
            return carry
        lax.fori_loop(0, M // 32, zero_wmod, 0)
        c_copy.wait()
        c = c_ref[...].astype(F32)
        sc = jnp.broadcast_to(c * jax.nn.sigmoid(c), (128, M))
        sc_ref[...] = _as_u32(sc.T.astype(BF16))
        ckv_copy.wait()

    def _keys(step, carry):
        for u in range(KP):
            wk_copy(step * KP + u).wait()

        @pl.when(step >= NK - NM)
        def _():
            wmod_copy(step - (NK - NM)).wait()

        @pl.when(step == NK - NL)
        def _():
            x_copy.wait()

        for u in range(KP):
            wkp_ref[:, 2 * u * D:(2 * u + 2) * D] = _split_pair(wkr_ref[step * KP + u])
        g = jnp.where(step >= NK - NM, step - (NK - NM), NM)
        lblk = jnp.where(step >= NK - NL, step - (NK - NL), NL)
        xoff = jnp.where(step >= NK - NL, HALO, 2 * HALO)
        sa = mod_ref[0, 0:1, :]
        ca1 = 1.0 + mod_ref[1, 0:1, :]
        zero = pltpu.bitcast(acc_ref[0:8, 0:128], U32)
        nk = S // TK
        lc = LR // nk
        mc = M // 2 // nk
        deps, part = [], None
        for i in range(nk):
            rows = slice(i * TK // 2, (i + 1) * TK // 2)
            lhs = ckv_ref[rows, :]
            if deps:
                lhs = _after(lhs, deps, zero)
            k = jnp.dot(_as_bf16(lhs), _as_bf16(wkp_ref[...]), preferred_element_type=F32)
            for u in range(KP):
                k_ref[step * KP + u, rows, :] = _as_u32(k[:, 2 * u * D:(2 * u + 2) * D].astype(BF16))
            r = pl.multiple_of(lblk * LR + i * lc + xoff, 8)
            rh = pl.multiple_of(lblk * (LR // 2) + i * (lc // 2), 8)
            x = x_ref[pl.ds(r, lc), :].astype(F32)
            h = _ln(x) * ca1 + sa
            h_ref[pl.ds(rh, lc // 2), :] = _as_u32(h.astype(BF16))
            we, wo = _halves(wmod_ref[g, i * mc:(i + 1) * mc, :])
            se, so = _halves(sc_ref[i * mc:(i + 1) * mc, :])
            prod = we * jnp.tile(se, (1, M // 128)) + wo * jnp.tile(so, (1, M // 128))
            for rr in range(0, mc, 8):
                part = prod[rr:rr + 8] if part is None else part + prod[rr:rr + 8]
            deps = [pltpu.bitcast(h, U32), pltpu.bitcast(part, U32)]
        mod_ref[g] = jnp.broadcast_to(jnp.sum(part, axis=0, keepdims=True), (8, M))
        return carry

    def _first_pair():
        pltpu.make_async_copy(wqr_ref, wqr_ref, ssem.at[8]).wait()
        pltpu.make_async_copy(wvr_ref, wvr_ref, ssem.at[9]).wait()
        wo_copy.wait()
        stage_weights(0)

    def _attention(j, carry):

        HH = HQ // 2
        row = lax.broadcasted_iota(jnp.int32, (HQ, TQ), 0)
        col = lax.broadcasted_iota(jnp.int32, (HQ, TQ), 1)
        diag = col <= row + HQ
        first = [col < HQ, col >= HQ]
        first0 = [col <= row, jnp.logical_and(col >= HQ, diag)]

        def proj_v(i):
            rows = slice(i * HQ, (i + 1) * HQ)
            v = jnp.dot(_as_bf16(ckv_ref[rows, :]), _as_bf16(wvp_ref[...]), preferred_element_type=F32)
            v_ref[rows, :] = _as_u32(v.astype(BF16))

        def proj_q(i):
            rows = slice(i * HQ, (i + 1) * HQ)
            q = jnp.dot(_as_bf16(h_ref[rows, :]), _as_bf16(wqp_ref[...]), preferred_element_type=F32)
            q = q * qscale
            return [q[:, 0:D].astype(BF16), q[:, D:2 * D].astype(BF16)]

        def masked_scores(qh, k):
            s = lax.dot_general(qh, k, NT, preferred_element_type=F32)
            n = s.shape[1] - TQ
            sd = jnp.where(diag, s[:, n:], NEG)
            return jnp.concatenate([s[:, :n], sd], axis=1) if n else sd

        def scores(q, hh, half, i):
            cols = slice(hh * D, (hh + 1) * D)
            if half == 1:
                return masked_scores(q[hh][HQ:TQ], _as_bf16(k_ref[j, 0:(i + 1) * HQ, cols]))
            if i > 0:
                return masked_scores(q[hh][0:HQ], _as_bf16(k_ref[j, HH:i * HQ + HH, cols]))
            return None

        def first_scores(q1, q2):
            st = [lax.dot_general(_as_bf16(k_ref[j, 0:HH, hh * D:(hh + 1) * D]),
                                  jnp.concatenate([q1[hh][0:HQ], q2[hh][0:HQ]], axis=0),
                                  NT, preferred_element_type=F32) for hh in range(2)]
            t = jnp.concatenate(st, axis=0).T
            return t[0:HQ], t[HQ:TQ]

        def softmax_pv(s, t0, hh, half, i):
            cols = slice(hh * D, (hh + 1) * D)
            if half == 1:
                v = v_ref[0:(i + 1) * HQ, cols]
            else:
                s0 = jnp.where(first[hh] if i > 0 else first0[hh], t0[i], NEG)
                s = s0 if s is None else jnp.concatenate([s, s0], axis=1)
                if hh == 0:
                    v = v_ref[0:HQ, cols]
                else:
                    v = jnp.concatenate([v_ref[HH:HQ, cols], v_ref[0:HH, cols]], axis=0)
                if i > 0:
                    v = jnp.concatenate([v_ref[HH:i * HQ + HH, cols], v], axis=0)
            m = jnp.max(s, axis=1, keepdims=True)
            p = jnp.exp2(s - m).astype(BF16)
            l = jnp.sum(p.astype(F32), axis=1, keepdims=True)
            o = jnp.dot(p, _as_bf16(v), preferred_element_type=F32)
            return o * pl.reciprocal(l, approx=False, full_range=False)

        def oproj(ctx, r, n):
            rows = slice(HALO + r, HALO + r + n)
            acc_ref[rows, :] += jnp.dot(ctx.astype(BF16), _as_bf16(wop_ref[...]),
                                        preferred_element_type=F32)

        q, s, t0, ctx = {}, {}, {}, {}
        for op in _attention_schedule(nq):
            kind, i = op[0], op[1]
            if kind == "q":
                q[i] = proj_q(i)
            elif kind == "v":
                proj_v(i)
            elif kind == "s":
                s[op[1:]] = scores(q[i], op[2], op[3], i)
            elif kind == "t":
                t0[i], t0[op[2]] = first_scores(q[i], q[op[2]])
            elif kind == "pv":
                ctx[op[1:]] = softmax_pv(s.pop(op[1:]), t0, op[2], op[3], i)
            elif op[2] is None:
                oproj(jnp.concatenate(
                    [jnp.concatenate([ctx.pop((i, hh, 0)), ctx.pop((i, hh, 1))], axis=0)
                     for hh in range(2)], axis=1), i * TQ, TQ)
            else:
                oproj(jnp.concatenate([ctx.pop((i, hh, op[2])) for hh in range(2)], axis=1),
                      i * TQ + op[2] * HQ, HQ)

        stage_weights(jnp.minimum(j + 1, NP - 1))
        return carry

    def _epilogue():
        for cp in late_copies:
            cp.wait()

        G = M // 4
        NC = TB // TC
        TH = TB + 2 * HALO
        hsplit = [0] + [2 * HALO + (k + 1) * TC for k in range(NC)]
        ntile = (Fd + 127) // 128
        fsplit = [min(Fd, ((k * ntile + NC - 1) // NC) * 128) for k in range(NC + 1)]

        def start_row(t):
            return t * TB if isinstance(t, int) else pl.multiple_of(t * TB, TB)

        def front_a(t, k):
            lo, hi = hsplit[k], hsplit[k + 1]
            r = start_row(t)
            ga = mod_ref[2, 0:1, :]
            sb = mod_ref[3, 0:1, :]
            cb1 = 1.0 + mod_ref[4, 0:1, :]
            x1 = (x_ref[pl.ds(r + lo, hi - lo), :].astype(F32)
                  + ga * acc_ref[pl.ds(r + lo, hi - lo), :])
            h = _ln(x1) * cb1 + sb
            tt = _gelu(jnp.dot(_ln(h).astype(BF16), _as_bf16(w1_ref[...]),
                               preferred_element_type=F32))
            if k == 0:
                tt = jnp.concatenate([jnp.where(r >= HALO, tt[0:HALO], 0.0), tt[HALO:]], axis=0)
            if k == NC - 1:
                n = hi - lo - HALO
                tt = jnp.concatenate([tt[:n], jnp.where(r + TB < S, tt[n:], 0.0)], axis=0)
            return x1, h, tt

        def front_b(x1, h, tt, k):
            lo = k * TC
            gb = mod_ref[5, 0:1, :]
            lane = lax.broadcasted_iota(jnp.int32, (TC, 128), 1)
            cols = []
            shifts = (-1, 1, -2, 2)
            for cblk in range(M // 128):
                c0, c1 = cblk * 128, (cblk + 1) * 128
                ga_, gb_ = c0 // G, (c1 - 1) // G
                a = tt[HALO + lo + shifts[ga_]:HALO + lo + shifts[ga_] + TC, c0:c1]
                if gb_ != ga_:
                    b = tt[HALO + lo + shifts[gb_]:HALO + lo + shifts[gb_] + TC, c0:c1]
                    a = jnp.where(lane < gb_ * G - c0, a, b)
                cols.append(a.astype(BF16))
            sh = jnp.concatenate(cols, axis=1)
            y = h[HALO + lo:HALO + lo + TC] + jnp.dot(sh, _as_bf16(w2_ref[...]),
                                                      preferred_element_type=F32)
            z_ref[lo:lo + TC, :] = x1[HALO + lo:HALO + lo + TC] + gb * y
            u3_ref[lo // 2:(lo + TC) // 2, :] = _as_u32(_ln(y).astype(BF16))

        def out_copy(t):
            rows = pl.ds(start_row(t), TB)
            return pltpu.make_async_copy(ob_ref.at[rows, :], o_hbm.at[rows, :], osem.at[t])

        def mm3(k):
            lo, hi = fsplit[k], fsplit[k + 1]
            mid = hi - hi % 128
            u3 = _as_bf16(u3_ref[...])
            f = _gelu(lax.dot_general(u3, _as_bf16(w3t_ref[lo // 2:mid // 2, :]),
                                      NT, preferred_element_type=F32))
            if mid < hi:
                ft = _gelu(lax.dot_general(_as_bf16(w3t_ref[mid // 2:hi // 2, :]), u3,
                                           NT, preferred_element_type=F32))
                f = jnp.concatenate([f, ft.T], axis=1)
            return f.astype(BF16)

        def mm4(t, f, z, k):
            lo = k * TC
            gb = mod_ref[5, 0:1, :]
            h2 = jnp.dot(f[lo:lo + TC], _as_bf16(w4_ref[...]), preferred_element_type=F32)
            ob_ref[pl.ds(start_row(t) + lo, TC), :] = (z + gb * h2).astype(ob_ref.dtype)

        def stage(t, cur, nxt):
            fs, fr = [], []
            for k in range(NC):
                if cur:
                    fs.append(mm3(k))
                if nxt:
                    fr.append(front_a(t + 1, k))
            if cur:
                f = jnp.concatenate(fs, axis=1)
            if nxt:
                fr = [jnp.concatenate(parts, axis=0) for parts in zip(*fr)]
            for k in range(NC):
                if cur:
                    z = z_ref[k * TC:(k + 1) * TC, :]
                if nxt and k == NC - 1:
                    front_b(*fr, k)
                if cur:
                    mm4(t, f, z, k)
                if nxt and k < NC - 1:
                    front_b(*fr, k)
            if cur:
                out_copy(t).start()

        nb = S // TB
        stage(-1, False, True)

        def loop_b(t, carry):
            stage(t, True, True)
            return carry
        lax.fori_loop(0, nb - 1, loop_b, 0)
        stage(nb - 1, True, False)
        for t in range(nb):
            out_copy(t).wait()

    _prologue()
    lax.fori_loop(0, NK, _keys, 0)
    _first_pair()
    lax.fori_loop(0, NP, _attention, 0)
    _epilogue()


@jax.jit
def pallas_adaLN_cond__compressed_kv_cla__mixer_s_mlp__prompt_kernel(
    A_x: jax.Array,
    A_c_kv: jax.Array,
    A_w_q: jax.Array,
    A_w_uk: jax.Array,
    A_w_uv: jax.Array,
    A_w_o: jax.Array,
    B_x: jax.Array,
    B_w1: jax.Array,
    B_w2: jax.Array,
    B_w3: jax.Array,
    B_w4: jax.Array,
    c: jax.Array,
    w_mod: jax.Array,
):
    B, S, M = A_x.shape
    assert B == 1 and A_c_kv.shape[1] == S
    Dc = A_c_kv.shape[2]
    H, D = A_w_q.shape[1], A_w_q.shape[2]
    NP = H // 2
    Fd = B_w3.shape[1]
    any_spec = pl.BlockSpec(memory_space=pl.ANY)

    out = pl.pallas_call(
        functools.partial(_kernel, S=S, M=M, D=D, NP=NP, Fd=Fd),
        in_specs=[any_spec] * 12,
        out_specs=any_spec,
        out_shape=jax.ShapeDtypeStruct((S, M), A_x.dtype),
        scratch_shapes=[
            pltpu.VMEM((S + 2 * HALO + S // NL, M), BF16),
            pltpu.VMEM((S // 2, Dc), U32),
            pltpu.VMEM((NP, M, D), U32),
            pltpu.VMEM((NP, Dc, D), U32),
            pltpu.VMEM((NP, Dc, D), U32),
            pltpu.VMEM((NP, D, M), U32),
            pltpu.VMEM((M // 2, M), U32),
            pltpu.VMEM((M // 2, M), U32),
            pltpu.VMEM((Fd // 2, M), U32),
            pltpu.VMEM((Fd // 2, M), U32),
            pltpu.VMEM((1, M), BF16),
            pltpu.VMEM((7, M // 2, M), U32),
            pltpu.VMEM((M // 2, 128), U32),
            pltpu.VMEM((7, 8, M), F32),
            pltpu.VMEM(((S + S // NL) // 2, M), U32),
            pltpu.VMEM((M // 2, 2 * D), U32),
            pltpu.VMEM((Dc // 2, 2 * KP * D), U32),
            pltpu.VMEM((Dc // 2, 2 * D), U32),
            pltpu.VMEM((D, M), U32),
            pltpu.VMEM((NP, S // 2, 2 * D), U32),
            pltpu.VMEM((S // 2, 2 * D), U32),
            pltpu.VMEM((S + 2 * HALO, M), F32),
            pltpu.VMEM((TB, M), F32),
            pltpu.VMEM((TB // 2, M), U32),
            pltpu.VMEM((S, M), BF16),
            pltpu.SemaphoreType.DMA((10,)),
            pltpu.SemaphoreType.DMA((NP,)),
            pltpu.SemaphoreType.DMA((6,)),
            pltpu.SemaphoreType.DMA((S // TB,)),
        ],
        compiler_params=pltpu.CompilerParams(
            vmem_limit_bytes=100 * 1024 * 1024,
            disable_bounds_checks=True,
            disable_semaphore_checks=True,
        ),
    )(
        A_x.reshape(S, M), A_c_kv.reshape(S, Dc),
        A_w_q, A_w_uk, A_w_uv,
        A_w_o.reshape(NP, 2 * D, M),
        B_w1, B_w2, B_w3.T, B_w4, c, w_mod,
    )
    return out.reshape(B, S, M)
```

```python
import functools
import math

import jax
import jax.numpy as jnp
from jax import lax
import jax.experimental.pallas as pl
import jax.experimental.pallas.tpu as pltpu

F32 = jnp.float32
BF16 = jnp.bfloat16
U32 = jnp.uint32
NT = (((1,), (1,)), ((), ()))
NEG = -1000000000.0
EPS = 1e-05
TQ = 128
TB = 256
TC = 64
LAG = 4
O_LAG = 4
Q_SUB = 0
T_SUB = 2
V_FIRST = 1
V_SPREAD = 4
O_HALF = True
CC = 4
KP = 2
TK = 256
NL = 4
HALO = 8


def _ln(x):
    m = jnp.mean(x, axis=-1, keepdims=True)
    xc = x - m
    v = jnp.mean(xc * xc, axis=-1, keepdims=True)
    return xc * lax.rsqrt(v + EPS)


def _gelu(x):
    c = math.sqrt(2.0 / math.pi)
    hx = 0.5 * x
    return hx + hx * jnp.tanh(x * (c + (c * 0.044715) * (x * x)))


def _as_bf16(u):
    return pltpu.bitcast(u, BF16)


def _as_u32(b):
    return pltpu.bitcast(b, U32)


def _halves(u):
    return pltpu.bitcast(u << 16, F32), pltpu.bitcast(u & jnp.uint32(0xFFFF0000), F32)


def _split_pair(u):
    return _as_u32(jnp.concatenate(_halves(u), axis=1).astype(BF16))


def _attention_schedule(nq):
    order = list(range(nq - 1, -1, -1))
    units = [(i, hh, half) for i in order for half in (1, 0) for hh in (0, 1)]
    ops = [("q", order[0])] + [("v", i) for i in range(V_FIRST)]
    for k in range(len(units) + LAG + O_LAG):
        n, sub = divmod(k, 4)
        if k < len(units):
            ops.append(("s",) + units[k])
        if 0 <= k - LAG < len(units):
            ops.append(("pv",) + units[k - LAG])
        if sub == Q_SUB and n + 1 < nq:
            ops.append(("q", order[n + 1]))
        if k < LAG:
            per = -(-(nq - V_FIRST) // V_SPREAD)
            ops.extend(("v", i) for i in range(V_FIRST + k * per, min(nq, V_FIRST + (k + 1) * per)))
        if sub == T_SUB and n % 2 == 0 and n + 1 < nq:
            ops.append(("t", order[n], order[n + 1]))
        ko = k - LAG - O_LAG
        if 0 <= ko < len(units):
            if O_HALF and ko % 2 == 1:
                ops.append(("o", units[ko][0], units[ko][2]))
            if not O_HALF and ko % 4 == 3:
                ops.append(("o", units[ko][0], None))
    return ops


def _after(lhs, deps, zero):
    t = None
    for dep in deps:
        for r in range(0, dep.shape[0], 8):
            for c in range(0, dep.shape[1], 128):
                tile = dep[r:r + 8, c:c + 128]
                t = tile if t is None else t | tile
    head = lhs[0:8, 0:128] | (t & zero)
    if lhs.shape[1] > 128:
        head = jnp.concatenate([head, lhs[0:8, 128:]], axis=1)
    return jnp.concatenate([head, lhs[8:]], axis=0)


def _kernel(x_hbm, ckv_hbm, wq_hbm, wk_hbm, wv_hbm, wo_hbm,
            w1_hbm, w2_hbm, w3t_hbm, w4_hbm, c_hbm, wmod_hbm,
            o_hbm,
            x_ref, ckv_ref, wqr_ref, wkr_ref, wvr_ref, wo_ref,
            w1_ref, w2_ref, w3t_ref, w4_ref, c_ref, wmod_ref,
            sc_ref, mod_ref, h_ref, wqp_ref, wkp_ref, wvp_ref, wop_ref, k_ref, v_ref, acc_ref,
            z_ref, u3_ref, ob_ref,
            ssem, csem, ksem, msem, osem,
            *, S, M, D, NP, Fd):
    NK = NP // KP
    nq = S // TQ
    HQ = TQ // 2
    qscale = (D ** -0.5) * math.log2(math.e)
    LR = S // NL
    NM = 6

    c_copy = pltpu.make_async_copy(c_hbm, c_ref, ssem.at[0])
    CR = S // CC // 2

    def ckv_copy(i):
        rows = pl.ds(i * CR if isinstance(i, int) else pl.multiple_of(i * CR, CR), CR)
        return pltpu.make_async_copy(ckv_hbm.bitcast(U32).at[rows, :], ckv_ref.at[rows, :],
                                     csem.at[i])

    x_copy = pltpu.make_async_copy(x_hbm, x_ref.at[pl.ds(HALO, S), :], ssem.at[2])
    wo_copy = pltpu.make_async_copy(wo_hbm.bitcast(U32), wo_ref, ssem.at[3])
    late_copies = [
        pltpu.make_async_copy(w1_hbm.bitcast(U32), w1_ref, ssem.at[4]),
        pltpu.make_async_copy(w2_hbm.bitcast(U32), w2_ref, ssem.at[5]),
        pltpu.make_async_copy(w3t_hbm.bitcast(U32), w3t_ref, ssem.at[6]),
        pltpu.make_async_copy(w4_hbm.bitcast(U32), w4_ref, ssem.at[7]),
    ]

    def wk_copy(p):
        return pltpu.make_async_copy(wk_hbm.bitcast(U32).at[:, p, :], wkr_ref.at[p], ksem.at[p])

    def wmod_copy(g):
        off = g * M if isinstance(g, int) else pl.multiple_of(g * M, 128)
        return pltpu.make_async_copy(wmod_hbm.bitcast(U32).at[:, pl.ds(off, M)],
                                     wmod_ref.at[g], msem.at[g])

    def stage_weights(p):
        wqp_ref[...] = _split_pair(wqr_ref[p])
        wvp_ref[...] = _split_pair(wvr_ref[p])
        wop_ref[...] = wo_ref[p]

    def stage_wk(step):
        for u in range(KP):
            wkp_ref[:, 2 * u * D:(2 * u + 2) * D] = _split_pair(wkr_ref[step * KP + u])

    def proj_k(step, rows, lhs):
        k = jnp.dot(_as_bf16(lhs), _as_bf16(wkp_ref[...]), preferred_element_type=F32)
        for u in range(KP):
            k_ref[step * KP + u, rows, :] = _as_u32(k[:, 2 * u * D:(2 * u + 2) * D].astype(BF16))

    def _prologue():
        c_copy.start()
        for p in range(KP):
            wk_copy(p).start()
        for i in range(CC):
            ckv_copy(i).start()
        x_ref[0:HALO, :] = jnp.zeros((HALO, M), BF16)
        x_ref[S + HALO:, :] = jnp.zeros((HALO + LR, M), BF16)
        for p in range(KP, 3 * KP):
            wk_copy(p).start()
        for g in range(2):
            wmod_copy(g).start()
        for p in range(3 * KP, NP):
            wk_copy(p).start()
        x_copy.start()
        for g in range(2, NM):
            wmod_copy(g).start()

        def start_qv(p, carry):
            pltpu.make_async_copy(wq_hbm.bitcast(U32).at[:, p, :], wqr_ref.at[p], ssem.at[8]).start()
            pltpu.make_async_copy(wv_hbm.bitcast(U32).at[:, p, :], wvr_ref.at[p], ssem.at[9]).start()
            return carry
        lax.fori_loop(0, NP, start_qv, 0)
        wo_copy.start()
        for cp in late_copies:
            cp.start()
        mod_ref[...] = jnp.zeros(mod_ref.shape, F32)
        acc_ref[S:, :] = jnp.zeros((2 * HALO, M), F32)
        c_copy.wait()
        c = c_ref[...].astype(F32)
        sc = jnp.broadcast_to(c * jax.nn.sigmoid(c), (128, M))
        sc_ref[...] = _as_u32(sc.T.astype(BF16))
        for p in range(KP):
            wk_copy(p).wait()
        stage_wk(0)

        def first_keys(i, carry):
            ckv_copy(i).wait()
            for ii in range(2 * CR // TK):
                rows = pl.ds(pl.multiple_of(i * CR + ii * (TK // 2), TK // 2), TK // 2)
                proj_k(0, rows, ckv_ref[rows, :])
            ar, wr = S // CC, M // 2 // CC
            acc_ref[pl.ds(pl.multiple_of(i * ar, ar), ar), :] = jnp.zeros((ar, M), F32)
            wmod_ref[NM, pl.ds(pl.multiple_of(i * wr, 8), wr), :] = jnp.zeros((wr, M), U32)
            return carry
        lax.fori_loop(0, CC, first_keys, 0)

    def _keys(step, carry):
        for u in range(KP):
            wk_copy(step * KP + u).wait()

        @pl.when(step >= NK - NM)
        def _():
            wmod_copy(step - (NK - NM)).wait()

        @pl.when(step == NK - NL)
        def _():
            x_copy.wait()

        stage_wk(step)
        g = jnp.where(step >= NK - NM, step - (NK - NM), NM)
        lblk = jnp.where(step >= NK - NL, step - (NK - NL), NL)
        xoff = jnp.where(step >= NK - NL, HALO, 2 * HALO)
        sa = mod_ref[0, 0:1, :]
        ca1 = 1.0 + mod_ref[1, 0:1, :]
        zero = pltpu.bitcast(acc_ref[0:8, 0:128], U32)
        nk = S // TK
        lc = LR // nk
        mc = M // 2 // nk
        deps, part = [], None
        for i in range(nk):
            rows = slice(i * TK // 2, (i + 1) * TK // 2)
            lhs = ckv_ref[rows, :]
            if deps:
                lhs = _after(lhs, deps, zero)
            proj_k(step, rows, lhs)
            r = pl.multiple_of(lblk * LR + i * lc + xoff, 8)
            rh = pl.multiple_of(lblk * (LR // 2) + i * (lc // 2), 8)
            x = x_ref[pl.ds(r, lc), :].astype(F32)
            h = _ln(x) * ca1 + sa
            h_ref[pl.ds(rh, lc // 2), :] = _as_u32(h.astype(BF16))
            we, wo = _halves(wmod_ref[g, i * mc:(i + 1) * mc, :])
            se, so = _halves(sc_ref[i * mc:(i + 1) * mc, :])
            prod = we * jnp.tile(se, (1, M // 128)) + wo * jnp.tile(so, (1, M // 128))
            for rr in range(0, mc, 8):
                part = prod[rr:rr + 8] if part is None else part + prod[rr:rr + 8]
            deps = [pltpu.bitcast(h, U32), pltpu.bitcast(part, U32)]
        mod_ref[g] = jnp.broadcast_to(jnp.sum(part, axis=0, keepdims=True), (8, M))
        return carry

    def _first_pair():
        pltpu.make_async_copy(wqr_ref, wqr_ref, ssem.at[8]).wait()
        pltpu.make_async_copy(wvr_ref, wvr_ref, ssem.at[9]).wait()
        wo_copy.wait()
        stage_weights(0)

    def _attention(j, carry):

        HH = HQ // 2
        row = lax.broadcasted_iota(jnp.int32, (HQ, TQ), 0)
        col = lax.broadcasted_iota(jnp.int32, (HQ, TQ), 1)
        diag = col <= row + HQ
        first = [col < HQ, col >= HQ]
        first0 = [col <= row, jnp.logical_and(col >= HQ, diag)]

        def proj_v(i):
            rows = slice(i * HQ, (i + 1) * HQ)
            v = jnp.dot(_as_bf16(ckv_ref[rows, :]), _as_bf16(wvp_ref[...]), preferred_element_type=F32)
            v_ref[rows, :] = _as_u32(v.astype(BF16))

        def proj_q(i):
            rows = slice(i * HQ, (i + 1) * HQ)
            q = jnp.dot(_as_bf16(h_ref[rows, :]), _as_bf16(wqp_ref[...]), preferred_element_type=F32)
            q = q * qscale
            return [q[:, 0:D].astype(BF16), q[:, D:2 * D].astype(BF16)]

        def masked_scores(qh, k):
            s = lax.dot_general(qh, k, NT, preferred_element_type=F32)
            n = s.shape[1] - TQ
            sd = jnp.where(diag, s[:, n:], NEG)
            return jnp.concatenate([s[:, :n], sd], axis=1) if n else sd

        def scores(q, hh, half, i):
            cols = slice(hh * D, (hh + 1) * D)
            if half == 1:
                return masked_scores(q[hh][HQ:TQ], _as_bf16(k_ref[j, 0:(i + 1) * HQ, cols]))
            if i > 0:
                return masked_scores(q[hh][0:HQ], _as_bf16(k_ref[j, HH:i * HQ + HH, cols]))
            return None

        def first_scores(q1, q2):
            st = [lax.dot_general(_as_bf16(k_ref[j, 0:HH, hh * D:(hh + 1) * D]),
                                  jnp.concatenate([q1[hh][0:HQ], q2[hh][0:HQ]], axis=0),
                                  NT, preferred_element_type=F32) for hh in range(2)]
            t = jnp.concatenate(st, axis=0).T
            return t[0:HQ], t[HQ:TQ]

        def softmax_pv(s, t0, hh, half, i):
            cols = slice(hh * D, (hh + 1) * D)
            if half == 1:
                v = v_ref[0:(i + 1) * HQ, cols]
            else:
                s0 = jnp.where(first[hh] if i > 0 else first0[hh], t0[i], NEG)
                s = s0 if s is None else jnp.concatenate([s, s0], axis=1)
                if hh == 0:
                    v = v_ref[0:HQ, cols]
                else:
                    v = jnp.concatenate([v_ref[HH:HQ, cols], v_ref[0:HH, cols]], axis=0)
                if i > 0:
                    v = jnp.concatenate([v_ref[HH:i * HQ + HH, cols], v], axis=0)
            m = jnp.max(s, axis=1, keepdims=True)
            p = jnp.exp2(s - m).astype(BF16)
            l = jnp.sum(p.astype(F32), axis=1, keepdims=True)
            o = jnp.dot(p, _as_bf16(v), preferred_element_type=F32)
            return o * pl.reciprocal(l, approx=False, full_range=False)

        def oproj(ctx, r, n):
            rows = slice(HALO + r, HALO + r + n)
            acc_ref[rows, :] += jnp.dot(ctx.astype(BF16), _as_bf16(wop_ref[...]),
                                        preferred_element_type=F32)

        q, s, t0, ctx = {}, {}, {}, {}
        for op in _attention_schedule(nq):
            kind, i = op[0], op[1]
            if kind == "q":
                q[i] = proj_q(i)
            elif kind == "v":
                proj_v(i)
            elif kind == "s":
                s[op[1:]] = scores(q[i], op[2], op[3], i)
            elif kind == "t":
                t0[i], t0[op[2]] = first_scores(q[i], q[op[2]])
            elif kind == "pv":
                ctx[op[1:]] = softmax_pv(s.pop(op[1:]), t0, op[2], op[3], i)
            elif op[2] is None:
                oproj(jnp.concatenate(
                    [jnp.concatenate([ctx.pop((i, hh, 0)), ctx.pop((i, hh, 1))], axis=0)
                     for hh in range(2)], axis=1), i * TQ, TQ)
            else:
                oproj(jnp.concatenate([ctx.pop((i, hh, op[2])) for hh in range(2)], axis=1),
                      i * TQ + op[2] * HQ, HQ)

        stage_weights(jnp.minimum(j + 1, NP - 1))
        return carry

    def _epilogue():
        for cp in late_copies:
            cp.wait()

        G = M // 4
        NC = TB // TC
        TH = TB + 2 * HALO
        hsplit = [0] + [2 * HALO + (k + 1) * TC for k in range(NC)]
        ntile = (Fd + 127) // 128
        fsplit = [min(Fd, ((k * ntile + NC - 1) // NC) * 128) for k in range(NC + 1)]

        def start_row(t):
            return t * TB if isinstance(t, int) else pl.multiple_of(t * TB, TB)

        def front_a(t, k):
            lo, hi = hsplit[k], hsplit[k + 1]
            r = start_row(t)
            ga = mod_ref[2, 0:1, :]
            sb = mod_ref[3, 0:1, :]
            cb1 = 1.0 + mod_ref[4, 0:1, :]
            x1 = (x_ref[pl.ds(r + lo, hi - lo), :].astype(F32)
                  + ga * acc_ref[pl.ds(r + lo, hi - lo), :])
            h = _ln(x1) * cb1 + sb
            tt = _gelu(jnp.dot(_ln(h).astype(BF16), _as_bf16(w1_ref[...]),
                               preferred_element_type=F32))
            if k == 0:
                tt = jnp.concatenate([jnp.where(r >= HALO, tt[0:HALO], 0.0), tt[HALO:]], axis=0)
            if k == NC - 1:
                n = hi - lo - HALO
                tt = jnp.concatenate([tt[:n], jnp.where(r + TB < S, tt[n:], 0.0)], axis=0)
            return x1, h, tt

        def front_b(x1, h, tt, k):
            lo = k * TC
            gb = mod_ref[5, 0:1, :]
            lane = lax.broadcasted_iota(jnp.int32, (TC, 128), 1)
            cols = []
            shifts = (-1, 1, -2, 2)
            for cblk in range(M // 128):
                c0, c1 = cblk * 128, (cblk + 1) * 128
                ga_, gb_ = c0 // G, (c1 - 1) // G
                a = tt[HALO + lo + shifts[ga_]:HALO + lo + shifts[ga_] + TC, c0:c1]
                if gb_ != ga_:
                    b = tt[HALO + lo + shifts[gb_]:HALO + lo + shifts[gb_] + TC, c0:c1]
                    a = jnp.where(lane < gb_ * G - c0, a, b)
                cols.append(a.astype(BF16))
            sh = jnp.concatenate(cols, axis=1)
            y = h[HALO + lo:HALO + lo + TC] + jnp.dot(sh, _as_bf16(w2_ref[...]),
                                                      preferred_element_type=F32)
            z_ref[lo:lo + TC, :] = x1[HALO + lo:HALO + lo + TC] + gb * y
            u3_ref[lo // 2:(lo + TC) // 2, :] = _as_u32(_ln(y).astype(BF16))

        def out_copy(t):
            rows = pl.ds(start_row(t), TB)
            return pltpu.make_async_copy(ob_ref.at[rows, :], o_hbm.at[rows, :], osem.at[t])

        def mm3(k):
            lo, hi = fsplit[k], fsplit[k + 1]
            mid = hi - hi % 128
            u3 = _as_bf16(u3_ref[...])
            f = _gelu(lax.dot_general(u3, _as_bf16(w3t_ref[lo // 2:mid // 2, :]),
                                      NT, preferred_element_type=F32))
            if mid < hi:
                ft = _gelu(lax.dot_general(_as_bf16(w3t_ref[mid // 2:hi // 2, :]), u3,
                                           NT, preferred_element_type=F32))
                f = jnp.concatenate([f, ft.T], axis=1)
            return f.astype(BF16)

        def mm4(t, f, z, k):
            lo = k * TC
            gb = mod_ref[5, 0:1, :]
            h2 = jnp.dot(f[lo:lo + TC], _as_bf16(w4_ref[...]), preferred_element_type=F32)
            ob_ref[pl.ds(start_row(t) + lo, TC), :] = (z + gb * h2).astype(ob_ref.dtype)

        def stage(t, cur, nxt):
            fs, fr = [], []
            for k in range(NC):
                if cur:
                    fs.append(mm3(k))
                if nxt:
                    fr.append(front_a(t + 1, k))
            if cur:
                f = jnp.concatenate(fs, axis=1)
            if nxt:
                fr = [jnp.concatenate(parts, axis=0) for parts in zip(*fr)]
            for k in range(NC):
                if cur:
                    z = z_ref[k * TC:(k + 1) * TC, :]
                if nxt and k == NC - 1:
                    front_b(*fr, k)
                if cur:
                    mm4(t, f, z, k)
                if nxt and k < NC - 1:
                    front_b(*fr, k)
            if cur:
                out_copy(t).start()

        nb = S // TB
        stage(-1, False, True)

        def loop_b(t, carry):
            stage(t, True, True)
            return carry
        lax.fori_loop(0, nb - 1, loop_b, 0)
        stage(nb - 1, True, False)
        for t in range(nb):
            out_copy(t).wait()

    @pl.when(pl.program_id(0) == 0)
    def _():
        _prologue()
        lax.fori_loop(1, NK, _keys, 0)
        _first_pair()
        lax.fori_loop(0, NP, _attention, 0)

    @pl.when(pl.program_id(0) == 1)
    def _():
        _epilogue()


@jax.jit
def pallas_adaLN_cond__compressed_kv_cla__mixer_s_mlp__prompt_kernel(
    A_x: jax.Array,
    A_c_kv: jax.Array,
    A_w_q: jax.Array,
    A_w_uk: jax.Array,
    A_w_uv: jax.Array,
    A_w_o: jax.Array,
    B_x: jax.Array,
    B_w1: jax.Array,
    B_w2: jax.Array,
    B_w3: jax.Array,
    B_w4: jax.Array,
    c: jax.Array,
    w_mod: jax.Array,
):
    B, S, M = A_x.shape
    assert B == 1 and A_c_kv.shape[1] == S
    Dc = A_c_kv.shape[2]
    H, D = A_w_q.shape[1], A_w_q.shape[2]
    NP = H // 2
    Fd = B_w3.shape[1]
    any_spec = pl.BlockSpec(memory_space=pl.ANY)

    out = pl.pallas_call(
        functools.partial(_kernel, S=S, M=M, D=D, NP=NP, Fd=Fd),
        grid=(2,),
        in_specs=[any_spec] * 12,
        out_specs=any_spec,
        out_shape=jax.ShapeDtypeStruct((S, M), A_x.dtype),
        scratch_shapes=[
            pltpu.VMEM((S + 2 * HALO + S // NL, M), BF16),
            pltpu.VMEM((S // 2, Dc), U32),
            pltpu.VMEM((NP, M, D), U32),
            pltpu.VMEM((NP, Dc, D), U32),
            pltpu.VMEM((NP, Dc, D), U32),
            pltpu.VMEM((NP, D, M), U32),
            pltpu.VMEM((M // 2, M), U32),
            pltpu.VMEM((M // 2, M), U32),
            pltpu.VMEM((Fd // 2, M), U32),
            pltpu.VMEM((Fd // 2, M), U32),
            pltpu.VMEM((1, M), BF16),
            pltpu.VMEM((7, M // 2, M), U32),
            pltpu.VMEM((M // 2, 128), U32),
            pltpu.VMEM((7, 8, M), F32),
            pltpu.VMEM(((S + S // NL) // 2, M), U32),
            pltpu.VMEM((M // 2, 2 * D), U32),
            pltpu.VMEM((Dc // 2, 2 * KP * D), U32),
            pltpu.VMEM((Dc // 2, 2 * D), U32),
            pltpu.VMEM((D, M), U32),
            pltpu.VMEM((NP, S // 2, 2 * D), U32),
            pltpu.VMEM((S // 2, 2 * D), U32),
            pltpu.VMEM((S + 2 * HALO, M), F32),
            pltpu.VMEM((TB, M), F32),
            pltpu.VMEM((TB // 2, M), U32),
            pltpu.VMEM((S, M), BF16),
            pltpu.SemaphoreType.DMA((10,)),
            pltpu.SemaphoreType.DMA((CC,)),
            pltpu.SemaphoreType.DMA((NP,)),
            pltpu.SemaphoreType.DMA((6,)),
            pltpu.SemaphoreType.DMA((S // TB,)),
        ],
        compiler_params=pltpu.CompilerParams(
            vmem_limit_bytes=100 * 1024 * 1024,
            disable_bounds_checks=True,
            disable_semaphore_checks=True,
        ),
    )(
        A_x.reshape(S, M), A_c_kv.reshape(S, Dc),
        A_w_q, A_w_uk, A_w_uv,
        A_w_o.reshape(NP, 2 * D, M),
        B_w1, B_w2, B_w3.T, B_w4, c, w_mod,
    )
    return out.reshape(B, S, M)
```

```python
import functools
import math

import jax
import jax.numpy as jnp
from jax import lax
import jax.experimental.pallas as pl
import jax.experimental.pallas.tpu as pltpu

F32 = jnp.float32
BF16 = jnp.bfloat16
U32 = jnp.uint32
NT = (((1,), (1,)), ((), ()))
NEG = -1000000000.0
EPS = 1e-05
TQ = 128
TB = 256
TC = 64
LAG = 4
O_LAG = 4
Q_SUB = 0
T_SUB = 2
V_FIRST = 1
V_SPREAD = 4
O_HALF = True
CC = 4
KP = 2
TK = 256
NL = 4
HALO = 8


def _ln(x):
    m = jnp.mean(x, axis=-1, keepdims=True)
    xc = x - m
    v = jnp.mean(xc * xc, axis=-1, keepdims=True)
    return xc * lax.rsqrt(v + EPS)


def _gelu(x):
    c = math.sqrt(2.0 / math.pi)
    hx = 0.5 * x
    return hx + hx * jnp.tanh(x * (c + (c * 0.044715) * (x * x)))


def _as_bf16(u):
    return pltpu.bitcast(u, BF16)


def _as_u32(b):
    return pltpu.bitcast(b, U32)


def _halves(u):
    return pltpu.bitcast(u << 16, F32), pltpu.bitcast(u & jnp.uint32(0xFFFF0000), F32)


def _split_pair(u):
    return _as_u32(jnp.concatenate(_halves(u), axis=1).astype(BF16))


def _attention_schedule(nq):
    order = list(range(nq - 1, -1, -1))
    units = [(i, hh, half) for i in order for half in (1, 0) for hh in (0, 1)]
    ops = [("q", order[0])] + [("v", i) for i in range(V_FIRST)]
    for k in range(len(units) + LAG + O_LAG):
        n, sub = divmod(k, 4)
        if k < len(units):
            ops.append(("s",) + units[k])
        if 0 <= k - LAG < len(units):
            ops.append(("pv",) + units[k - LAG])
        if sub == Q_SUB and n + 1 < nq:
            ops.append(("q", order[n + 1]))
        if k < LAG:
            per = -(-(nq - V_FIRST) // V_SPREAD)
            ops.extend(("v", i) for i in range(V_FIRST + k * per, min(nq, V_FIRST + (k + 1) * per)))
        if sub == T_SUB and n % 2 == 0 and n + 1 < nq:
            ops.append(("t", order[n], order[n + 1]))
        ko = k - LAG - O_LAG
        if 0 <= ko < len(units):
            if O_HALF and ko % 2 == 1:
                ops.append(("o", units[ko][0], units[ko][2]))
            if not O_HALF and ko % 4 == 3:
                ops.append(("o", units[ko][0], None))
    return ops


def _after(lhs, deps, zero):
    t = None
    for dep in deps:
        for r in range(0, dep.shape[0], 8):
            for c in range(0, dep.shape[1], 128):
                tile = dep[r:r + 8, c:c + 128]
                t = tile if t is None else t | tile
    head = lhs[0:8, 0:128] | (t & zero)
    if lhs.shape[1] > 128:
        head = jnp.concatenate([head, lhs[0:8, 128:]], axis=1)
    return jnp.concatenate([head, lhs[8:]], axis=0)


def _kernel(x_hbm, ckv_hbm, wq_hbm, wk_hbm, wv_hbm, wo_hbm,
            w1_hbm, w2_hbm, w3t_hbm, w4_hbm, c_hbm, wmod_hbm,
            o_hbm,
            x_ref, ckv_ref, wqr_ref, wkr_ref, wvr_ref, wo_ref,
            w1_ref, w2_ref, w3t_ref, w4_ref, c_ref, wmod_ref,
            sc_ref, mod_ref, h_ref, wqp_ref, wkp_ref, wvp_ref, wop_ref, k_ref, v_ref, acc_ref,
            cr_ref, z_ref, u3_ref, ob_ref,
            ssem, csem, ksem, msem, osem,
            *, S, M, D, NP, Fd):
    NK = NP // KP
    nq = S // TQ
    HQ = TQ // 2
    qscale = (D ** -0.5) * math.log2(math.e)
    LR = S // NL
    NM = 6

    c_copy = pltpu.make_async_copy(c_hbm, c_ref, ssem.at[0])
    CR = S // CC // 2

    def ckv_copy(i):
        rows = pl.ds(i * CR if isinstance(i, int) else pl.multiple_of(i * CR, CR), CR)
        return pltpu.make_async_copy(ckv_hbm.bitcast(U32).at[rows, :], ckv_ref.at[rows, :],
                                     csem.at[i])

    x_copy = pltpu.make_async_copy(x_hbm, x_ref.at[pl.ds(HALO, S), :], ssem.at[2])
    wo_copy = pltpu.make_async_copy(wo_hbm.bitcast(U32), wo_ref, ssem.at[3])
    late_copies = [
        pltpu.make_async_copy(w1_hbm.bitcast(U32), w1_ref, ssem.at[4]),
        pltpu.make_async_copy(w2_hbm.bitcast(U32), w2_ref, ssem.at[5]),
        pltpu.make_async_copy(w3t_hbm.bitcast(U32), w3t_ref, ssem.at[6]),
        pltpu.make_async_copy(w4_hbm.bitcast(U32), w4_ref, ssem.at[7]),
    ]

    def wk_copy(p):
        return pltpu.make_async_copy(wk_hbm.bitcast(U32).at[:, p, :], wkr_ref.at[p], ksem.at[p])

    def wmod_copy(g):
        off = g * M if isinstance(g, int) else pl.multiple_of(g * M, 128)
        return pltpu.make_async_copy(wmod_hbm.bitcast(U32).at[:, pl.ds(off, M)],
                                     wmod_ref.at[g], msem.at[g])

    def stage_weights(p):
        wqp_ref[...] = _split_pair(wqr_ref[p])
        wvp_ref[...] = _split_pair(wvr_ref[p])
        wop_ref[...] = wo_ref[p]

    def stage_wk(step):
        for u in range(KP):
            wkp_ref[:, 2 * u * D:(2 * u + 2) * D] = _split_pair(wkr_ref[step * KP + u])

    def proj_k(step, rows, lhs):
        k = jnp.dot(_as_bf16(lhs), _as_bf16(wkp_ref[...]), preferred_element_type=F32)
        for u in range(KP):
            k_ref[step * KP + u, rows, :] = _as_u32(k[:, 2 * u * D:(2 * u + 2) * D].astype(BF16))

    def _prologue():
        c_copy.start()
        for p in range(KP):
            wk_copy(p).start()
        for i in range(CC):
            ckv_copy(i).start()
        x_ref[0:HALO, :] = jnp.zeros((HALO, M), BF16)
        x_ref[S + HALO:, :] = jnp.zeros((HALO + LR, M), BF16)
        for p in range(KP, 3 * KP):
            wk_copy(p).start()
        for g in range(2):
            wmod_copy(g).start()
        for p in range(3 * KP, NP):
            wk_copy(p).start()
        x_copy.start()
        for g in range(2, NM):
            wmod_copy(g).start()

        def start_qv(p, carry):
            pltpu.make_async_copy(wq_hbm.bitcast(U32).at[:, p, :], wqr_ref.at[p], ssem.at[8]).start()
            pltpu.make_async_copy(wv_hbm.bitcast(U32).at[:, p, :], wvr_ref.at[p], ssem.at[9]).start()
            return carry
        lax.fori_loop(0, NP, start_qv, 0)
        wo_copy.start()
        for cp in late_copies:
            cp.start()
        mod_ref[...] = jnp.zeros(mod_ref.shape, F32)
        acc_ref[S:, :] = jnp.zeros((2 * HALO, M), F32)
        c_copy.wait()
        c = c_ref[...].astype(F32)
        sc = jnp.broadcast_to(c * jax.nn.sigmoid(c), (128, M))
        sc_ref[...] = _as_u32(sc.T.astype(BF16))
        for p in range(KP):
            wk_copy(p).wait()
        stage_wk(0)

        def first_keys(i, carry):
            ckv_copy(i).wait()
            for ii in range(2 * CR // TK):
                rows = pl.ds(pl.multiple_of(i * CR + ii * (TK // 2), TK // 2), TK // 2)
                proj_k(0, rows, ckv_ref[rows, :])
            ar, wr = S // CC, M // 2 // CC
            acc_ref[pl.ds(pl.multiple_of(i * ar, ar), ar), :] = jnp.zeros((ar, M), F32)
            wmod_ref[NM, pl.ds(pl.multiple_of(i * wr, 8), wr), :] = jnp.zeros((wr, M), U32)
            return carry
        lax.fori_loop(0, CC, first_keys, 0)

    def _keys(step, carry):
        for u in range(KP):
            wk_copy(step * KP + u).wait()

        @pl.when(step >= NK - NM)
        def _():
            wmod_copy(step - (NK - NM)).wait()

        @pl.when(step == NK - NL)
        def _():
            x_copy.wait()

        stage_wk(step)
        g = jnp.where(step >= NK - NM, step - (NK - NM), NM)
        lblk = jnp.where(step >= NK - NL, step - (NK - NL), NL)
        xoff = jnp.where(step >= NK - NL, HALO, 2 * HALO)
        sa = mod_ref[0, 0:1, :]
        ca1 = 1.0 + mod_ref[1, 0:1, :]
        zero = pltpu.bitcast(acc_ref[0:8, 0:128], U32)
        nk = S // TK
        lc = LR // nk
        mc = M // 2 // nk
        deps, part = [], None
        for i in range(nk):
            rows = slice(i * TK // 2, (i + 1) * TK // 2)
            lhs = ckv_ref[rows, :]
            if deps:
                lhs = _after(lhs, deps, zero)
            proj_k(step, rows, lhs)
            r = pl.multiple_of(lblk * LR + i * lc + xoff, 8)
            rh = pl.multiple_of(lblk * (LR // 2) + i * (lc // 2), 8)
            x = x_ref[pl.ds(r, lc), :].astype(F32)
            h = _ln(x) * ca1 + sa
            h_ref[pl.ds(rh, lc // 2), :] = _as_u32(h.astype(BF16))
            we, wo = _halves(wmod_ref[g, i * mc:(i + 1) * mc, :])
            se, so = _halves(sc_ref[i * mc:(i + 1) * mc, :])
            prod = we * jnp.tile(se, (1, M // 128)) + wo * jnp.tile(so, (1, M // 128))
            for rr in range(0, mc, 8):
                part = prod[rr:rr + 8] if part is None else part + prod[rr:rr + 8]
            deps = [pltpu.bitcast(h, U32), pltpu.bitcast(part, U32)]
        mod_ref[g] = jnp.broadcast_to(jnp.sum(part, axis=0, keepdims=True), (8, M))
        return carry

    def _first_pair():
        pltpu.make_async_copy(wqr_ref, wqr_ref, ssem.at[8]).wait()
        pltpu.make_async_copy(wvr_ref, wvr_ref, ssem.at[9]).wait()
        wo_copy.wait()
        stage_weights(0)

    def _attention(j, carry):

        HH = HQ // 2
        row = lax.broadcasted_iota(jnp.int32, (HQ, TQ), 0)
        col = lax.broadcasted_iota(jnp.int32, (HQ, TQ), 1)
        diag = col <= row + HQ
        first = [col < HQ, col >= HQ]
        first0 = [col <= row, jnp.logical_and(col >= HQ, diag)]

        def proj_v(i):
            rows = slice(i * HQ, (i + 1) * HQ)
            v = jnp.dot(_as_bf16(ckv_ref[rows, :]), _as_bf16(wvp_ref[...]), preferred_element_type=F32)
            v_ref[rows, :] = _as_u32(v.astype(BF16))

        def proj_q(i):
            rows = slice(i * HQ, (i + 1) * HQ)
            q = jnp.dot(_as_bf16(h_ref[rows, :]), _as_bf16(wqp_ref[...]), preferred_element_type=F32)
            q = q * qscale
            return [q[:, 0:D].astype(BF16), q[:, D:2 * D].astype(BF16)]

        def masked_scores(qh, k):
            s = lax.dot_general(qh, k, NT, preferred_element_type=F32)
            n = s.shape[1] - TQ
            sd = jnp.where(diag, s[:, n:], NEG)
            return jnp.concatenate([s[:, :n], sd], axis=1) if n else sd

        def scores(q, hh, half, i):
            cols = slice(hh * D, (hh + 1) * D)
            if half == 1:
                return masked_scores(q[hh][HQ:TQ], _as_bf16(k_ref[j, 0:(i + 1) * HQ, cols]))
            if i > 0:
                return masked_scores(q[hh][0:HQ], _as_bf16(k_ref[j, HH:i * HQ + HH, cols]))
            return None

        def first_scores(q1, q2):
            st = [lax.dot_general(_as_bf16(k_ref[j, 0:HH, hh * D:(hh + 1) * D]),
                                  jnp.concatenate([q1[hh][0:HQ], q2[hh][0:HQ]], axis=0),
                                  NT, preferred_element_type=F32) for hh in range(2)]
            t = jnp.concatenate(st, axis=0).T
            return t[0:HQ], t[HQ:TQ]

        def softmax_pv(s, t0, hh, half, i):
            cols = slice(hh * D, (hh + 1) * D)
            if half == 1:
                v = v_ref[0:(i + 1) * HQ, cols]
            else:
                s0 = jnp.where(first[hh] if i > 0 else first0[hh], t0[i], NEG)
                s = s0 if s is None else jnp.concatenate([s, s0], axis=1)
                if hh == 0:
                    v = v_ref[0:HQ, cols]
                else:
                    v = jnp.concatenate([v_ref[HH:HQ, cols], v_ref[0:HH, cols]], axis=0)
                if i > 0:
                    v = jnp.concatenate([v_ref[HH:i * HQ + HH, cols], v], axis=0)
            m = jnp.max(s, axis=1, keepdims=True)
            p = jnp.exp2(s - m).astype(BF16)
            l = jnp.sum(p.astype(F32), axis=1, keepdims=True)
            o = jnp.dot(p, _as_bf16(v), preferred_element_type=F32)
            return o * pl.reciprocal(l, approx=False, full_range=False)

        def oproj(ctx, r, n):
            rows = slice(HALO + r, HALO + r + n)
            acc_ref[rows, :] += jnp.dot(ctx.astype(BF16), _as_bf16(wop_ref[...]),
                                        preferred_element_type=F32)

        q, s, t0, ctx = {}, {}, {}, {}
        for op in _attention_schedule(nq):
            kind, i = op[0], op[1]
            if kind == "q":
                q[i] = proj_q(i)
            elif kind == "v":
                proj_v(i)
            elif kind == "s":
                s[op[1:]] = scores(q[i], op[2], op[3], i)
            elif kind == "t":
                t0[i], t0[op[2]] = first_scores(q[i], q[op[2]])
            elif kind == "pv":
                ctx[op[1:]] = softmax_pv(s.pop(op[1:]), t0, op[2], op[3], i)
            elif op[2] is None:
                oproj(jnp.concatenate(
                    [jnp.concatenate([ctx.pop((i, hh, 0)), ctx.pop((i, hh, 1))], axis=0)
                     for hh in range(2)], axis=1), i * TQ, TQ)
            else:
                oproj(jnp.concatenate([ctx.pop((i, hh, op[2])) for hh in range(2)], axis=1),
                      i * TQ + op[2] * HQ, HQ)

        stage_weights(jnp.minimum(j + 1, NP - 1))
        return carry

    def _epilogue():
        for cp in late_copies:
            cp.wait()

        G = M // 4
        NC = TB // TC
        TH = TB + 2 * HALO
        hsplit = [0] + [2 * HALO + (k + 1) * TC for k in range(NC)]
        ntile = (Fd + 127) // 128
        fsplit = [min(Fd, ((k * ntile + NC - 1) // NC) * 128) for k in range(NC + 1)]

        def start_row(t):
            return t * TB if isinstance(t, int) else pl.multiple_of(t * TB, TB)

        def front_a(t, k, first):
            lo, hi = hsplit[k], hsplit[k + 1]
            if k == 0 and not first:
                lo = 2 * HALO
            r = start_row(t)
            ga = mod_ref[2, 0:1, :]
            sb = mod_ref[3, 0:1, :]
            cb1 = 1.0 + mod_ref[4, 0:1, :]
            x1 = (x_ref[pl.ds(r + lo, hi - lo), :].astype(F32)
                  + ga * acc_ref[pl.ds(r + lo, hi - lo), :])
            h = _ln(x1) * cb1 + sb
            tt = _gelu(jnp.dot(_ln(h).astype(BF16), _as_bf16(w1_ref[...]),
                               preferred_element_type=F32))
            if k == 0 and first:
                tt = jnp.concatenate([jnp.zeros((HALO, M), F32), tt[HALO:]], axis=0)
            if k == 0 and not first:
                x1, h, tt = [jnp.concatenate([cr_ref[a], v], axis=0)
                             for a, v in enumerate((x1, h, tt))]
            if k == NC - 1:
                n = hi - lo - HALO
                tt = jnp.concatenate([tt[:n], jnp.where(r + TB < S, tt[n:], 0.0)], axis=0)
                for a, v in enumerate((x1, h, tt)):
                    cr_ref[a] = v[n - HALO:]
            return x1, h, tt

        def front_b(x1, h, tt, k):
            lo = k * TC
            gb = mod_ref[5, 0:1, :]
            lane = lax.broadcasted_iota(jnp.int32, (TC, 128), 1)
            cols = []
            shifts = (-1, 1, -2, 2)
            for cblk in range(M // 128):
                c0, c1 = cblk * 128, (cblk + 1) * 128
                ga_, gb_ = c0 // G, (c1 - 1) // G
                a = tt[HALO + lo + shifts[ga_]:HALO + lo + shifts[ga_] + TC, c0:c1]
                if gb_ != ga_:
                    b = tt[HALO + lo + shifts[gb_]:HALO + lo + shifts[gb_] + TC, c0:c1]
                    a = jnp.where(lane < gb_ * G - c0, a, b)
                cols.append(a.astype(BF16))
            sh = jnp.concatenate(cols, axis=1)
            y = h[HALO + lo:HALO + lo + TC] + jnp.dot(sh, _as_bf16(w2_ref[...]),
                                                      preferred_element_type=F32)
            z_ref[lo:lo + TC, :] = x1[HALO + lo:HALO + lo + TC] + gb * y
            u3_ref[lo // 2:(lo + TC) // 2, :] = _as_u32(_ln(y).astype(BF16))

        def out_copy(t):
            rows = pl.ds(start_row(t), TB)
            return pltpu.make_async_copy(ob_ref.at[rows, :], o_hbm.at[rows, :], osem.at[t])

        def mm3(k):
            lo, hi = fsplit[k], fsplit[k + 1]
            mid = hi - hi % 128
            u3 = _as_bf16(u3_ref[...])
            f = _gelu(lax.dot_general(u3, _as_bf16(w3t_ref[lo // 2:mid // 2, :]),
                                      NT, preferred_element_type=F32))
            if mid < hi:
                ft = _gelu(lax.dot_general(_as_bf16(w3t_ref[mid // 2:hi // 2, :]), u3,
                                           NT, preferred_element_type=F32))
                f = jnp.concatenate([f, ft.T], axis=1)
            return f.astype(BF16)

        def mm4(t, f, z, k):
            lo = k * TC
            gb = mod_ref[5, 0:1, :]
            h2 = jnp.dot(f[lo:lo + TC], _as_bf16(w4_ref[...]), preferred_element_type=F32)
            ob_ref[pl.ds(start_row(t) + lo, TC), :] = (z + gb * h2).astype(ob_ref.dtype)

        def stage(t, cur, nxt):
            fs, fr = [], []
            for k in range(NC):
                if cur:
                    fs.append(mm3(k))
                if nxt:
                    fr.append(front_a(t + 1, k, not cur))
            if cur:
                f = jnp.concatenate(fs, axis=1)
            if nxt:
                fr = [jnp.concatenate(parts, axis=0) for parts in zip(*fr)]
            for k in range(NC):
                if cur:
                    z = z_ref[k * TC:(k + 1) * TC, :]
                if nxt and k == NC - 1:
                    front_b(*fr, k)
                if cur:
                    mm4(t, f, z, k)
                if nxt and k < NC - 1:
                    front_b(*fr, k)
            if cur:
                out_copy(t).start()

        nb = S // TB
        stage(-1, False, True)

        def loop_b(t, carry):
            stage(t, True, True)
            return carry
        lax.fori_loop(0, nb - 1, loop_b, 0)
        stage(nb - 1, True, False)
        for t in range(nb):
            out_copy(t).wait()

    @pl.when(pl.program_id(0) == 0)
    def _():
        _prologue()
        lax.fori_loop(1, NK, _keys, 0)
        _first_pair()
        lax.fori_loop(0, NP, _attention, 0)

    @pl.when(pl.program_id(0) == 1)
    def _():
        _epilogue()


@jax.jit
def pallas_adaLN_cond__compressed_kv_cla__mixer_s_mlp__prompt_kernel(
    A_x: jax.Array,
    A_c_kv: jax.Array,
    A_w_q: jax.Array,
    A_w_uk: jax.Array,
    A_w_uv: jax.Array,
    A_w_o: jax.Array,
    B_x: jax.Array,
    B_w1: jax.Array,
    B_w2: jax.Array,
    B_w3: jax.Array,
    B_w4: jax.Array,
    c: jax.Array,
    w_mod: jax.Array,
):
    B, S, M = A_x.shape
    assert B == 1 and A_c_kv.shape[1] == S
    Dc = A_c_kv.shape[2]
    H, D = A_w_q.shape[1], A_w_q.shape[2]
    NP = H // 2
    Fd = B_w3.shape[1]
    any_spec = pl.BlockSpec(memory_space=pl.ANY)

    out = pl.pallas_call(
        functools.partial(_kernel, S=S, M=M, D=D, NP=NP, Fd=Fd),
        grid=(2,),
        in_specs=[any_spec] * 12,
        out_specs=any_spec,
        out_shape=jax.ShapeDtypeStruct((S, M), A_x.dtype),
        scratch_shapes=[
            pltpu.VMEM((S + 2 * HALO + S // NL, M), BF16),
            pltpu.VMEM((S // 2, Dc), U32),
            pltpu.VMEM((NP, M, D), U32),
            pltpu.VMEM((NP, Dc, D), U32),
            pltpu.VMEM((NP, Dc, D), U32),
            pltpu.VMEM((NP, D, M), U32),
            pltpu.VMEM((M // 2, M), U32),
            pltpu.VMEM((M // 2, M), U32),
            pltpu.VMEM((Fd // 2, M), U32),
            pltpu.VMEM((Fd // 2, M), U32),
            pltpu.VMEM((1, M), BF16),
            pltpu.VMEM((7, M // 2, M), U32),
            pltpu.VMEM((M // 2, 128), U32),
            pltpu.VMEM((7, 8, M), F32),
            pltpu.VMEM(((S + S // NL) // 2, M), U32),
            pltpu.VMEM((M // 2, 2 * D), U32),
            pltpu.VMEM((Dc // 2, 2 * KP * D), U32),
            pltpu.VMEM((Dc // 2, 2 * D), U32),
            pltpu.VMEM((D, M), U32),
            pltpu.VMEM((NP, S // 2, 2 * D), U32),
            pltpu.VMEM((S // 2, 2 * D), U32),
            pltpu.VMEM((S + 2 * HALO, M), F32),
            pltpu.VMEM((3, 2 * HALO, M), F32),
            pltpu.VMEM((TB, M), F32),
            pltpu.VMEM((TB // 2, M), U32),
            pltpu.VMEM((S, M), BF16),
            pltpu.SemaphoreType.DMA((10,)),
            pltpu.SemaphoreType.DMA((CC,)),
            pltpu.SemaphoreType.DMA((NP,)),
            pltpu.SemaphoreType.DMA((6,)),
            pltpu.SemaphoreType.DMA((S // TB,)),
        ],
        compiler_params=pltpu.CompilerParams(
            vmem_limit_bytes=100 * 1024 * 1024,
            disable_bounds_checks=True,
            disable_semaphore_checks=True,
        ),
    )(
        A_x.reshape(S, M), A_c_kv.reshape(S, Dc),
        A_w_q, A_w_uk, A_w_uv,
        A_w_o.reshape(NP, 2 * D, M),
        B_w1, B_w2, B_w3.T, B_w4, c, w_mod,
    )
    return out.reshape(B, S, M)
```

```python
import functools
import math

import jax
import jax.numpy as jnp
from jax import lax
import jax.experimental.pallas as pl
import jax.experimental.pallas.tpu as pltpu

F32 = jnp.float32
BF16 = jnp.bfloat16
U32 = jnp.uint32
NT = (((1,), (1,)), ((), ()))
NEG = -1000000000.0
EPS = 1e-05
TQ = 128
TB = 256
TC = 64
LAG = 4
O_LAG = 4
Q_SUB = 0
T_SUB = 2
V_FIRST = 1
V_SPREAD = 4
O_HALF = True
CC = 4
KP = 2
TK = 256
NL = 4
HALO = 8


def _ln(x):
    m = jnp.mean(x, axis=-1, keepdims=True)
    xc = x - m
    v = jnp.mean(xc * xc, axis=-1, keepdims=True)
    return xc * lax.rsqrt(v + EPS)


def _gelu(x):
    c = math.sqrt(2.0 / math.pi)
    hx = 0.5 * x
    return hx + hx * jnp.tanh(x * (c + (c * 0.044715) * (x * x)))


def _as_bf16(u):
    return pltpu.bitcast(u, BF16)


def _as_u32(b):
    return pltpu.bitcast(b, U32)


def _halves(u):
    return pltpu.bitcast(u << 16, F32), pltpu.bitcast(u & jnp.uint32(0xFFFF0000), F32)


def _split_pair(u):
    return _as_u32(jnp.concatenate(_halves(u), axis=1).astype(BF16))


def _attention_schedule(nq):
    order = list(range(nq - 1, -1, -1))
    units = [(i, hh, half) for i in order for half in (1, 0) for hh in (0, 1)]
    ops = [("q", order[0])] + [("v", i) for i in range(V_FIRST)]
    for k in range(len(units) + LAG + O_LAG):
        n, sub = divmod(k, 4)
        if k < len(units):
            ops.append(("s",) + units[k])
        if 0 <= k - LAG < len(units):
            ops.append(("pv",) + units[k - LAG])
        if sub == Q_SUB and n + 1 < nq:
            ops.append(("q", order[n + 1]))
        if k < LAG:
            per = -(-(nq - V_FIRST) // V_SPREAD)
            ops.extend(("v", i) for i in range(V_FIRST + k * per, min(nq, V_FIRST + (k + 1) * per)))
        if sub == T_SUB and n % 2 == 0 and n + 1 < nq:
            ops.append(("t", order[n], order[n + 1]))
        ko = k - LAG - O_LAG
        if 0 <= ko < len(units):
            if O_HALF and ko % 2 == 1:
                ops.append(("o", units[ko][0], units[ko][2]))
            if not O_HALF and ko % 4 == 3:
                ops.append(("o", units[ko][0], None))
    return ops


def _after(lhs, deps, zero):
    t = None
    for dep in deps:
        for r in range(0, dep.shape[0], 8):
            for c in range(0, dep.shape[1], 128):
                tile = dep[r:r + 8, c:c + 128]
                t = tile if t is None else t | tile
    head = lhs[0:8, 0:128] | (t & zero)
    if lhs.shape[1] > 128:
        head = jnp.concatenate([head, lhs[0:8, 128:]], axis=1)
    return jnp.concatenate([head, lhs[8:]], axis=0)


def _kernel(x_hbm, ckv_hbm, wq_hbm, wk_hbm, wv_hbm, wo_hbm,
            w1_hbm, w2_hbm, w3t_hbm, w4_hbm, c_hbm, wmod_hbm,
            o_hbm,
            x_ref, ckv_ref, wqr_ref, wkr_ref, wvr_ref, wo_ref,
            w1_ref, w2_ref, w3t_ref, w4_ref, c_ref, wmod_ref,
            sc_ref, mod_ref, h_ref, wqp_ref, wkp_ref, wvp_ref, wop_ref, k_ref, v_ref, acc_ref,
            cr_ref, z_ref, u3_ref, ob_ref,
            ssem, csem, ksem, msem, osem,
            *, S, M, D, NP, Fd):
    NK = NP // KP
    nq = S // TQ
    HQ = TQ // 2
    qscale = (D ** -0.5) * math.log2(math.e)
    LR = S // NL
    NM = 6

    c_copy = pltpu.make_async_copy(c_hbm, c_ref, ssem.at[0])
    CR = S // CC // 2

    def ckv_copy(i):
        rows = pl.ds(i * CR if isinstance(i, int) else pl.multiple_of(i * CR, CR), CR)
        return pltpu.make_async_copy(ckv_hbm.bitcast(U32).at[rows, :], ckv_ref.at[rows, :],
                                     csem.at[i])

    x_copy = pltpu.make_async_copy(x_hbm, x_ref.at[pl.ds(HALO, S), :], ssem.at[2])
    wo_copy = pltpu.make_async_copy(wo_hbm.bitcast(U32), wo_ref, ssem.at[3])
    late_copies = [
        pltpu.make_async_copy(w1_hbm.bitcast(U32), w1_ref, ssem.at[4]),
        pltpu.make_async_copy(w2_hbm.bitcast(U32), w2_ref, ssem.at[5]),
        pltpu.make_async_copy(w3t_hbm.bitcast(U32), w3t_ref, ssem.at[6]),
        pltpu.make_async_copy(w4_hbm.bitcast(U32), w4_ref, ssem.at[7]),
    ]

    def wk_copy(p):
        return pltpu.make_async_copy(wk_hbm.bitcast(U32).at[:, p, :], wkr_ref.at[p], ksem.at[p])

    def wmod_copy(g):
        off = g * M if isinstance(g, int) else pl.multiple_of(g * M, 128)
        return pltpu.make_async_copy(wmod_hbm.bitcast(U32).at[:, pl.ds(off, M)],
                                     wmod_ref.at[g], msem.at[g])

    def stage_weights(p):
        wqp_ref[...] = _split_pair(wqr_ref[p])
        wvp_ref[...] = _split_pair(wvr_ref[p])
        wop_ref[...] = wo_ref[p]

    def stage_wk(step):
        for u in range(KP):
            wkp_ref[:, 2 * u * D:(2 * u + 2) * D] = _split_pair(wkr_ref[step * KP + u])

    def k_rows(p, lo, n):
        off = p * (S // 2) + lo
        return pl.ds(off if isinstance(off, int) else pl.multiple_of(off, 8), n)

    def proj_k(step, lo, lhs):
        k = jnp.dot(_as_bf16(lhs), _as_bf16(wkp_ref[...]), preferred_element_type=F32)
        for u in range(KP):
            k_ref[k_rows(step * KP + u, lo, TK // 2), :] = _as_u32(
                k[:, 2 * u * D:(2 * u + 2) * D].astype(BF16))

    def _prologue():
        c_copy.start()
        for p in range(KP):
            wk_copy(p).start()
        for i in range(CC):
            ckv_copy(i).start()
        x_ref[0:HALO, :] = jnp.zeros((HALO, M), BF16)
        x_ref[S + HALO:, :] = jnp.zeros((HALO + LR, M), BF16)
        for p in range(KP, 3 * KP):
            wk_copy(p).start()
        for g in range(2):
            wmod_copy(g).start()
        for p in range(3 * KP, NP):
            wk_copy(p).start()
        x_copy.start()
        for g in range(2, NM):
            wmod_copy(g).start()

        def start_qv(p, carry):
            pltpu.make_async_copy(wq_hbm.bitcast(U32).at[:, p, :], wqr_ref.at[p], ssem.at[8]).start()
            pltpu.make_async_copy(wv_hbm.bitcast(U32).at[:, p, :], wvr_ref.at[p], ssem.at[9]).start()
            return carry
        lax.fori_loop(0, NP, start_qv, 0)
        wo_copy.start()
        for cp in late_copies:
            cp.start()
        mod_ref[...] = jnp.zeros(mod_ref.shape, F32)
        acc_ref[S:, :] = jnp.zeros((2 * HALO, M), F32)

        def zero_fill(i, carry):
            ar, wr = S // 20 // 8 * 8 + 8, M // 2 // 20
            acc_ref[pl.ds(pl.multiple_of(jnp.minimum(i * ar, S - ar), 8), ar), :] = (
                jnp.zeros((ar, M), F32))
            wmod_ref[NM, pl.ds(pl.multiple_of(i * wr, 8), wr), :] = jnp.zeros((wr, M), U32)
            return carry
        lax.fori_loop(0, 20, zero_fill, 0)
        c_copy.wait()
        c = c_ref[...].astype(F32)
        sc = jnp.broadcast_to(c * jax.nn.sigmoid(c), (128, M))
        sc_ref[...] = _as_u32(sc.T.astype(BF16))
        for p in range(KP):
            wk_copy(p).wait()
        stage_wk(0)

        def first_keys(i, carry):
            ckv_copy(i).wait()
            for ii in range(2 * CR // TK):
                lo = pl.multiple_of(i * CR + ii * (TK // 2), TK // 2)
                proj_k(0, lo, ckv_ref[pl.ds(lo, TK // 2), :])
            return carry
        lax.fori_loop(0, CC, first_keys, 0)

    def _keys(step, carry):
        for u in range(KP):
            wk_copy(step * KP + u).wait()

        @pl.when(step >= NK - NM)
        def _():
            wmod_copy(step - (NK - NM)).wait()

        @pl.when(step == NK - NL)
        def _():
            x_copy.wait()

        stage_wk(step)
        g = jnp.where(step >= NK - NM, step - (NK - NM), NM)
        lblk = jnp.where(step >= NK - NL, step - (NK - NL), NL)
        xoff = jnp.where(step >= NK - NL, HALO, 2 * HALO)
        sa = mod_ref[0, 0:1, :]
        ca1 = 1.0 + mod_ref[1, 0:1, :]
        zero = pltpu.bitcast(acc_ref[0:8, 0:128], U32)
        nk = S // TK
        lc = LR // nk
        mc = M // 2 // nk
        deps, part = [], None
        for i in range(nk):
            rows = slice(i * TK // 2, (i + 1) * TK // 2)
            lhs = ckv_ref[rows, :]
            if deps:
                lhs = _after(lhs, deps, zero)
            proj_k(step, i * TK // 2, lhs)
            r = pl.multiple_of(lblk * LR + i * lc + xoff, 8)
            rh = pl.multiple_of(lblk * (LR // 2) + i * (lc // 2), 8)
            x = x_ref[pl.ds(r, lc), :].astype(F32)
            h = _ln(x) * ca1 + sa
            h_ref[pl.ds(rh, lc // 2), :] = _as_u32(h.astype(BF16))
            we, wo = _halves(wmod_ref[g, i * mc:(i + 1) * mc, :])
            se, so = _halves(sc_ref[i * mc:(i + 1) * mc, :])
            prod = we * jnp.tile(se, (1, M // 128)) + wo * jnp.tile(so, (1, M // 128))
            for rr in range(0, mc, 8):
                part = prod[rr:rr + 8] if part is None else part + prod[rr:rr + 8]
            deps = [pltpu.bitcast(h, U32), pltpu.bitcast(part, U32)]
        mod_ref[g] = jnp.broadcast_to(jnp.sum(part, axis=0, keepdims=True), (8, M))
        return carry

    def _first_pair():
        pltpu.make_async_copy(wqr_ref, wqr_ref, ssem.at[8]).wait()
        pltpu.make_async_copy(wvr_ref, wvr_ref, ssem.at[9]).wait()
        wo_copy.wait()
        stage_weights(0)

    def _attention(j, carry):

        HH = HQ // 2
        row = lax.broadcasted_iota(jnp.int32, (HQ, TQ), 0)
        col = lax.broadcasted_iota(jnp.int32, (HQ, TQ), 1)
        diag = col <= row + HQ
        first = [col < HQ, col >= HQ]
        first0 = [col <= row, jnp.logical_and(col >= HQ, diag)]

        def proj_v(i):
            rows = slice(i * HQ, (i + 1) * HQ)
            v = jnp.dot(_as_bf16(ckv_ref[rows, :]), _as_bf16(wvp_ref[...]), preferred_element_type=F32)
            v_ref[rows, :] = _as_u32(v.astype(BF16))

        def proj_q(i):
            rows = slice(i * HQ, (i + 1) * HQ)
            q = jnp.dot(_as_bf16(h_ref[rows, :]), _as_bf16(wqp_ref[...]), preferred_element_type=F32)
            q = q * qscale
            return [[q[half * HQ:(half + 1) * HQ, hh * D:(hh + 1) * D].astype(BF16)
                     for half in range(2)] for hh in range(2)]

        def masked_scores(qh, k):
            s = lax.dot_general(qh, k, NT, preferred_element_type=F32)
            n = s.shape[1] - TQ
            sd = jnp.where(diag, s[:, n:], NEG)
            return jnp.concatenate([s[:, :n], sd], axis=1) if n else sd

        def scores(q, hh, half, i):
            cols = slice(hh * D, (hh + 1) * D)
            if half == 1:
                return masked_scores(q[hh][1], _as_bf16(k_ref[k_rows(j, 0, (i + 1) * HQ), cols]))
            if i > 0:
                return masked_scores(q[hh][0], _as_bf16(k_ref[k_rows(j, HH, i * HQ), cols]))
            return None

        def first_scores(q1, q2):
            st = [lax.dot_general(_as_bf16(k_ref[k_rows(j, 0, HH), hh * D:(hh + 1) * D]),
                                  jnp.concatenate([q1[hh][0], q2[hh][0]], axis=0),
                                  NT, preferred_element_type=F32) for hh in range(2)]
            t = jnp.concatenate(st, axis=0).T
            return t[0:HQ], t[HQ:TQ]

        def softmax_pv(s, t0, hh, half, i):
            cols = slice(hh * D, (hh + 1) * D)
            if half == 1:
                v = v_ref[0:(i + 1) * HQ, cols]
            else:
                s0 = jnp.where(first[hh] if i > 0 else first0[hh], t0[i], NEG)
                s = s0 if s is None else jnp.concatenate([s, s0], axis=1)
                if hh == 0:
                    v = v_ref[0:HQ, cols]
                else:
                    v = jnp.concatenate([v_ref[HH:HQ, cols], v_ref[0:HH, cols]], axis=0)
                if i > 0:
                    v = jnp.concatenate([v_ref[HH:i * HQ + HH, cols], v], axis=0)
            m = jnp.max(s, axis=1, keepdims=True)
            p = jnp.exp2(s - m).astype(BF16)
            l = jnp.sum(p.astype(F32), axis=1, keepdims=True)
            o = jnp.dot(p, _as_bf16(v), preferred_element_type=F32)
            return o * pl.reciprocal(l, approx=False, full_range=False)

        def oproj(ctx, r, n):
            rows = slice(HALO + r, HALO + r + n)
            acc_ref[rows, :] += jnp.dot(ctx.astype(BF16), _as_bf16(wop_ref[...]),
                                        preferred_element_type=F32)

        q, s, t0, ctx = {}, {}, {}, {}
        for op in _attention_schedule(nq):
            kind, i = op[0], op[1]
            if kind == "q":
                q[i] = proj_q(i)
            elif kind == "v":
                proj_v(i)
            elif kind == "s":
                s[op[1:]] = scores(q[i], op[2], op[3], i)
            elif kind == "t":
                t0[i], t0[op[2]] = first_scores(q[i], q[op[2]])
            elif kind == "pv":
                ctx[op[1:]] = softmax_pv(s.pop(op[1:]), t0, op[2], op[3], i)
            elif op[2] is None:
                oproj(jnp.concatenate(
                    [jnp.concatenate([ctx.pop((i, hh, 0)), ctx.pop((i, hh, 1))], axis=0)
                     for hh in range(2)], axis=1), i * TQ, TQ)
            else:
                oproj(jnp.concatenate([ctx.pop((i, hh, op[2])) for hh in range(2)], axis=1),
                      i * TQ + op[2] * HQ, HQ)

        stage_weights(jnp.minimum(j + 1, NP - 1))
        return carry

    def _epilogue():
        for cp in late_copies:
            cp.wait()

        G = M // 4
        NC = TB // TC
        TH = TB + 2 * HALO
        hsplit = [0] + [2 * HALO + (k + 1) * TC for k in range(NC)]
        ntile = (Fd + 127) // 128
        fsplit = [min(Fd, ((k * ntile + NC - 1) // NC) * 128) for k in range(NC + 1)]

        def start_row(t):
            return t * TB if isinstance(t, int) else pl.multiple_of(t * TB, TB)

        def front_a(t, k, first):
            lo, hi = hsplit[k], hsplit[k + 1]
            if k == 0 and not first:
                lo = 2 * HALO
            r = start_row(t)
            ga = mod_ref[2, 0:1, :]
            sb = mod_ref[3, 0:1, :]
            cb1 = 1.0 + mod_ref[4, 0:1, :]
            x1 = (x_ref[pl.ds(r + lo, hi - lo), :].astype(F32)
                  + ga * acc_ref[pl.ds(r + lo, hi - lo), :])
            h = _ln(x1) * cb1 + sb
            tt = _gelu(jnp.dot(_ln(h).astype(BF16), _as_bf16(w1_ref[...]),
                               preferred_element_type=F32))
            if k == 0 and first:
                tt = jnp.concatenate([jnp.zeros((HALO, M), F32), tt[HALO:]], axis=0)
            if k == 0 and not first:
                x1, h, tt = [jnp.concatenate([cr_ref[a], v], axis=0)
                             for a, v in enumerate((x1, h, tt))]
            if k == NC - 1:
                n = hi - lo - HALO
                tt = jnp.concatenate([tt[:n], jnp.where(r + TB < S, tt[n:], 0.0)], axis=0)
                for a, v in enumerate((x1, h, tt)):
                    cr_ref[a] = v[n - HALO:]
            return x1, h, tt

        def front_b(x1, h, tt, k):
            lo = k * TC
            gb = mod_ref[5, 0:1, :]
            lane = lax.broadcasted_iota(jnp.int32, (TC, 128), 1)
            cols = []
            shifts = (-1, 1, -2, 2)
            for cblk in range(M // 128):
                c0, c1 = cblk * 128, (cblk + 1) * 128
                ga_, gb_ = c0 // G, (c1 - 1) // G
                a = tt[HALO + lo + shifts[ga_]:HALO + lo + shifts[ga_] + TC, c0:c1]
                if gb_ != ga_:
                    b = tt[HALO + lo + shifts[gb_]:HALO + lo + shifts[gb_] + TC, c0:c1]
                    a = jnp.where(lane < gb_ * G - c0, a, b)
                cols.append(a)
            sh = jnp.concatenate(cols, axis=1).astype(BF16)
            y = h[HALO + lo:HALO + lo + TC] + jnp.dot(sh, _as_bf16(w2_ref[...]),
                                                      preferred_element_type=F32)
            z_ref[lo:lo + TC, :] = x1[HALO + lo:HALO + lo + TC] + gb * y
            u3_ref[lo // 2:(lo + TC) // 2, :] = _as_u32(_ln(y).astype(BF16))

        def out_copy(t):
            rows = pl.ds(start_row(t), TB)
            return pltpu.make_async_copy(ob_ref.at[rows, :], o_hbm.at[rows, :], osem.at[t])

        def mm3(k):
            lo, hi = fsplit[k], fsplit[k + 1]
            mid = hi - hi % 128
            u3 = _as_bf16(u3_ref[...])
            f = _gelu(lax.dot_general(u3, _as_bf16(w3t_ref[lo // 2:mid // 2, :]),
                                      NT, preferred_element_type=F32))
            if mid < hi:
                ft = _gelu(lax.dot_general(_as_bf16(w3t_ref[mid // 2:hi // 2, :]), u3,
                                           NT, preferred_element_type=F32))
                f = jnp.concatenate([f, ft.T], axis=1)
            return [f[kk * TC:(kk + 1) * TC].astype(BF16) for kk in range(NC)]

        def mm4(t, f, z, k):
            lo = k * TC
            gb = mod_ref[5, 0:1, :]
            h2 = jnp.dot(jnp.concatenate([fk[k] for fk in f], axis=1), _as_bf16(w4_ref[...]),
                         preferred_element_type=F32)
            ob_ref[pl.ds(start_row(t) + lo, TC), :] = (z + gb * h2).astype(ob_ref.dtype)

        def stage(t, cur, nxt):
            fs, fr = [], []
            for k in range(NC):
                if cur:
                    fs.append(mm3(k))
                if nxt:
                    fr.append(front_a(t + 1, k, not cur))
            if nxt:
                fr = [jnp.concatenate(parts, axis=0) for parts in zip(*fr)]
            for k in range(NC):
                if cur:
                    z = z_ref[k * TC:(k + 1) * TC, :]
                if nxt and k == NC - 1:
                    front_b(*fr, k)
                if cur:
                    mm4(t, fs, z, k)
                if nxt and k < NC - 1:
                    front_b(*fr, k)
            if cur:
                out_copy(t).start()

        nb = S // TB
        stage(-1, False, True)

        def loop_b(t, carry):
            stage(t, True, True)
            return carry
        lax.fori_loop(0, nb - 1, loop_b, 0)
        stage(nb - 1, True, False)
        for t in range(nb):
            out_copy(t).wait()

    @pl.when(pl.program_id(0) == 0)
    def _():
        _prologue()
        lax.fori_loop(1, NK, _keys, 0)
        _first_pair()
        lax.fori_loop(0, NP, _attention, 0)

    @pl.when(pl.program_id(0) == 1)
    def _():
        _epilogue()


@jax.jit
def pallas_adaLN_cond__compressed_kv_cla__mixer_s_mlp__prompt_kernel(
    A_x: jax.Array,
    A_c_kv: jax.Array,
    A_w_q: jax.Array,
    A_w_uk: jax.Array,
    A_w_uv: jax.Array,
    A_w_o: jax.Array,
    B_x: jax.Array,
    B_w1: jax.Array,
    B_w2: jax.Array,
    B_w3: jax.Array,
    B_w4: jax.Array,
    c: jax.Array,
    w_mod: jax.Array,
):
    B, S, M = A_x.shape
    assert B == 1 and A_c_kv.shape[1] == S
    Dc = A_c_kv.shape[2]
    H, D = A_w_q.shape[1], A_w_q.shape[2]
    NP = H // 2
    Fd = B_w3.shape[1]
    any_spec = pl.BlockSpec(memory_space=pl.ANY)

    out = pl.pallas_call(
        functools.partial(_kernel, S=S, M=M, D=D, NP=NP, Fd=Fd),
        grid=(2,),
        in_specs=[any_spec] * 12,
        out_specs=any_spec,
        out_shape=jax.ShapeDtypeStruct((S, M), A_x.dtype),
        scratch_shapes=[
            pltpu.VMEM((S + 2 * HALO + S // NL, M), BF16),
            pltpu.VMEM((S // 2, Dc), U32),
            pltpu.VMEM((NP, M, D), U32),
            pltpu.VMEM((NP, Dc, D), U32),
            pltpu.VMEM((NP, Dc, D), U32),
            pltpu.VMEM((NP, D, M), U32),
            pltpu.VMEM((M // 2, M), U32),
            pltpu.VMEM((M // 2, M), U32),
            pltpu.VMEM((Fd // 2, M), U32),
            pltpu.VMEM((Fd // 2, M), U32),
            pltpu.VMEM((1, M), BF16),
            pltpu.VMEM((7, M // 2, M), U32),
            pltpu.VMEM((M // 2, 128), U32),
            pltpu.VMEM((7, 8, M), F32),
            pltpu.VMEM(((S + S // NL) // 2, M), U32),
            pltpu.VMEM((M // 2, 2 * D), U32),
            pltpu.VMEM((Dc // 2, 2 * KP * D), U32),
            pltpu.VMEM((Dc // 2, 2 * D), U32),
            pltpu.VMEM((D, M), U32),
            pltpu.VMEM((NP * S // 2, 2 * D), U32),
            pltpu.VMEM((S // 2, 2 * D), U32),
            pltpu.VMEM((S + 2 * HALO, M), F32),
            pltpu.VMEM((3, 2 * HALO, M), F32),
            pltpu.VMEM((TB, M), F32),
            pltpu.VMEM((TB // 2, M), U32),
            pltpu.VMEM((S, M), BF16),
            pltpu.SemaphoreType.DMA((10,)),
            pltpu.SemaphoreType.DMA((CC,)),
            pltpu.SemaphoreType.DMA((NP,)),
            pltpu.SemaphoreType.DMA((6,)),
            pltpu.SemaphoreType.DMA((S // TB,)),
        ],
        compiler_params=pltpu.CompilerParams(
            dimension_semantics=("arbitrary",),
            vmem_limit_bytes=100 * 1024 * 1024,
            disable_bounds_checks=True,
            disable_semaphore_checks=True,
        ),
    )(
        A_x.reshape(S, M), A_c_kv.reshape(S, Dc),
        A_w_q, A_w_uk, A_w_uv,
        A_w_o.reshape(NP, 2 * D, M),
        B_w1, B_w2, B_w3.T, B_w4, c, w_mod,
    )
    return out.reshape(B, S, M)
```

```python
import functools
import math

import jax
import jax.numpy as jnp
from jax import lax
import jax.experimental.pallas as pl
import jax.experimental.pallas.tpu as pltpu

F32 = jnp.float32
BF16 = jnp.bfloat16
U32 = jnp.uint32
NT = (((1,), (1,)), ((), ()))
NEG = -1000000000.0
EPS = 1e-05
TQ = 128
TB = 128
NS = 3
TC = 64
LAG = 4
O_LAG = 4
Q_SUB = 0
T_SUB = 2
V_FIRST = 1
V_SPREAD = 4
O_HALF = True
CC = 4
KP = 2
TK = 256
NL = 4
HALO = 8


def _ln(x):
    m = jnp.mean(x, axis=-1, keepdims=True)
    xc = x - m
    v = jnp.mean(xc * xc, axis=-1, keepdims=True)
    return xc * lax.rsqrt(v + EPS)


def _gelu(x):
    c = math.sqrt(2.0 / math.pi)
    hx = 0.5 * x
    return hx + hx * jnp.tanh(x * (c + (c * 0.044715) * (x * x)))


def _as_bf16(u):
    return pltpu.bitcast(u, BF16)


def _as_u32(b):
    return pltpu.bitcast(b, U32)


def _halves(u):
    return pltpu.bitcast(u << 16, F32), pltpu.bitcast(u & jnp.uint32(0xFFFF0000), F32)


def _split_pair(u):
    return _as_u32(jnp.concatenate(_halves(u), axis=1).astype(BF16))


def _attention_schedule(nq):
    order = list(range(nq - 1, -1, -1))
    units = [(i, hh, half) for i in order for half in (1, 0) for hh in (0, 1)]
    ops = [("q", order[0])] + [("v", i) for i in range(V_FIRST)]
    for k in range(len(units) + LAG + O_LAG):
        n, sub = divmod(k, 4)
        if k < len(units):
            ops.append(("s",) + units[k])
        if 0 <= k - LAG < len(units):
            ops.append(("pv",) + units[k - LAG])
        if sub == Q_SUB and n + 1 < nq:
            ops.append(("q", order[n + 1]))
        if k < LAG:
            per = -(-(nq - V_FIRST) // V_SPREAD)
            ops.extend(("v", i) for i in range(V_FIRST + k * per, min(nq, V_FIRST + (k + 1) * per)))
        if sub == T_SUB and n % 2 == 0 and n + 1 < nq:
            ops.append(("t", order[n], order[n + 1]))
        ko = k - LAG - O_LAG
        if 0 <= ko < len(units):
            if O_HALF and ko % 2 == 1:
                ops.append(("o", units[ko][0], units[ko][2]))
            if not O_HALF and ko % 4 == 3:
                ops.append(("o", units[ko][0], None))
    return ops


def _after(lhs, deps, zero):
    t = None
    for dep in deps:
        for r in range(0, dep.shape[0], 8):
            for c in range(0, dep.shape[1], 128):
                tile = dep[r:r + 8, c:c + 128]
                t = tile if t is None else t | tile
    head = lhs[0:8, 0:128] | (t & zero)
    if lhs.shape[1] > 128:
        head = jnp.concatenate([head, lhs[0:8, 128:]], axis=1)
    return jnp.concatenate([head, lhs[8:]], axis=0)


def _kernel(x_hbm, ckv_hbm, wq_hbm, wk_hbm, wv_hbm, wo_hbm,
            w1_hbm, w2_hbm, w3t_hbm, w4_hbm, c_hbm, wmod_hbm,
            o_hbm,
            x_ref, ckv_ref, wqr_ref, wkr_ref, wvr_ref, wo_ref,
            w1_ref, w2_ref, w3t_ref, w4_ref, c_ref, wmod_ref,
            sc_ref, mod_ref, h_ref, wqp_ref, wkp_ref, wvp_ref, wop_ref, k_ref, v_ref, acc_ref,
            cr_ref, z_ref, u3_ref, ob_ref,
            ssem, csem, ksem, msem, osem,
            *, S, M, D, NP, Fd):
    NK = NP // KP
    nq = S // TQ
    HQ = TQ // 2
    qscale = (D ** -0.5) * math.log2(math.e)
    LR = S // NL
    NM = 6

    c_copy = pltpu.make_async_copy(c_hbm, c_ref, ssem.at[0])
    CR = S // CC // 2

    def ckv_copy(i):
        rows = pl.ds(i * CR if isinstance(i, int) else pl.multiple_of(i * CR, CR), CR)
        return pltpu.make_async_copy(ckv_hbm.bitcast(U32).at[rows, :], ckv_ref.at[rows, :],
                                     csem.at[i])

    x_copy = pltpu.make_async_copy(x_hbm, x_ref.at[pl.ds(HALO, S), :], ssem.at[2])
    wo_copy = pltpu.make_async_copy(wo_hbm.bitcast(U32), wo_ref, ssem.at[3])
    late_copies = [
        pltpu.make_async_copy(w1_hbm.bitcast(U32), w1_ref, ssem.at[4]),
        pltpu.make_async_copy(w2_hbm.bitcast(U32), w2_ref, ssem.at[5]),
        pltpu.make_async_copy(w3t_hbm.bitcast(U32), w3t_ref, ssem.at[6]),
        pltpu.make_async_copy(w4_hbm.bitcast(U32), w4_ref, ssem.at[7]),
    ]

    def wk_copy(p):
        return pltpu.make_async_copy(wk_hbm.bitcast(U32).at[:, p, :], wkr_ref.at[p], ksem.at[p])

    def wmod_copy(g):
        off = g * M if isinstance(g, int) else pl.multiple_of(g * M, 128)
        return pltpu.make_async_copy(wmod_hbm.bitcast(U32).at[:, pl.ds(off, M)],
                                     wmod_ref.at[g], msem.at[g])

    def stage_weights(p):
        wqp_ref[...] = _split_pair(wqr_ref[p])
        wvp_ref[...] = _split_pair(wvr_ref[p])
        wop_ref[...] = wo_ref[p]

    def stage_wk(step):
        for u in range(KP):
            wkp_ref[:, 2 * u * D:(2 * u + 2) * D] = _split_pair(wkr_ref[step * KP + u])

    def k_rows(p, lo, n):
        off = p * (S // 2) + lo
        return pl.ds(off if isinstance(off, int) else pl.multiple_of(off, 8), n)

    def proj_k(step, lo, lhs):
        k = jnp.dot(_as_bf16(lhs), _as_bf16(wkp_ref[...]), preferred_element_type=F32)
        for u in range(KP):
            k_ref[k_rows(step * KP + u, lo, TK // 2), :] = _as_u32(
                k[:, 2 * u * D:(2 * u + 2) * D].astype(BF16))

    def _prologue():
        c_copy.start()
        for p in range(KP):
            wk_copy(p).start()
        for i in range(CC):
            ckv_copy(i).start()
        x_ref[0:HALO, :] = jnp.zeros((HALO, M), BF16)
        x_ref[S + HALO:, :] = jnp.zeros((HALO + LR, M), BF16)
        for p in range(KP, 3 * KP):
            wk_copy(p).start()
        for g in range(2):
            wmod_copy(g).start()
        for p in range(3 * KP, NP):
            wk_copy(p).start()
        x_copy.start()
        for g in range(2, NM):
            wmod_copy(g).start()

        def start_qv(p, carry):
            pltpu.make_async_copy(wq_hbm.bitcast(U32).at[:, p, :], wqr_ref.at[p], ssem.at[8]).start()
            pltpu.make_async_copy(wv_hbm.bitcast(U32).at[:, p, :], wvr_ref.at[p], ssem.at[9]).start()
            return carry
        lax.fori_loop(0, NP, start_qv, 0)
        wo_copy.start()
        for cp in late_copies:
            cp.start()
        mod_ref[...] = jnp.zeros(mod_ref.shape, F32)
        acc_ref[S:, :] = jnp.zeros((2 * HALO, M), F32)

        def zero_fill(i, carry):
            ar, wr = S // 20 // 8 * 8 + 8, M // 2 // 20
            acc_ref[pl.ds(pl.multiple_of(jnp.minimum(i * ar, S - ar), 8), ar), :] = (
                jnp.zeros((ar, M), F32))
            wmod_ref[NM, pl.ds(pl.multiple_of(i * wr, 8), wr), :] = jnp.zeros((wr, M), U32)
            return carry
        lax.fori_loop(0, 20, zero_fill, 0)
        c_copy.wait()
        c = c_ref[...].astype(F32)
        sc = jnp.broadcast_to(c * jax.nn.sigmoid(c), (128, M))
        sc_ref[...] = _as_u32(sc.T.astype(BF16))
        for p in range(KP):
            wk_copy(p).wait()
        stage_wk(0)

        def first_keys(i, carry):
            ckv_copy(i).wait()
            for ii in range(2 * CR // TK):
                lo = pl.multiple_of(i * CR + ii * (TK // 2), TK // 2)
                proj_k(0, lo, ckv_ref[pl.ds(lo, TK // 2), :])
            return carry
        lax.fori_loop(0, CC, first_keys, 0)

    def _keys(step, carry):
        for u in range(KP):
            wk_copy(step * KP + u).wait()

        @pl.when(step >= NK - NM)
        def _():
            wmod_copy(step - (NK - NM)).wait()

        @pl.when(step == NK - NL)
        def _():
            x_copy.wait()

        stage_wk(step)
        g = jnp.where(step >= NK - NM, step - (NK - NM), NM)
        lblk = jnp.where(step >= NK - NL, step - (NK - NL), NL)
        xoff = jnp.where(step >= NK - NL, HALO, 2 * HALO)
        sa = mod_ref[0, 0:1, :]
        ca1 = 1.0 + mod_ref[1, 0:1, :]
        zero = pltpu.bitcast(acc_ref[0:8, 0:128], U32)
        nk = S // TK
        lc = LR // nk
        mc = M // 2 // nk
        deps, part = [], None
        for i in range(nk):
            rows = slice(i * TK // 2, (i + 1) * TK // 2)
            lhs = ckv_ref[rows, :]
            if deps:
                lhs = _after(lhs, deps, zero)
            proj_k(step, i * TK // 2, lhs)
            r = pl.multiple_of(lblk * LR + i * lc + xoff, 8)
            rh = pl.multiple_of(lblk * (LR // 2) + i * (lc // 2), 8)
            x = x_ref[pl.ds(r, lc), :].astype(F32)
            h = _ln(x) * ca1 + sa
            h_ref[pl.ds(rh, lc // 2), :] = _as_u32(h.astype(BF16))
            we, wo = _halves(wmod_ref[g, i * mc:(i + 1) * mc, :])
            se, so = _halves(sc_ref[i * mc:(i + 1) * mc, :])
            prod = we * jnp.tile(se, (1, M // 128)) + wo * jnp.tile(so, (1, M // 128))
            for rr in range(0, mc, 8):
                part = prod[rr:rr + 8] if part is None else part + prod[rr:rr + 8]
            deps = [pltpu.bitcast(h, U32), pltpu.bitcast(part, U32)]
        mod_ref[g] = jnp.broadcast_to(jnp.sum(part, axis=0, keepdims=True), (8, M))
        return carry

    def _first_pair():
        pltpu.make_async_copy(wqr_ref, wqr_ref, ssem.at[8]).wait()
        pltpu.make_async_copy(wvr_ref, wvr_ref, ssem.at[9]).wait()
        wo_copy.wait()
        stage_weights(0)

    def _attention(j, carry):

        HH = HQ // 2
        row = lax.broadcasted_iota(jnp.int32, (HQ, TQ), 0)
        col = lax.broadcasted_iota(jnp.int32, (HQ, TQ), 1)
        diag = col <= row + HQ
        first = [col < HQ, col >= HQ]
        first0 = [col <= row, jnp.logical_and(col >= HQ, diag)]

        def proj_v(i):
            rows = slice(i * HQ, (i + 1) * HQ)
            v = jnp.dot(_as_bf16(ckv_ref[rows, :]), _as_bf16(wvp_ref[...]), preferred_element_type=F32)
            v_ref[rows, :] = _as_u32(v.astype(BF16))

        def proj_q(i):
            rows = slice(i * HQ, (i + 1) * HQ)
            q = jnp.dot(_as_bf16(h_ref[rows, :]), _as_bf16(wqp_ref[...]), preferred_element_type=F32)
            q = q * qscale
            return [[q[half * HQ:(half + 1) * HQ, hh * D:(hh + 1) * D].astype(BF16)
                     for half in range(2)] for hh in range(2)]

        def masked_scores(qh, k):
            s = lax.dot_general(qh, k, NT, preferred_element_type=F32)
            n = s.shape[1] - TQ
            sd = jnp.where(diag, s[:, n:], NEG)
            return jnp.concatenate([s[:, :n], sd], axis=1) if n else sd

        def scores(q, hh, half, i):
            cols = slice(hh * D, (hh + 1) * D)
            if half == 1:
                return masked_scores(q[hh][1], _as_bf16(k_ref[k_rows(j, 0, (i + 1) * HQ), cols]))
            if i > 0:
                return masked_scores(q[hh][0], _as_bf16(k_ref[k_rows(j, HH, i * HQ), cols]))
            return None

        def first_scores(q1, q2):
            st = [lax.dot_general(_as_bf16(k_ref[k_rows(j, 0, HH), hh * D:(hh + 1) * D]),
                                  jnp.concatenate([q1[hh][0], q2[hh][0]], axis=0),
                                  NT, preferred_element_type=F32) for hh in range(2)]
            t = jnp.concatenate(st, axis=0).T
            return t[0:HQ], t[HQ:TQ]

        def softmax_pv(s, t0, hh, half, i):
            cols = slice(hh * D, (hh + 1) * D)
            if half == 1:
                v = v_ref[0:(i + 1) * HQ, cols]
            else:
                s0 = jnp.where(first[hh] if i > 0 else first0[hh], t0[i], NEG)
                s = s0 if s is None else jnp.concatenate([s, s0], axis=1)
                if hh == 0:
                    v = v_ref[0:HQ, cols]
                else:
                    v = jnp.concatenate([v_ref[HH:HQ, cols], v_ref[0:HH, cols]], axis=0)
                if i > 0:
                    v = jnp.concatenate([v_ref[HH:i * HQ + HH, cols], v], axis=0)
            m = jnp.max(s, axis=1, keepdims=True)
            p = jnp.exp2(s - m).astype(BF16)
            l = jnp.sum(p.astype(F32), axis=1, keepdims=True)
            o = jnp.dot(p, _as_bf16(v), preferred_element_type=F32)
            return o * pl.reciprocal(l, approx=False, full_range=False)

        def oproj(ctx, r, n):
            rows = slice(HALO + r, HALO + r + n)
            acc_ref[rows, :] += jnp.dot(ctx.astype(BF16), _as_bf16(wop_ref[...]),
                                        preferred_element_type=F32)

        q, s, t0, ctx = {}, {}, {}, {}
        for op in _attention_schedule(nq):
            kind, i = op[0], op[1]
            if kind == "q":
                q[i] = proj_q(i)
            elif kind == "v":
                proj_v(i)
            elif kind == "s":
                s[op[1:]] = scores(q[i], op[2], op[3], i)
            elif kind == "t":
                t0[i], t0[op[2]] = first_scores(q[i], q[op[2]])
            elif kind == "pv":
                ctx[op[1:]] = softmax_pv(s.pop(op[1:]), t0, op[2], op[3], i)
            elif op[2] is None:
                oproj(jnp.concatenate(
                    [jnp.concatenate([ctx.pop((i, hh, 0)), ctx.pop((i, hh, 1))], axis=0)
                     for hh in range(2)], axis=1), i * TQ, TQ)
            else:
                oproj(jnp.concatenate([ctx.pop((i, hh, op[2])) for hh in range(2)], axis=1),
                      i * TQ + op[2] * HQ, HQ)

        stage_weights(jnp.minimum(j + 1, NP - 1))
        return carry

    def _epilogue():
        for cp in late_copies:
            cp.wait()

        G = M // 4
        NC = TB // TC
        TH = TB + 2 * HALO
        hsplit = [0] + [2 * HALO + (k + 1) * TC for k in range(NC)]
        ntile = (Fd + 127) // 128
        fsplit = [min(Fd, ((k * ntile + NC - 1) // NC) * 128) for k in range(NC + 1)]

        def start_row(t):
            return t * TB if isinstance(t, int) else pl.multiple_of(t * TB, TB)

        def front_a(t, k, first):
            lo, hi = hsplit[k], hsplit[k + 1]
            if k == 0 and not first:
                lo = 2 * HALO
            r = start_row(t)
            ga = mod_ref[2, 0:1, :]
            sb = mod_ref[3, 0:1, :]
            cb1 = 1.0 + mod_ref[4, 0:1, :]
            x1 = (x_ref[pl.ds(r + lo, hi - lo), :].astype(F32)
                  + ga * acc_ref[pl.ds(r + lo, hi - lo), :])
            h = _ln(x1) * cb1 + sb
            tt = _gelu(jnp.dot(_ln(h).astype(BF16), _as_bf16(w1_ref[...]),
                               preferred_element_type=F32))
            if k == 0 and first:
                tt = jnp.concatenate([jnp.zeros((HALO, M), F32), tt[HALO:]], axis=0)
            if k == 0 and not first:
                x1, h, tt = [jnp.concatenate([cr_ref[a], v], axis=0)
                             for a, v in enumerate((x1, h, tt))]
            if k == NC - 1:
                n = hi - lo - HALO
                tt = jnp.concatenate([tt[:n], jnp.where(r + TB < S, tt[n:], 0.0)], axis=0)
                for a, v in enumerate((x1, h, tt)):
                    cr_ref[a] = v[n - HALO:]
            return x1, h, tt

        def front_b(x1, h, tt, k):
            lo = k * TC
            gb = mod_ref[5, 0:1, :]
            lane = lax.broadcasted_iota(jnp.int32, (TC, 128), 1)
            cols = []
            shifts = (-1, 1, -2, 2)
            for cblk in range(M // 128):
                c0, c1 = cblk * 128, (cblk + 1) * 128
                ga_, gb_ = c0 // G, (c1 - 1) // G
                a = tt[HALO + lo + shifts[ga_]:HALO + lo + shifts[ga_] + TC, c0:c1]
                if gb_ != ga_:
                    b = tt[HALO + lo + shifts[gb_]:HALO + lo + shifts[gb_] + TC, c0:c1]
                    a = jnp.where(lane < gb_ * G - c0, a, b)
                cols.append(a)
            sh = jnp.concatenate(cols, axis=1).astype(BF16)
            y = h[HALO + lo:HALO + lo + TC] + jnp.dot(sh, _as_bf16(w2_ref[...]),
                                                      preferred_element_type=F32)
            z_ref[lo:lo + TC, :] = x1[HALO + lo:HALO + lo + TC] + gb * y
            u3_ref[lo // 2:(lo + TC) // 2, :] = _as_u32(_ln(y).astype(BF16))

        def out_copy(it, n):
            rows = pl.ds(start_row(it * NS), n * TB)
            return pltpu.make_async_copy(ob_ref.at[rows, :], o_hbm.at[rows, :], osem.at[it])

        def mm3(k):
            lo, hi = fsplit[k], fsplit[k + 1]
            mid = hi - hi % 128
            u3 = _as_bf16(u3_ref[...])
            f = _gelu(lax.dot_general(u3, _as_bf16(w3t_ref[lo // 2:mid // 2, :]),
                                      NT, preferred_element_type=F32))
            if mid < hi:
                ft = _gelu(lax.dot_general(_as_bf16(w3t_ref[mid // 2:hi // 2, :]), u3,
                                           NT, preferred_element_type=F32))
                f = jnp.concatenate([f, ft.T], axis=1)
            return [f[kk * TC:(kk + 1) * TC].astype(BF16) for kk in range(NC)]

        def mm4(t, f, z, k):
            lo = k * TC
            gb = mod_ref[5, 0:1, :]
            h2 = jnp.dot(jnp.concatenate([fk[k] for fk in f], axis=1), _as_bf16(w4_ref[...]),
                         preferred_element_type=F32)
            ob_ref[pl.ds(start_row(t) + lo, TC), :] = (z + gb * h2).astype(ob_ref.dtype)

        def stage(t, cur, nxt):
            fs, fr = [], []
            for k in range(NC):
                if cur:
                    fs.append(mm3(k))
                if nxt:
                    fr.append(front_a(t + 1, k, not cur))
            if nxt:
                fr = [jnp.concatenate(parts, axis=0) for parts in zip(*fr)]
            for k in range(NC):
                if cur:
                    z = z_ref[k * TC:(k + 1) * TC, :]
                if nxt and k == NC - 1:
                    front_b(*fr, k)
                if cur:
                    mm4(t, fs, z, k)
                if nxt and k < NC - 1:
                    front_b(*fr, k)

        nb = S // TB
        ni = (nb - 1) // NS
        assert ni * NS == nb - 1
        stage(-1, False, True)

        def loop_b(it, carry):
            for u in range(NS):
                stage(it * NS + u, True, True)
            out_copy(it, NS).start()
            return carry
        lax.fori_loop(0, ni, loop_b, 0)
        stage(nb - 1, True, False)
        out_copy(ni, 1).start()
        for it in range(ni):
            out_copy(it, NS).wait()
        out_copy(ni, 1).wait()

    @pl.when(pl.program_id(0) == 0)
    def _():
        _prologue()
        lax.fori_loop(1, NK, _keys, 0)
        _first_pair()
        lax.fori_loop(0, NP, _attention, 0)

    @pl.when(pl.program_id(0) == 1)
    def _():
        _epilogue()


@jax.jit
def pallas_adaLN_cond__compressed_kv_cla__mixer_s_mlp__prompt_kernel(
    A_x: jax.Array,
    A_c_kv: jax.Array,
    A_w_q: jax.Array,
    A_w_uk: jax.Array,
    A_w_uv: jax.Array,
    A_w_o: jax.Array,
    B_x: jax.Array,
    B_w1: jax.Array,
    B_w2: jax.Array,
    B_w3: jax.Array,
    B_w4: jax.Array,
    c: jax.Array,
    w_mod: jax.Array,
):
    B, S, M = A_x.shape
    assert B == 1 and A_c_kv.shape[1] == S
    Dc = A_c_kv.shape[2]
    H, D = A_w_q.shape[1], A_w_q.shape[2]
    NP = H // 2
    Fd = B_w3.shape[1]
    any_spec = pl.BlockSpec(memory_space=pl.ANY)

    out = pl.pallas_call(
        functools.partial(_kernel, S=S, M=M, D=D, NP=NP, Fd=Fd),
        grid=(2,),
        in_specs=[any_spec] * 12,
        out_specs=any_spec,
        out_shape=jax.ShapeDtypeStruct((S, M), A_x.dtype),
        scratch_shapes=[
            pltpu.VMEM((S + 2 * HALO + S // NL, M), BF16),
            pltpu.VMEM((S // 2, Dc), U32),
            pltpu.VMEM((NP, M, D), U32),
            pltpu.VMEM((NP, Dc, D), U32),
            pltpu.VMEM((NP, Dc, D), U32),
            pltpu.VMEM((NP, D, M), U32),
            pltpu.VMEM((M // 2, M), U32),
            pltpu.VMEM((M // 2, M), U32),
            pltpu.VMEM((Fd // 2, M), U32),
            pltpu.VMEM((Fd // 2, M), U32),
            pltpu.VMEM((1, M), BF16),
            pltpu.VMEM((7, M // 2, M), U32),
            pltpu.VMEM((M // 2, 128), U32),
            pltpu.VMEM((7, 8, M), F32),
            pltpu.VMEM(((S + S // NL) // 2, M), U32),
            pltpu.VMEM((M // 2, 2 * D), U32),
            pltpu.VMEM((Dc // 2, 2 * KP * D), U32),
            pltpu.VMEM((Dc // 2, 2 * D), U32),
            pltpu.VMEM((D, M), U32),
            pltpu.VMEM((NP * S // 2, 2 * D), U32),
            pltpu.VMEM((S // 2, 2 * D), U32),
            pltpu.VMEM((S + 2 * HALO, M), F32),
            pltpu.VMEM((3, 2 * HALO, M), F32),
            pltpu.VMEM((TB, M), F32),
            pltpu.VMEM((TB // 2, M), U32),
            pltpu.VMEM((S, M), BF16),
            pltpu.SemaphoreType.DMA((10,)),
            pltpu.SemaphoreType.DMA((CC,)),
            pltpu.SemaphoreType.DMA((NP,)),
            pltpu.SemaphoreType.DMA((6,)),
            pltpu.SemaphoreType.DMA(((S // TB - 1) // NS + 1,)),
        ],
        compiler_params=pltpu.CompilerParams(
            dimension_semantics=("arbitrary",),
            vmem_limit_bytes=100 * 1024 * 1024,
            disable_bounds_checks=True,
            disable_semaphore_checks=True,
        ),
    )(
        A_x.reshape(S, M), A_c_kv.reshape(S, Dc),
        A_w_q, A_w_uk, A_w_uv,
        A_w_o.reshape(NP, 2 * D, M),
        B_w1, B_w2, B_w3.T, B_w4, c, w_mod,
    )
    return out.reshape(B, S, M)
```

```python
import functools
import math

import jax
import jax.numpy as jnp
from jax import lax
import jax.experimental.pallas as pl
import jax.experimental.pallas.tpu as pltpu

F32 = jnp.float32
BF16 = jnp.bfloat16
U32 = jnp.uint32
NT = (((1,), (1,)), ((), ()))
NEG = -1000000000.0
EPS = 1e-05
TQ = 128
TB = 128
NS = 3
TC = 64
LAG = 4
O_LAG = 4
Q_SUB = 0
T_SUB = 2
V_FIRST = 1
V_SPREAD = 4
O_HALF = True
CC = 4
KP = 2
TK = 256
NL = 4
HALO = 8


def _ln(x):
    m = jnp.mean(x, axis=-1, keepdims=True)
    xc = x - m
    v = jnp.mean(xc * xc, axis=-1, keepdims=True)
    return xc * lax.rsqrt(v + EPS)


def _gelu(x):
    c = math.sqrt(2.0 / math.pi)
    hx = 0.5 * x
    return hx + hx * jnp.tanh(x * (c + (c * 0.044715) * (x * x)))


def _as_bf16(u):
    return pltpu.bitcast(u, BF16)


def _as_u32(b):
    return pltpu.bitcast(b, U32)


def _halves(u):
    return pltpu.bitcast(u << 16, F32), pltpu.bitcast(u & jnp.uint32(0xFFFF0000), F32)


def _split_pair(u):
    return _as_u32(jnp.concatenate(_halves(u), axis=1).astype(BF16))


def _attention_schedule(nq):
    order = list(range(nq - 1, -1, -1))
    units = [(i, hh, half) for i in order for half in (1, 0) for hh in (0, 1)]
    ops = [("q", order[0])] + [("v", i) for i in range(V_FIRST)]
    for k in range(len(units) + LAG + O_LAG):
        n, sub = divmod(k, 4)
        if k < len(units):
            ops.append(("s",) + units[k])
        if 0 <= k - LAG < len(units):
            ops.append(("pv",) + units[k - LAG])
        if sub == Q_SUB and n + 1 < nq:
            ops.append(("q", order[n + 1]))
        if k < LAG:
            per = -(-(nq - V_FIRST) // V_SPREAD)
            ops.extend(("v", i) for i in range(V_FIRST + k * per, min(nq, V_FIRST + (k + 1) * per)))
        if sub == T_SUB and n % 2 == 0 and n + 1 < nq:
            ops.append(("t", order[n], order[n + 1]))
        ko = k - LAG - O_LAG
        if 0 <= ko < len(units):
            if O_HALF and ko % 2 == 1:
                ops.append(("o", units[ko][0], units[ko][2]))
            if not O_HALF and ko % 4 == 3:
                ops.append(("o", units[ko][0], None))
    return ops


def _after(lhs, deps, zero):
    t = None
    for dep in deps:
        for r in range(0, dep.shape[0], 8):
            for c in range(0, dep.shape[1], 128):
                tile = dep[r:r + 8, c:c + 128]
                t = tile if t is None else t | tile
    head = lhs[0:8, 0:128] | (t & zero)
    if lhs.shape[1] > 128:
        head = jnp.concatenate([head, lhs[0:8, 128:]], axis=1)
    return jnp.concatenate([head, lhs[8:]], axis=0)


def _kernel(x_hbm, ckv_hbm, wq_hbm, wk_hbm, wv_hbm, wo_hbm,
            w1_hbm, w2_hbm, w3t_hbm, w4_hbm, c_hbm, wmod_hbm,
            o_hbm,
            x_ref, ckv_ref, wqr_ref, wkr_ref, wvr_ref, wo_ref,
            w1_ref, w2_ref, w3t_ref, w4_ref, c_ref, wmod_ref,
            zero_ref, sc_ref, mod_ref, h_ref, wqp_ref, wkp_ref, wvp_ref, wop_ref, k_ref, v_ref, acc_ref,
            cr_ref, z_ref, u3_ref, ob_ref,
            ssem, csem, ksem, msem, osem,
            *, S, M, D, NP, Fd):
    NK = NP // KP
    nq = S // TQ
    HQ = TQ // 2
    qscale = (D ** -0.5) * math.log2(math.e)
    LR = S // NL
    NM = 6
    nk = S // TK
    LC = LR // nk
    assert NK - 1 >= NM and NK - NL >= 3

    c_copy = pltpu.make_async_copy(c_hbm, c_ref, ssem.at[0])
    CR = S // CC // 2
    HK = TK // 2

    def ckv_copy(lo, n, sem):
        rows = pl.ds(lo if isinstance(lo, int) else pl.multiple_of(lo, HK), n)
        return pltpu.make_async_copy(ckv_hbm.bitcast(U32).at[rows, :], ckv_ref.at[rows, :],
                                     csem.at[sem])

    def ckv_head(i):
        return ckv_copy(i * HK, HK, i)

    def ckv_chunk(i):
        return ckv_copy(i * CR, CR, CR // HK - 1 + i)

    x_copy = pltpu.make_async_copy(x_hbm, x_ref.at[pl.ds(HALO, S), :], ssem.at[2])
    wo_copy = pltpu.make_async_copy(wo_hbm.bitcast(U32), wo_ref, ssem.at[3])
    late_copies = [
        pltpu.make_async_copy(w1_hbm.bitcast(U32), w1_ref, ssem.at[4]),
        pltpu.make_async_copy(w2_hbm.bitcast(U32), w2_ref, ssem.at[5]),
        pltpu.make_async_copy(w3t_hbm.bitcast(U32), w3t_ref, ssem.at[6]),
        pltpu.make_async_copy(w4_hbm.bitcast(U32), w4_ref, ssem.at[7]),
    ]

    def wk_copy(p):
        return pltpu.make_async_copy(wk_hbm.bitcast(U32).at[:, p, :], wkr_ref.at[p], ksem.at[p])

    def wmod_copy(g):
        off = g * M if isinstance(g, int) else pl.multiple_of(g * M, 128)
        return pltpu.make_async_copy(wmod_hbm.bitcast(U32).at[:, pl.ds(off, M)],
                                     wmod_ref.at[g], msem.at[g])

    def stage_weights(p):
        wqp_ref[...] = _split_pair(wqr_ref[p])
        wvp_ref[...] = _split_pair(wvr_ref[p])
        wop_ref[...] = wo_ref[p]

    def stage_wk(step, us=tuple(range(KP))):
        for u in us:
            wkp_ref[:, 2 * u * D:(2 * u + 2) * D] = _split_pair(wkr_ref[step * KP + u])

    def k_rows(p, lo, n):
        off = p * (S // 2) + lo
        return pl.ds(off if isinstance(off, int) else pl.multiple_of(off, 8), n)

    def proj_k(step, lo, lhs, u0=0, u1=KP):
        k = jnp.dot(_as_bf16(lhs), _as_bf16(wkp_ref[:, 2 * u0 * D:2 * u1 * D]),
                    preferred_element_type=F32)
        for u in range(u0, u1):
            k_ref[k_rows(step * KP + u, lo, HK), :] = _as_u32(
                k[:, 2 * (u - u0) * D:2 * (u - u0 + 1) * D].astype(BF16))

    def _prologue():
        c_copy.start()
        wk_copy(0).start()
        for i in range(CR // HK):
            ckv_head(i).start()
        for p in range(1, KP):
            wk_copy(p).start()
        for i in range(1, CC):
            ckv_chunk(i).start()
        x_ref[0:HALO, :] = jnp.zeros((HALO, M), BF16)
        x_ref[S + HALO:, :] = jnp.zeros((HALO + LC, M), BF16)
        for g in range(2):
            for p in range((g + 1) * KP, (g + 2) * KP):
                wk_copy(p).start()
            wmod_copy(g).start()

        def start_wk(p, carry):
            wk_copy(p).start()
            return carry
        lax.fori_loop(3 * KP, NP, start_wk, 0)
        wmod_copy(2).start()
        x_copy.start()
        for g in range(3, NM):
            wmod_copy(g).start()

        def start_qv(p, carry):
            pltpu.make_async_copy(wq_hbm.bitcast(U32).at[:, p, :], wqr_ref.at[p], ssem.at[8]).start()
            pltpu.make_async_copy(wv_hbm.bitcast(U32).at[:, p, :], wvr_ref.at[p], ssem.at[9]).start()
            return carry
        lax.fori_loop(0, NP, start_qv, 0)
        wo_copy.start()
        for cp in late_copies:
            cp.start()
        mod_ref[0:2] = jnp.zeros((2, 8, M), F32)
        zero_ref[...] = jnp.zeros(zero_ref.shape, U32)
        c_copy.wait()
        c = c_ref[...].astype(F32)
        sc = jnp.broadcast_to(c * jax.nn.sigmoid(c), (128, M))
        sc_ref[...] = _as_u32(sc.T.astype(BF16))
        wk_copy(0).wait()
        stage_wk(0, (0,))

        def head_keys(i, carry):
            ckv_head(i).wait()
            lo = pl.multiple_of(i * HK, HK)
            proj_k(0, lo, ckv_ref[pl.ds(lo, HK), :], 0, 1)
            return carry
        lax.fori_loop(0, CR // HK, head_keys, 0)
        for p in range(1, KP):
            wk_copy(p).wait()
        stage_wk(0, tuple(range(1, KP)))
        for i in range(CR // HK):
            proj_k(0, i * HK, ckv_ref[i * HK:(i + 1) * HK, :], 1, KP)

        def first_keys(i, carry):
            ckv_chunk(i).wait()
            for ii in range(CR // HK):
                lo = pl.multiple_of(i * CR + ii * HK, HK)
                proj_k(0, lo, ckv_ref[pl.ds(lo, HK), :])
            return carry
        lax.fori_loop(1, CC, first_keys, 0)

    def _keys(step, carry):
        for u in range(KP):
            wk_copy(step * KP + u).wait()

        @pl.when(step <= NM)
        def _():
            wmod_copy(step - 1).wait()

        @pl.when(step == NK - NL)
        def _():
            x_copy.wait()

        stage_wk(step)
        g = jnp.minimum(step - 1, NM - 1)
        live = step >= NK - NL
        lblk = step - (NK - NL)
        sa = mod_ref[0, 0:1, :]
        ca1 = 1.0 + mod_ref[1, 0:1, :]
        zero = zero_ref[...]
        mc = M // 2 // nk
        ar = -(-(S + 2 * HALO) // ((NK - 1) * nk * 8)) * 8
        deps, part = [], None
        for i in range(nk):
            lhs = ckv_ref[i * HK:(i + 1) * HK, :]
            if deps:
                lhs = _after(lhs, deps, zero)
            proj_k(step, i * HK, lhs)
            r = pl.multiple_of(jnp.where(live, HALO + lblk * LR + i * LC, S + 2 * HALO), 8)
            rh = pl.multiple_of(jnp.where(live, (lblk * LR + i * LC) // 2, S // 2), 8)
            x = x_ref[pl.ds(r, LC), :].astype(F32)
            h = _ln(x) * ca1 + sa
            h_ref[pl.ds(rh, LC // 2), :] = _as_u32(h.astype(BF16))
            we, wo = _halves(wmod_ref[g, i * mc:(i + 1) * mc, :])
            se, so = _halves(sc_ref[i * mc:(i + 1) * mc, :])
            prod = we * jnp.tile(se, (1, M // 128)) + wo * jnp.tile(so, (1, M // 128))
            for rr in range(0, mc, 8):
                part = prod[rr:rr + 8] if part is None else part + prod[rr:rr + 8]
            deps = [pltpu.bitcast(h, U32), pltpu.bitcast(part, U32)]
            zt = pltpu.bitcast(deps[1][:, 0:128] & zero, F32)
            ra = jnp.minimum(((step - 1) * nk + i) * ar, S + 2 * HALO - ar)
            acc_ref[pl.ds(pl.multiple_of(ra, 8), ar), :] = jnp.tile(zt, (ar // 8, M // 128))
        mod_ref[g] = jnp.broadcast_to(jnp.sum(part, axis=0, keepdims=True), (8, M))
        return carry

    def _first_pair():
        pltpu.make_async_copy(wqr_ref, wqr_ref, ssem.at[8]).wait()
        pltpu.make_async_copy(wvr_ref, wvr_ref, ssem.at[9]).wait()
        wo_copy.wait()
        stage_weights(0)

    def _attention(j, carry):

        HH = HQ // 2
        row = lax.broadcasted_iota(jnp.int32, (HQ, TQ), 0)
        col = lax.broadcasted_iota(jnp.int32, (HQ, TQ), 1)
        diag = col <= row + HQ
        first = [col < HQ, col >= HQ]
        first0 = [col <= row, jnp.logical_and(col >= HQ, diag)]

        def proj_v(i):
            rows = slice(i * HQ, (i + 1) * HQ)
            v = jnp.dot(_as_bf16(ckv_ref[rows, :]), _as_bf16(wvp_ref[...]), preferred_element_type=F32)
            v_ref[rows, :] = _as_u32(v.astype(BF16))

        def proj_q(i):
            rows = slice(i * HQ, (i + 1) * HQ)
            q = jnp.dot(_as_bf16(h_ref[rows, :]), _as_bf16(wqp_ref[...]), preferred_element_type=F32)
            q = q * qscale
            return [[q[half * HQ:(half + 1) * HQ, hh * D:(hh + 1) * D].astype(BF16)
                     for half in range(2)] for hh in range(2)]

        def masked_scores(qh, k):
            s = lax.dot_general(qh, k, NT, preferred_element_type=F32)
            n = s.shape[1] - TQ
            sd = jnp.where(diag, s[:, n:], NEG)
            return jnp.concatenate([s[:, :n], sd], axis=1) if n else sd

        def scores(q, hh, half, i):
            cols = slice(hh * D, (hh + 1) * D)
            if half == 1:
                return masked_scores(q[hh][1], _as_bf16(k_ref[k_rows(j, 0, (i + 1) * HQ), cols]))
            if i > 0:
                return masked_scores(q[hh][0], _as_bf16(k_ref[k_rows(j, HH, i * HQ), cols]))
            return None

        def first_scores(q1, q2):
            st = [lax.dot_general(_as_bf16(k_ref[k_rows(j, 0, HH), hh * D:(hh + 1) * D]),
                                  jnp.concatenate([q1[hh][0], q2[hh][0]], axis=0),
                                  NT, preferred_element_type=F32) for hh in range(2)]
            t = jnp.concatenate(st, axis=0).T
            return t[0:HQ], t[HQ:TQ]

        def softmax_pv(s, t0, hh, half, i):
            cols = slice(hh * D, (hh + 1) * D)
            if half == 1:
                v = v_ref[0:(i + 1) * HQ, cols]
            else:
                s0 = jnp.where(first[hh] if i > 0 else first0[hh], t0[i], NEG)
                s = s0 if s is None else jnp.concatenate([s, s0], axis=1)
                if hh == 0:
                    v = v_ref[0:HQ, cols]
                else:
                    v = jnp.concatenate([v_ref[HH:HQ, cols], v_ref[0:HH, cols]], axis=0)
                if i > 0:
                    v = jnp.concatenate([v_ref[HH:i * HQ + HH, cols], v], axis=0)
            m = jnp.max(s, axis=1, keepdims=True)
            p = jnp.exp2(s - m).astype(BF16)
            l = jnp.sum(p.astype(F32), axis=1, keepdims=True)
            o = jnp.dot(p, _as_bf16(v), preferred_element_type=F32)
            return o * pl.reciprocal(l, approx=False, full_range=False)

        def oproj(ctx, r, n):
            rows = slice(HALO + r, HALO + r + n)
            acc_ref[rows, :] += jnp.dot(ctx.astype(BF16), _as_bf16(wop_ref[...]),
                                        preferred_element_type=F32)

        q, s, t0, ctx = {}, {}, {}, {}
        for op in _attention_schedule(nq):
            kind, i = op[0], op[1]
            if kind == "q":
                q[i] = proj_q(i)
            elif kind == "v":
                proj_v(i)
            elif kind == "s":
                s[op[1:]] = scores(q[i], op[2], op[3], i)
            elif kind == "t":
                t0[i], t0[op[2]] = first_scores(q[i], q[op[2]])
            elif kind == "pv":
                ctx[op[1:]] = softmax_pv(s.pop(op[1:]), t0, op[2], op[3], i)
            elif op[2] is None:
                oproj(jnp.concatenate(
                    [jnp.concatenate([ctx.pop((i, hh, 0)), ctx.pop((i, hh, 1))], axis=0)
                     for hh in range(2)], axis=1), i * TQ, TQ)
            else:
                oproj(jnp.concatenate([ctx.pop((i, hh, op[2])) for hh in range(2)], axis=1),
                      i * TQ + op[2] * HQ, HQ)

        stage_weights(jnp.minimum(j + 1, NP - 1))
        return carry

    def _epilogue():
        for cp in late_copies:
            cp.wait()

        G = M // 4
        NC = TB // TC
        TH = TB + 2 * HALO
        hsplit = [0] + [2 * HALO + (k + 1) * TC for k in range(NC)]
        ntile = (Fd + 127) // 128
        fsplit = [min(Fd, ((k * ntile + NC - 1) // NC) * 128) for k in range(NC + 1)]

        def start_row(t):
            return t * TB if isinstance(t, int) else pl.multiple_of(t * TB, TB)

        def front_a(t, k, first):
            lo, hi = hsplit[k], hsplit[k + 1]
            if k == 0 and not first:
                lo = 2 * HALO
            r = start_row(t)
            ga = mod_ref[2, 0:1, :]
            sb = mod_ref[3, 0:1, :]
            cb1 = 1.0 + mod_ref[4, 0:1, :]
            x1 = (x_ref[pl.ds(r + lo, hi - lo), :].astype(F32)
                  + ga * acc_ref[pl.ds(r + lo, hi - lo), :])
            h = _ln(x1) * cb1 + sb
            tt = _gelu(jnp.dot(_ln(h).astype(BF16), _as_bf16(w1_ref[...]),
                               preferred_element_type=F32))
            if k == 0 and first:
                tt = jnp.concatenate([jnp.zeros((HALO, M), F32), tt[HALO:]], axis=0)
            if k == 0 and not first:
                x1, h, tt = [jnp.concatenate([cr_ref[a], v], axis=0)
                             for a, v in enumerate((x1, h, tt))]
            if k == NC - 1:
                n = hi - lo - HALO
                tt = jnp.concatenate([tt[:n], jnp.where(r + TB < S, tt[n:], 0.0)], axis=0)
                for a, v in enumerate((x1, h, tt)):
                    cr_ref[a] = v[n - HALO:]
            return x1, h, tt

        def front_b(x1, h, tt, k):
            lo = k * TC
            gb = mod_ref[5, 0:1, :]
            lane = lax.broadcasted_iota(jnp.int32, (TC, 128), 1)
            cols = []
            shifts = (-1, 1, -2, 2)
            for cblk in range(M // 128):
                c0, c1 = cblk * 128, (cblk + 1) * 128
                ga_, gb_ = c0 // G, (c1 - 1) // G
                a = tt[HALO + lo + shifts[ga_]:HALO + lo + shifts[ga_] + TC, c0:c1]
                if gb_ != ga_:
                    b = tt[HALO + lo + shifts[gb_]:HALO + lo + shifts[gb_] + TC, c0:c1]
                    a = jnp.where(lane < gb_ * G - c0, a, b)
                cols.append(a)
            sh = jnp.concatenate(cols, axis=1).astype(BF16)
            y = h[HALO + lo:HALO + lo + TC] + jnp.dot(sh, _as_bf16(w2_ref[...]),
                                                      preferred_element_type=F32)
            z_ref[lo:lo + TC, :] = x1[HALO + lo:HALO + lo + TC] + gb * y
            u3_ref[lo // 2:(lo + TC) // 2, :] = _as_u32(_ln(y).astype(BF16))

        def out_copy(it, n):
            rows = pl.ds(start_row(it * NS), n * TB)
            return pltpu.make_async_copy(ob_ref.at[rows, :], o_hbm.at[rows, :], osem.at[it])

        def mm3(k):
            lo, hi = fsplit[k], fsplit[k + 1]
            mid = hi - hi % 128
            u3 = _as_bf16(u3_ref[...])
            f = _gelu(lax.dot_general(u3, _as_bf16(w3t_ref[lo // 2:mid // 2, :]),
                                      NT, preferred_element_type=F32))
            if mid < hi:
                ft = _gelu(lax.dot_general(_as_bf16(w3t_ref[mid // 2:hi // 2, :]), u3,
                                           NT, preferred_element_type=F32))
                f = jnp.concatenate([f, ft.T], axis=1)
            return [f[kk * TC:(kk + 1) * TC].astype(BF16) for kk in range(NC)]

        def mm4(t, f, z, k):
            lo = k * TC
            gb = mod_ref[5, 0:1, :]
            h2 = jnp.dot(jnp.concatenate([fk[k] for fk in f], axis=1), _as_bf16(w4_ref[...]),
                         preferred_element_type=F32)
            ob_ref[pl.ds(start_row(t) + lo, TC), :] = (z + gb * h2).astype(ob_ref.dtype)

        def stage(t, cur, nxt):
            fs, fr = [], []
            for k in range(NC):
                if cur:
                    fs.append(mm3(k))
                if nxt:
                    fr.append(front_a(t + 1, k, not cur))
            if nxt:
                fr = [jnp.concatenate(parts, axis=0) for parts in zip(*fr)]
            for k in range(NC):
                if cur:
                    z = z_ref[k * TC:(k + 1) * TC, :]
                if nxt and k == NC - 1:
                    front_b(*fr, k)
                if cur:
                    mm4(t, fs, z, k)
                if nxt and k < NC - 1:
                    front_b(*fr, k)

        nb = S // TB
        ni = (nb - 1) // NS
        assert ni * NS == nb - 1
        stage(-1, False, True)

        def loop_b(it, carry):
            for u in range(NS):
                stage(it * NS + u, True, True)
            out_copy(it, NS).start()
            return carry
        lax.fori_loop(0, ni, loop_b, 0)
        stage(nb - 1, True, False)
        out_copy(ni, 1).start()
        for it in range(ni):
            out_copy(it, NS).wait()
        out_copy(ni, 1).wait()

    @pl.when(pl.program_id(0) == 0)
    def _():
        _prologue()
        lax.fori_loop(1, NK, _keys, 0)
        _first_pair()
        lax.fori_loop(0, NP, _attention, 0)

    @pl.when(pl.program_id(0) == 1)
    def _():
        _epilogue()


@jax.jit
def pallas_adaLN_cond__compressed_kv_cla__mixer_s_mlp__prompt_kernel(
    A_x: jax.Array,
    A_c_kv: jax.Array,
    A_w_q: jax.Array,
    A_w_uk: jax.Array,
    A_w_uv: jax.Array,
    A_w_o: jax.Array,
    B_x: jax.Array,
    B_w1: jax.Array,
    B_w2: jax.Array,
    B_w3: jax.Array,
    B_w4: jax.Array,
    c: jax.Array,
    w_mod: jax.Array,
):
    B, S, M = A_x.shape
    assert B == 1 and A_c_kv.shape[1] == S
    Dc = A_c_kv.shape[2]
    H, D = A_w_q.shape[1], A_w_q.shape[2]
    NP = H // 2
    Fd = B_w3.shape[1]
    LC = TK // NL
    any_spec = pl.BlockSpec(memory_space=pl.ANY)

    out = pl.pallas_call(
        functools.partial(_kernel, S=S, M=M, D=D, NP=NP, Fd=Fd),
        grid=(2,),
        in_specs=[any_spec] * 12,
        out_specs=any_spec,
        out_shape=jax.ShapeDtypeStruct((S, M), A_x.dtype),
        scratch_shapes=[
            pltpu.VMEM((S + 2 * HALO + LC, M), BF16),
            pltpu.VMEM((S // 2, Dc), U32),
            pltpu.VMEM((NP, M, D), U32),
            pltpu.VMEM((NP, Dc, D), U32),
            pltpu.VMEM((NP, Dc, D), U32),
            pltpu.VMEM((NP, D, M), U32),
            pltpu.VMEM((M // 2, M), U32),
            pltpu.VMEM((M // 2, M), U32),
            pltpu.VMEM((Fd // 2, M), U32),
            pltpu.VMEM((Fd // 2, M), U32),
            pltpu.VMEM((1, M), BF16),
            pltpu.VMEM((6, M // 2, M), U32),
            pltpu.VMEM((8, 128), U32),
            pltpu.VMEM((M // 2, 128), U32),
            pltpu.VMEM((6, 8, M), F32),
            pltpu.VMEM(((S + LC) // 2, M), U32),
            pltpu.VMEM((M // 2, 2 * D), U32),
            pltpu.VMEM((Dc // 2, 2 * KP * D), U32),
            pltpu.VMEM((Dc // 2, 2 * D), U32),
            pltpu.VMEM((D, M), U32),
            pltpu.VMEM((NP * S // 2, 2 * D), U32),
            pltpu.VMEM((S // 2, 2 * D), U32),
            pltpu.VMEM((S + 2 * HALO, M), F32),
            pltpu.VMEM((3, 2 * HALO, M), F32),
            pltpu.VMEM((TB, M), F32),
            pltpu.VMEM((TB // 2, M), U32),
            pltpu.VMEM((S, M), BF16),
            pltpu.SemaphoreType.DMA((10,)),
            pltpu.SemaphoreType.DMA((CC - 1 + S // CC // TK,)),
            pltpu.SemaphoreType.DMA((NP,)),
            pltpu.SemaphoreType.DMA((6,)),
            pltpu.SemaphoreType.DMA(((S // TB - 1) // NS + 1,)),
        ],
        compiler_params=pltpu.CompilerParams(
            dimension_semantics=("arbitrary",),
            vmem_limit_bytes=100 * 1024 * 1024,
            disable_bounds_checks=True,
            disable_semaphore_checks=True,
        ),
    )(
        A_x.reshape(S, M), A_c_kv.reshape(S, Dc),
        A_w_q, A_w_uk, A_w_uv,
        A_w_o.reshape(NP, 2 * D, M),
        B_w1, B_w2, B_w3.T, B_w4, c, w_mod,
    )
    return out.reshape(B, S, M)
```

```python
import functools
import math

import jax
import jax.numpy as jnp
from jax import lax
import jax.experimental.pallas as pl
import jax.experimental.pallas.tpu as pltpu

F32 = jnp.float32
BF16 = jnp.bfloat16
U32 = jnp.uint32
NT = (((1,), (1,)), ((), ()))
NEG = -1000000000.0
EPS = 1e-05
TQ = 128
TB = 128
NS = 3
TC = 64
LAG = 4
O_LAG = 4
Q_SUB = 0
T_SUB = 2
V_FIRST = 1
V_SPREAD = 4
O_HALF = True
ZC = 3
CC = 4
KP = 2
TK = 256
NL = 4
HALO = 8


def _ln(x):
    m = jnp.mean(x, axis=-1, keepdims=True)
    xc = x - m
    v = jnp.mean(xc * xc, axis=-1, keepdims=True)
    return xc * lax.rsqrt(v + EPS)


def _gelu(x):
    c = math.sqrt(2.0 / math.pi)
    hx = 0.5 * x
    return hx + hx * jnp.tanh(x * (c + (c * 0.044715) * (x * x)))


def _as_bf16(u):
    return pltpu.bitcast(u, BF16)


def _as_u32(b):
    return pltpu.bitcast(b, U32)


def _halves(u):
    return pltpu.bitcast(u << 16, F32), pltpu.bitcast(u & jnp.uint32(0xFFFF0000), F32)


def _split_pair(u):
    return _as_u32(jnp.concatenate(_halves(u), axis=1).astype(BF16))


def _attention_schedule(nq):
    order = list(range(nq - 1, -1, -1))
    units = [(i, hh, half) for i in order for half in (1, 0) for hh in (0, 1)]
    ops = [("q", order[0])] + [("v", i) for i in range(V_FIRST)]
    for k in range(len(units) + LAG + O_LAG):
        n, sub = divmod(k, 4)
        if k < len(units):
            ops.append(("s",) + units[k])
        if 0 <= k - LAG < len(units):
            ops.append(("pv",) + units[k - LAG])
        if sub == Q_SUB and n + 1 < nq:
            ops.append(("q", order[n + 1]))
        if k < LAG:
            per = -(-(nq - V_FIRST) // V_SPREAD)
            ops.extend(("v", i) for i in range(V_FIRST + k * per, min(nq, V_FIRST + (k + 1) * per)))
        if sub == T_SUB and n % 2 == 0 and n + 1 < nq:
            ops.append(("t", order[n], order[n + 1]))
        ko = k - LAG - O_LAG
        if 0 <= ko < len(units):
            if O_HALF and ko % 2 == 1:
                ops.append(("o", units[ko][0], units[ko][2]))
            if not O_HALF and ko % 4 == 3:
                ops.append(("o", units[ko][0], None))
    return ops


def _after(lhs, deps, zero):
    t = None
    for dep in deps:
        for r in range(0, dep.shape[0], 8):
            for c in range(0, dep.shape[1], 128):
                tile = dep[r:r + 8, c:c + 128]
                t = tile if t is None else t | tile
    head = lhs[0:8, 0:128] | (t & zero)
    if lhs.shape[1] > 128:
        head = jnp.concatenate([head, lhs[0:8, 128:]], axis=1)
    return jnp.concatenate([head, lhs[8:]], axis=0)


def _kernel(x_hbm, ckv_hbm, wq_hbm, wk_hbm, wv_hbm, wo_hbm,
            w1_hbm, w2_hbm, w3t_hbm, w4_hbm, c_hbm, wmod_hbm,
            o_hbm,
            x_ref, ckv_ref, wqr_ref, wkr_ref, wvr_ref, wo_ref,
            w1_ref, w2_ref, w3t_ref, w4_ref, c_ref, wmod_ref,
            zero_ref, sc_ref, mod_ref, h_ref, wqp_ref, wkp_ref, wvp_ref, wop_ref, k_ref, v_ref, acc_ref,
            cr_ref, z_ref, u3_ref, ob_ref,
            ssem, csem, ksem, msem, osem,
            *, S, M, D, NP, Fd):
    NK = NP // KP
    nq = S // TQ
    HQ = TQ // 2
    qscale = (D ** -0.5) * math.log2(math.e)
    LR = S // NL
    NM = 6
    nk = S // TK
    LC = LR // nk
    assert NK - 1 >= NM and NK - NL >= 3

    c_copy = pltpu.make_async_copy(c_hbm, c_ref, ssem.at[0])
    CR = S // CC // 2
    HK = TK // 2

    def ckv_copy(lo, n, sem):
        rows = pl.ds(lo if isinstance(lo, int) else pl.multiple_of(lo, HK), n)
        return pltpu.make_async_copy(ckv_hbm.bitcast(U32).at[rows, :], ckv_ref.at[rows, :],
                                     csem.at[sem])

    def ckv_head(i):
        return ckv_copy(i * HK, HK, i)

    def ckv_chunk(i):
        return ckv_copy(i * CR, CR, CR // HK - 1 + i)

    x_copy = pltpu.make_async_copy(x_hbm, x_ref.at[pl.ds(HALO, S), :], ssem.at[2])
    wo_copy = pltpu.make_async_copy(wo_hbm.bitcast(U32), wo_ref, ssem.at[3])
    late_copies = [
        pltpu.make_async_copy(w1_hbm.bitcast(U32), w1_ref, ssem.at[4]),
        pltpu.make_async_copy(w2_hbm.bitcast(U32), w2_ref, ssem.at[5]),
        pltpu.make_async_copy(w3t_hbm.bitcast(U32), w3t_ref, ssem.at[6]),
        pltpu.make_async_copy(w4_hbm.bitcast(U32), w4_ref, ssem.at[7]),
    ]

    def wk_copy(p):
        return pltpu.make_async_copy(wk_hbm.bitcast(U32).at[:, p, :], wkr_ref.at[p], ksem.at[p])

    def wmod_copy(g):
        off = g * M if isinstance(g, int) else pl.multiple_of(g * M, 128)
        return pltpu.make_async_copy(wmod_hbm.bitcast(U32).at[:, pl.ds(off, M)],
                                     wmod_ref.at[g], msem.at[g])

    def stage_weights(p):
        wqp_ref[...] = _split_pair(wqr_ref[p])
        wvp_ref[...] = _split_pair(wvr_ref[p])
        wop_ref[...] = wo_ref[p]

    def stage_wk(step, us=tuple(range(KP))):
        for u in us:
            wkp_ref[:, 2 * u * D:(2 * u + 2) * D] = _split_pair(wkr_ref[step * KP + u])

    def k_rows(p, lo, n):
        off = p * (S // 2) + lo
        return pl.ds(off if isinstance(off, int) else pl.multiple_of(off, 8), n)

    def proj_k(step, lo, lhs, u0=0, u1=KP, w=None):
        if w is None:
            w = _as_bf16(wkp_ref[:, 2 * u0 * D:2 * u1 * D])
        k = jnp.dot(_as_bf16(lhs), w, preferred_element_type=F32)
        for u in range(u0, u1):
            k_ref[k_rows(step * KP + u, lo, HK), :] = _as_u32(
                k[:, 2 * (u - u0) * D:2 * (u - u0 + 1) * D].astype(BF16))
        return k

    def _prologue():
        c_copy.start()
        wk_copy(0).start()
        for i in range(CR // HK):
            ckv_head(i).start()
        for p in range(1, KP):
            wk_copy(p).start()
        for i in range(1, CC):
            ckv_chunk(i).start()
        x_ref[0:HALO, :] = jnp.zeros((HALO, M), BF16)
        x_ref[S + HALO:, :] = jnp.zeros((HALO + LC, M), BF16)
        for g in range(2):
            for p in range((g + 1) * KP, (g + 2) * KP):
                wk_copy(p).start()
            wmod_copy(g).start()

        def start_wk(p, carry):
            wk_copy(p).start()
            return carry
        lax.fori_loop(3 * KP, NP, start_wk, 0)
        wmod_copy(2).start()
        x_copy.start()
        for g in range(3, NM):
            wmod_copy(g).start()

        def start_qv(p, carry):
            pltpu.make_async_copy(wq_hbm.bitcast(U32).at[:, p, :], wqr_ref.at[p], ssem.at[8]).start()
            pltpu.make_async_copy(wv_hbm.bitcast(U32).at[:, p, :], wvr_ref.at[p], ssem.at[9]).start()
            return carry
        lax.fori_loop(0, NP, start_qv, 0)
        wo_copy.start()
        for cp in late_copies:
            cp.start()
        mod_ref[0:2] = jnp.zeros((2, 8, M), F32)
        zero_ref[...] = jnp.zeros(zero_ref.shape, U32)
        c_copy.wait()
        c = c_ref[...].astype(F32)
        sc = jnp.broadcast_to(c * jax.nn.sigmoid(c), (128, M))
        sc_ref[...] = _as_u32(sc.T.astype(BF16))
        wk_copy(0).wait()
        stage_wk(0, (0,))

        def head_keys(i, carry):
            ckv_head(i).wait()
            lo = pl.multiple_of(i * HK, HK)
            proj_k(0, lo, ckv_ref[pl.ds(lo, HK), :], 0, 1)
            return carry
        lax.fori_loop(0, CR // HK, head_keys, 0)
        for p in range(1, KP):
            wk_copy(p).wait()
        stage_wk(0, tuple(range(1, KP)))
        for i in range(CR // HK):
            proj_k(0, i * HK, ckv_ref[i * HK:(i + 1) * HK, :], 1, KP)

        def first_keys(i, carry):
            ckv_chunk(i).wait()
            for ii in range(CR // HK):
                lo = pl.multiple_of(i * CR + ii * HK, HK)
                proj_k(0, lo, ckv_ref[pl.ds(lo, HK), :])
            return carry
        lax.fori_loop(1, CC, first_keys, 0)

    def _keys(step, carry):
        for u in range(KP):
            wk_copy(step * KP + u).wait()

        @pl.when(step <= NM)
        def _():
            wmod_copy(step - 1).wait()

        @pl.when(step == NK - NL)
        def _():
            x_copy.wait()

        wk = jnp.concatenate([half for u in range(KP) for half in _halves(wkr_ref[step * KP + u])],
                             axis=1).astype(BF16)
        g = jnp.minimum(step - 1, NM - 1)
        live = step >= NK - NL
        lblk = step - (NK - NL)
        sa = mod_ref[0, 0:1, :]
        ca1 = 1.0 + mod_ref[1, 0:1, :]
        zero = zero_ref[...]
        mc = M // 2 // nk
        ar = -(-(S + 2 * HALO) // ((NK - 1) * nk * 8)) * 8
        deps, part = [], None
        for i in range(nk):
            lhs = ckv_ref[i * HK:(i + 1) * HK, :]
            if deps:
                lhs = _after(lhs, deps, zero)
            k = proj_k(step, i * HK, lhs, w=wk)
            r = pl.multiple_of(jnp.where(live, HALO + lblk * LR + i * LC, S + 2 * HALO), 8)
            rh = pl.multiple_of(jnp.where(live, (lblk * LR + i * LC) // 2, S // 2), 8)
            x = x_ref[pl.ds(r, LC), :].astype(F32)
            h = _ln(x) * ca1 + sa
            h_ref[pl.ds(rh, LC // 2), :] = _as_u32(h.astype(BF16))
            we, wo = _halves(wmod_ref[g, i * mc:(i + 1) * mc, :])
            se, so = _halves(sc_ref[i * mc:(i + 1) * mc, :])
            prod = we * jnp.tile(se, (1, M // 128)) + wo * jnp.tile(so, (1, M // 128))
            for rr in range(0, mc, 8):
                part = prod[rr:rr + 8] if part is None else part + prod[rr:rr + 8]
            deps = [pltpu.bitcast(h, U32), pltpu.bitcast(part, U32)]
            zt = pltpu.bitcast(pltpu.bitcast(k[0:8, ZC * D:(ZC + 1) * D], U32) & zero, F32)
            ra = jnp.minimum(((step - 1) * nk + i) * ar, S + 2 * HALO - ar)
            acc_ref[pl.ds(pl.multiple_of(ra, 8), ar), :] = jnp.tile(zt, (ar // 8, M // 128))
        mod_ref[g] = jnp.broadcast_to(jnp.sum(part, axis=0, keepdims=True), (8, M))
        return carry

    def _first_pair():
        pltpu.make_async_copy(wqr_ref, wqr_ref, ssem.at[8]).wait()
        pltpu.make_async_copy(wvr_ref, wvr_ref, ssem.at[9]).wait()
        wo_copy.wait()
        stage_weights(0)

    def _attention(j, carry):

        HH = HQ // 2
        row = lax.broadcasted_iota(jnp.int32, (HQ, TQ), 0)
        col = lax.broadcasted_iota(jnp.int32, (HQ, TQ), 1)
        diag = col <= row + HQ
        first = [col < HQ, col >= HQ]
        first0 = [col <= row, jnp.logical_and(col >= HQ, diag)]

        def proj_v(i):
            rows = slice(i * HQ, (i + 1) * HQ)
            v = jnp.dot(_as_bf16(ckv_ref[rows, :]), _as_bf16(wvp_ref[...]), preferred_element_type=F32)
            v_ref[rows, :] = _as_u32(v.astype(BF16))

        def proj_q(i):
            rows = slice(i * HQ, (i + 1) * HQ)
            q = jnp.dot(_as_bf16(h_ref[rows, :]), _as_bf16(wqp_ref[...]), preferred_element_type=F32)
            q = q * qscale
            return [[q[half * HQ:(half + 1) * HQ, hh * D:(hh + 1) * D].astype(BF16)
                     for half in range(2)] for hh in range(2)]

        def masked_scores(qh, k):
            s = lax.dot_general(qh, k, NT, preferred_element_type=F32)
            n = s.shape[1] - TQ
            sd = jnp.where(diag, s[:, n:], NEG)
            return jnp.concatenate([s[:, :n], sd], axis=1) if n else sd

        def scores(q, hh, half, i):
            cols = slice(hh * D, (hh + 1) * D)
            if half == 1:
                return masked_scores(q[hh][1], _as_bf16(k_ref[k_rows(j, 0, (i + 1) * HQ), cols]))
            if i > 0:
                return masked_scores(q[hh][0], _as_bf16(k_ref[k_rows(j, HH, i * HQ), cols]))
            return None

        def first_scores(q1, q2):
            st = [lax.dot_general(_as_bf16(k_ref[k_rows(j, 0, HH), hh * D:(hh + 1) * D]),
                                  jnp.concatenate([q1[hh][0], q2[hh][0]], axis=0),
                                  NT, preferred_element_type=F32) for hh in range(2)]
            t = jnp.concatenate(st, axis=0).T
            return t[0:HQ], t[HQ:TQ]

        def softmax_pv(s, t0, hh, half, i):
            cols = slice(hh * D, (hh + 1) * D)
            if half == 1:
                v = v_ref[0:(i + 1) * HQ, cols]
            else:
                s0 = jnp.where(first[hh] if i > 0 else first0[hh], t0[i], NEG)
                s = s0 if s is None else jnp.concatenate([s, s0], axis=1)
                if hh == 0:
                    v = v_ref[0:HQ, cols]
                else:
                    v = jnp.concatenate([v_ref[HH:HQ, cols], v_ref[0:HH, cols]], axis=0)
                if i > 0:
                    v = jnp.concatenate([v_ref[HH:i * HQ + HH, cols], v], axis=0)
            m = jnp.max(s, axis=1, keepdims=True)
            p = jnp.exp2(s - m).astype(BF16)
            l = jnp.sum(p.astype(F32), axis=1, keepdims=True)
            o = jnp.dot(p, _as_bf16(v), preferred_element_type=F32)
            return o * pl.reciprocal(l, approx=False, full_range=False)

        def oproj(ctx, r, n):
            rows = slice(HALO + r, HALO + r + n)
            acc_ref[rows, :] += jnp.dot(ctx.astype(BF16), _as_bf16(wop_ref[...]),
                                        preferred_element_type=F32)

        q, s, t0, ctx = {}, {}, {}, {}
        for op in _attention_schedule(nq):
            kind, i = op[0], op[1]
            if kind == "q":
                q[i] = proj_q(i)
            elif kind == "v":
                proj_v(i)
            elif kind == "s":
                s[op[1:]] = scores(q[i], op[2], op[3], i)
            elif kind == "t":
                t0[i], t0[op[2]] = first_scores(q[i], q[op[2]])
            elif kind == "pv":
                ctx[op[1:]] = softmax_pv(s.pop(op[1:]), t0, op[2], op[3], i)
            elif op[2] is None:
                oproj(jnp.concatenate(
                    [jnp.concatenate([ctx.pop((i, hh, 0)), ctx.pop((i, hh, 1))], axis=0)
                     for hh in range(2)], axis=1), i * TQ, TQ)
            else:
                oproj(jnp.concatenate([ctx.pop((i, hh, op[2])) for hh in range(2)], axis=1),
                      i * TQ + op[2] * HQ, HQ)

        stage_weights(jnp.minimum(j + 1, NP - 1))
        return carry

    def _epilogue():
        for cp in late_copies:
            cp.wait()

        G = M // 4
        NC = TB // TC
        TH = TB + 2 * HALO
        hsplit = [0] + [2 * HALO + (k + 1) * TC for k in range(NC)]
        ntile = (Fd + 127) // 128
        fsplit = [min(Fd, ((k * ntile + NC - 1) // NC) * 128) for k in range(NC + 1)]

        def start_row(t):
            return t * TB if isinstance(t, int) else pl.multiple_of(t * TB, TB)

        def front_a(t, k, first):
            lo, hi = hsplit[k], hsplit[k + 1]
            if k == 0 and not first:
                lo = 2 * HALO
            r = start_row(t)
            ga = mod_ref[2, 0:1, :]
            sb = mod_ref[3, 0:1, :]
            cb1 = 1.0 + mod_ref[4, 0:1, :]
            x1 = (x_ref[pl.ds(r + lo, hi - lo), :].astype(F32)
                  + ga * acc_ref[pl.ds(r + lo, hi - lo), :])
            h = _ln(x1) * cb1 + sb
            tt = _gelu(jnp.dot(_ln(h).astype(BF16), _as_bf16(w1_ref[...]),
                               preferred_element_type=F32))
            if k == 0 and first:
                tt = jnp.concatenate([jnp.zeros((HALO, M), F32), tt[HALO:]], axis=0)
            if k == 0 and not first:
                x1, h, tt = [jnp.concatenate([cr_ref[a], v], axis=0)
                             for a, v in enumerate((x1, h, tt))]
            if k == NC - 1:
                n = hi - lo - HALO
                tt = jnp.concatenate([tt[:n], jnp.where(r + TB < S, tt[n:], 0.0)], axis=0)
                for a, v in enumerate((x1, h, tt)):
                    cr_ref[a] = v[n - HALO:]
            return x1, h, tt

        def front_b(x1, h, tt, k):
            lo = k * TC
            gb = mod_ref[5, 0:1, :]
            lane = lax.broadcasted_iota(jnp.int32, (TC, 128), 1)
            cols = []
            shifts = (-1, 1, -2, 2)
            for cblk in range(M // 128):
                c0, c1 = cblk * 128, (cblk + 1) * 128
                ga_, gb_ = c0 // G, (c1 - 1) // G
                a = tt[HALO + lo + shifts[ga_]:HALO + lo + shifts[ga_] + TC, c0:c1]
                if gb_ != ga_:
                    b = tt[HALO + lo + shifts[gb_]:HALO + lo + shifts[gb_] + TC, c0:c1]
                    a = jnp.where(lane < gb_ * G - c0, a, b)
                cols.append(a)
            sh = jnp.concatenate(cols, axis=1).astype(BF16)
            y = h[HALO + lo:HALO + lo + TC] + jnp.dot(sh, _as_bf16(w2_ref[...]),
                                                      preferred_element_type=F32)
            z_ref[lo:lo + TC, :] = x1[HALO + lo:HALO + lo + TC] + gb * y
            u3_ref[lo // 2:(lo + TC) // 2, :] = _as_u32(_ln(y).astype(BF16))

        def out_copy(it, n):
            rows = pl.ds(start_row(it * NS), n * TB)
            return pltpu.make_async_copy(ob_ref.at[rows, :], o_hbm.at[rows, :], osem.at[it])

        def mm3(k):
            lo, hi = fsplit[k], fsplit[k + 1]
            mid = hi - hi % 128
            u3 = _as_bf16(u3_ref[...])
            f = _gelu(lax.dot_general(u3, _as_bf16(w3t_ref[lo // 2:mid // 2, :]),
                                      NT, preferred_element_type=F32))
            if mid < hi:
                ft = _gelu(lax.dot_general(_as_bf16(w3t_ref[mid // 2:hi // 2, :]), u3,
                                           NT, preferred_element_type=F32))
                f = jnp.concatenate([f, ft.T], axis=1)
            return [f[kk * TC:(kk + 1) * TC].astype(BF16) for kk in range(NC)]

        def mm4(t, f, z, k):
            lo = k * TC
            gb = mod_ref[5, 0:1, :]
            h2 = jnp.dot(jnp.concatenate([fk[k] for fk in f], axis=1), _as_bf16(w4_ref[...]),
                         preferred_element_type=F32)
            ob_ref[pl.ds(start_row(t) + lo, TC), :] = (z + gb * h2).astype(ob_ref.dtype)

        def stage(t, cur, nxt):
            fs, fr = [], []
            for k in range(NC):
                if cur:
                    fs.append(mm3(k))
                if nxt:
                    fr.append(front_a(t + 1, k, not cur))
            if nxt:
                fr = [jnp.concatenate(parts, axis=0) for parts in zip(*fr)]
            for k in range(NC):
                if cur:
                    z = z_ref[k * TC:(k + 1) * TC, :]
                if nxt and k == NC - 1:
                    front_b(*fr, k)
                if cur:
                    mm4(t, fs, z, k)
                if nxt and k < NC - 1:
                    front_b(*fr, k)

        nb = S // TB
        ni = (nb - 1) // NS
        assert ni * NS == nb - 1
        stage(-1, False, True)

        def loop_b(it, carry):
            for u in range(NS):
                stage(it * NS + u, True, True)
            out_copy(it, NS).start()
            return carry
        lax.fori_loop(0, ni, loop_b, 0)
        stage(nb - 1, True, False)
        out_copy(ni, 1).start()
        for it in range(ni):
            out_copy(it, NS).wait()
        out_copy(ni, 1).wait()

    @pl.when(pl.program_id(0) == 0)
    def _():
        _prologue()
        lax.fori_loop(1, NK, _keys, 0)
        _first_pair()
        lax.fori_loop(0, NP, _attention, 0)

    @pl.when(pl.program_id(0) == 1)
    def _():
        _epilogue()


@jax.jit
def pallas_adaLN_cond__compressed_kv_cla__mixer_s_mlp__prompt_kernel(
    A_x: jax.Array,
    A_c_kv: jax.Array,
    A_w_q: jax.Array,
    A_w_uk: jax.Array,
    A_w_uv: jax.Array,
    A_w_o: jax.Array,
    B_x: jax.Array,
    B_w1: jax.Array,
    B_w2: jax.Array,
    B_w3: jax.Array,
    B_w4: jax.Array,
    c: jax.Array,
    w_mod: jax.Array,
):
    B, S, M = A_x.shape
    assert B == 1 and A_c_kv.shape[1] == S
    Dc = A_c_kv.shape[2]
    H, D = A_w_q.shape[1], A_w_q.shape[2]
    NP = H // 2
    Fd = B_w3.shape[1]
    LC = TK // NL
    any_spec = pl.BlockSpec(memory_space=pl.ANY)

    out = pl.pallas_call(
        functools.partial(_kernel, S=S, M=M, D=D, NP=NP, Fd=Fd),
        grid=(2,),
        in_specs=[any_spec] * 12,
        out_specs=any_spec,
        out_shape=jax.ShapeDtypeStruct((S, M), A_x.dtype),
        scratch_shapes=[
            pltpu.VMEM((S + 2 * HALO + LC, M), BF16),
            pltpu.VMEM((S // 2, Dc), U32),
            pltpu.VMEM((NP, M, D), U32),
            pltpu.VMEM((NP, Dc, D), U32),
            pltpu.VMEM((NP, Dc, D), U32),
            pltpu.VMEM((NP, D, M), U32),
            pltpu.VMEM((M // 2, M), U32),
            pltpu.VMEM((M // 2, M), U32),
            pltpu.VMEM((Fd // 2, M), U32),
            pltpu.VMEM((Fd // 2, M), U32),
            pltpu.VMEM((1, M), BF16),
            pltpu.VMEM((6, M // 2, M), U32),
            pltpu.VMEM((8, 128), U32),
            pltpu.VMEM((M // 2, 128), U32),
            pltpu.VMEM((6, 8, M), F32),
            pltpu.VMEM(((S + LC) // 2, M), U32),
            pltpu.VMEM((M // 2, 2 * D), U32),
            pltpu.VMEM((Dc // 2, 2 * KP * D), U32),
            pltpu.VMEM((Dc // 2, 2 * D), U32),
            pltpu.VMEM((D, M), U32),
            pltpu.VMEM((NP * S // 2, 2 * D), U32),
            pltpu.VMEM((S // 2, 2 * D), U32),
            pltpu.VMEM((S + 2 * HALO, M), F32),
            pltpu.VMEM((3, 2 * HALO, M), F32),
            pltpu.VMEM((TB, M), F32),
            pltpu.VMEM((TB // 2, M), U32),
            pltpu.VMEM((S, M), BF16),
            pltpu.SemaphoreType.DMA((10,)),
            pltpu.SemaphoreType.DMA((CC - 1 + S // CC // TK,)),
            pltpu.SemaphoreType.DMA((NP,)),
            pltpu.SemaphoreType.DMA((6,)),
            pltpu.SemaphoreType.DMA(((S // TB - 1) // NS + 1,)),
        ],
        compiler_params=pltpu.CompilerParams(
            dimension_semantics=("arbitrary",),
            vmem_limit_bytes=100 * 1024 * 1024,
            disable_bounds_checks=True,
            disable_semaphore_checks=True,
        ),
    )(
        A_x.reshape(S, M), A_c_kv.reshape(S, Dc),
        A_w_q, A_w_uk, A_w_uv,
        A_w_o.reshape(NP, 2 * D, M),
        B_w1, B_w2, B_w3.T, B_w4, c, w_mod,
    )
    return out.reshape(B, S, M)
```

```python
import functools
import math

import jax
import jax.numpy as jnp
from jax import lax
import jax.experimental.pallas as pl
import jax.experimental.pallas.tpu as pltpu

F32 = jnp.float32
BF16 = jnp.bfloat16
U32 = jnp.uint32
NT = (((1,), (1,)), ((), ()))
NEG = -1000000000.0
EPS = 1e-05
TQ = 128
TB = 128
NS = 3
TC = 64
LAG = 4
O_LAG = 4
Q_SUB = 0
T_SUB = 2
V_FIRST = 1
V_SPREAD = 4
O_HALF = True
ZC = 3
CC = 4
KP = 2
TK = 256
NL = 4
HALO = 8


def _ln(x):
    m = jnp.mean(x, axis=-1, keepdims=True)
    xc = x - m
    v = jnp.mean(xc * xc, axis=-1, keepdims=True)
    return xc * lax.rsqrt(v + EPS)


def _gelu(x):
    c = math.sqrt(2.0 / math.pi)
    hx = 0.5 * x
    return hx + hx * jnp.tanh(x * (c + (c * 0.044715) * (x * x)))


def _as_bf16(u):
    return pltpu.bitcast(u, BF16)


def _as_u32(b):
    return pltpu.bitcast(b, U32)


def _halves(u):
    return pltpu.bitcast(u << 16, F32), pltpu.bitcast(u & jnp.uint32(0xFFFF0000), F32)


def _split_pair(u):
    return _as_u32(jnp.concatenate(_halves(u), axis=1).astype(BF16))


def _attention_schedule(nq):
    order = list(range(nq - 1, -1, -1))
    units = [(i, hh, half) for i in order for half in (1, 0) for hh in (0, 1)]
    ops = [("q", order[0])] + [("v", i) for i in range(V_FIRST)]
    for k in range(len(units) + LAG + O_LAG):
        n, sub = divmod(k, 4)
        if k < len(units):
            ops.append(("s",) + units[k])
        if 0 <= k - LAG < len(units):
            ops.append(("pv",) + units[k - LAG])
        if sub == Q_SUB and n + 1 < nq:
            ops.append(("q", order[n + 1]))
        if k < LAG:
            per = -(-(nq - V_FIRST) // V_SPREAD)
            ops.extend(("v", i) for i in range(V_FIRST + k * per, min(nq, V_FIRST + (k + 1) * per)))
        if sub == T_SUB and n % 2 == 0 and n + 1 < nq:
            ops.append(("t", order[n], order[n + 1]))
        ko = k - LAG - O_LAG
        if 0 <= ko < len(units):
            if O_HALF and ko % 2 == 1:
                ops.append(("o", units[ko][0], units[ko][2]))
            if not O_HALF and ko % 4 == 3:
                ops.append(("o", units[ko][0], None))
    return ops


def _after(lhs, deps, zero):
    t = None
    for dep in deps:
        for r in range(0, dep.shape[0], 8):
            for c in range(0, dep.shape[1], 128):
                tile = dep[r:r + 8, c:c + 128]
                t = tile if t is None else t | tile
    head = lhs[0:8, 0:128] | (t & zero)
    if lhs.shape[1] > 128:
        head = jnp.concatenate([head, lhs[0:8, 128:]], axis=1)
    return jnp.concatenate([head, lhs[8:]], axis=0)


def _kernel(x_hbm, ckv_hbm, wq_hbm, wk_hbm, wv_hbm, wo_hbm,
            w1_hbm, w2_hbm, w3t_hbm, w4_hbm, c_hbm, wmod_hbm,
            o_hbm,
            x_ref, ckv_ref, wqr_ref, wkr_ref, wvr_ref, wo_ref,
            w1_ref, w2_ref, w3t_ref, w4_ref, c_ref, wmod_ref,
            zero_ref, sc_ref, mod_ref, h_ref, wqp_ref, wkp_ref, wvp_ref, wop_ref, k_ref, v_ref, acc_ref,
            w3h_ref, cr_ref, z_ref, u3_ref, ob_ref,
            ssem, csem, ksem, msem, osem,
            *, S, M, D, NP, Fd):
    NK = NP // KP
    nq = S // TQ
    HQ = TQ // 2
    qscale = (D ** -0.5) * math.log2(math.e)
    LR = S // NL
    NM = 6
    nk = S // TK
    LC = LR // nk
    assert NK - 1 >= NM and NK - NL >= 3

    c_copy = pltpu.make_async_copy(c_hbm, c_ref, ssem.at[0])
    CR = S // CC // 2
    HK = TK // 2

    def ckv_copy(lo, n, sem):
        rows = pl.ds(lo if isinstance(lo, int) else pl.multiple_of(lo, HK), n)
        return pltpu.make_async_copy(ckv_hbm.bitcast(U32).at[rows, :], ckv_ref.at[rows, :],
                                     csem.at[sem])

    def ckv_head(i):
        return ckv_copy(i * HK, HK, i)

    def ckv_chunk(i):
        return ckv_copy(i * CR, CR, CR // HK - 1 + i)

    x_copy = pltpu.make_async_copy(x_hbm, x_ref.at[pl.ds(HALO, S), :], ssem.at[2])
    wo_copy = pltpu.make_async_copy(wo_hbm.bitcast(U32), wo_ref, ssem.at[3])
    late_copies = [
        pltpu.make_async_copy(w1_hbm.bitcast(U32), w1_ref, ssem.at[4]),
        pltpu.make_async_copy(w2_hbm.bitcast(U32), w2_ref, ssem.at[5]),
        pltpu.make_async_copy(w3t_hbm.bitcast(U32), w3t_ref, ssem.at[6]),
        pltpu.make_async_copy(w4_hbm.bitcast(U32), w4_ref, ssem.at[7]),
    ]

    def wk_copy(p):
        return pltpu.make_async_copy(wk_hbm.bitcast(U32).at[:, p, :], wkr_ref.at[p], ksem.at[p])

    def wmod_copy(g):
        off = g * M if isinstance(g, int) else pl.multiple_of(g * M, 128)
        return pltpu.make_async_copy(wmod_hbm.bitcast(U32).at[:, pl.ds(off, M)],
                                     wmod_ref.at[g], msem.at[g])

    def stage_weights(p):
        wqp_ref[...] = _split_pair(wqr_ref[p])
        wvp_ref[...] = _split_pair(wvr_ref[p])
        wop_ref[...] = wo_ref[p]

    def stage_wk(step, us=tuple(range(KP))):
        for u in us:
            wkp_ref[:, 2 * u * D:(2 * u + 2) * D] = _split_pair(wkr_ref[step * KP + u])

    def k_rows(p, lo, n):
        off = p * (S // 2) + lo
        return pl.ds(off if isinstance(off, int) else pl.multiple_of(off, 8), n)

    def proj_k(step, lo, lhs, u0=0, u1=KP, w=None):
        if w is None:
            w = _as_bf16(wkp_ref[:, 2 * u0 * D:2 * u1 * D])
        k = jnp.dot(_as_bf16(lhs), w, preferred_element_type=F32)
        for u in range(u0, u1):
            k_ref[k_rows(step * KP + u, lo, HK), :] = _as_u32(
                k[:, 2 * (u - u0) * D:2 * (u - u0 + 1) * D].astype(BF16))
        return k

    def _prologue():
        c_copy.start()
        wk_copy(0).start()
        for i in range(CR // HK):
            ckv_head(i).start()
        for p in range(1, KP):
            wk_copy(p).start()
        for i in range(1, CC):
            ckv_chunk(i).start()
        x_ref[0:HALO, :] = jnp.zeros((HALO, M), BF16)
        x_ref[S + HALO:, :] = jnp.zeros((HALO + LC, M), BF16)
        for g in range(2):
            for p in range((g + 1) * KP, (g + 2) * KP):
                wk_copy(p).start()
            wmod_copy(g).start()

        def start_wk(p, carry):
            wk_copy(p).start()
            return carry
        lax.fori_loop(3 * KP, NP, start_wk, 0)
        wmod_copy(2).start()
        x_copy.start()
        for g in range(3, NM):
            wmod_copy(g).start()

        def start_qv(p, carry):
            pltpu.make_async_copy(wq_hbm.bitcast(U32).at[:, p, :], wqr_ref.at[p], ssem.at[8]).start()
            pltpu.make_async_copy(wv_hbm.bitcast(U32).at[:, p, :], wvr_ref.at[p], ssem.at[9]).start()
            return carry
        lax.fori_loop(0, NP, start_qv, 0)
        wo_copy.start()
        for cp in late_copies:
            cp.start()
        mod_ref[0:2] = jnp.zeros((2, 8, M), F32)
        zero_ref[...] = jnp.zeros(zero_ref.shape, U32)
        c_copy.wait()
        c = c_ref[...].astype(F32)
        sc = jnp.broadcast_to(c * jax.nn.sigmoid(c), (128, M))
        sc_ref[...] = _as_u32(sc.T.astype(BF16))
        wk_copy(0).wait()
        stage_wk(0, (0,))

        def head_keys(i, carry):
            ckv_head(i).wait()
            lo = pl.multiple_of(i * HK, HK)
            proj_k(0, lo, ckv_ref[pl.ds(lo, HK), :], 0, 1)
            return carry
        lax.fori_loop(0, CR // HK, head_keys, 0)
        for p in range(1, KP):
            wk_copy(p).wait()
        stage_wk(0, tuple(range(1, KP)))
        for i in range(CR // HK):
            proj_k(0, i * HK, ckv_ref[i * HK:(i + 1) * HK, :], 1, KP)

        def first_keys(i, carry):
            ckv_chunk(i).wait()
            for ii in range(CR // HK):
                lo = pl.multiple_of(i * CR + ii * HK, HK)
                proj_k(0, lo, ckv_ref[pl.ds(lo, HK), :])
            return carry
        lax.fori_loop(1, CC, first_keys, 0)

    def _keys(step, carry):
        for u in range(KP):
            wk_copy(step * KP + u).wait()

        @pl.when(step <= NM)
        def _():
            wmod_copy(step - 1).wait()

        @pl.when(step == NK - NL)
        def _():
            x_copy.wait()

        wk = jnp.concatenate([half for u in range(KP) for half in _halves(wkr_ref[step * KP + u])],
                             axis=1).astype(BF16)
        g = jnp.minimum(step - 1, NM - 1)
        live = step >= NK - NL
        lblk = step - (NK - NL)
        sa = mod_ref[0, 0:1, :]
        ca1 = 1.0 + mod_ref[1, 0:1, :]
        zero = zero_ref[...]
        mc = M // 2 // nk
        ar = -(-(S + 2 * HALO) // ((NK - 1) * nk * 8)) * 8
        deps, part = [], None
        for i in range(nk):
            lhs = ckv_ref[i * HK:(i + 1) * HK, :]
            if deps:
                lhs = _after(lhs, deps, zero)
            k = proj_k(step, i * HK, lhs, w=wk)
            r = pl.multiple_of(jnp.where(live, HALO + lblk * LR + i * LC, S + 2 * HALO), 8)
            rh = pl.multiple_of(jnp.where(live, (lblk * LR + i * LC) // 2, S // 2), 8)
            x = x_ref[pl.ds(r, LC), :].astype(F32)
            h = _ln(x) * ca1 + sa
            h_ref[pl.ds(rh, LC // 2), :] = _as_u32(h.astype(BF16))
            we, wo = _halves(wmod_ref[g, i * mc:(i + 1) * mc, :])
            se, so = _halves(sc_ref[i * mc:(i + 1) * mc, :])
            prod = we * jnp.tile(se, (1, M // 128)) + wo * jnp.tile(so, (1, M // 128))
            for rr in range(0, mc, 8):
                part = prod[rr:rr + 8] if part is None else part + prod[rr:rr + 8]
            deps = [pltpu.bitcast(h, U32), pltpu.bitcast(part, U32)]
            zt = pltpu.bitcast(pltpu.bitcast(k[0:8, ZC * D:(ZC + 1) * D], U32) & zero, F32)
            ra = jnp.minimum(((step - 1) * nk + i) * ar, S + 2 * HALO - ar)
            acc_ref[pl.ds(pl.multiple_of(ra, 8), ar), :] = jnp.tile(zt, (ar // 8, M // 128))
        mod_ref[g] = jnp.broadcast_to(jnp.sum(part, axis=0, keepdims=True), (8, M))
        return carry

    def _first_pair():
        pltpu.make_async_copy(wqr_ref, wqr_ref, ssem.at[8]).wait()
        pltpu.make_async_copy(wvr_ref, wvr_ref, ssem.at[9]).wait()
        wo_copy.wait()
        stage_weights(0)

    def _attention(j, carry):

        HH = HQ // 2
        row = lax.broadcasted_iota(jnp.int32, (HQ, TQ), 0)
        col = lax.broadcasted_iota(jnp.int32, (HQ, TQ), 1)
        diag = col <= row + HQ
        first = [col < HQ, col >= HQ]
        first0 = [col <= row, jnp.logical_and(col >= HQ, diag)]

        def proj_v(i):
            rows = slice(i * HQ, (i + 1) * HQ)
            v = jnp.dot(_as_bf16(ckv_ref[rows, :]), _as_bf16(wvp_ref[...]), preferred_element_type=F32)
            v_ref[rows, :] = _as_u32(v.astype(BF16))

        def proj_q(i):
            rows = slice(i * HQ, (i + 1) * HQ)
            q = jnp.dot(_as_bf16(h_ref[rows, :]), _as_bf16(wqp_ref[...]), preferred_element_type=F32)
            q = q * qscale
            return [[q[half * HQ:(half + 1) * HQ, hh * D:(hh + 1) * D].astype(BF16)
                     for half in range(2)] for hh in range(2)]

        def masked_scores(qh, k):
            s = lax.dot_general(qh, k, NT, preferred_element_type=F32)
            n = s.shape[1] - TQ
            sd = jnp.where(diag, s[:, n:], NEG)
            return jnp.concatenate([s[:, :n], sd], axis=1) if n else sd

        def scores(q, hh, half, i):
            cols = slice(hh * D, (hh + 1) * D)
            if half == 1:
                return masked_scores(q[hh][1], _as_bf16(k_ref[k_rows(j, 0, (i + 1) * HQ), cols]))
            if i > 0:
                return masked_scores(q[hh][0], _as_bf16(k_ref[k_rows(j, HH, i * HQ), cols]))
            return None

        def first_scores(q1, q2):
            st = [lax.dot_general(_as_bf16(k_ref[k_rows(j, 0, HH), hh * D:(hh + 1) * D]),
                                  jnp.concatenate([q1[hh][0], q2[hh][0]], axis=0),
                                  NT, preferred_element_type=F32) for hh in range(2)]
            t = jnp.concatenate(st, axis=0).T
            return t[0:HQ], t[HQ:TQ]

        def softmax_pv(s, t0, hh, half, i):
            cols = slice(hh * D, (hh + 1) * D)
            if half == 1:
                v = v_ref[0:(i + 1) * HQ, cols]
            else:
                s0 = jnp.where(first[hh] if i > 0 else first0[hh], t0[i], NEG)
                s = s0 if s is None else jnp.concatenate([s, s0], axis=1)
                if hh == 0:
                    v = v_ref[0:HQ, cols]
                else:
                    v = jnp.concatenate([v_ref[HH:HQ, cols], v_ref[0:HH, cols]], axis=0)
                if i > 0:
                    v = jnp.concatenate([v_ref[HH:i * HQ + HH, cols], v], axis=0)
            m = jnp.max(s, axis=1, keepdims=True)
            p = jnp.exp2(s - m).astype(BF16)
            l = jnp.sum(p.astype(F32), axis=1, keepdims=True)
            o = jnp.dot(p, _as_bf16(v), preferred_element_type=F32)
            return o * pl.reciprocal(l, approx=False, full_range=False)

        def oproj(ctx, r, n):
            rows = slice(HALO + r, HALO + r + n)
            acc_ref[rows, :] += jnp.dot(ctx.astype(BF16), _as_bf16(wop_ref[...]),
                                        preferred_element_type=F32)

        q, s, t0, ctx = {}, {}, {}, {}
        for op in _attention_schedule(nq):
            kind, i = op[0], op[1]
            if kind == "q":
                q[i] = proj_q(i)
            elif kind == "v":
                proj_v(i)
            elif kind == "s":
                s[op[1:]] = scores(q[i], op[2], op[3], i)
            elif kind == "t":
                t0[i], t0[op[2]] = first_scores(q[i], q[op[2]])
            elif kind == "pv":
                ctx[op[1:]] = softmax_pv(s.pop(op[1:]), t0, op[2], op[3], i)
            elif op[2] is None:
                oproj(jnp.concatenate(
                    [jnp.concatenate([ctx.pop((i, hh, 0)), ctx.pop((i, hh, 1))], axis=0)
                     for hh in range(2)], axis=1), i * TQ, TQ)
            else:
                oproj(jnp.concatenate([ctx.pop((i, hh, op[2])) for hh in range(2)], axis=1),
                      i * TQ + op[2] * HQ, HQ)

        stage_weights(jnp.minimum(j + 1, NP - 1))
        return carry

    def _epilogue():
        for cp in late_copies:
            cp.wait()

        G = M // 4
        NC = TB // TC
        TH = TB + 2 * HALO
        hsplit = [0] + [2 * HALO + (k + 1) * TC for k in range(NC)]
        ntile = (Fd + 127) // 128
        fsplit = [min(Fd, ((k * ntile + NC - 1) // NC) * 128) for k in range(NC + 1)]

        def start_row(t):
            return t * TB if isinstance(t, int) else pl.multiple_of(t * TB, TB)

        def front_a(t, k, first):
            lo, hi = hsplit[k], hsplit[k + 1]
            if k == 0 and not first:
                lo = 2 * HALO
            r = start_row(t)
            ga = mod_ref[2, 0:1, :]
            sb = mod_ref[3, 0:1, :]
            cb1 = 1.0 + mod_ref[4, 0:1, :]
            x1 = (x_ref[pl.ds(r + lo, hi - lo), :].astype(F32)
                  + ga * acc_ref[pl.ds(r + lo, hi - lo), :])
            h = _ln(x1) * cb1 + sb
            tt = _gelu(jnp.dot(_ln(h).astype(BF16), _as_bf16(w1_ref[...]),
                               preferred_element_type=F32))
            if k == 0 and first:
                tt = jnp.concatenate([jnp.zeros((HALO, M), F32), tt[HALO:]], axis=0)
            if k == 0 and not first:
                x1, h, tt = [jnp.concatenate([cr_ref[a], v], axis=0)
                             for a, v in enumerate((x1, h, tt))]
            if k == NC - 1:
                n = hi - lo - HALO
                tt = jnp.concatenate([tt[:n], jnp.where(r + TB < S, tt[n:], 0.0)], axis=0)
                for a, v in enumerate((x1, h, tt)):
                    cr_ref[a] = v[n - HALO:]
            return x1, h, tt

        def front_b(x1, h, tt, k):
            lo = k * TC
            gb = mod_ref[5, 0:1, :]
            lane = lax.broadcasted_iota(jnp.int32, (TC, 128), 1)
            cols = []
            shifts = (-1, 1, -2, 2)
            for cblk in range(M // 128):
                c0, c1 = cblk * 128, (cblk + 1) * 128
                ga_, gb_ = c0 // G, (c1 - 1) // G
                a = tt[HALO + lo + shifts[ga_]:HALO + lo + shifts[ga_] + TC, c0:c1]
                if gb_ != ga_:
                    b = tt[HALO + lo + shifts[gb_]:HALO + lo + shifts[gb_] + TC, c0:c1]
                    a = jnp.where(lane < gb_ * G - c0, a, b)
                cols.append(a)
            sh = jnp.concatenate(cols, axis=1).astype(BF16)
            y = h[HALO + lo:HALO + lo + TC] + jnp.dot(sh, _as_bf16(w2_ref[...]),
                                                      preferred_element_type=F32)
            z_ref[lo:lo + TC, :] = x1[HALO + lo:HALO + lo + TC] + gb * y
            u3_ref[lo // 2:(lo + TC) // 2, :] = _as_u32(_ln(y).astype(BF16))

        def out_copy(it, n):
            rows = pl.ds(start_row(it * NS), n * TB)
            return pltpu.make_async_copy(ob_ref.at[rows, :], o_hbm.at[rows, :], osem.at[it])

        w3h_ref[...] = _as_u32(_as_bf16(w3t_ref[0:64, :]).astype(F32).T.astype(BF16))

        def mm3(k, opens):
            lo, hi = fsplit[k], fsplit[k + 1]
            mid = hi - hi % 128
            u3 = _as_bf16(u3_ref[...])
            fs = []
            if opens:
                fs.append(jnp.dot(u3, _as_bf16(w3h_ref[...]), preferred_element_type=F32))
                lo += 128
            fs.append(lax.dot_general(u3, _as_bf16(w3t_ref[lo // 2:mid // 2, :]),
                                      NT, preferred_element_type=F32))
            f = _gelu(jnp.concatenate(fs, axis=1))
            if mid < hi:
                ft = _gelu(lax.dot_general(_as_bf16(w3t_ref[mid // 2:hi // 2, :]), u3,
                                           NT, preferred_element_type=F32))
                f = jnp.concatenate([f, ft.T], axis=1)
            return [f[kk * TC:(kk + 1) * TC].astype(BF16) for kk in range(NC)]

        def mm4(t, f, z, k):
            lo = k * TC
            gb = mod_ref[5, 0:1, :]
            h2 = jnp.dot(jnp.concatenate([fk[k] for fk in f], axis=1), _as_bf16(w4_ref[...]),
                         preferred_element_type=F32)
            ob_ref[pl.ds(start_row(t) + lo, TC), :] = (z + gb * h2).astype(ob_ref.dtype)

        def stage(t, cur, nxt, opens):
            fs, fr = [], []
            for k in range(NC):
                if cur:
                    fs.append(mm3(k, opens and k == 0))
                if nxt:
                    fr.append(front_a(t + 1, k, not cur))
            if nxt:
                fr = [jnp.concatenate(parts, axis=0) for parts in zip(*fr)]
            for k in range(NC):
                if cur:
                    z = z_ref[k * TC:(k + 1) * TC, :]
                if nxt and k == NC - 1:
                    front_b(*fr, k)
                if cur:
                    mm4(t, fs, z, k)
                if nxt and k < NC - 1:
                    front_b(*fr, k)

        nb = S // TB
        ni = (nb - 1) // NS
        assert ni * NS == nb - 1
        stage(-1, False, True, True)

        def loop_b(it, carry):
            for u in range(NS):
                stage(it * NS + u, True, True, u == 0)
            out_copy(it, NS).start()
            return carry
        lax.fori_loop(0, ni, loop_b, 0)
        stage(nb - 1, True, False, True)
        out_copy(ni, 1).start()
        for it in range(ni):
            out_copy(it, NS).wait()
        out_copy(ni, 1).wait()

    @pl.when(pl.program_id(0) == 0)
    def _():
        _prologue()
        lax.fori_loop(1, NK, _keys, 0)
        _first_pair()
        lax.fori_loop(0, NP, _attention, 0)

    @pl.when(pl.program_id(0) == 1)
    def _():
        _epilogue()


@jax.jit
def pallas_adaLN_cond__compressed_kv_cla__mixer_s_mlp__prompt_kernel(
    A_x: jax.Array,
    A_c_kv: jax.Array,
    A_w_q: jax.Array,
    A_w_uk: jax.Array,
    A_w_uv: jax.Array,
    A_w_o: jax.Array,
    B_x: jax.Array,
    B_w1: jax.Array,
    B_w2: jax.Array,
    B_w3: jax.Array,
    B_w4: jax.Array,
    c: jax.Array,
    w_mod: jax.Array,
):
    B, S, M = A_x.shape
    assert B == 1 and A_c_kv.shape[1] == S
    Dc = A_c_kv.shape[2]
    H, D = A_w_q.shape[1], A_w_q.shape[2]
    NP = H // 2
    Fd = B_w3.shape[1]
    LC = TK // NL
    any_spec = pl.BlockSpec(memory_space=pl.ANY)

    out = pl.pallas_call(
        functools.partial(_kernel, S=S, M=M, D=D, NP=NP, Fd=Fd),
        grid=(2,),
        in_specs=[any_spec] * 12,
        out_specs=any_spec,
        out_shape=jax.ShapeDtypeStruct((S, M), A_x.dtype),
        scratch_shapes=[
            pltpu.VMEM((S + 2 * HALO + LC, M), BF16),
            pltpu.VMEM((S // 2, Dc), U32),
            pltpu.VMEM((NP, M, D), U32),
            pltpu.VMEM((NP, Dc, D), U32),
            pltpu.VMEM((NP, Dc, D), U32),
            pltpu.VMEM((NP, D, M), U32),
            pltpu.VMEM((M // 2, M), U32),
            pltpu.VMEM((M // 2, M), U32),
            pltpu.VMEM((Fd // 2, M), U32),
            pltpu.VMEM((Fd // 2, M), U32),
            pltpu.VMEM((1, M), BF16),
            pltpu.VMEM((6, M // 2, M), U32),
            pltpu.VMEM((8, 128), U32),
            pltpu.VMEM((M // 2, 128), U32),
            pltpu.VMEM((6, 8, M), F32),
            pltpu.VMEM(((S + LC) // 2, M), U32),
            pltpu.VMEM((M // 2, 2 * D), U32),
            pltpu.VMEM((Dc // 2, 2 * KP * D), U32),
            pltpu.VMEM((Dc // 2, 2 * D), U32),
            pltpu.VMEM((D, M), U32),
            pltpu.VMEM((NP * S // 2, 2 * D), U32),
            pltpu.VMEM((S // 2, 2 * D), U32),
            pltpu.VMEM((S + 2 * HALO, M), F32),
            pltpu.VMEM((M // 2, 128), U32),
            pltpu.VMEM((3, 2 * HALO, M), F32),
            pltpu.VMEM((TB, M), F32),
            pltpu.VMEM((TB // 2, M), U32),
            pltpu.VMEM((S, M), BF16),
            pltpu.SemaphoreType.DMA((10,)),
            pltpu.SemaphoreType.DMA((CC - 1 + S // CC // TK,)),
            pltpu.SemaphoreType.DMA((NP,)),
            pltpu.SemaphoreType.DMA((6,)),
            pltpu.SemaphoreType.DMA(((S // TB - 1) // NS + 1,)),
        ],
        compiler_params=pltpu.CompilerParams(
            dimension_semantics=("arbitrary",),
            vmem_limit_bytes=100 * 1024 * 1024,
            disable_bounds_checks=True,
            disable_semaphore_checks=True,
        ),
    )(
        A_x.reshape(S, M), A_c_kv.reshape(S, Dc),
        A_w_q, A_w_uk, A_w_uv,
        A_w_o.reshape(NP, 2 * D, M),
        B_w1, B_w2, B_w3.T, B_w4, c, w_mod,
    )
    return out.reshape(B, S, M)
```

```python
import functools
import math

import jax
import jax.numpy as jnp
from jax import lax
import jax.experimental.pallas as pl
import jax.experimental.pallas.tpu as pltpu

F32 = jnp.float32
BF16 = jnp.bfloat16
U32 = jnp.uint32
NT = (((1,), (1,)), ((), ()))
NEG = -1000000000.0
EPS = 1e-05
TQ = 128
TB = 128
NS = 3
TC = 64
LAG = 4
O_LAG = 4
Q_SUB = 0
T_SUB = 2
V_FIRST = 1
V_SPREAD = 4
O_HALF = True
ZC = 3
ZS = 2
CC = 4
KP = 2
TK = 256
NL = 4
HALO = 8


def _ln(x):
    m = jnp.mean(x, axis=-1, keepdims=True)
    xc = x - m
    v = jnp.mean(xc * xc, axis=-1, keepdims=True)
    return xc * lax.rsqrt(v + EPS)


def _gelu(x):
    c = math.sqrt(2.0 / math.pi)
    hx = 0.5 * x
    return hx + hx * jnp.tanh(x * (c + (c * 0.044715) * (x * x)))


def _as_bf16(u):
    return pltpu.bitcast(u, BF16)


def _as_u32(b):
    return pltpu.bitcast(b, U32)


def _halves(u):
    return pltpu.bitcast(u << 16, F32), pltpu.bitcast(u & jnp.uint32(0xFFFF0000), F32)


def _split_pair(u):
    return _as_u32(jnp.concatenate(_halves(u), axis=1).astype(BF16))


def _attention_schedule(nq):
    order = list(range(nq - 1, -1, -1))
    units = [(i, hh, half) for i in order for half in (1, 0) for hh in (0, 1)]
    ops = [("q", order[0])] + [("v", i) for i in range(V_FIRST)]
    for k in range(len(units) + LAG + O_LAG):
        n, sub = divmod(k, 4)
        if k < len(units):
            ops.append(("s",) + units[k])
        if 0 <= k - LAG < len(units):
            ops.append(("pv",) + units[k - LAG])
        if sub == Q_SUB and n + 1 < nq:
            ops.append(("q", order[n + 1]))
        if k < LAG:
            per = -(-(nq - V_FIRST) // V_SPREAD)
            ops.extend(("v", i) for i in range(V_FIRST + k * per, min(nq, V_FIRST + (k + 1) * per)))
        if sub == T_SUB and n % 2 == 0 and n + 1 < nq:
            ops.append(("t", order[n], order[n + 1]))
        ko = k - LAG - O_LAG
        if 0 <= ko < len(units):
            if O_HALF and ko % 2 == 1:
                ops.append(("o", units[ko][0], units[ko][2]))
            if not O_HALF and ko % 4 == 3:
                ops.append(("o", units[ko][0], None))
    return ops


def _after(lhs, deps, zero):
    t = None
    for dep in deps:
        for r in range(0, dep.shape[0], 8):
            for c in range(0, dep.shape[1], 128):
                tile = dep[r:r + 8, c:c + 128]
                t = tile if t is None else t | tile
    head = lhs[0:8, 0:128] | (t & zero)
    if lhs.shape[1] > 128:
        head = jnp.concatenate([head, lhs[0:8, 128:]], axis=1)
    return jnp.concatenate([head, lhs[8:]], axis=0)


def _kernel(x_hbm, ckv_hbm, wq_hbm, wk_hbm, wv_hbm, wo_hbm,
            w1_hbm, w2_hbm, w3t_hbm, w4_hbm, c_hbm, wmod_hbm,
            o_hbm,
            x_ref, ckv_ref, wqr_ref, wkr_ref, wvr_ref, wo_ref,
            w1_ref, w2_ref, w3t_ref, w4_ref, c_ref, wmod_ref,
            zero_ref, sc_ref, mod_ref, h_ref, wqp_ref, wkp_ref, wvp_ref, wop_ref, k_ref, v_ref, acc_ref,
            w3h_ref, cr_ref, z_ref, u3_ref, ob_ref,
            ssem, csem, ksem, msem, osem,
            *, S, M, D, NP, Fd):
    NK = NP // KP
    nq = S // TQ
    HQ = TQ // 2
    qscale = (D ** -0.5) * math.log2(math.e)
    LR = S // NL
    NM = 6
    nk = S // TK
    LC = LR // nk
    assert NK - 1 >= NM and NK - NL >= 3

    c_copy = pltpu.make_async_copy(c_hbm, c_ref, ssem.at[0])
    CR = S // CC // 2
    HK = TK // 2

    def ckv_copy(lo, n, sem):
        rows = pl.ds(lo if isinstance(lo, int) else pl.multiple_of(lo, HK), n)
        return pltpu.make_async_copy(ckv_hbm.bitcast(U32).at[rows, :], ckv_ref.at[rows, :],
                                     csem.at[sem])

    def ckv_head(i):
        return ckv_copy(i * HK, HK, i)

    def ckv_chunk(i):
        return ckv_copy(i * CR, CR, CR // HK - 1 + i)

    x_copy = pltpu.make_async_copy(x_hbm, x_ref.at[pl.ds(HALO, S), :], ssem.at[2])
    rest = pl.ds(1, NP - 1)
    wo_copy = pltpu.make_async_copy(wo_hbm.bitcast(U32).at[rest], wo_ref.at[rest], ssem.at[3])
    pair0_copies = [
        pltpu.make_async_copy(wq_hbm.bitcast(U32).at[:, 0, :], wqr_ref.at[0], ssem.at[1]),
        pltpu.make_async_copy(wv_hbm.bitcast(U32).at[:, 0, :], wvr_ref.at[0], ssem.at[10]),
        pltpu.make_async_copy(wo_hbm.bitcast(U32).at[0], wop_ref, ssem.at[11]),
    ]
    late_copies = [
        pltpu.make_async_copy(w1_hbm.bitcast(U32), w1_ref, ssem.at[4]),
        pltpu.make_async_copy(w2_hbm.bitcast(U32), w2_ref, ssem.at[5]),
        pltpu.make_async_copy(w3t_hbm.bitcast(U32), w3t_ref, ssem.at[6]),
        pltpu.make_async_copy(w4_hbm.bitcast(U32), w4_ref, ssem.at[7]),
    ]

    def wk_copy(p):
        return pltpu.make_async_copy(wk_hbm.bitcast(U32).at[:, p, :], wkr_ref.at[p], ksem.at[p])

    def wmod_copy(g):
        off = g * M if isinstance(g, int) else pl.multiple_of(g * M, 128)
        return pltpu.make_async_copy(wmod_hbm.bitcast(U32).at[:, pl.ds(off, M)],
                                     wmod_ref.at[g], msem.at[g])

    def stage_weights(p):
        wqp_ref[...] = _split_pair(wqr_ref[p])
        wvp_ref[...] = _split_pair(wvr_ref[p])
        wop_ref[...] = wo_ref[p]

    def stage_wk(step, us=tuple(range(KP))):
        for u in us:
            wkp_ref[:, 2 * u * D:(2 * u + 2) * D] = _split_pair(wkr_ref[step * KP + u])

    def k_rows(p, lo, n):
        off = p * (S // 2) + lo
        return pl.ds(off if isinstance(off, int) else pl.multiple_of(off, 8), n)

    def proj_k(step, lo, lhs, u0=0, u1=KP, w=None):
        if w is None:
            w = _as_bf16(wkp_ref[:, 2 * u0 * D:2 * u1 * D])
        k = jnp.dot(_as_bf16(lhs), w, preferred_element_type=F32)
        for u in range(u0, u1):
            k_ref[k_rows(step * KP + u, lo, HK), :] = _as_u32(
                k[:, 2 * (u - u0) * D:2 * (u - u0 + 1) * D].astype(BF16))
        return k

    def _prologue():
        c_copy.start()
        wk_copy(0).start()
        for i in range(CR // HK):
            ckv_head(i).start()
        for p in range(1, KP):
            wk_copy(p).start()
        for i in range(1, CC):
            ckv_chunk(i).start()
        x_ref[0:HALO, :] = jnp.zeros((HALO, M), BF16)
        x_ref[S + HALO:, :] = jnp.zeros((HALO + LC, M), BF16)
        for g in range(2):
            for p in range((g + 1) * KP, (g + 2) * KP):
                wk_copy(p).start()
            wmod_copy(g).start()
            if g == 0:
                for cp in pair0_copies[:2]:
                    cp.start()
        pair0_copies[2].start()

        def start_wk(p, carry):
            wk_copy(p).start()
            return carry
        lax.fori_loop(3 * KP, NP, start_wk, 0)
        wmod_copy(2).start()
        x_copy.start()
        for g in range(3, NM):
            wmod_copy(g).start()

        def start_qv(p, carry):
            pltpu.make_async_copy(wq_hbm.bitcast(U32).at[:, p, :], wqr_ref.at[p], ssem.at[8]).start()
            pltpu.make_async_copy(wv_hbm.bitcast(U32).at[:, p, :], wvr_ref.at[p], ssem.at[9]).start()
            return carry
        lax.fori_loop(1, NP, start_qv, 0)
        wo_copy.start()
        for cp in late_copies:
            cp.start()
        mod_ref[0:2] = jnp.zeros((2, 8, M), F32)
        zero_ref[...] = jnp.zeros(zero_ref.shape, U32)
        c_copy.wait()
        c = c_ref[...].astype(F32)
        sc = jnp.broadcast_to(c * jax.nn.sigmoid(c), (128, M))
        sc_ref[...] = _as_u32(sc.T.astype(BF16))
        wk_copy(0).wait()
        stage_wk(0, (0,))

        def head_keys(i, carry):
            ckv_head(i).wait()
            lo = pl.multiple_of(i * HK, HK)
            proj_k(0, lo, ckv_ref[pl.ds(lo, HK), :], 0, 1)
            return carry
        lax.fori_loop(0, CR // HK, head_keys, 0)
        for p in range(1, KP):
            wk_copy(p).wait()
        stage_wk(0, tuple(range(1, KP)))
        for i in range(CR // HK):
            proj_k(0, i * HK, ckv_ref[i * HK:(i + 1) * HK, :], 1, KP)

        def first_keys(i, carry):
            ckv_chunk(i).wait()
            for ii in range(CR // HK):
                lo = pl.multiple_of(i * CR + ii * HK, HK)
                proj_k(0, lo, ckv_ref[pl.ds(lo, HK), :])
            return carry
        lax.fori_loop(1, CC, first_keys, 0)
        for cp in pair0_copies[:2]:
            cp.wait()

    def _keys(step, carry):
        for u in range(KP):
            wk_copy(step * KP + u).wait()

        @pl.when(step <= NM)
        def _():
            wmod_copy(step - 1).wait()

        @pl.when(step == NK - NL)
        def _():
            x_copy.wait()

        wk = jnp.concatenate([half for u in range(KP) for half in _halves(wkr_ref[step * KP + u])],
                             axis=1).astype(BF16)
        g = jnp.minimum(step - 1, NM - 1)
        live = step >= NK - NL
        lblk = step - (NK - NL)
        sa = mod_ref[0, 0:1, :]
        ca1 = 1.0 + mod_ref[1, 0:1, :]
        zero = zero_ref[...]
        mc = M // 2 // nk
        ar = -(-(S + 2 * HALO) // ((NK - 1) * nk * 8)) * 8
        deps, part = [], None
        for i in range(nk):
            lhs = ckv_ref[i * HK:(i + 1) * HK, :]
            if deps:
                lhs = _after(lhs, deps, zero)
            k = proj_k(step, i * HK, lhs, w=wk)
            r = pl.multiple_of(jnp.where(live, HALO + lblk * LR + i * LC, S + 2 * HALO), 8)
            rh = pl.multiple_of(jnp.where(live, (lblk * LR + i * LC) // 2, S // 2), 8)
            x = x_ref[pl.ds(r, LC), :].astype(F32)
            h = _ln(x) * ca1 + sa
            h_ref[pl.ds(rh, LC // 2), :] = _as_u32(h.astype(BF16))
            we, wo = _halves(wmod_ref[g, i * mc:(i + 1) * mc, :])
            se, so = _halves(sc_ref[i * mc:(i + 1) * mc, :])
            prod = we * jnp.tile(se, (1, M // 128)) + wo * jnp.tile(so, (1, M // 128))
            for rr in range(0, mc, 8):
                part = prod[rr:rr + 8] if part is None else part + prod[rr:rr + 8]
            deps = [pltpu.bitcast(h, U32), pltpu.bitcast(part, U32)]
            zt = pltpu.bitcast(pltpu.bitcast(k[0:8, ZC * D:(ZC + 1) * D], U32) & zero, F32)
            ra = jnp.minimum(((step - 1) * nk + i) * ar, S + 2 * HALO - ar)
            acc_ref[pl.ds(pl.multiple_of(ra, 8), ar), :] = jnp.tile(zt, (ar // 8, M // 128))
            zu = pltpu.bitcast(k[0:8, ZS * D:(ZS + 1) * D], U32) & zero
            for raw_ref, dst_ref in ((wqr_ref, wqp_ref), (wvr_ref, wvp_ref)):
                n = raw_ref.shape[1] // nk
                raw = raw_ref[0, i * n:(i + 1) * n, :] | jnp.tile(zu, (n // 8, 1))
                dst_ref[i * n // 2:(i + 1) * n // 2, :] = _split_pair(raw)
        mod_ref[g] = jnp.broadcast_to(jnp.sum(part, axis=0, keepdims=True), (8, M))
        return carry

    def _first_pair():
        pltpu.make_async_copy(wqr_ref.at[rest], wqr_ref.at[rest], ssem.at[8]).wait()
        pltpu.make_async_copy(wvr_ref.at[rest], wvr_ref.at[rest], ssem.at[9]).wait()
        wo_copy.wait()
        pair0_copies[2].wait()

    def _attention(j, carry):

        HH = HQ // 2
        row = lax.broadcasted_iota(jnp.int32, (HQ, TQ), 0)
        col = lax.broadcasted_iota(jnp.int32, (HQ, TQ), 1)
        diag = col <= row + HQ
        first = [col < HQ, col >= HQ]
        first0 = [col <= row, jnp.logical_and(col >= HQ, diag)]

        def proj_v(i):
            rows = slice(i * HQ, (i + 1) * HQ)
            v = jnp.dot(_as_bf16(ckv_ref[rows, :]), _as_bf16(wvp_ref[...]), preferred_element_type=F32)
            v_ref[rows, :] = _as_u32(v.astype(BF16))

        def proj_q(i):
            rows = slice(i * HQ, (i + 1) * HQ)
            q = jnp.dot(_as_bf16(h_ref[rows, :]), _as_bf16(wqp_ref[...]), preferred_element_type=F32)
            q = q * qscale
            return [[q[half * HQ:(half + 1) * HQ, hh * D:(hh + 1) * D].astype(BF16)
                     for half in range(2)] for hh in range(2)]

        def masked_scores(qh, k):
            s = lax.dot_general(qh, k, NT, preferred_element_type=F32)
            n = s.shape[1] - TQ
            sd = jnp.where(diag, s[:, n:], NEG)
            return jnp.concatenate([s[:, :n], sd], axis=1) if n else sd

        def scores(q, hh, half, i):
            cols = slice(hh * D, (hh + 1) * D)
            if half == 1:
                return masked_scores(q[hh][1], _as_bf16(k_ref[k_rows(j, 0, (i + 1) * HQ), cols]))
            if i > 0:
                return masked_scores(q[hh][0], _as_bf16(k_ref[k_rows(j, HH, i * HQ), cols]))
            return None

        def first_scores(q1, q2):
            st = [lax.dot_general(_as_bf16(k_ref[k_rows(j, 0, HH), hh * D:(hh + 1) * D]),
                                  jnp.concatenate([q1[hh][0], q2[hh][0]], axis=0),
                                  NT, preferred_element_type=F32) for hh in range(2)]
            t = jnp.concatenate(st, axis=0).T
            return t[0:HQ], t[HQ:TQ]

        def softmax_pv(s, t0, hh, half, i):
            cols = slice(hh * D, (hh + 1) * D)
            if half == 1:
                v = v_ref[0:(i + 1) * HQ, cols]
            else:
                s0 = jnp.where(first[hh] if i > 0 else first0[hh], t0[i], NEG)
                s = s0 if s is None else jnp.concatenate([s, s0], axis=1)
                if hh == 0:
                    v = v_ref[0:HQ, cols]
                else:
                    v = jnp.concatenate([v_ref[HH:HQ, cols], v_ref[0:HH, cols]], axis=0)
                if i > 0:
                    v = jnp.concatenate([v_ref[HH:i * HQ + HH, cols], v], axis=0)
            m = jnp.max(s, axis=1, keepdims=True)
            p = jnp.exp2(s - m).astype(BF16)
            l = jnp.sum(p.astype(F32), axis=1, keepdims=True)
            o = jnp.dot(p, _as_bf16(v), preferred_element_type=F32)
            return o * pl.reciprocal(l, approx=False, full_range=False)

        def oproj(ctx, r, n):
            rows = slice(HALO + r, HALO + r + n)
            acc_ref[rows, :] += jnp.dot(ctx.astype(BF16), _as_bf16(wop_ref[...]),
                                        preferred_element_type=F32)

        q, s, t0, ctx = {}, {}, {}, {}
        for op in _attention_schedule(nq):
            kind, i = op[0], op[1]
            if kind == "q":
                q[i] = proj_q(i)
            elif kind == "v":
                proj_v(i)
            elif kind == "s":
                s[op[1:]] = scores(q[i], op[2], op[3], i)
            elif kind == "t":
                t0[i], t0[op[2]] = first_scores(q[i], q[op[2]])
            elif kind == "pv":
                ctx[op[1:]] = softmax_pv(s.pop(op[1:]), t0, op[2], op[3], i)
            elif op[2] is None:
                oproj(jnp.concatenate(
                    [jnp.concatenate([ctx.pop((i, hh, 0)), ctx.pop((i, hh, 1))], axis=0)
                     for hh in range(2)], axis=1), i * TQ, TQ)
            else:
                oproj(jnp.concatenate([ctx.pop((i, hh, op[2])) for hh in range(2)], axis=1),
                      i * TQ + op[2] * HQ, HQ)

        stage_weights(jnp.minimum(j + 1, NP - 1))
        return carry

    def _epilogue():
        for cp in late_copies:
            cp.wait()

        G = M // 4
        NC = TB // TC
        TH = TB + 2 * HALO
        hsplit = [0] + [2 * HALO + (k + 1) * TC for k in range(NC)]
        ntile = (Fd + 127) // 128
        fsplit = [min(Fd, ((k * ntile + NC - 1) // NC) * 128) for k in range(NC + 1)]

        def start_row(t):
            return t * TB if isinstance(t, int) else pl.multiple_of(t * TB, TB)

        def front_a(t, k, first):
            lo, hi = hsplit[k], hsplit[k + 1]
            if k == 0 and not first:
                lo = 2 * HALO
            r = start_row(t)
            ga = mod_ref[2, 0:1, :]
            sb = mod_ref[3, 0:1, :]
            cb1 = 1.0 + mod_ref[4, 0:1, :]
            x1 = (x_ref[pl.ds(r + lo, hi - lo), :].astype(F32)
                  + ga * acc_ref[pl.ds(r + lo, hi - lo), :])
            h = _ln(x1) * cb1 + sb
            tt = _gelu(jnp.dot(_ln(h).astype(BF16), _as_bf16(w1_ref[...]),
                               preferred_element_type=F32))
            if k == 0 and first:
                tt = jnp.concatenate([jnp.zeros((HALO, M), F32), tt[HALO:]], axis=0)
            if k == 0 and not first:
                x1, h, tt = [jnp.concatenate([cr_ref[a], v], axis=0)
                             for a, v in enumerate((x1, h, tt))]
            if k == NC - 1:
                n = hi - lo - HALO
                tt = jnp.concatenate([tt[:n], jnp.where(r + TB < S, tt[n:], 0.0)], axis=0)
                for a, v in enumerate((x1, h, tt)):
                    cr_ref[a] = v[n - HALO:]
            return x1, h, tt

        def front_b(x1, h, tt, k):
            lo = k * TC
            gb = mod_ref[5, 0:1, :]
            lane = lax.broadcasted_iota(jnp.int32, (TC, 128), 1)
            cols = []
            shifts = (-1, 1, -2, 2)
            for cblk in range(M // 128):
                c0, c1 = cblk * 128, (cblk + 1) * 128
                ga_, gb_ = c0 // G, (c1 - 1) // G
                a = tt[HALO + lo + shifts[ga_]:HALO + lo + shifts[ga_] + TC, c0:c1]
                if gb_ != ga_:
                    b = tt[HALO + lo + shifts[gb_]:HALO + lo + shifts[gb_] + TC, c0:c1]
                    a = jnp.where(lane < gb_ * G - c0, a, b)
                cols.append(a)
            sh = jnp.concatenate(cols, axis=1).astype(BF16)
            y = h[HALO + lo:HALO + lo + TC] + jnp.dot(sh, _as_bf16(w2_ref[...]),
                                                      preferred_element_type=F32)
            z_ref[lo:lo + TC, :] = x1[HALO + lo:HALO + lo + TC] + gb * y
            u3_ref[lo // 2:(lo + TC) // 2, :] = _as_u32(_ln(y).astype(BF16))

        def out_copy(it, n):
            rows = pl.ds(start_row(it * NS), n * TB)
            return pltpu.make_async_copy(ob_ref.at[rows, :], o_hbm.at[rows, :], osem.at[it])

        w3h_ref[...] = _as_u32(_as_bf16(w3t_ref[0:64, :]).astype(F32).T.astype(BF16))

        def mm3(k, opens):
            lo, hi = fsplit[k], fsplit[k + 1]
            mid = hi - hi % 128
            u3 = _as_bf16(u3_ref[...])
            fs = []
            if opens:
                fs.append(jnp.dot(u3, _as_bf16(w3h_ref[...]), preferred_element_type=F32))
                lo += 128
            fs.append(lax.dot_general(u3, _as_bf16(w3t_ref[lo // 2:mid // 2, :]),
                                      NT, preferred_element_type=F32))
            f = _gelu(jnp.concatenate(fs, axis=1))
            if mid < hi:
                ft = _gelu(lax.dot_general(_as_bf16(w3t_ref[mid // 2:hi // 2, :]), u3,
                                           NT, preferred_element_type=F32))
                f = jnp.concatenate([f, ft.T], axis=1)
            return [f[kk * TC:(kk + 1) * TC].astype(BF16) for kk in range(NC)]

        def mm4(t, f, z, k):
            lo = k * TC
            gb = mod_ref[5, 0:1, :]
            h2 = jnp.dot(jnp.concatenate([fk[k] for fk in f], axis=1), _as_bf16(w4_ref[...]),
                         preferred_element_type=F32)
            ob_ref[pl.ds(start_row(t) + lo, TC), :] = (z + gb * h2).astype(ob_ref.dtype)

        def stage(t, cur, nxt, opens):
            fs, fr = [], []
            for k in range(NC):
                if cur:
                    fs.append(mm3(k, opens and k == 0))
                if nxt:
                    fr.append(front_a(t + 1, k, not cur))
            if nxt:
                fr = [jnp.concatenate(parts, axis=0) for parts in zip(*fr)]
            for k in range(NC):
                if cur:
                    z = z_ref[k * TC:(k + 1) * TC, :]
                if nxt and k == NC - 1:
                    front_b(*fr, k)
                if cur:
                    mm4(t, fs, z, k)
                if nxt and k < NC - 1:
                    front_b(*fr, k)

        nb = S // TB
        ni = (nb - 1) // NS
        assert ni * NS == nb - 1
        stage(-1, False, True, True)

        def loop_b(it, carry):
            for u in range(NS):
                stage(it * NS + u, True, True, u == 0)
            out_copy(it, NS).start()
            return carry
        lax.fori_loop(0, ni, loop_b, 0)
        stage(nb - 1, True, False, True)
        out_copy(ni, 1).start()
        for it in range(ni):
            out_copy(it, NS).wait()
        out_copy(ni, 1).wait()

    @pl.when(pl.program_id(0) == 0)
    def _():
        _prologue()
        lax.fori_loop(1, NK, _keys, 0)
        _first_pair()
        lax.fori_loop(0, NP, _attention, 0)

    @pl.when(pl.program_id(0) == 1)
    def _():
        _epilogue()


@jax.jit
def pallas_adaLN_cond__compressed_kv_cla__mixer_s_mlp__prompt_kernel(
    A_x: jax.Array,
    A_c_kv: jax.Array,
    A_w_q: jax.Array,
    A_w_uk: jax.Array,
    A_w_uv: jax.Array,
    A_w_o: jax.Array,
    B_x: jax.Array,
    B_w1: jax.Array,
    B_w2: jax.Array,
    B_w3: jax.Array,
    B_w4: jax.Array,
    c: jax.Array,
    w_mod: jax.Array,
):
    B, S, M = A_x.shape
    assert B == 1 and A_c_kv.shape[1] == S
    Dc = A_c_kv.shape[2]
    H, D = A_w_q.shape[1], A_w_q.shape[2]
    NP = H // 2
    Fd = B_w3.shape[1]
    LC = TK // NL
    any_spec = pl.BlockSpec(memory_space=pl.ANY)

    out = pl.pallas_call(
        functools.partial(_kernel, S=S, M=M, D=D, NP=NP, Fd=Fd),
        grid=(2,),
        in_specs=[any_spec] * 12,
        out_specs=any_spec,
        out_shape=jax.ShapeDtypeStruct((S, M), A_x.dtype),
        scratch_shapes=[
            pltpu.VMEM((S + 2 * HALO + LC, M), BF16),
            pltpu.VMEM((S // 2, Dc), U32),
            pltpu.VMEM((NP, M, D), U32),
            pltpu.VMEM((NP, Dc, D), U32),
            pltpu.VMEM((NP, Dc, D), U32),
            pltpu.VMEM((NP, D, M), U32),
            pltpu.VMEM((M // 2, M), U32),
            pltpu.VMEM((M // 2, M), U32),
            pltpu.VMEM((Fd // 2, M), U32),
            pltpu.VMEM((Fd // 2, M), U32),
            pltpu.VMEM((1, M), BF16),
            pltpu.VMEM((6, M // 2, M), U32),
            pltpu.VMEM((8, 128), U32),
            pltpu.VMEM((M // 2, 128), U32),
            pltpu.VMEM((6, 8, M), F32),
            pltpu.VMEM(((S + LC) // 2, M), U32),
            pltpu.VMEM((M // 2, 2 * D), U32),
            pltpu.VMEM((Dc // 2, 2 * KP * D), U32),
            pltpu.VMEM((Dc // 2, 2 * D), U32),
            pltpu.VMEM((D, M), U32),
            pltpu.VMEM((NP * S // 2, 2 * D), U32),
            pltpu.VMEM((S // 2, 2 * D), U32),
            pltpu.VMEM((S + 2 * HALO, M), F32),
            pltpu.VMEM((M // 2, 128), U32),
            pltpu.VMEM((3, 2 * HALO, M), F32),
            pltpu.VMEM((TB, M), F32),
            pltpu.VMEM((TB // 2, M), U32),
            pltpu.VMEM((S, M), BF16),
            pltpu.SemaphoreType.DMA((12,)),
            pltpu.SemaphoreType.DMA((CC - 1 + S // CC // TK,)),
            pltpu.SemaphoreType.DMA((NP,)),
            pltpu.SemaphoreType.DMA((6,)),
            pltpu.SemaphoreType.DMA(((S // TB - 1) // NS + 1,)),
        ],
        compiler_params=pltpu.CompilerParams(
            dimension_semantics=("arbitrary",),
            vmem_limit_bytes=100 * 1024 * 1024,
            disable_bounds_checks=True,
            disable_semaphore_checks=True,
        ),
    )(
        A_x.reshape(S, M), A_c_kv.reshape(S, Dc),
        A_w_q, A_w_uk, A_w_uv,
        A_w_o.reshape(NP, 2 * D, M),
        B_w1, B_w2, B_w3.T, B_w4, c, w_mod,
    )
    return out.reshape(B, S, M)
```

```python
import functools
import math

import jax
import jax.numpy as jnp
from jax import lax
import jax.experimental.pallas as pl
import jax.experimental.pallas.tpu as pltpu

F32 = jnp.float32
BF16 = jnp.bfloat16
U32 = jnp.uint32
NT = (((1,), (1,)), ((), ()))
NEG = -1000000000.0
EPS = 1e-05
CC = 4
KP = 2
TK = 256
NL = 4
ZC, ZS = 3, 2
TQ = 128
LAG = 4
O_LAG = 4
Q_SUB = 0
T_SUB = 2
TB = 128
NS = 3
TC = 64
HALO = 8
FILL_A = (0, 96, 144)
FILL_B = (0, 64, 128)


def _ln(x):
    m = jnp.mean(x, axis=-1, keepdims=True)
    xc = x - m
    v = jnp.mean(xc * xc, axis=-1, keepdims=True)
    return xc * lax.rsqrt(v + EPS)


def _gelu(x):
    c = math.sqrt(2.0 / math.pi)
    hx = 0.5 * x
    return hx + hx * jnp.tanh(x * (c + (c * 0.044715) * (x * x)))


def _as_bf16(u):
    return pltpu.bitcast(u, BF16)


def _as_u32(b):
    return pltpu.bitcast(b, U32)


def _halves(u):
    return pltpu.bitcast(u << 16, F32), pltpu.bitcast(u & jnp.uint32(0xFFFF0000), F32)


def _split_pair(u):
    return _as_u32(jnp.concatenate(_halves(u), axis=1).astype(BF16))


def _attention_schedule(nq):
    order = list(range(nq - 1, -1, -1))
    units = [(i, hh, half) for i in order for half in (1, 0) for hh in (0, 1)]
    ops = [("q", order[0]), ("v", 0)]
    per = -(-(nq - 1) // LAG)
    for k in range(len(units) + LAG + O_LAG):
        n, sub = divmod(k, 4)
        if k < len(units):
            ops.append(("s",) + units[k])
        if 0 <= k - LAG < len(units):
            ops.append(("pv",) + units[k - LAG])
        if sub == Q_SUB and n + 1 < nq:
            ops.append(("q", order[n + 1]))
        if k < LAG:
            ops.extend(("v", i) for i in range(1 + k * per, min(nq, 1 + (k + 1) * per)))
        if sub == T_SUB and n % 2 == 0 and n + 1 < nq:
            ops.append(("t", order[n], order[n + 1]))
        ko = k - LAG - O_LAG
        if 0 <= ko < len(units) and ko % 2 == 1:
            ops.append(("o", units[ko][0], units[ko][2]))
    return ops


def _after(lhs, deps, zero):
    t = None
    for dep in deps:
        for r in range(0, dep.shape[0], 8):
            for c in range(0, dep.shape[1], 128):
                tile = dep[r:r + 8, c:c + 128]
                t = tile if t is None else t | tile
    head = lhs[0:8, 0:128] | (t & zero)
    if lhs.shape[1] > 128:
        head = jnp.concatenate([head, lhs[0:8, 128:]], axis=1)
    return jnp.concatenate([head, lhs[8:]], axis=0)


def _kernel(x_hbm, ckv_hbm, wq_hbm, wk_hbm, wv_hbm, wo_hbm,
            w1_hbm, w2_hbm, w3t_hbm, w4_hbm, c_hbm, wmod_hbm,
            o_hbm,
            x_ref, ckv_ref, wqr_ref, wkr_ref, wvr_ref, wo_ref,
            w1_ref, w2_ref, w3t_ref, w4_ref, c_ref, wmod_ref,
            zero_ref, sc_ref, mod_ref, h_ref, wqp_ref, wkp_ref, wvp_ref, wop_ref, k_ref, v_ref, acc_ref,
            w3h_ref, cr_ref, z_ref, u3_ref, ob_ref,
            ssem, csem, ksem, msem, osem,
            *, S, M, D, NP, Fd):
    NK = NP // KP
    nq = S // TQ
    HQ = TQ // 2
    qscale = (D ** -0.5) * math.log2(math.e)
    LR = S // NL
    NM = 6
    nk = S // TK
    LC = LR // nk
    assert NK - 1 >= NM and NK - NL >= 3

    c_copy = pltpu.make_async_copy(c_hbm, c_ref, ssem.at[0])
    CR = S // CC // 2
    HK = TK // 2

    def ckv_copy(lo, n, sem):
        rows = pl.ds(lo if isinstance(lo, int) else pl.multiple_of(lo, HK), n)
        return pltpu.make_async_copy(ckv_hbm.bitcast(U32).at[rows, :], ckv_ref.at[rows, :],
                                     csem.at[sem])

    def ckv_head(i):
        return ckv_copy(i * HK, HK, i)

    def ckv_chunk(i):
        return ckv_copy(i * CR, CR, CR // HK - 1 + i)

    x_copy = pltpu.make_async_copy(x_hbm, x_ref.at[pl.ds(HALO, S), :], ssem.at[2])
    rest = pl.ds(1, NP - 1)
    wo_copy = pltpu.make_async_copy(wo_hbm.bitcast(U32).at[rest], wo_ref.at[rest], ssem.at[3])
    pair0_copies = [
        pltpu.make_async_copy(wq_hbm.bitcast(U32).at[:, 0, :], wqr_ref.at[0], ssem.at[1]),
        pltpu.make_async_copy(wv_hbm.bitcast(U32).at[:, 0, :], wvr_ref.at[0], ssem.at[10]),
        pltpu.make_async_copy(wo_hbm.bitcast(U32).at[0], wop_ref, ssem.at[11]),
    ]
    late_copies = [
        pltpu.make_async_copy(w1_hbm.bitcast(U32), w1_ref, ssem.at[4]),
        pltpu.make_async_copy(w2_hbm.bitcast(U32), w2_ref, ssem.at[5]),
        pltpu.make_async_copy(w3t_hbm.bitcast(U32), w3t_ref, ssem.at[6]),
        pltpu.make_async_copy(w4_hbm.bitcast(U32), w4_ref, ssem.at[7]),
    ]

    def wk_copy(p):
        return pltpu.make_async_copy(wk_hbm.bitcast(U32).at[:, p, :], wkr_ref.at[p], ksem.at[p])

    def wmod_copy(g):
        off = g * M if isinstance(g, int) else pl.multiple_of(g * M, 128)
        return pltpu.make_async_copy(wmod_hbm.bitcast(U32).at[:, pl.ds(off, M)],
                                     wmod_ref.at[g], msem.at[g])

    def stage_weights(p):
        wqp_ref[...] = _split_pair(wqr_ref[p])
        wvp_ref[...] = _split_pair(wvr_ref[p])
        wop_ref[...] = wo_ref[p]

    def stage_wk(step, us=tuple(range(KP))):
        for u in us:
            wkp_ref[:, 2 * u * D:(2 * u + 2) * D] = _split_pair(wkr_ref[step * KP + u])

    def k_rows(p, lo, n):
        off = p * (S // 2) + lo
        return pl.ds(off if isinstance(off, int) else pl.multiple_of(off, 8), n)

    def proj_k(step, lo, lhs, u0=0, u1=KP, w=None):
        if w is None:
            w = _as_bf16(wkp_ref[:, 2 * u0 * D:2 * u1 * D])
        k = jnp.dot(_as_bf16(lhs), w, preferred_element_type=F32)
        for u in range(u0, u1):
            k_ref[k_rows(step * KP + u, lo, HK), :] = _as_u32(
                k[:, 2 * (u - u0) * D:2 * (u - u0 + 1) * D].astype(BF16))
        return k

    def _prologue():
        wk_copy(0).start()
        for i in range(CR // HK):
            ckv_head(i).start()
        c_copy.start()
        for p in range(1, KP):
            wk_copy(p).start()
        for i in range(1, CC):
            ckv_chunk(i).start()
        x_ref[0:HALO, :] = jnp.zeros((HALO, M), BF16)
        x_ref[S + HALO:, :] = jnp.zeros((HALO + LC, M), BF16)
        for g in range(2):
            for p in range((g + 1) * KP, (g + 2) * KP):
                wk_copy(p).start()
            wmod_copy(g).start()
            if g == 0:
                for cp in pair0_copies[:2]:
                    cp.start()
        pair0_copies[2].start()

        def start_wk(p, carry):
            wk_copy(p).start()
            return carry
        lax.fori_loop(3 * KP, NP, start_wk, 0)
        wmod_copy(2).start()
        x_copy.start()
        for g in range(3, NM):
            wmod_copy(g).start()

        def start_qv(p, carry):
            pltpu.make_async_copy(wq_hbm.bitcast(U32).at[:, p, :], wqr_ref.at[p], ssem.at[8]).start()
            pltpu.make_async_copy(wv_hbm.bitcast(U32).at[:, p, :], wvr_ref.at[p], ssem.at[9]).start()
            return carry
        lax.fori_loop(1, NP, start_qv, 0)
        wo_copy.start()
        for cp in late_copies:
            cp.start()
        mod_ref[0:2] = jnp.zeros((2, 8, M), F32)
        zero_ref[...] = jnp.zeros(zero_ref.shape, U32)
        wk_copy(0).wait()
        stage_wk(0, (0,))

        def head_keys(i, carry):
            ckv_head(i).wait()
            lo = pl.multiple_of(i * HK, HK)
            proj_k(0, lo, ckv_ref[pl.ds(lo, HK), :], 0, 1)
            return carry
        lax.fori_loop(0, CR // HK, head_keys, 0)
        for p in range(1, KP):
            wk_copy(p).wait()
        c_copy.wait()
        c = c_ref[...].astype(F32)
        sc = jnp.broadcast_to(c * jax.nn.sigmoid(c), (128, M))
        sc_ref[...] = _as_u32(sc.T.astype(BF16))
        stage_wk(0, tuple(range(1, KP)))
        for i in range(CR // HK):
            proj_k(0, i * HK, ckv_ref[i * HK:(i + 1) * HK, :], 1, KP)

        def first_keys(i, carry):
            ckv_chunk(i).wait()
            for ii in range(CR // HK):
                lo = pl.multiple_of(i * CR + ii * HK, HK)
                proj_k(0, lo, ckv_ref[pl.ds(lo, HK), :])
            return carry
        lax.fori_loop(1, CC, first_keys, 0)
        for cp in pair0_copies[:2]:
            cp.wait()

    def _keys(step, carry):
        for u in range(KP):
            wk_copy(step * KP + u).wait()

        @pl.when(step <= NM)
        def _():
            wmod_copy(step - 1).wait()

        @pl.when(step == NK - NL)
        def _():
            x_copy.wait()

        wk = jnp.concatenate([half for u in range(KP) for half in _halves(wkr_ref[step * KP + u])],
                             axis=1).astype(BF16)
        g = jnp.minimum(step - 1, NM - 1)
        live = step >= NK - NL
        lblk = step - (NK - NL)
        sa = mod_ref[0, 0:1, :]
        ca1 = 1.0 + mod_ref[1, 0:1, :]
        zero = zero_ref[...]
        mc = M // 2 // nk
        ar = -(-(S + 2 * HALO) // ((NK - 1) * nk * 8)) * 8
        deps, part = [], None
        for i in range(nk):
            lhs = ckv_ref[i * HK:(i + 1) * HK, :]
            if deps:
                lhs = _after(lhs, deps, zero)
            k = proj_k(step, i * HK, lhs, w=wk)
            r = pl.multiple_of(jnp.where(live, HALO + lblk * LR + i * LC, S + 2 * HALO), 8)
            rh = pl.multiple_of(jnp.where(live, (lblk * LR + i * LC) // 2, S // 2), 8)
            x = x_ref[pl.ds(r, LC), :].astype(F32)
            h = _ln(x) * ca1 + sa
            h_ref[pl.ds(rh, LC // 2), :] = _as_u32(h.astype(BF16))
            we, wo = _halves(wmod_ref[g, i * mc:(i + 1) * mc, :])
            se, so = _halves(sc_ref[i * mc:(i + 1) * mc, :])
            prod = we * jnp.tile(se, (1, M // 128)) + wo * jnp.tile(so, (1, M // 128))
            for rr in range(0, mc, 8):
                part = prod[rr:rr + 8] if part is None else part + prod[rr:rr + 8]
            deps = [pltpu.bitcast(h, U32), pltpu.bitcast(part, U32)]
            zt = pltpu.bitcast(pltpu.bitcast(k[0:8, ZC * D:(ZC + 1) * D], U32) & zero, F32)
            ra = jnp.minimum(((step - 1) * nk + i) * ar, S + 2 * HALO - ar)
            acc_ref[pl.ds(pl.multiple_of(ra, 8), ar), :] = jnp.tile(zt, (ar // 8, M // 128))
            zu = pltpu.bitcast(k[0:8, ZS * D:(ZS + 1) * D], U32) & zero
            for raw_ref, dst_ref in ((wqr_ref, wqp_ref), (wvr_ref, wvp_ref)):
                n = raw_ref.shape[1] // nk
                raw = raw_ref[0, i * n:(i + 1) * n, :] | jnp.tile(zu, (n // 8, 1))
                dst_ref[i * n // 2:(i + 1) * n // 2, :] = _split_pair(raw)
        mod_ref[g] = jnp.broadcast_to(jnp.sum(part, axis=0, keepdims=True), (8, M))
        return carry

    def _wait_pair_weights():
        pltpu.make_async_copy(wqr_ref.at[rest], wqr_ref.at[rest], ssem.at[8]).wait()
        pltpu.make_async_copy(wvr_ref.at[rest], wvr_ref.at[rest], ssem.at[9]).wait()
        wo_copy.wait()
        pair0_copies[2].wait()

    def _attention(j, carry):
        HH = HQ // 2
        row = lax.broadcasted_iota(jnp.int32, (HQ, TQ), 0)
        col = lax.broadcasted_iota(jnp.int32, (HQ, TQ), 1)
        diag = col <= row + HQ
        first = [col < HQ, col >= HQ]
        first0 = [col <= row, jnp.logical_and(col >= HQ, diag)]

        def proj_v(i):
            rows = slice(i * HQ, (i + 1) * HQ)
            v = jnp.dot(_as_bf16(ckv_ref[rows, :]), _as_bf16(wvp_ref[...]), preferred_element_type=F32)
            v_ref[rows, :] = _as_u32(v.astype(BF16))

        def proj_q(i):
            rows = slice(i * HQ, (i + 1) * HQ)
            q = jnp.dot(_as_bf16(h_ref[rows, :]), _as_bf16(wqp_ref[...]), preferred_element_type=F32)
            q = q * qscale
            return [[q[half * HQ:(half + 1) * HQ, hh * D:(hh + 1) * D].astype(BF16)
                     for half in range(2)] for hh in range(2)]

        def masked_scores(qh, k):
            s = lax.dot_general(qh, k, NT, preferred_element_type=F32)
            n = s.shape[1] - TQ
            sd = jnp.where(diag, s[:, n:], NEG)
            return jnp.concatenate([s[:, :n], sd], axis=1) if n else sd

        def scores(q, hh, half, i):
            cols = slice(hh * D, (hh + 1) * D)
            if half == 1:
                return masked_scores(q[hh][1], _as_bf16(k_ref[k_rows(j, 0, (i + 1) * HQ), cols]))
            if i > 0:
                return masked_scores(q[hh][0], _as_bf16(k_ref[k_rows(j, HH, i * HQ), cols]))
            return None

        def first_scores(q1, q2):
            st = [lax.dot_general(_as_bf16(k_ref[k_rows(j, 0, HH), hh * D:(hh + 1) * D]),
                                  jnp.concatenate([q1[hh][0], q2[hh][0]], axis=0),
                                  NT, preferred_element_type=F32) for hh in range(2)]
            t = jnp.concatenate(st, axis=0).T
            return t[0:HQ], t[HQ:TQ]

        def softmax_pv(s, t0, hh, half, i):
            cols = slice(hh * D, (hh + 1) * D)
            if half == 1:
                v = v_ref[0:(i + 1) * HQ, cols]
            else:
                s0 = jnp.where(first[hh] if i > 0 else first0[hh], t0[i], NEG)
                s = s0 if s is None else jnp.concatenate([s, s0], axis=1)
                if hh == 0:
                    v = v_ref[0:HQ, cols]
                else:
                    v = jnp.concatenate([v_ref[HH:HQ, cols], v_ref[0:HH, cols]], axis=0)
                if i > 0:
                    v = jnp.concatenate([v_ref[HH:i * HQ + HH, cols], v], axis=0)
            m = jnp.max(s, axis=1, keepdims=True)
            p = jnp.exp2(s - m).astype(BF16)
            l = jnp.sum(p.astype(F32), axis=1, keepdims=True)
            o = jnp.dot(p, _as_bf16(v), preferred_element_type=F32)
            return o * pl.reciprocal(l, approx=False, full_range=False)

        def oproj(ctx, r, n):
            rows = slice(HALO + r, HALO + r + n)
            acc_ref[rows, :] += jnp.dot(ctx.astype(BF16), _as_bf16(wop_ref[...]),
                                        preferred_element_type=F32)

        q, s, t0, ctx = {}, {}, {}, {}
        for op in _attention_schedule(nq):
            kind, i = op[0], op[1]
            if kind == "q":
                q[i] = proj_q(i)
            elif kind == "v":
                proj_v(i)
            elif kind == "s":
                s[op[1:]] = scores(q[i], op[2], op[3], i)
            elif kind == "t":
                t0[i], t0[op[2]] = first_scores(q[i], q[op[2]])
            elif kind == "pv":
                ctx[op[1:]] = softmax_pv(s.pop(op[1:]), t0, op[2], op[3], i)
            else:
                oproj(jnp.concatenate([ctx.pop((i, hh, op[2])) for hh in range(2)], axis=1),
                      i * TQ + op[2] * HQ, HQ)

        stage_weights(jnp.minimum(j + 1, NP - 1))
        return carry

    def _epilogue():
        for cp in late_copies:
            cp.wait()

        G = M // 4
        NC = TB // TC
        TH = TB + 2 * HALO
        ntile = (Fd + 127) // 128
        fsplit = [min(Fd, ((k * ntile + NC - 1) // NC) * 128) for k in range(NC + 1)]

        def start_row(t):
            return t * TB if isinstance(t, int) else pl.multiple_of(t * TB, TB)

        def front_a(t, lo, hi):
            r = start_row(t)
            ga = mod_ref[2, 0:1, :]
            sb = mod_ref[3, 0:1, :]
            cb1 = 1.0 + mod_ref[4, 0:1, :]
            x1 = (x_ref[pl.ds(r + lo, hi - lo), :].astype(F32)
                  + ga * acc_ref[pl.ds(r + lo, hi - lo), :])
            h = _ln(x1) * cb1 + sb
            tt = _gelu(jnp.dot(_ln(h).astype(BF16), _as_bf16(w1_ref[...]),
                               preferred_element_type=F32))
            if lo == 0:
                tt = jnp.concatenate([jnp.zeros((HALO, M), F32), tt[HALO:]], axis=0)
            if lo == 2 * HALO:
                x1, h, tt = [jnp.concatenate([cr_ref[a], v], axis=0)
                             for a, v in enumerate((x1, h, tt))]
            if hi == TH:
                n = hi - lo - HALO
                tt = jnp.concatenate([tt[:n], jnp.where(r + TB < S, tt[n:], 0.0)], axis=0)
                for a, v in enumerate((x1, h, tt)):
                    cr_ref[a] = v[n - HALO:]
            return x1, h, tt

        def front_b(x1, h, tt, lo, n):
            gb = mod_ref[5, 0:1, :]
            lane = lax.broadcasted_iota(jnp.int32, (n, 128), 1)
            cols = []
            shifts = (-1, 1, -2, 2)
            for cblk in range(M // 128):
                c0, c1 = cblk * 128, (cblk + 1) * 128
                ga_, gb_ = c0 // G, (c1 - 1) // G
                a = tt[HALO + lo + shifts[ga_]:HALO + lo + shifts[ga_] + n, c0:c1]
                if gb_ != ga_:
                    b = tt[HALO + lo + shifts[gb_]:HALO + lo + shifts[gb_] + n, c0:c1]
                    a = jnp.where(lane < gb_ * G - c0, a, b)
                cols.append(a)
            sh = jnp.concatenate(cols, axis=1).astype(BF16)
            y = h[HALO + lo:HALO + lo + n] + jnp.dot(sh, _as_bf16(w2_ref[...]),
                                                     preferred_element_type=F32)
            z_ref[lo:lo + n, :] = x1[HALO + lo:HALO + lo + n] + gb * y
            u3_ref[lo // 2:(lo + n) // 2, :] = _as_u32(_ln(y).astype(BF16))

        def out_copy(it, n):
            rows = pl.ds(start_row(it * NS), n * TB)
            return pltpu.make_async_copy(ob_ref.at[rows, :], o_hbm.at[rows, :], osem.at[it])

        w3h_ref[...] = _as_u32(_as_bf16(w3t_ref[0:64, :]).astype(F32).T.astype(BF16))

        def mm3(k, opens):
            lo, hi = fsplit[k], fsplit[k + 1]
            mid = hi - hi % 128
            u3 = _as_bf16(u3_ref[...])
            fs = []
            if opens:
                fs.append(jnp.dot(u3, _as_bf16(w3h_ref[...]), preferred_element_type=F32))
                lo += 128
            fs.append(lax.dot_general(u3, _as_bf16(w3t_ref[lo // 2:mid // 2, :]),
                                      NT, preferred_element_type=F32))
            f = _gelu(jnp.concatenate(fs, axis=1))
            if mid < hi:
                ft = _gelu(lax.dot_general(_as_bf16(w3t_ref[mid // 2:hi // 2, :]), u3,
                                           NT, preferred_element_type=F32))
                f = jnp.concatenate([f, ft.T], axis=1)
            return [f[kk * TC:(kk + 1) * TC].astype(BF16) for kk in range(NC)]

        def mm4(t, f, z, k):
            lo = k * TC
            gb = mod_ref[5, 0:1, :]
            h2 = jnp.dot(jnp.concatenate([fk[k] for fk in f], axis=1), _as_bf16(w4_ref[...]),
                         preferred_element_type=F32)
            ob_ref[pl.ds(start_row(t) + lo, TC), :] = (z + gb * h2).astype(ob_ref.dtype)

        def stage(t, nxt, opens):
            fs, fr = [], []
            for k in range(NC):
                fs.append(mm3(k, opens and k == 0))
                if nxt:
                    fr.append(front_a(t + 1, 2 * HALO + k * TC, 2 * HALO + (k + 1) * TC))
            if nxt:
                fr = [jnp.concatenate(parts, axis=0) for parts in zip(*fr)]
            for k in range(NC):
                z = z_ref[k * TC:(k + 1) * TC, :]
                if nxt and k == NC - 1:
                    front_b(*fr, k * TC, TC)
                mm4(t, fs, z, k)
                if nxt and k < NC - 1:
                    front_b(*fr, k * TC, TC)

        nb = S // TB
        ni = (nb - 1) // NS
        assert ni * NS == nb - 1
        fr = [front_a(0, lo, hi) for lo, hi in zip(FILL_A[:-1], FILL_A[1:])]
        fr = [jnp.concatenate(parts, axis=0) for parts in zip(*fr)]
        for lo, hi in zip(FILL_B[:-1], FILL_B[1:]):
            front_b(*fr, lo, hi - lo)

        def loop_b(it, carry):
            for u in range(NS):
                stage(it * NS + u, True, u == 0)
            out_copy(it, NS).start()
            return carry
        lax.fori_loop(0, ni, loop_b, 0)
        stage(nb - 1, False, True)
        out_copy(ni, 1).start()
        for it in range(ni):
            out_copy(it, NS).wait()
        out_copy(ni, 1).wait()

    @pl.when(pl.program_id(0) == 0)
    def _():
        _prologue()
        lax.fori_loop(1, NK, _keys, 0)
        _wait_pair_weights()
        lax.fori_loop(0, NP, _attention, 0)

    @pl.when(pl.program_id(0) == 1)
    def _():
        _epilogue()


@jax.jit
def pallas_adaLN_cond__compressed_kv_cla__mixer_s_mlp__prompt_kernel(
    A_x: jax.Array,
    A_c_kv: jax.Array,
    A_w_q: jax.Array,
    A_w_uk: jax.Array,
    A_w_uv: jax.Array,
    A_w_o: jax.Array,
    B_x: jax.Array,
    B_w1: jax.Array,
    B_w2: jax.Array,
    B_w3: jax.Array,
    B_w4: jax.Array,
    c: jax.Array,
    w_mod: jax.Array,
):
    B, S, M = A_x.shape
    assert B == 1 and A_c_kv.shape[1] == S
    Dc = A_c_kv.shape[2]
    H, D = A_w_q.shape[1], A_w_q.shape[2]
    NP = H // 2
    Fd = B_w3.shape[1]
    LC = TK // NL
    any_spec = pl.BlockSpec(memory_space=pl.ANY)

    out = pl.pallas_call(
        functools.partial(_kernel, S=S, M=M, D=D, NP=NP, Fd=Fd),
        grid=(2,),
        in_specs=[any_spec] * 12,
        out_specs=any_spec,
        out_shape=jax.ShapeDtypeStruct((S, M), A_x.dtype),
        scratch_shapes=[
            pltpu.VMEM((S + 2 * HALO + LC, M), BF16),
            pltpu.VMEM((S // 2, Dc), U32),
            pltpu.VMEM((NP, M, D), U32),
            pltpu.VMEM((NP, Dc, D), U32),
            pltpu.VMEM((NP, Dc, D), U32),
            pltpu.VMEM((NP, D, M), U32),
            pltpu.VMEM((M // 2, M), U32),
            pltpu.VMEM((M // 2, M), U32),
            pltpu.VMEM((Fd // 2, M), U32),
            pltpu.VMEM((Fd // 2, M), U32),
            pltpu.VMEM((1, M), BF16),
            pltpu.VMEM((6, M // 2, M), U32),
            pltpu.VMEM((8, 128), U32),
            pltpu.VMEM((M // 2, 128), U32),
            pltpu.VMEM((6, 8, M), F32),
            pltpu.VMEM(((S + LC) // 2, M), U32),
            pltpu.VMEM((M // 2, 2 * D), U32),
            pltpu.VMEM((Dc // 2, 2 * KP * D), U32),
            pltpu.VMEM((Dc // 2, 2 * D), U32),
            pltpu.VMEM((D, M), U32),
            pltpu.VMEM((NP * S // 2, 2 * D), U32),
            pltpu.VMEM((S // 2, 2 * D), U32),
            pltpu.VMEM((S + 2 * HALO, M), F32),
            pltpu.VMEM((M // 2, 128), U32),
            pltpu.VMEM((3, 2 * HALO, M), F32),
            pltpu.VMEM((TB, M), F32),
            pltpu.VMEM((TB // 2, M), U32),
            pltpu.VMEM((S, M), BF16),
            pltpu.SemaphoreType.DMA((12,)),
            pltpu.SemaphoreType.DMA((CC - 1 + S // CC // TK,)),
            pltpu.SemaphoreType.DMA((NP,)),
            pltpu.SemaphoreType.DMA((6,)),
            pltpu.SemaphoreType.DMA(((S // TB - 1) // NS + 1,)),
        ],
        compiler_params=pltpu.CompilerParams(
            dimension_semantics=("arbitrary",),
            vmem_limit_bytes=100 * 1024 * 1024,
            disable_bounds_checks=True,
            disable_semaphore_checks=True,
        ),
    )(
        A_x.reshape(S, M), A_c_kv.reshape(S, Dc),
        A_w_q, A_w_uk, A_w_uv,
        A_w_o.reshape(NP, 2 * D, M),
        B_w1, B_w2, B_w3.T, B_w4, c, w_mod,
    )
    return out.reshape(B, S, M)
```

```python
import functools
import math

import jax
import jax.numpy as jnp
from jax import lax
import jax.experimental.pallas as pl
import jax.experimental.pallas.tpu as pltpu

F32 = jnp.float32
BF16 = jnp.bfloat16
U32 = jnp.uint32
NT = (((1,), (1,)), ((), ()))
NEG = -1000000000.0
EPS = 1e-05
CC = 4
KP = 2
TK = 256
NL = 4
ZC, ZS = 3, 2
TQ = 128
LAG = 4
O_LAG = 4
Q_SUB = 0
T_SUB = 2
TB = 128
NS = 3
TC = 64
HALO = 8
FILL_A = (0, 96, 144)
FILL_B = (0, 64, 128)


def _ln(x):
    m = jnp.mean(x, axis=-1, keepdims=True)
    xc = x - m
    v = jnp.mean(xc * xc, axis=-1, keepdims=True)
    return xc * lax.rsqrt(v + EPS)


def _gelu(x):
    c = math.sqrt(2.0 / math.pi)
    hx = 0.5 * x
    return hx + hx * jnp.tanh(x * (c + (c * 0.044715) * (x * x)))


def _as_bf16(u):
    return pltpu.bitcast(u, BF16)


def _as_u32(b):
    return pltpu.bitcast(b, U32)


def _halves(u):
    return pltpu.bitcast(u << 16, F32), pltpu.bitcast(u & jnp.uint32(0xFFFF0000), F32)


def _split_pair(u):
    return _as_u32(jnp.concatenate(_halves(u), axis=1).astype(BF16))


def _attention_schedule(nq):
    order = list(range(nq - 1, -1, -1))
    units = [(i, hh, half) for i in order for half in (1, 0) for hh in (0, 1)]
    ops = [("q", order[0]), ("v", 0)]
    per = -(-(nq - 1) // LAG)
    for k in range(len(units) + LAG + O_LAG):
        n, sub = divmod(k, 4)
        if k < len(units):
            ops.append(("s",) + units[k])
        if 0 <= k - LAG < len(units):
            ops.append(("pv",) + units[k - LAG])
        if sub == Q_SUB and n + 1 < nq:
            ops.append(("q", order[n + 1]))
        if k < LAG:
            ops.extend(("v", i) for i in range(1 + k * per, min(nq, 1 + (k + 1) * per)))
        if sub == T_SUB and n % 2 == 0 and n + 1 < nq:
            ops.append(("t", order[n], order[n + 1]))
        ko = k - LAG - O_LAG
        if 0 <= ko < len(units) and ko % 2 == 1:
            ops.append(("o", units[ko][0], units[ko][2]))
    return ops


def _after(lhs, deps, zero):
    t = None
    for dep in deps:
        for r in range(0, dep.shape[0], 8):
            for c in range(0, dep.shape[1], 128):
                tile = dep[r:r + 8, c:c + 128]
                t = tile if t is None else t | tile
    head = lhs[0:8, 0:128] | (t & zero)
    if lhs.shape[1] > 128:
        head = jnp.concatenate([head, lhs[0:8, 128:]], axis=1)
    return jnp.concatenate([head, lhs[8:]], axis=0)


def _kernel(x_hbm, ckv_hbm, wq_hbm, wk_hbm, wv_hbm, wo_hbm,
            w1_hbm, w2_hbm, w3t_hbm, w4_hbm, c_hbm, wmod_hbm,
            o_hbm,
            x_ref, ckv_ref, wqr_ref, wkr_ref, wvr_ref, wo_ref,
            w1_ref, w2_ref, w3t_ref, w4_ref, wmod_ref, k_ref, acc_ref, h_ref, ob_ref,
            sc_ref, wqp_ref, wkp_ref, wvp_ref, wop_ref, v_ref, w3h_ref, z_ref, u3_ref,
            mod_ref, cr_ref, zero_ref, c_ref,
            ssem, csem, ksem, msem, osem,
            *, S, M, D, NP, Fd):
    NK = NP // KP
    nq = S // TQ
    HQ = TQ // 2
    qscale = (D ** -0.5) * math.log2(math.e)
    LR = S // NL
    NM = 6
    nk = S // TK
    LC = LR // nk
    assert NK - 1 >= NM and NK - NL >= 3

    c_copy = pltpu.make_async_copy(c_hbm, c_ref, ssem.at[0])
    CR = S // CC // 2
    HK = TK // 2

    def ckv_copy(lo, n, sem):
        rows = pl.ds(lo if isinstance(lo, int) else pl.multiple_of(lo, HK), n)
        return pltpu.make_async_copy(ckv_hbm.bitcast(U32).at[rows, :], ckv_ref.at[rows, :],
                                     csem.at[sem])

    def ckv_head(i):
        return ckv_copy(i * HK, HK, i)

    def ckv_chunk(i):
        return ckv_copy(i * CR, CR, CR // HK - 1 + i)

    x_copy = pltpu.make_async_copy(x_hbm, x_ref.at[pl.ds(HALO, S), :], ssem.at[2])
    rest = pl.ds(1, NP - 1)
    wo_copy = pltpu.make_async_copy(wo_hbm.bitcast(U32).at[rest], wo_ref.at[rest], ssem.at[3])
    pair0_copies = [
        pltpu.make_async_copy(wq_hbm.bitcast(U32).at[:, 0, :], wqr_ref.at[0], ssem.at[1]),
        pltpu.make_async_copy(wv_hbm.bitcast(U32).at[:, 0, :], wvr_ref.at[0], ssem.at[10]),
        pltpu.make_async_copy(wo_hbm.bitcast(U32).at[0], wop_ref, ssem.at[11]),
    ]
    late_copies = [
        pltpu.make_async_copy(w1_hbm.bitcast(U32), w1_ref, ssem.at[4]),
        pltpu.make_async_copy(w2_hbm.bitcast(U32), w2_ref, ssem.at[5]),
        pltpu.make_async_copy(w3t_hbm.bitcast(U32), w3t_ref, ssem.at[6]),
        pltpu.make_async_copy(w4_hbm.bitcast(U32), w4_ref, ssem.at[7]),
    ]

    def wk_copy(p):
        return pltpu.make_async_copy(wk_hbm.bitcast(U32).at[:, p, :], wkr_ref.at[p], ksem.at[p])

    def wmod_copy(g):
        off = g * M if isinstance(g, int) else pl.multiple_of(g * M, 128)
        return pltpu.make_async_copy(wmod_hbm.bitcast(U32).at[:, pl.ds(off, M)],
                                     wmod_ref.at[g], msem.at[g])

    def stage_weights(p):
        wqp_ref[...] = _split_pair(wqr_ref[p])
        wvp_ref[...] = _split_pair(wvr_ref[p])
        wop_ref[...] = wo_ref[p]

    def stage_wk(step, us=tuple(range(KP))):
        for u in us:
            wkp_ref[:, 2 * u * D:(2 * u + 2) * D] = _split_pair(wkr_ref[step * KP + u])

    def k_rows(p, lo, n):
        off = p * (S // 2) + lo
        return pl.ds(off if isinstance(off, int) else pl.multiple_of(off, 8), n)

    def proj_k(step, lo, lhs, u0=0, u1=KP, w=None):
        if w is None:
            w = _as_bf16(wkp_ref[:, 2 * u0 * D:2 * u1 * D])
        k = jnp.dot(_as_bf16(lhs), w, preferred_element_type=F32)
        for u in range(u0, u1):
            k_ref[k_rows(step * KP + u, lo, HK), :] = _as_u32(
                k[:, 2 * (u - u0) * D:2 * (u - u0 + 1) * D].astype(BF16))
        return k

    def _prologue():
        wk_copy(0).start()
        for i in range(CR // HK):
            ckv_head(i).start()
        c_copy.start()
        for p in range(1, KP):
            wk_copy(p).start()
        for i in range(1, CC):
            ckv_chunk(i).start()
        x_ref[0:HALO, :] = jnp.zeros((HALO, M), BF16)
        x_ref[S + HALO:S + HALO + 2 * LC, :] = jnp.zeros((2 * LC, M), BF16)
        for g in range(2):
            for p in range((g + 1) * KP, (g + 2) * KP):
                wk_copy(p).start()
            wmod_copy(g).start()
            if g == 0:
                for cp in pair0_copies[:2]:
                    cp.start()
        pair0_copies[2].start()

        def start_wk(p, carry):
            wk_copy(p).start()
            return carry
        lax.fori_loop(3 * KP, NP, start_wk, 0)
        wmod_copy(2).start()
        x_copy.start()
        for g in range(3, NM):
            wmod_copy(g).start()

        def start_qv(p, carry):
            pltpu.make_async_copy(wq_hbm.bitcast(U32).at[:, p, :], wqr_ref.at[p], ssem.at[8]).start()
            pltpu.make_async_copy(wv_hbm.bitcast(U32).at[:, p, :], wvr_ref.at[p], ssem.at[9]).start()
            return carry
        lax.fori_loop(1, NP, start_qv, 0)
        wo_copy.start()
        for cp in late_copies:
            cp.start()
        mod_ref[0:2] = jnp.zeros((2, 8, M), F32)
        zero_ref[...] = jnp.zeros(zero_ref.shape, U32)
        wk_copy(0).wait()
        stage_wk(0, (0,))

        def head_keys(i, carry):
            ckv_head(i).wait()
            lo = pl.multiple_of(i * HK, HK)
            proj_k(0, lo, ckv_ref[pl.ds(lo, HK), :], 0, 1)
            return carry
        lax.fori_loop(0, CR // HK, head_keys, 0)
        for p in range(1, KP):
            wk_copy(p).wait()
        c_copy.wait()
        c = c_ref[...].astype(F32)
        sc = jnp.broadcast_to(c * jax.nn.sigmoid(c), (128, M))
        sc_ref[...] = _as_u32(sc.T.astype(BF16))
        stage_wk(0, tuple(range(1, KP)))
        for i in range(CR // HK):
            proj_k(0, i * HK, ckv_ref[i * HK:(i + 1) * HK, :], 1, KP)

        def first_keys(i, carry):
            ckv_chunk(i).wait()
            for ii in range(CR // HK):
                lo = pl.multiple_of(i * CR + ii * HK, HK)
                proj_k(0, lo, ckv_ref[pl.ds(lo, HK), :])
            return carry
        lax.fori_loop(1, CC, first_keys, 0)
        for cp in pair0_copies[:2]:
            cp.wait()

    def _keys(step, carry):
        for u in range(KP):
            wk_copy(step * KP + u).wait()

        @pl.when(step <= NM)
        def _():
            wmod_copy(step - 1).wait()

        @pl.when(step == NK - NL)
        def _():
            x_copy.wait()

        wk = jnp.concatenate([half for u in range(KP) for half in _halves(wkr_ref[step * KP + u])],
                             axis=1).astype(BF16)
        g = jnp.minimum(step - 1, NM - 1)
        live = step >= NK - NL
        lblk = step - (NK - NL)
        sa = mod_ref[0, 0:1, :]
        ca1 = 1.0 + mod_ref[1, 0:1, :]
        zero = zero_ref[...]
        mc = M // 2 // nk
        ar = -(-(S + 2 * HALO) // ((NK - 1) * nk * 8)) * 8
        deps, part = [], None
        for i in range(nk):
            lhs = ckv_ref[i * HK:(i + 1) * HK, :]
            if deps:
                lhs = _after(lhs, deps, zero)
            k = proj_k(step, i * HK, lhs, w=wk)
            r = pl.multiple_of(jnp.where(live, lblk * LR + i * LC, S + LC), LC)
            rh = pl.multiple_of(jnp.where(live, (lblk * LR + i * LC) // 2, S // 2), 8)
            x = x_ref.at[pl.ds(r, LC + HALO), :][HALO:, :].astype(F32)
            h = _ln(x) * ca1 + sa
            h_ref[pl.ds(rh, LC // 2), :] = _as_u32(h.astype(BF16))
            we, wo = _halves(wmod_ref[g, i * mc:(i + 1) * mc, :])
            se, so = _halves(sc_ref[i * mc:(i + 1) * mc, :])
            prod = we * jnp.tile(se, (1, M // 128)) + wo * jnp.tile(so, (1, M // 128))
            for rr in range(0, mc, 8):
                part = prod[rr:rr + 8] if part is None else part + prod[rr:rr + 8]
            deps = [pltpu.bitcast(h, U32), pltpu.bitcast(part, U32)]
            zt = pltpu.bitcast(pltpu.bitcast(k[0:8, ZC * D:(ZC + 1) * D], U32) & zero, F32)
            ra = jnp.minimum(((step - 1) * nk + i) * ar, S + 2 * HALO - ar)
            acc_ref[pl.ds(pl.multiple_of(ra, 8), ar), :] = jnp.tile(zt, (ar // 8, M // 128))
            zu = pltpu.bitcast(k[0:8, ZS * D:(ZS + 1) * D], U32) & zero
            for raw_ref, dst_ref in ((wqr_ref, wqp_ref), (wvr_ref, wvp_ref)):
                n = raw_ref.shape[1] // nk
                raw = raw_ref[0, i * n:(i + 1) * n, :] | jnp.tile(zu, (n // 8, 1))
                dst_ref[i * n // 2:(i + 1) * n // 2, :] = _split_pair(raw)
        mod_ref[g] = jnp.broadcast_to(jnp.sum(part, axis=0, keepdims=True), (8, M))
        return carry

    def _wait_pair_weights():
        pltpu.make_async_copy(wqr_ref.at[rest], wqr_ref.at[rest], ssem.at[8]).wait()
        pltpu.make_async_copy(wvr_ref.at[rest], wvr_ref.at[rest], ssem.at[9]).wait()
        wo_copy.wait()
        pair0_copies[2].wait()

    def _attention(j, carry):
        HH = HQ // 2
        row = lax.broadcasted_iota(jnp.int32, (HQ, TQ), 0)
        col = lax.broadcasted_iota(jnp.int32, (HQ, TQ), 1)
        diag = col <= row + HQ
        first = [col < HQ, col >= HQ]
        first0 = [col <= row, jnp.logical_and(col >= HQ, diag)]

        def proj_v(i):
            rows = slice(i * HQ, (i + 1) * HQ)
            v = jnp.dot(_as_bf16(ckv_ref[rows, :]), _as_bf16(wvp_ref[...]), preferred_element_type=F32)
            v_ref[rows, :] = _as_u32(v.astype(BF16))

        def proj_q(i):
            rows = slice(i * HQ, (i + 1) * HQ)
            q = jnp.dot(_as_bf16(h_ref[rows, :]), _as_bf16(wqp_ref[...]), preferred_element_type=F32)
            q = q * qscale
            return [[q[half * HQ:(half + 1) * HQ, hh * D:(hh + 1) * D].astype(BF16)
                     for half in range(2)] for hh in range(2)]

        def masked_scores(qh, k):
            s = lax.dot_general(qh, k, NT, preferred_element_type=F32)
            n = s.shape[1] - TQ
            sd = jnp.where(diag, s[:, n:], NEG)
            return jnp.concatenate([s[:, :n], sd], axis=1) if n else sd

        def scores(q, hh, half, i):
            cols = slice(hh * D, (hh + 1) * D)
            if half == 1:
                return masked_scores(q[hh][1], _as_bf16(k_ref[k_rows(j, 0, (i + 1) * HQ), cols]))
            if i > 0:
                return masked_scores(q[hh][0], _as_bf16(k_ref[k_rows(j, HH, i * HQ), cols]))
            return None

        def first_scores(q1, q2):
            st = [lax.dot_general(_as_bf16(k_ref[k_rows(j, 0, HH), hh * D:(hh + 1) * D]),
                                  jnp.concatenate([q1[hh][0], q2[hh][0]], axis=0),
                                  NT, preferred_element_type=F32) for hh in range(2)]
            t = jnp.concatenate(st, axis=0).T
            return t[0:HQ], t[HQ:TQ]

        def softmax_pv(s, t0, hh, half, i):
            cols = slice(hh * D, (hh + 1) * D)
            if half == 1:
                v = v_ref[0:(i + 1) * HQ, cols]
            else:
                s0 = jnp.where(first[hh] if i > 0 else first0[hh], t0[i], NEG)
                s = s0 if s is None else jnp.concatenate([s, s0], axis=1)
                if hh == 0:
                    v = v_ref[0:HQ, cols]
                else:
                    v = jnp.concatenate([v_ref[HH:HQ, cols], v_ref[0:HH, cols]], axis=0)
                if i > 0:
                    v = jnp.concatenate([v_ref[HH:i * HQ + HH, cols], v], axis=0)
            m = jnp.max(s, axis=1, keepdims=True)
            p = jnp.exp2(s - m).astype(BF16)
            l = jnp.sum(p.astype(F32), axis=1, keepdims=True)
            o = jnp.dot(p, _as_bf16(v), preferred_element_type=F32)
            return o * pl.reciprocal(l, approx=False, full_range=False)

        def oproj(ctx, r, n):
            rows = slice(HALO + r, HALO + r + n)
            acc_ref[rows, :] += jnp.dot(ctx.astype(BF16), _as_bf16(wop_ref[...]),
                                        preferred_element_type=F32)

        q, s, t0, ctx = {}, {}, {}, {}
        for op in _attention_schedule(nq):
            kind, i = op[0], op[1]
            if kind == "q":
                q[i] = proj_q(i)
            elif kind == "v":
                proj_v(i)
            elif kind == "s":
                s[op[1:]] = scores(q[i], op[2], op[3], i)
            elif kind == "t":
                t0[i], t0[op[2]] = first_scores(q[i], q[op[2]])
            elif kind == "pv":
                ctx[op[1:]] = softmax_pv(s.pop(op[1:]), t0, op[2], op[3], i)
            else:
                oproj(jnp.concatenate([ctx.pop((i, hh, op[2])) for hh in range(2)], axis=1),
                      i * TQ + op[2] * HQ, HQ)

        stage_weights(jnp.minimum(j + 1, NP - 1))
        return carry

    def _epilogue():
        for cp in late_copies:
            cp.wait()

        G = M // 4
        NC = TB // TC
        TH = TB + 2 * HALO
        ntile = (Fd + 127) // 128
        fsplit = [min(Fd, ((k * ntile + NC - 1) // NC) * 128) for k in range(NC + 1)]

        def start_row(t):
            return t * TB if isinstance(t, int) else pl.multiple_of(t * TB, TB)

        def front_a(t, lo, hi):
            r = start_row(t)
            ga = mod_ref[2, 0:1, :]
            sb = mod_ref[3, 0:1, :]
            cb1 = 1.0 + mod_ref[4, 0:1, :]
            x1 = (x_ref.at[pl.ds(r, TH), :][lo:hi, :].astype(F32)
                  + ga * acc_ref.at[pl.ds(r, TH), :][lo:hi, :])
            h = _ln(x1) * cb1 + sb
            tt = _gelu(jnp.dot(_ln(h).astype(BF16), _as_bf16(w1_ref[...]),
                               preferred_element_type=F32))
            if lo == 0:
                tt = jnp.concatenate([jnp.zeros((HALO, M), F32), tt[HALO:]], axis=0)
            if lo == 2 * HALO:
                x1, h, tt = [jnp.concatenate([cr_ref[a], v], axis=0)
                             for a, v in enumerate((x1, h, tt))]
            if hi == TH:
                n = hi - lo - HALO
                tt = jnp.concatenate([tt[:n], jnp.where(r + TB < S, tt[n:], 0.0)], axis=0)
                for a, v in enumerate((x1, h, tt)):
                    cr_ref[a] = v[n - HALO:]
            return x1, h, tt

        def front_b(x1, h, tt, lo, n):
            gb = mod_ref[5, 0:1, :]
            lane = lax.broadcasted_iota(jnp.int32, (n, 128), 1)
            cols = []
            shifts = (-1, 1, -2, 2)
            for cblk in range(M // 128):
                c0, c1 = cblk * 128, (cblk + 1) * 128
                ga_, gb_ = c0 // G, (c1 - 1) // G
                a = tt[HALO + lo + shifts[ga_]:HALO + lo + shifts[ga_] + n, c0:c1]
                if gb_ != ga_:
                    b = tt[HALO + lo + shifts[gb_]:HALO + lo + shifts[gb_] + n, c0:c1]
                    a = jnp.where(lane < gb_ * G - c0, a, b)
                cols.append(a)
            sh = jnp.concatenate(cols, axis=1).astype(BF16)
            y = h[HALO + lo:HALO + lo + n] + jnp.dot(sh, _as_bf16(w2_ref[...]),
                                                     preferred_element_type=F32)
            z_ref[lo:lo + n, :] = x1[HALO + lo:HALO + lo + n] + gb * y
            u3_ref[lo // 2:(lo + n) // 2, :] = _as_u32(_ln(y).astype(BF16))

        def out_copy(it, n):
            rows = pl.ds(start_row(it * NS), n * TB)
            return pltpu.make_async_copy(ob_ref.at[rows, :], o_hbm.at[rows, :], osem.at[it])

        w3h_ref[...] = _as_u32(_as_bf16(w3t_ref[0:64, :]).astype(F32).T.astype(BF16))

        def mm3(k, opens):
            lo, hi = fsplit[k], fsplit[k + 1]
            mid = hi - hi % 128
            u3 = _as_bf16(u3_ref[...])
            fs = []
            if opens:
                fs.append(jnp.dot(u3, _as_bf16(w3h_ref[...]), preferred_element_type=F32))
                lo += 128
            fs.append(lax.dot_general(u3, _as_bf16(w3t_ref[lo // 2:mid // 2, :]),
                                      NT, preferred_element_type=F32))
            f = _gelu(jnp.concatenate(fs, axis=1))
            if mid < hi:
                ft = _gelu(lax.dot_general(_as_bf16(w3t_ref[mid // 2:hi // 2, :]), u3,
                                           NT, preferred_element_type=F32))
                f = jnp.concatenate([f, ft.T], axis=1)
            return [f[kk * TC:(kk + 1) * TC].astype(BF16) for kk in range(NC)]

        def mm4(t, f, z, k):
            lo = k * TC
            gb = mod_ref[5, 0:1, :]
            h2 = jnp.dot(jnp.concatenate([fk[k] for fk in f], axis=1), _as_bf16(w4_ref[...]),
                         preferred_element_type=F32)
            ob_ref[pl.ds(start_row(t) + lo, TC), :] = (z + gb * h2).astype(ob_ref.dtype)

        def stage(t, nxt, opens):
            fs, fr = [], []
            for k in range(NC):
                fs.append(mm3(k, opens and k == 0))
                if nxt:
                    fr.append(front_a(t + 1, 2 * HALO + k * TC, 2 * HALO + (k + 1) * TC))
            if nxt:
                fr = [jnp.concatenate(parts, axis=0) for parts in zip(*fr)]
            for k in range(NC):
                z = z_ref[k * TC:(k + 1) * TC, :]
                if nxt and k == NC - 1:
                    front_b(*fr, k * TC, TC)
                mm4(t, fs, z, k)
                if nxt and k < NC - 1:
                    front_b(*fr, k * TC, TC)

        nb = S // TB
        ni = (nb - 1) // NS
        assert ni * NS == nb - 1
        fr = [front_a(0, lo, hi) for lo, hi in zip(FILL_A[:-1], FILL_A[1:])]
        fr = [jnp.concatenate(parts, axis=0) for parts in zip(*fr)]
        for lo, hi in zip(FILL_B[:-1], FILL_B[1:]):
            front_b(*fr, lo, hi - lo)

        def loop_b(it, carry):
            for u in range(NS):
                stage(it * NS + u, True, u == 0)
            out_copy(it, NS).start()
            return carry
        lax.fori_loop(0, ni, loop_b, 0)
        stage(nb - 1, False, True)
        out_copy(ni, 1).start()
        for it in range(ni):
            out_copy(it, NS).wait()
        out_copy(ni, 1).wait()

    @pl.when(pl.program_id(0) == 0)
    def _():
        _prologue()
        lax.fori_loop(1, NK, _keys, 0)
        _wait_pair_weights()
        lax.fori_loop(0, NP, _attention, 0)

    @pl.when(pl.program_id(0) == 1)
    def _():
        _epilogue()


@jax.jit
def pallas_adaLN_cond__compressed_kv_cla__mixer_s_mlp__prompt_kernel(
    A_x: jax.Array,
    A_c_kv: jax.Array,
    A_w_q: jax.Array,
    A_w_uk: jax.Array,
    A_w_uv: jax.Array,
    A_w_o: jax.Array,
    B_x: jax.Array,
    B_w1: jax.Array,
    B_w2: jax.Array,
    B_w3: jax.Array,
    B_w4: jax.Array,
    c: jax.Array,
    w_mod: jax.Array,
):
    B, S, M = A_x.shape
    assert B == 1 and A_c_kv.shape[1] == S
    Dc = A_c_kv.shape[2]
    H, D = A_w_q.shape[1], A_w_q.shape[2]
    NP = H // 2
    Fd = B_w3.shape[1]
    LC = TK // NL
    any_spec = pl.BlockSpec(memory_space=pl.ANY)

    out = pl.pallas_call(
        functools.partial(_kernel, S=S, M=M, D=D, NP=NP, Fd=Fd),
        grid=(2,),
        in_specs=[any_spec] * 12,
        out_specs=any_spec,
        out_shape=jax.ShapeDtypeStruct((S, M), A_x.dtype),
        scratch_shapes=[
            pltpu.VMEM((S + 3 * LC, M), BF16),
            pltpu.VMEM((S // 2, Dc), U32),
            pltpu.VMEM((NP, M, D), U32),
            pltpu.VMEM((NP, Dc, D), U32),
            pltpu.VMEM((NP, Dc, D), U32),
            pltpu.VMEM((NP, D, M), U32),
            pltpu.VMEM((M // 2, M), U32),
            pltpu.VMEM((M // 2, M), U32),
            pltpu.VMEM((Fd // 2, M), U32),
            pltpu.VMEM((Fd // 2, M), U32),
            pltpu.VMEM((6, M // 2, M), U32),
            pltpu.VMEM((NP * S // 2, 2 * D), U32),
            pltpu.VMEM((S + 4 * HALO, M), F32),
            pltpu.VMEM(((S + LC) // 2, M), U32),
            pltpu.VMEM((S, M), BF16),
            pltpu.VMEM((M // 2, 128), U32),
            pltpu.VMEM((M // 2, 2 * D), U32),
            pltpu.VMEM((Dc // 2, 2 * KP * D), U32),
            pltpu.VMEM((Dc // 2, 2 * D), U32),
            pltpu.VMEM((D, M), U32),
            pltpu.VMEM((S // 2, 2 * D), U32),
            pltpu.VMEM((M // 2, 128), U32),
            pltpu.VMEM((TB, M), F32),
            pltpu.VMEM((TB // 2, M), U32),
            pltpu.VMEM((6, 8, M), F32),
            pltpu.VMEM((3, 2 * HALO, M), F32),
            pltpu.VMEM((8, 128), U32),
            pltpu.VMEM((1, M), BF16),
            pltpu.SemaphoreType.DMA((12,)),
            pltpu.SemaphoreType.DMA((CC - 1 + S // CC // TK,)),
            pltpu.SemaphoreType.DMA((NP,)),
            pltpu.SemaphoreType.DMA((6,)),
            pltpu.SemaphoreType.DMA(((S // TB - 1) // NS + 1,)),
        ],
        compiler_params=pltpu.CompilerParams(
            dimension_semantics=("arbitrary",),
            vmem_limit_bytes=100 * 1024 * 1024,
            disable_bounds_checks=True,
            disable_semaphore_checks=True,
        ),
    )(
        A_x.reshape(S, M), A_c_kv.reshape(S, Dc),
        A_w_q, A_w_uk, A_w_uv,
        A_w_o.reshape(NP, 2 * D, M),
        B_w1, B_w2, B_w3.T, B_w4, c, w_mod,
    )
    return out.reshape(B, S, M)
```

```python
import functools
import math

import jax
import jax.numpy as jnp
from jax import lax
import jax.experimental.pallas as pl
import jax.experimental.pallas.tpu as pltpu

F32 = jnp.float32
BF16 = jnp.bfloat16
U32 = jnp.uint32
NT = (((1,), (1,)), ((), ()))
NEG = -1000000000.0
EPS = 1e-05
CC = 4
KP = 2
TK = 256
NL = 4
ZC, ZS = 3, 2
TQ = 128
LAG = 4
O_LAG = 6
T_SUB = 2
TB = 128
NS = 3
TC = 64
HALO = 8
FILL_A = (0, 96, 144)
FILL_B = (0, 64, 128)


def _ln(x):
    m = jnp.mean(x, axis=-1, keepdims=True)
    xc = x - m
    v = jnp.mean(xc * xc, axis=-1, keepdims=True)
    return xc * lax.rsqrt(v + EPS)


def _gelu(x):
    c = math.sqrt(2.0 / math.pi)
    hx = 0.5 * x
    return hx + hx * jnp.tanh(x * (c + (c * 0.044715) * (x * x)))


def _as_bf16(u):
    return pltpu.bitcast(u, BF16)


def _as_u32(b):
    return pltpu.bitcast(b, U32)


def _halves(u):
    return pltpu.bitcast(u << 16, F32), pltpu.bitcast(u & jnp.uint32(0xFFFF0000), F32)


def _split_pair(u):
    return _as_u32(jnp.concatenate(_halves(u), axis=1).astype(BF16))


def _attention_schedule(nq):
    order = list(range(nq - 1, -1, -1))
    units = [(i, hh, half) for i in order for half in (1, 0) for hh in (0, 1)]
    ops = [("q", order[0]), ("v", 0)]
    per = -(-(nq - 1) // LAG)
    for k in range(len(units) + LAG + O_LAG):
        n, sub = divmod(k, 4)
        if sub == 0 and 1 <= n < nq - 1:
            ops.append(("q", order[n + 1]))
        if 0 <= k - LAG < len(units):
            ops.append(("pv",) + units[k - LAG])
        if k < len(units):
            ops.append(("s",) + units[k])
        if k == 0:
            ops.append(("q", order[1]))
        if k < LAG:
            ops.extend(("v", i) for i in range(1 + k * per, min(nq, 1 + (k + 1) * per)))
        if sub == T_SUB and n % 2 == 0 and n + 1 < nq:
            ops.append(("t", order[n], order[n + 1]))
        ko = k - LAG - O_LAG
        if 0 <= ko < len(units) and ko % 2 == 1:
            ops.append(("o", units[ko][0], units[ko][2]))
    return ops


def _after(lhs, deps, zero):
    t = None
    for dep in deps:
        for r in range(0, dep.shape[0], 8):
            for c in range(0, dep.shape[1], 128):
                tile = dep[r:r + 8, c:c + 128]
                t = tile if t is None else t | tile
    head = lhs[0:8, 0:128] | (t & zero)
    if lhs.shape[1] > 128:
        head = jnp.concatenate([head, lhs[0:8, 128:]], axis=1)
    return jnp.concatenate([head, lhs[8:]], axis=0)


def _kernel(x_hbm, ckv_hbm, wq_hbm, wk_hbm, wv_hbm, wo_hbm,
            w1_hbm, w2_hbm, w3t_hbm, w4_hbm, c_hbm, wmod_hbm,
            o_hbm,
            x_ref, ckv_ref, wqr_ref, wkr_ref, wvr_ref, wo_ref,
            w1_ref, w2_ref, w3t_ref, w4_ref, wmod_ref, k_ref, acc_ref, h_ref, ob_ref,
            sc_ref, wqp_ref, wkp_ref, wvp_ref, wop_ref, v_ref, w3h_ref, z_ref, u3_ref,
            mod_ref, cr_ref, zero_ref, c_ref,
            ssem, csem, ksem, msem, osem,
            *, S, M, D, NP, Fd):
    NK = NP // KP
    nq = S // TQ
    HQ = TQ // 2
    qscale = (D ** -0.5) * math.log2(math.e)
    LR = S // NL
    NM = 6
    nk = S // TK
    LC = LR // nk
    assert NK - 1 >= NM and NK - NL >= 3

    c_copy = pltpu.make_async_copy(c_hbm, c_ref, ssem.at[0])
    CR = S // CC // 2
    HK = TK // 2

    def ckv_copy(lo, n, sem):
        rows = pl.ds(lo if isinstance(lo, int) else pl.multiple_of(lo, HK), n)
        return pltpu.make_async_copy(ckv_hbm.bitcast(U32).at[rows, :], ckv_ref.at[rows, :],
                                     csem.at[sem])

    def ckv_head(i):
        return ckv_copy(i * HK, HK, i)

    def ckv_chunk(i):
        return ckv_copy(i * CR, CR, CR // HK - 1 + i)

    x_copy = pltpu.make_async_copy(x_hbm, x_ref.at[pl.ds(HALO, S), :], ssem.at[2])
    rest = pl.ds(1, NP - 1)
    wo_copy = pltpu.make_async_copy(wo_hbm.bitcast(U32).at[rest], wo_ref.at[rest], ssem.at[3])
    pair0_copies = [
        pltpu.make_async_copy(wq_hbm.bitcast(U32).at[:, 0, :], wqr_ref.at[0], ssem.at[1]),
        pltpu.make_async_copy(wv_hbm.bitcast(U32).at[:, 0, :], wvr_ref.at[0], ssem.at[10]),
        pltpu.make_async_copy(wo_hbm.bitcast(U32).at[0], wop_ref, ssem.at[11]),
    ]
    late_copies = [
        pltpu.make_async_copy(w1_hbm.bitcast(U32), w1_ref, ssem.at[4]),
        pltpu.make_async_copy(w2_hbm.bitcast(U32), w2_ref, ssem.at[5]),
        pltpu.make_async_copy(w3t_hbm.bitcast(U32), w3t_ref, ssem.at[6]),
        pltpu.make_async_copy(w4_hbm.bitcast(U32), w4_ref, ssem.at[7]),
    ]

    def wk_copy(p):
        return pltpu.make_async_copy(wk_hbm.bitcast(U32).at[:, p, :], wkr_ref.at[p], ksem.at[p])

    def wmod_copy(g):
        off = g * M if isinstance(g, int) else pl.multiple_of(g * M, 128)
        return pltpu.make_async_copy(wmod_hbm.bitcast(U32).at[:, pl.ds(off, M)],
                                     wmod_ref.at[g], msem.at[g])

    def stage_weights(p):
        wqp_ref[...] = _split_pair(wqr_ref[p])
        wvp_ref[...] = _split_pair(wvr_ref[p])
        wop_ref[...] = wo_ref[p]

    def stage_wk(step, us=tuple(range(KP))):
        for u in us:
            wkp_ref[:, 2 * u * D:(2 * u + 2) * D] = _split_pair(wkr_ref[step * KP + u])

    def k_rows(p, lo, n):
        off = p * (S // 2) + lo
        return pl.ds(off if isinstance(off, int) else pl.multiple_of(off, 8), n)

    def proj_k(step, lo, lhs, u0=0, u1=KP, w=None):
        if w is None:
            w = _as_bf16(wkp_ref[:, 2 * u0 * D:2 * u1 * D])
        k = jnp.dot(_as_bf16(lhs), w, preferred_element_type=F32)
        for u in range(u0, u1):
            k_ref[k_rows(step * KP + u, lo, HK), :] = _as_u32(
                k[:, 2 * (u - u0) * D:2 * (u - u0 + 1) * D].astype(BF16))
        return k

    def _prologue():
        wk_copy(0).start()
        for i in range(CR // HK):
            ckv_head(i).start()
        c_copy.start()
        for p in range(1, KP):
            wk_copy(p).start()
        for i in range(1, CC):
            ckv_chunk(i).start()
        x_ref[0:HALO, :] = jnp.zeros((HALO, M), BF16)
        x_ref[S + HALO:S + HALO + 2 * LC, :] = jnp.zeros((2 * LC, M), BF16)
        for g in range(2):
            for p in range((g + 1) * KP, (g + 2) * KP):
                wk_copy(p).start()
            wmod_copy(g).start()
            if g == 0:
                for cp in pair0_copies[:2]:
                    cp.start()
        pair0_copies[2].start()

        def start_wk(p, carry):
            wk_copy(p).start()
            return carry
        lax.fori_loop(3 * KP, NP, start_wk, 0)
        wmod_copy(2).start()
        x_copy.start()
        for g in range(3, NM):
            wmod_copy(g).start()

        def start_qv(p, carry):
            pltpu.make_async_copy(wq_hbm.bitcast(U32).at[:, p, :], wqr_ref.at[p], ssem.at[8]).start()
            pltpu.make_async_copy(wv_hbm.bitcast(U32).at[:, p, :], wvr_ref.at[p], ssem.at[9]).start()
            return carry
        lax.fori_loop(1, NP, start_qv, 0)
        wo_copy.start()
        for cp in late_copies:
            cp.start()
        mod_ref[0:2] = jnp.zeros((2, 8, M), F32)
        zero_ref[...] = jnp.zeros(zero_ref.shape, U32)
        wk_copy(0).wait()
        stage_wk(0, (0,))

        def head_keys(i, carry):
            ckv_head(i).wait()
            lo = pl.multiple_of(i * HK, HK)
            proj_k(0, lo, ckv_ref[pl.ds(lo, HK), :], 0, 1)
            return carry
        lax.fori_loop(0, CR // HK, head_keys, 0)
        for p in range(1, KP):
            wk_copy(p).wait()
        c_copy.wait()
        c = c_ref[...].astype(F32)
        sc = jnp.broadcast_to(c * jax.nn.sigmoid(c), (128, M))
        sc_ref[...] = _as_u32(sc.T.astype(BF16))
        stage_wk(0, tuple(range(1, KP)))
        for i in range(CR // HK):
            proj_k(0, i * HK, ckv_ref[i * HK:(i + 1) * HK, :], 1, KP)

        def first_keys(i, carry):
            ckv_chunk(i).wait()
            for ii in range(CR // HK):
                lo = pl.multiple_of(i * CR + ii * HK, HK)
                proj_k(0, lo, ckv_ref[pl.ds(lo, HK), :])
            return carry
        lax.fori_loop(1, CC, first_keys, 0)
        for cp in pair0_copies[:2]:
            cp.wait()

    def _keys(step, carry):
        for u in range(KP):
            wk_copy(step * KP + u).wait()

        @pl.when(step <= NM)
        def _():
            wmod_copy(step - 1).wait()

        @pl.when(step == NK - NL)
        def _():
            x_copy.wait()

        wk = jnp.concatenate([half for u in range(KP) for half in _halves(wkr_ref[step * KP + u])],
                             axis=1).astype(BF16)
        g = jnp.minimum(step - 1, NM - 1)
        live = step >= NK - NL
        lblk = step - (NK - NL)
        sa = mod_ref[0, 0:1, :]
        ca1 = 1.0 + mod_ref[1, 0:1, :]
        zero = zero_ref[...]
        mc = M // 2 // nk
        ar = -(-(S + 2 * HALO) // ((NK - 1) * nk * 8)) * 8
        deps, part = [], None
        for i in range(nk):
            lhs = ckv_ref[i * HK:(i + 1) * HK, :]
            if deps:
                lhs = _after(lhs, deps, zero)
            k = proj_k(step, i * HK, lhs, w=wk)
            r = pl.multiple_of(jnp.where(live, lblk * LR + i * LC, S + LC), LC)
            rh = pl.multiple_of(jnp.where(live, (lblk * LR + i * LC) // 2, S // 2), 8)
            x = x_ref.at[pl.ds(r, LC + HALO), :][HALO:, :].astype(F32)
            h = _ln(x) * ca1 + sa
            h_ref[pl.ds(rh, LC // 2), :] = _as_u32(h.astype(BF16))
            we, wo = _halves(wmod_ref[g, i * mc:(i + 1) * mc, :])
            se, so = _halves(sc_ref[i * mc:(i + 1) * mc, :])
            prod = we * jnp.tile(se, (1, M // 128)) + wo * jnp.tile(so, (1, M // 128))
            for rr in range(0, mc, 8):
                part = prod[rr:rr + 8] if part is None else part + prod[rr:rr + 8]
            deps = [pltpu.bitcast(h, U32), pltpu.bitcast(part, U32)]
            zt = pltpu.bitcast(pltpu.bitcast(k[0:8, ZC * D:(ZC + 1) * D], U32) & zero, F32)
            ra = jnp.minimum(((step - 1) * nk + i) * ar, S + 2 * HALO - ar)
            acc_ref[pl.ds(pl.multiple_of(ra, 8), ar), :] = jnp.tile(zt, (ar // 8, M // 128))
            zu = pltpu.bitcast(k[0:8, ZS * D:(ZS + 1) * D], U32) & zero
            for raw_ref, dst_ref in ((wqr_ref, wqp_ref), (wvr_ref, wvp_ref)):
                n = raw_ref.shape[1] // nk
                raw = raw_ref[0, i * n:(i + 1) * n, :] | jnp.tile(zu, (n // 8, 1))
                dst_ref[i * n // 2:(i + 1) * n // 2, :] = _split_pair(raw)
        mod_ref[g] = jnp.broadcast_to(jnp.sum(part, axis=0, keepdims=True), (8, M))
        return carry

    def _wait_pair_weights():
        pltpu.make_async_copy(wqr_ref.at[rest], wqr_ref.at[rest], ssem.at[8]).wait()
        pltpu.make_async_copy(wvr_ref.at[rest], wvr_ref.at[rest], ssem.at[9]).wait()
        wo_copy.wait()
        pair0_copies[2].wait()

    def _attention(j, carry):
        HH = HQ // 2
        row = lax.broadcasted_iota(jnp.int32, (HQ, TQ), 0)
        col = lax.broadcasted_iota(jnp.int32, (HQ, TQ), 1)
        diag = col <= row + HQ
        first = [col < HQ, col >= HQ]
        first0 = [col <= row, jnp.logical_and(col >= HQ, diag)]

        def proj_v(i):
            rows = slice(i * HQ, (i + 1) * HQ)
            v = jnp.dot(_as_bf16(ckv_ref[rows, :]), _as_bf16(wvp_ref[...]), preferred_element_type=F32)
            v_ref[rows, :] = _as_u32(v.astype(BF16))

        def proj_q(i):
            rows = slice(i * HQ, (i + 1) * HQ)
            q = jnp.dot(_as_bf16(h_ref[rows, :]), _as_bf16(wqp_ref[...]), preferred_element_type=F32)
            q = q * qscale
            return [[q[half * HQ:(half + 1) * HQ, hh * D:(hh + 1) * D].astype(BF16)
                     for half in range(2)] for hh in range(2)]

        def masked_scores(qh, k):
            s = lax.dot_general(qh, k, NT, preferred_element_type=F32)
            n = s.shape[1] - TQ
            sd = jnp.where(diag, s[:, n:], NEG)
            return jnp.concatenate([s[:, :n], sd], axis=1) if n else sd

        def scores(q, hh, half, i):
            cols = slice(hh * D, (hh + 1) * D)
            if half == 1:
                return masked_scores(q[hh][1], _as_bf16(k_ref[k_rows(j, 0, (i + 1) * HQ), cols]))
            if i > 0:
                return masked_scores(q[hh][0], _as_bf16(k_ref[k_rows(j, HH, i * HQ), cols]))
            return None

        def first_scores(q1, q2):
            st = [lax.dot_general(_as_bf16(k_ref[k_rows(j, 0, HH), hh * D:(hh + 1) * D]),
                                  jnp.concatenate([q1[hh][0], q2[hh][0]], axis=0),
                                  NT, preferred_element_type=F32) for hh in range(2)]
            t = jnp.concatenate(st, axis=0).T
            return t[0:HQ], t[HQ:TQ]

        def softmax_pv(s, t0, hh, half, i):
            cols = slice(hh * D, (hh + 1) * D)
            if half == 1:
                v = v_ref[0:(i + 1) * HQ, cols]
            else:
                s0 = jnp.where(first[hh] if i > 0 else first0[hh], t0[i], NEG)
                s = s0 if s is None else jnp.concatenate([s, s0], axis=1)
                if hh == 0:
                    v = v_ref[0:HQ, cols]
                else:
                    v = jnp.concatenate([v_ref[HH:HQ, cols], v_ref[0:HH, cols]], axis=0)
                if i > 0:
                    v = jnp.concatenate([v_ref[HH:i * HQ + HH, cols], v], axis=0)
            m = jnp.max(s, axis=1, keepdims=True)
            p = jnp.exp2(s - m).astype(BF16)
            l = jnp.sum(p.astype(F32), axis=1, keepdims=True)
            o = jnp.dot(p, _as_bf16(v), preferred_element_type=F32)
            return o * pl.reciprocal(l, approx=False, full_range=False)

        def oproj(ctx, r, n):
            rows = slice(HALO + r, HALO + r + n)
            acc_ref[rows, :] += jnp.dot(ctx.astype(BF16), _as_bf16(wop_ref[...]),
                                        preferred_element_type=F32)

        q, s, t0, ctx = {}, {}, {}, {}
        for op in _attention_schedule(nq):
            kind, i = op[0], op[1]
            if kind == "q":
                q[i] = proj_q(i)
            elif kind == "v":
                proj_v(i)
            elif kind == "s":
                s[op[1:]] = scores(q[i], op[2], op[3], i)
            elif kind == "t":
                t0[i], t0[op[2]] = first_scores(q[i], q[op[2]])
            elif kind == "pv":
                ctx[op[1:]] = softmax_pv(s.pop(op[1:]), t0, op[2], op[3], i)
            else:
                oproj(jnp.concatenate([ctx.pop((i, hh, op[2])) for hh in range(2)], axis=1),
                      i * TQ + op[2] * HQ, HQ)

        stage_weights(jnp.minimum(j + 1, NP - 1))
        return carry

    def _epilogue():
        for cp in late_copies:
            cp.wait()

        G = M // 4
        NC = TB // TC
        TH = TB + 2 * HALO
        ntile = (Fd + 127) // 128
        fsplit = [min(Fd, ((k * ntile + NC - 1) // NC) * 128) for k in range(NC + 1)]

        def start_row(t):
            return t * TB if isinstance(t, int) else pl.multiple_of(t * TB, TB)

        def front_a(t, lo, hi):
            r = start_row(t)
            ga = mod_ref[2, 0:1, :]
            sb = mod_ref[3, 0:1, :]
            cb1 = 1.0 + mod_ref[4, 0:1, :]
            x1 = (x_ref.at[pl.ds(r, TH), :][lo:hi, :].astype(F32)
                  + ga * acc_ref.at[pl.ds(r, TH), :][lo:hi, :])
            h = _ln(x1) * cb1 + sb
            tt = _gelu(jnp.dot(_ln(h).astype(BF16), _as_bf16(w1_ref[...]),
                               preferred_element_type=F32))
            if lo == 0:
                tt = jnp.concatenate([jnp.zeros((HALO, M), F32), tt[HALO:]], axis=0)
            if lo == 2 * HALO:
                x1, h, tt = [jnp.concatenate([cr_ref[a], v], axis=0)
                             for a, v in enumerate((x1, h, tt))]
            if hi == TH:
                n = hi - lo - HALO
                tt = jnp.concatenate([tt[:n], jnp.where(r + TB < S, tt[n:], 0.0)], axis=0)
                for a, v in enumerate((x1, h, tt)):
                    cr_ref[a] = v[n - HALO:]
            return x1, h, tt

        def front_b(x1, h, tt, lo, n):
            gb = mod_ref[5, 0:1, :]
            lane = lax.broadcasted_iota(jnp.int32, (n, 128), 1)
            cols = []
            shifts = (-1, 1, -2, 2)
            for cblk in range(M // 128):
                c0, c1 = cblk * 128, (cblk + 1) * 128
                ga_, gb_ = c0 // G, (c1 - 1) // G
                a = tt[HALO + lo + shifts[ga_]:HALO + lo + shifts[ga_] + n, c0:c1]
                if gb_ != ga_:
                    b = tt[HALO + lo + shifts[gb_]:HALO + lo + shifts[gb_] + n, c0:c1]
                    a = jnp.where(lane < gb_ * G - c0, a, b)
                cols.append(a)
            sh = jnp.concatenate(cols, axis=1).astype(BF16)
            y = h[HALO + lo:HALO + lo + n] + jnp.dot(sh, _as_bf16(w2_ref[...]),
                                                     preferred_element_type=F32)
            z_ref[lo:lo + n, :] = x1[HALO + lo:HALO + lo + n] + gb * y
            u3_ref[lo // 2:(lo + n) // 2, :] = _as_u32(_ln(y).astype(BF16))

        def out_copy(it, n):
            rows = pl.ds(start_row(it * NS), n * TB)
            return pltpu.make_async_copy(ob_ref.at[rows, :], o_hbm.at[rows, :], osem.at[it])

        w3h_ref[...] = _as_u32(_as_bf16(w3t_ref[0:64, :]).astype(F32).T.astype(BF16))

        def mm3(k, opens):
            lo, hi = fsplit[k], fsplit[k + 1]
            mid = hi - hi % 128
            u3 = _as_bf16(u3_ref[...])
            fs = []
            if opens:
                fs.append(jnp.dot(u3, _as_bf16(w3h_ref[...]), preferred_element_type=F32))
                lo += 128
            fs.append(lax.dot_general(u3, _as_bf16(w3t_ref[lo // 2:mid // 2, :]),
                                      NT, preferred_element_type=F32))
            f = _gelu(jnp.concatenate(fs, axis=1))
            if mid < hi:
                ft = _gelu(lax.dot_general(_as_bf16(w3t_ref[mid // 2:hi // 2, :]), u3,
                                           NT, preferred_element_type=F32))
                f = jnp.concatenate([f, ft.T], axis=1)
            return [f[kk * TC:(kk + 1) * TC].astype(BF16) for kk in range(NC)]

        def mm4(t, f, z, k):
            lo = k * TC
            gb = mod_ref[5, 0:1, :]
            h2 = jnp.dot(jnp.concatenate([fk[k] for fk in f], axis=1), _as_bf16(w4_ref[...]),
                         preferred_element_type=F32)
            ob_ref[pl.ds(start_row(t) + lo, TC), :] = (z + gb * h2).astype(ob_ref.dtype)

        def stage(t, nxt, opens):
            fs, fr = [], []
            for k in range(NC):
                fs.append(mm3(k, opens and k == 0))
                if nxt:
                    fr.append(front_a(t + 1, 2 * HALO + k * TC, 2 * HALO + (k + 1) * TC))
            if nxt:
                fr = [jnp.concatenate(parts, axis=0) for parts in zip(*fr)]
            for k in range(NC):
                z = z_ref[k * TC:(k + 1) * TC, :]
                if nxt and k == NC - 1:
                    front_b(*fr, k * TC, TC)
                mm4(t, fs, z, k)
                if nxt and k < NC - 1:
                    front_b(*fr, k * TC, TC)

        nb = S // TB
        ni = (nb - 1) // NS
        assert ni * NS == nb - 1
        fr = [front_a(0, lo, hi) for lo, hi in zip(FILL_A[:-1], FILL_A[1:])]
        fr = [jnp.concatenate(parts, axis=0) for parts in zip(*fr)]
        for lo, hi in zip(FILL_B[:-1], FILL_B[1:]):
            front_b(*fr, lo, hi - lo)

        def loop_b(it, carry):
            for u in range(NS):
                stage(it * NS + u, True, u == 0)
            out_copy(it, NS).start()
            return carry
        lax.fori_loop(0, ni, loop_b, 0)
        stage(nb - 1, False, True)
        out_copy(ni, 1).start()
        for it in range(ni):
            out_copy(it, NS).wait()
        out_copy(ni, 1).wait()

    @pl.when(pl.program_id(0) == 0)
    def _():
        _prologue()
        lax.fori_loop(1, NK, _keys, 0)
        _wait_pair_weights()
        lax.fori_loop(0, NP, _attention, 0)

    @pl.when(pl.program_id(0) == 1)
    def _():
        _epilogue()


@jax.jit
def pallas_adaLN_cond__compressed_kv_cla__mixer_s_mlp__prompt_kernel(
    A_x: jax.Array,
    A_c_kv: jax.Array,
    A_w_q: jax.Array,
    A_w_uk: jax.Array,
    A_w_uv: jax.Array,
    A_w_o: jax.Array,
    B_x: jax.Array,
    B_w1: jax.Array,
    B_w2: jax.Array,
    B_w3: jax.Array,
    B_w4: jax.Array,
    c: jax.Array,
    w_mod: jax.Array,
):
    B, S, M = A_x.shape
    assert B == 1 and A_c_kv.shape[1] == S
    Dc = A_c_kv.shape[2]
    H, D = A_w_q.shape[1], A_w_q.shape[2]
    NP = H // 2
    Fd = B_w3.shape[1]
    LC = TK // NL
    any_spec = pl.BlockSpec(memory_space=pl.ANY)

    out = pl.pallas_call(
        functools.partial(_kernel, S=S, M=M, D=D, NP=NP, Fd=Fd),
        grid=(2,),
        in_specs=[any_spec] * 12,
        out_specs=any_spec,
        out_shape=jax.ShapeDtypeStruct((S, M), A_x.dtype),
        scratch_shapes=[
            pltpu.VMEM((S + 3 * LC, M), BF16),
            pltpu.VMEM((S // 2, Dc), U32),
            pltpu.VMEM((NP, M, D), U32),
            pltpu.VMEM((NP, Dc, D), U32),
            pltpu.VMEM((NP, Dc, D), U32),
            pltpu.VMEM((NP, D, M), U32),
            pltpu.VMEM((M // 2, M), U32),
            pltpu.VMEM((M // 2, M), U32),
            pltpu.VMEM((Fd // 2, M), U32),
            pltpu.VMEM((Fd // 2, M), U32),
            pltpu.VMEM((6, M // 2, M), U32),
            pltpu.VMEM((NP * S // 2, 2 * D), U32),
            pltpu.VMEM((S + 4 * HALO, M), F32),
            pltpu.VMEM(((S + LC) // 2, M), U32),
            pltpu.VMEM((S, M), BF16),
            pltpu.VMEM((M // 2, 128), U32),
            pltpu.VMEM((M // 2, 2 * D), U32),
            pltpu.VMEM((Dc // 2, 2 * KP * D), U32),
            pltpu.VMEM((Dc // 2, 2 * D), U32),
            pltpu.VMEM((D, M), U32),
            pltpu.VMEM((S // 2, 2 * D), U32),
            pltpu.VMEM((M // 2, 128), U32),
            pltpu.VMEM((TB, M), F32),
            pltpu.VMEM((TB // 2, M), U32),
            pltpu.VMEM((6, 8, M), F32),
            pltpu.VMEM((3, 2 * HALO, M), F32),
            pltpu.VMEM((8, 128), U32),
            pltpu.VMEM((1, M), BF16),
            pltpu.SemaphoreType.DMA((12,)),
            pltpu.SemaphoreType.DMA((CC - 1 + S // CC // TK,)),
            pltpu.SemaphoreType.DMA((NP,)),
            pltpu.SemaphoreType.DMA((6,)),
            pltpu.SemaphoreType.DMA(((S // TB - 1) // NS + 1,)),
        ],
        compiler_params=pltpu.CompilerParams(
            dimension_semantics=("arbitrary",),
            vmem_limit_bytes=100 * 1024 * 1024,
            disable_bounds_checks=True,
            disable_semaphore_checks=True,
        ),
    )(
        A_x.reshape(S, M), A_c_kv.reshape(S, Dc),
        A_w_q, A_w_uk, A_w_uv,
        A_w_o.reshape(NP, 2 * D, M),
        B_w1, B_w2, B_w3.T, B_w4, c, w_mod,
    )
    return out.reshape(B, S, M)
```

```python
import functools
import math

import jax
import jax.numpy as jnp
from jax import lax
import jax.experimental.pallas as pl
import jax.experimental.pallas.tpu as pltpu

F32 = jnp.float32
BF16 = jnp.bfloat16
U32 = jnp.uint32
NT = (((1,), (1,)), ((), ()))
NEG = -1000000000.0
EPS = 1e-05
CC = 4
KP = 2
TK = 256
NL = 4
ZC, ZS = 3, 2
TQ = 128
LAG = 4
O_LAG = 6
T_SUB = 2
TB = 128
NS = 3
TC = 64
HALO = 8
F_CUTS = (0, 6)
FILL_A = (0, 96, 144)
FILL_B = (0, 64, 128)


def _ln(x):
    m = jnp.mean(x, axis=-1, keepdims=True)
    xc = x - m
    v = jnp.mean(xc * xc, axis=-1, keepdims=True)
    return xc * lax.rsqrt(v + EPS)


def _gelu(x):
    c = math.sqrt(2.0 / math.pi)
    hx = 0.5 * x
    return hx + hx * jnp.tanh(x * (c + (c * 0.044715) * (x * x)))


def _as_bf16(u):
    return pltpu.bitcast(u, BF16)


def _as_u32(b):
    return pltpu.bitcast(b, U32)


def _halves(u):
    return pltpu.bitcast(u << 16, F32), pltpu.bitcast(u & jnp.uint32(0xFFFF0000), F32)


def _split_pair(u):
    return _as_u32(jnp.concatenate(_halves(u), axis=1).astype(BF16))


def _attention_schedule(nq):
    order = list(range(nq - 1, -1, -1))
    units = [(i, hh, half) for i in order for half in (1, 0) for hh in (0, 1)]
    ops = [("q", order[0]), ("v", 0)]
    per = -(-(nq - 1) // LAG)
    for k in range(len(units) + LAG + O_LAG):
        n, sub = divmod(k, 4)
        if sub == 0 and 1 <= n < nq - 1:
            ops.append(("q", order[n + 1]))
        if 0 <= k - LAG < len(units):
            ops.append(("pv",) + units[k - LAG])
        if k < len(units):
            ops.append(("s",) + units[k])
        if k == 0:
            ops.append(("q", order[1]))
        if k < LAG:
            ops.extend(("v", i) for i in range(1 + k * per, min(nq, 1 + (k + 1) * per)))
        if sub == T_SUB and n % 2 == 0 and n + 1 < nq:
            ops.append(("t", order[n], order[n + 1]))
        ko = k - LAG - O_LAG
        if 0 <= ko < len(units) and ko % 2 == 1:
            ops.append(("o", units[ko][0], units[ko][2]))
    return ops


def _after(lhs, deps, zero):
    t = None
    for dep in deps:
        for r in range(0, dep.shape[0], 8):
            for c in range(0, dep.shape[1], 128):
                tile = dep[r:r + 8, c:c + 128]
                t = tile if t is None else t | tile
    head = lhs[0:8, 0:128] | (t & zero)
    if lhs.shape[1] > 128:
        head = jnp.concatenate([head, lhs[0:8, 128:]], axis=1)
    return jnp.concatenate([head, lhs[8:]], axis=0)


def _kernel(x_hbm, ckv_hbm, wq_hbm, wk_hbm, wv_hbm, wo_hbm,
            w1_hbm, w2_hbm, w3t_hbm, w4_hbm, c_hbm, wmod_hbm,
            o_hbm,
            x_ref, ckv_ref, wqr_ref, wkr_ref, wvr_ref, wo_ref,
            w1_ref, w2_ref, w3t_ref, w4_ref, wmod_ref, k_ref, acc_ref, h_ref, ob_ref,
            sc_ref, wqp_ref, wkp_ref, wvp_ref, wop_ref, v_ref, w3h_ref, z_ref, u3_ref,
            mod_ref, cr_ref, zero_ref, c_ref,
            ssem, csem, ksem, msem, osem,
            *, S, M, D, NP, Fd):
    NK = NP // KP
    nq = S // TQ
    HQ = TQ // 2
    qscale = (D ** -0.5) * math.log2(math.e)
    LR = S // NL
    NM = 6
    nk = S // TK
    LC = LR // nk
    assert NK - 1 >= NM and NK - NL >= 3

    c_copy = pltpu.make_async_copy(c_hbm, c_ref, ssem.at[0])
    CR = S // CC // 2
    HK = TK // 2

    def ckv_copy(lo, n, sem):
        rows = pl.ds(lo if isinstance(lo, int) else pl.multiple_of(lo, HK), n)
        return pltpu.make_async_copy(ckv_hbm.bitcast(U32).at[rows, :], ckv_ref.at[rows, :],
                                     csem.at[sem])

    def ckv_head(i):
        return ckv_copy(i * HK, HK, i)

    def ckv_chunk(i):
        return ckv_copy(i * CR, CR, CR // HK - 1 + i)

    x_copy = pltpu.make_async_copy(x_hbm, x_ref.at[pl.ds(HALO, S), :], ssem.at[2])
    rest = pl.ds(1, NP - 1)
    wo_copy = pltpu.make_async_copy(wo_hbm.bitcast(U32).at[rest], wo_ref.at[rest], ssem.at[3])
    pair0_copies = [
        pltpu.make_async_copy(wq_hbm.bitcast(U32).at[:, 0, :], wqr_ref.at[0], ssem.at[1]),
        pltpu.make_async_copy(wv_hbm.bitcast(U32).at[:, 0, :], wvr_ref.at[0], ssem.at[10]),
        pltpu.make_async_copy(wo_hbm.bitcast(U32).at[0], wop_ref, ssem.at[11]),
    ]
    late_copies = [
        pltpu.make_async_copy(w1_hbm.bitcast(U32), w1_ref, ssem.at[4]),
        pltpu.make_async_copy(w2_hbm.bitcast(U32), w2_ref, ssem.at[5]),
        pltpu.make_async_copy(w3t_hbm.bitcast(U32), w3t_ref, ssem.at[6]),
        pltpu.make_async_copy(w4_hbm.bitcast(U32), w4_ref, ssem.at[7]),
    ]

    def wk_copy(p):
        return pltpu.make_async_copy(wk_hbm.bitcast(U32).at[:, p, :], wkr_ref.at[p], ksem.at[p])

    def wmod_copy(g):
        off = g * M if isinstance(g, int) else pl.multiple_of(g * M, 128)
        return pltpu.make_async_copy(wmod_hbm.bitcast(U32).at[:, pl.ds(off, M)],
                                     wmod_ref.at[g], msem.at[g])

    def stage_weights(p):
        wqp_ref[...] = _split_pair(wqr_ref[p])
        wvp_ref[...] = _split_pair(wvr_ref[p])
        wop_ref[...] = wo_ref[p]

    def stage_wk(step, us=tuple(range(KP))):
        for u in us:
            wkp_ref[:, 2 * u * D:(2 * u + 2) * D] = _split_pair(wkr_ref[step * KP + u])

    def k_rows(p, lo, n):
        off = p * (S // 2) + lo
        return pl.ds(off if isinstance(off, int) else pl.multiple_of(off, 8), n)

    def proj_k(step, lo, lhs, u0=0, u1=KP, w=None):
        if w is None:
            w = _as_bf16(wkp_ref[:, 2 * u0 * D:2 * u1 * D])
        k = jnp.dot(_as_bf16(lhs), w, preferred_element_type=F32)
        for u in range(u0, u1):
            k_ref[k_rows(step * KP + u, lo, HK), :] = _as_u32(
                k[:, 2 * (u - u0) * D:2 * (u - u0 + 1) * D].astype(BF16))
        return k

    def _prologue():
        wk_copy(0).start()
        for i in range(CR // HK):
            ckv_head(i).start()
        c_copy.start()
        for p in range(1, KP):
            wk_copy(p).start()
        for i in range(1, CC):
            ckv_chunk(i).start()
        x_ref[0:HALO, :] = jnp.zeros((HALO, M), BF16)
        x_ref[S + HALO:S + HALO + 2 * LC, :] = jnp.zeros((2 * LC, M), BF16)
        for g in range(2):
            for p in range((g + 1) * KP, (g + 2) * KP):
                wk_copy(p).start()
            wmod_copy(g).start()
            if g == 0:
                for cp in pair0_copies[:2]:
                    cp.start()
        pair0_copies[2].start()

        def start_wk(p, carry):
            wk_copy(p).start()
            return carry
        lax.fori_loop(3 * KP, NP, start_wk, 0)
        wmod_copy(2).start()
        x_copy.start()
        for g in range(3, NM):
            wmod_copy(g).start()

        def start_qv(p, carry):
            pltpu.make_async_copy(wq_hbm.bitcast(U32).at[:, p, :], wqr_ref.at[p], ssem.at[8]).start()
            pltpu.make_async_copy(wv_hbm.bitcast(U32).at[:, p, :], wvr_ref.at[p], ssem.at[9]).start()
            return carry
        lax.fori_loop(1, NP, start_qv, 0)
        wo_copy.start()
        for cp in late_copies:
            cp.start()
        mod_ref[0:2] = jnp.zeros((2, 8, M), F32)
        zero_ref[...] = jnp.zeros(zero_ref.shape, U32)
        wk_copy(0).wait()
        stage_wk(0, (0,))

        def head_keys(i, carry):
            ckv_head(i).wait()
            lo = pl.multiple_of(i * HK, HK)
            proj_k(0, lo, ckv_ref[pl.ds(lo, HK), :], 0, 1)
            return carry
        lax.fori_loop(0, CR // HK, head_keys, 0)
        for p in range(1, KP):
            wk_copy(p).wait()
        c_copy.wait()
        c = c_ref[...].astype(F32)
        sc = jnp.broadcast_to(c * jax.nn.sigmoid(c), (128, M))
        sc_ref[...] = _as_u32(sc.T.astype(BF16))
        stage_wk(0, tuple(range(1, KP)))
        for i in range(CR // HK):
            proj_k(0, i * HK, ckv_ref[i * HK:(i + 1) * HK, :], 1, KP)

        def first_keys(i, carry):
            ckv_chunk(i).wait()
            for ii in range(CR // HK):
                lo = pl.multiple_of(i * CR + ii * HK, HK)
                proj_k(0, lo, ckv_ref[pl.ds(lo, HK), :])
            return carry
        lax.fori_loop(1, CC, first_keys, 0)
        for cp in pair0_copies[:2]:
            cp.wait()

    def _keys(step, carry):
        for u in range(KP):
            wk_copy(step * KP + u).wait()

        @pl.when(step <= NM)
        def _():
            wmod_copy(step - 1).wait()

        @pl.when(step == NK - NL)
        def _():
            x_copy.wait()

        wk = jnp.concatenate([half for u in range(KP) for half in _halves(wkr_ref[step * KP + u])],
                             axis=1).astype(BF16)
        g = jnp.minimum(step - 1, NM - 1)
        live = step >= NK - NL
        lblk = step - (NK - NL)
        sa = mod_ref[0, 0:1, :]
        ca1 = 1.0 + mod_ref[1, 0:1, :]
        zero = zero_ref[...]
        mc = M // 2 // nk
        ar = -(-(S + 2 * HALO) // ((NK - 1) * nk * 8)) * 8
        deps, part = [], None
        for i in range(nk):
            lhs = ckv_ref[i * HK:(i + 1) * HK, :]
            if deps:
                lhs = _after(lhs, deps, zero)
            k = proj_k(step, i * HK, lhs, w=wk)
            r = pl.multiple_of(jnp.where(live, lblk * LR + i * LC, S + LC), LC)
            rh = pl.multiple_of(jnp.where(live, (lblk * LR + i * LC) // 2, S // 2), 8)
            x = x_ref.at[pl.ds(r, LC + HALO), :][HALO:, :].astype(F32)
            h = _ln(x) * ca1 + sa
            h_ref[pl.ds(rh, LC // 2), :] = _as_u32(h.astype(BF16))
            we, wo = _halves(wmod_ref[g, i * mc:(i + 1) * mc, :])
            se, so = _halves(sc_ref[i * mc:(i + 1) * mc, :])
            prod = we * jnp.tile(se, (1, M // 128)) + wo * jnp.tile(so, (1, M // 128))
            for rr in range(0, mc, 8):
                part = prod[rr:rr + 8] if part is None else part + prod[rr:rr + 8]
            deps = [pltpu.bitcast(h, U32), pltpu.bitcast(part, U32)]
            zt = pltpu.bitcast(pltpu.bitcast(k[0:8, ZC * D:(ZC + 1) * D], U32) & zero, F32)
            ra = jnp.minimum(((step - 1) * nk + i) * ar, S + 2 * HALO - ar)
            acc_ref[pl.ds(pl.multiple_of(ra, 8), ar), :] = jnp.tile(zt, (ar // 8, M // 128))
            zu = pltpu.bitcast(k[0:8, ZS * D:(ZS + 1) * D], U32) & zero
            for raw_ref, dst_ref in ((wqr_ref, wqp_ref), (wvr_ref, wvp_ref)):
                n = raw_ref.shape[1] // nk
                raw = raw_ref[0, i * n:(i + 1) * n, :] | jnp.tile(zu, (n // 8, 1))
                dst_ref[i * n // 2:(i + 1) * n // 2, :] = _split_pair(raw)
        mod_ref[g] = jnp.broadcast_to(jnp.sum(part, axis=0, keepdims=True), (8, M))
        return carry

    def _wait_pair_weights():
        pltpu.make_async_copy(wqr_ref.at[rest], wqr_ref.at[rest], ssem.at[8]).wait()
        pltpu.make_async_copy(wvr_ref.at[rest], wvr_ref.at[rest], ssem.at[9]).wait()
        wo_copy.wait()
        pair0_copies[2].wait()

    def _attention(j, carry):
        HH = HQ // 2
        row = lax.broadcasted_iota(jnp.int32, (HQ, TQ), 0)
        col = lax.broadcasted_iota(jnp.int32, (HQ, TQ), 1)
        diag = col <= row + HQ
        first = [col < HQ, col >= HQ]
        first0 = [col <= row, jnp.logical_and(col >= HQ, diag)]

        def proj_v(i):
            rows = slice(i * HQ, (i + 1) * HQ)
            v = jnp.dot(_as_bf16(ckv_ref[rows, :]), _as_bf16(wvp_ref[...]), preferred_element_type=F32)
            v_ref[rows, :] = _as_u32(v.astype(BF16))

        def proj_q(i):
            rows = slice(i * HQ, (i + 1) * HQ)
            q = jnp.dot(_as_bf16(h_ref[rows, :]), _as_bf16(wqp_ref[...]), preferred_element_type=F32)
            q = q * qscale
            return [[q[half * HQ:(half + 1) * HQ, hh * D:(hh + 1) * D].astype(BF16)
                     for half in range(2)] for hh in range(2)]

        def masked_scores(qh, k):
            s = lax.dot_general(qh, k, NT, preferred_element_type=F32)
            n = s.shape[1] - TQ
            sd = jnp.where(diag, s[:, n:], NEG)
            return jnp.concatenate([s[:, :n], sd], axis=1) if n else sd

        def scores(q, hh, half, i):
            cols = slice(hh * D, (hh + 1) * D)
            if half == 1:
                return masked_scores(q[hh][1], _as_bf16(k_ref[k_rows(j, 0, (i + 1) * HQ), cols]))
            if i > 0:
                return masked_scores(q[hh][0], _as_bf16(k_ref[k_rows(j, HH, i * HQ), cols]))
            return None

        def first_scores(q1, q2):
            st = [lax.dot_general(_as_bf16(k_ref[k_rows(j, 0, HH), hh * D:(hh + 1) * D]),
                                  jnp.concatenate([q1[hh][0], q2[hh][0]], axis=0),
                                  NT, preferred_element_type=F32) for hh in range(2)]
            t = jnp.concatenate(st, axis=0).T
            return t[0:HQ], t[HQ:TQ]

        def softmax_pv(s, t0, hh, half, i):
            cols = slice(hh * D, (hh + 1) * D)
            if half == 1:
                v = v_ref[0:(i + 1) * HQ, cols]
            else:
                s0 = jnp.where(first[hh] if i > 0 else first0[hh], t0[i], NEG)
                s = s0 if s is None else jnp.concatenate([s, s0], axis=1)
                if hh == 0:
                    v = v_ref[0:HQ, cols]
                else:
                    v = jnp.concatenate([v_ref[HH:HQ, cols], v_ref[0:HH, cols]], axis=0)
                if i > 0:
                    v = jnp.concatenate([v_ref[HH:i * HQ + HH, cols], v], axis=0)
            m = jnp.max(s, axis=1, keepdims=True)
            p = jnp.exp2(s - m).astype(BF16)
            l = jnp.sum(p.astype(F32), axis=1, keepdims=True)
            o = jnp.dot(p, _as_bf16(v), preferred_element_type=F32)
            return o * pl.reciprocal(l, approx=False, full_range=False)

        def oproj(ctx, r, n):
            rows = slice(HALO + r, HALO + r + n)
            acc_ref[rows, :] += jnp.dot(ctx.astype(BF16), _as_bf16(wop_ref[...]),
                                        preferred_element_type=F32)

        q, s, t0, ctx = {}, {}, {}, {}
        for op in _attention_schedule(nq):
            kind, i = op[0], op[1]
            if kind == "q":
                q[i] = proj_q(i)
            elif kind == "v":
                proj_v(i)
            elif kind == "s":
                s[op[1:]] = scores(q[i], op[2], op[3], i)
            elif kind == "t":
                t0[i], t0[op[2]] = first_scores(q[i], q[op[2]])
            elif kind == "pv":
                ctx[op[1:]] = softmax_pv(s.pop(op[1:]), t0, op[2], op[3], i)
            else:
                oproj(jnp.concatenate([ctx.pop((i, hh, op[2])) for hh in range(2)], axis=1),
                      i * TQ + op[2] * HQ, HQ)

        stage_weights(jnp.minimum(j + 1, NP - 1))
        return carry

    def _epilogue():
        for cp in late_copies:
            cp.wait()

        G = M // 4
        NC = TB // TC
        TH = TB + 2 * HALO
        fsplit = [c * 128 for c in F_CUTS] + [Fd - Fd % 128]
        assert len(F_CUTS) == NC and Fd % 128

        def start_row(t):
            return t * TB if isinstance(t, int) else pl.multiple_of(t * TB, TB)

        def front_a(t, lo, hi):
            r = start_row(t)
            ga = mod_ref[2, 0:1, :]
            sb = mod_ref[3, 0:1, :]
            cb1 = 1.0 + mod_ref[4, 0:1, :]
            x1 = (x_ref.at[pl.ds(r, TH), :][lo:hi, :].astype(F32)
                  + ga * acc_ref.at[pl.ds(r, TH), :][lo:hi, :])
            h = _ln(x1) * cb1 + sb
            tt = _gelu(jnp.dot(_ln(h).astype(BF16), _as_bf16(w1_ref[...]),
                               preferred_element_type=F32))
            if lo == 0:
                tt = jnp.concatenate([jnp.zeros((HALO, M), F32), tt[HALO:]], axis=0)
            if lo == 2 * HALO:
                x1, h, tt = [jnp.concatenate([cr_ref[a], v], axis=0)
                             for a, v in enumerate((x1, h, tt))]
            if hi == TH:
                n = hi - lo - HALO
                tt = jnp.concatenate([tt[:n], jnp.where(r + TB < S, tt[n:], 0.0)], axis=0)
                for a, v in enumerate((x1, h, tt)):
                    cr_ref[a] = v[n - HALO:]
            return x1, h, tt

        def front_b(x1, h, tt, lo, n):
            gb = mod_ref[5, 0:1, :]
            lane = lax.broadcasted_iota(jnp.int32, (n, 128), 1)
            cols = []
            shifts = (-1, 1, -2, 2)
            for cblk in range(M // 128):
                c0, c1 = cblk * 128, (cblk + 1) * 128
                ga_, gb_ = c0 // G, (c1 - 1) // G
                a = tt[HALO + lo + shifts[ga_]:HALO + lo + shifts[ga_] + n, c0:c1]
                if gb_ != ga_:
                    b = tt[HALO + lo + shifts[gb_]:HALO + lo + shifts[gb_] + n, c0:c1]
                    a = jnp.where(lane < gb_ * G - c0, a, b)
                cols.append(a)
            sh = jnp.concatenate(cols, axis=1).astype(BF16)
            y = h[HALO + lo:HALO + lo + n] + jnp.dot(sh, _as_bf16(w2_ref[...]),
                                                     preferred_element_type=F32)
            z_ref[lo:lo + n, :] = x1[HALO + lo:HALO + lo + n] + gb * y
            u3_ref[lo // 2:(lo + n) // 2, :] = _as_u32(_ln(y).astype(BF16))

        def out_copy(it, n):
            rows = pl.ds(start_row(it * NS), n * TB)
            return pltpu.make_async_copy(ob_ref.at[rows, :], o_hbm.at[rows, :], osem.at[it])

        w3h_ref[...] = _as_u32(_as_bf16(w3t_ref[0:64, :]).astype(F32).T.astype(BF16))

        def rows_bf16(f):
            return [f[kk * TC:(kk + 1) * TC].astype(BF16) for kk in range(NC)]

        def mm3(k, opens):
            lo, hi = fsplit[k], fsplit[k + 1]
            u3 = _as_bf16(u3_ref[...])
            fs = []
            if opens:
                fs.append(jnp.dot(u3, _as_bf16(w3h_ref[...]), preferred_element_type=F32))
                lo += 128
            fs.append(lax.dot_general(u3, _as_bf16(w3t_ref[lo // 2:hi // 2, :]),
                                      NT, preferred_element_type=F32))
            return rows_bf16(_gelu(jnp.concatenate(fs, axis=1)))

        def mm3_rest():
            ft = _gelu(lax.dot_general(_as_bf16(w3t_ref[fsplit[-1] // 2:, :]), _as_bf16(u3_ref[...]),
                                       NT, preferred_element_type=F32))
            return rows_bf16(ft.T)

        def mm4(t, f, z, k):
            lo = k * TC
            gb = mod_ref[5, 0:1, :]
            h2 = jnp.dot(jnp.concatenate([fk[k] for fk in f], axis=1), _as_bf16(w4_ref[...]),
                         preferred_element_type=F32)
            ob_ref[pl.ds(start_row(t) + lo, TC), :] = (z + gb * h2).astype(ob_ref.dtype)

        def stage(t, nxt, opens):
            fs, fr = [], []
            for k in range(NC):
                fs.append(mm3(k, opens and k == 0))
                if k == 0:
                    rest = mm3_rest()
                if nxt:
                    fr.append(front_a(t + 1, 2 * HALO + k * TC, 2 * HALO + (k + 1) * TC))
            fs.append(rest)
            if nxt:
                fr = [jnp.concatenate(parts, axis=0) for parts in zip(*fr)]
            for k in range(NC):
                z = z_ref[k * TC:(k + 1) * TC, :]
                if nxt:
                    front_b(*fr, k * TC, TC)
                mm4(t, fs, z, k)

        nb = S // TB
        ni = (nb - 1) // NS
        assert ni * NS == nb - 1
        fr = [front_a(0, lo, hi) for lo, hi in zip(FILL_A[:-1], FILL_A[1:])]
        fr = [jnp.concatenate(parts, axis=0) for parts in zip(*fr)]
        for lo, hi in zip(FILL_B[:-1], FILL_B[1:]):
            front_b(*fr, lo, hi - lo)

        def loop_b(it, carry):
            for u in range(NS):
                stage(it * NS + u, True, u == 0)
            out_copy(it, NS).start()
            return carry
        lax.fori_loop(0, ni, loop_b, 0)
        stage(nb - 1, False, True)
        out_copy(ni, 1).start()
        for it in range(ni):
            out_copy(it, NS).wait()
        out_copy(ni, 1).wait()

    @pl.when(pl.program_id(0) == 0)
    def _():
        _prologue()
        lax.fori_loop(1, NK, _keys, 0)
        _wait_pair_weights()
        lax.fori_loop(0, NP, _attention, 0)

    @pl.when(pl.program_id(0) == 1)
    def _():
        _epilogue()


@jax.jit
def pallas_adaLN_cond__compressed_kv_cla__mixer_s_mlp__prompt_kernel(
    A_x: jax.Array,
    A_c_kv: jax.Array,
    A_w_q: jax.Array,
    A_w_uk: jax.Array,
    A_w_uv: jax.Array,
    A_w_o: jax.Array,
    B_x: jax.Array,
    B_w1: jax.Array,
    B_w2: jax.Array,
    B_w3: jax.Array,
    B_w4: jax.Array,
    c: jax.Array,
    w_mod: jax.Array,
):
    B, S, M = A_x.shape
    assert B == 1 and A_c_kv.shape[1] == S
    Dc = A_c_kv.shape[2]
    H, D = A_w_q.shape[1], A_w_q.shape[2]
    NP = H // 2
    Fd = B_w3.shape[1]
    LC = TK // NL
    any_spec = pl.BlockSpec(memory_space=pl.ANY)

    out = pl.pallas_call(
        functools.partial(_kernel, S=S, M=M, D=D, NP=NP, Fd=Fd),
        grid=(2,),
        in_specs=[any_spec] * 12,
        out_specs=any_spec,
        out_shape=jax.ShapeDtypeStruct((S, M), A_x.dtype),
        scratch_shapes=[
            pltpu.VMEM((S + 3 * LC, M), BF16),
            pltpu.VMEM((S // 2, Dc), U32),
            pltpu.VMEM((NP, M, D), U32),
            pltpu.VMEM((NP, Dc, D), U32),
            pltpu.VMEM((NP, Dc, D), U32),
            pltpu.VMEM((NP, D, M), U32),
            pltpu.VMEM((M // 2, M), U32),
            pltpu.VMEM((M // 2, M), U32),
            pltpu.VMEM((Fd // 2, M), U32),
            pltpu.VMEM((Fd // 2, M), U32),
            pltpu.VMEM((6, M // 2, M), U32),
            pltpu.VMEM((NP * S // 2, 2 * D), U32),
            pltpu.VMEM((S + 4 * HALO, M), F32),
            pltpu.VMEM(((S + LC) // 2, M), U32),
            pltpu.VMEM((S, M), BF16),
            pltpu.VMEM((M // 2, 128), U32),
            pltpu.VMEM((M // 2, 2 * D), U32),
            pltpu.VMEM((Dc // 2, 2 * KP * D), U32),
            pltpu.VMEM((Dc // 2, 2 * D), U32),
            pltpu.VMEM((D, M), U32),
            pltpu.VMEM((S // 2, 2 * D), U32),
            pltpu.VMEM((M // 2, 128), U32),
            pltpu.VMEM((TB, M), F32),
            pltpu.VMEM((TB // 2, M), U32),
            pltpu.VMEM((6, 8, M), F32),
            pltpu.VMEM((3, 2 * HALO, M), F32),
            pltpu.VMEM((8, 128), U32),
            pltpu.VMEM((1, M), BF16),
            pltpu.SemaphoreType.DMA((12,)),
            pltpu.SemaphoreType.DMA((CC - 1 + S // CC // TK,)),
            pltpu.SemaphoreType.DMA((NP,)),
            pltpu.SemaphoreType.DMA((6,)),
            pltpu.SemaphoreType.DMA(((S // TB - 1) // NS + 1,)),
        ],
        compiler_params=pltpu.CompilerParams(
            dimension_semantics=("arbitrary",),
            vmem_limit_bytes=100 * 1024 * 1024,
            disable_bounds_checks=True,
            disable_semaphore_checks=True,
        ),
    )(
        A_x.reshape(S, M), A_c_kv.reshape(S, Dc),
        A_w_q, A_w_uk, A_w_uv,
        A_w_o.reshape(NP, 2 * D, M),
        B_w1, B_w2, B_w3.T, B_w4, c, w_mod,
    )
    return out.reshape(B, S, M)
```
